```python
import jax
import jax.numpy as jnp

def _softmax(x, axis=-1):
    return jax.nn.softmax(x, axis=axis)

def _gelu(x):
    return jax.nn.gelu(x, approximate=True)

def _silu(x):
    return jax.nn.silu(x)

def _sigmoid(x):
    return jax.nn.sigmoid(x)

def _layernorm(x, axis=-1, eps=1e-05):
    m = jnp.mean(x, axis=axis, keepdims=True)
    v = jnp.var(x, axis=axis, keepdims=True)
    return (x - m) / jnp.sqrt(v + eps)

def _scatter_add(tgt, idx, src, axis=0):
    return tgt.at[idx].add(src)

def _segment_sum(src, seg, n):
    return jax.ops.segment_sum(src, seg, n)

class _Rng:

    def __init__(self, key):
        self._k = key

    def _next(self):
        self._k, sub = jax.random.split(self._k)
        return sub

    def normal(self, shape):
        return jax.random.normal(self._next(), shape, dtype=jnp.bfloat16)

    def randint(self, lo, hi, shape):
        return jax.random.randint(self._next(), shape, lo, hi, dtype=jnp.int32)

    def uniform(self, shape, lo=0.0, hi=1.0):
        return jax.random.uniform(self._next(), shape, jnp.bfloat16, lo, hi)

    def permutation(self, n):
        return jax.random.permutation(self._next(), n)
kernel_name = 'parallel_sum__memory_aug_infini_attn__moe_arch_mod__prompt'

def setup_inputs():
    _rng = _Rng(jax.random.key(int.from_bytes(__import__("os").urandom(4), "little")))
    _w = lambda a: (lambda t: t.astype(jnp.bfloat16) if jnp.issubdtype(t.dtype, jnp.floating) else t)(jnp.asarray(a))

    def _A_setup():
        B, S, D, H = (1, 2048, 576, 32)
        N = 4
        L = max(1, S // N)
        sc = D ** (-0.5)
        return {'x': _w((lambda *s: _rng.normal(s) * 0.05)(B, N * L, D)), 'wq': _w((lambda *s: _rng.normal(s) * 0.05)(D, D) * sc), 'wk': _w((lambda *s: _rng.normal(s) * 0.05)(D, D) * sc), 'wv': _w((lambda *s: _rng.normal(s) * 0.05)(D, D) * sc), 'wo': _w((lambda *s: _rng.normal(s) * 0.05)(D, D) * sc), 'beta': _w((lambda *s: _rng.normal(s) * 0.05)(H))}
    _A_in = _A_setup()

    def _B_setup():
        B, S, D, F, C = (1, 2048, 576, 4608, 2)
        return {'x': _w((lambda *s: _rng.normal(s) * 0.05)(B, S, D)), 'w_r': _w((lambda *s: _rng.normal(s) * 0.05)(D)), 'w_gate': _w((lambda *s: _rng.normal(s) * 0.05)(D, F)), 'w_up': _w((lambda *s: _rng.normal(s) * 0.05)(D, F)), 'w_down': _w((lambda *s: _rng.normal(s) * 0.05)(F, D))}
    _B_in = _B_setup()
    return {'A_x': _A_in['x'], 'A_wq': _A_in['wq'], 'A_wk': _A_in['wk'], 'A_wv': _A_in['wv'], 'A_wo': _A_in['wo'], 'A_beta': _A_in['beta'], 'B_x': _B_in['x'], 'B_w_r': _B_in['w_r'], 'B_w_gate': _B_in['w_gate'], 'B_w_up': _B_in['w_up'], 'B_w_down': _B_in['w_down']}

def reference(A_x, A_wq, A_wk, A_wv, A_wo, A_beta, B_x, B_w_r, B_w_gate, B_w_up, B_w_down):

    def _A_ref(x, wq, wk, wv, wo, beta):
        B, S, D = x.shape
        H = 32
        Dh = D // H
        N = 4
        L = S // N
        q = (lambda x, *d: x.transpose(*d))((x @ wq).reshape(B, S, H, Dh), 0, 2, 1, 3).reshape(B, H, N, L, Dh)
        k = (lambda x, *d: x.transpose(*d))((x @ wk).reshape(B, S, H, Dh), 0, 2, 1, 3).reshape(B, H, N, L, Dh)
        v = (lambda x, *d: x.transpose(*d))((x @ wv).reshape(B, S, H, Dh), 0, 2, 1, 3).reshape(B, H, N, L, Dh)
        phi = lambda t: jnp.where(t > 0, t + 1.0, jnp.exp(t))
        scale = Dh ** (-0.5)
        ar = jnp.arange(L)
        mask = (lambda x, dt: x.astype(dt))(ar[:, None] < ar[None, :], x.dtype) * -1000000000.0
        g = _sigmoid(beta).reshape(1, H, 1, 1)
        M = jnp.einsum('bhd,bhe->bhde', q[:, :, 0, 0, :] * 0.0, q[:, :, 0, 0, :] * 0.0)
        z = q[:, :, 0, 0, :] * 0.0
        outs = []
        for s in range(N):
            qs, ks, vs = (q[:, :, s].copy(), k[:, :, s].copy(), v[:, :, s].copy())
            logits = jnp.einsum('bhqd,bhkd->bhqk', qs, ks) * scale + mask
            p = _softmax(logits, axis=-1)
            a_dot = jnp.einsum('bhqk,bhkd->bhqd', p, vs)
            pq = phi(qs)
            num = jnp.einsum('bhld,bhde->bhle', pq, M)
            den = jnp.einsum('bhld,bhd->bhl', pq, z)[..., None] + 1e-06
            a_mem = num / den
            o = g * a_mem + (1.0 - g) * a_dot
            outs.append(o)
            pk = phi(ks)
            M = M + jnp.einsum('bhld,bhle->bhde', pk, vs)
            z = z + jnp.einsum('bhld->bhd', pk)
        o = (lambda x, *d: x.transpose(*d))(jnp.stack(outs, 2).reshape(B, H, S, Dh), 0, 2, 1, 3).reshape(B, S, D)
        return o @ wo

    def _B_ref(x, w_r, w_gate, w_up, w_down):
        B, S, D = x.shape
        C = 2
        r = x @ w_r
        idx = jnp.argsort(-r, axis=-1)[:, :C]
        idx_e = jnp.repeat(idx.reshape(B, C, 1), D, axis=2)
        x_sel = jnp.take_along_axis(x, idx_e, axis=1)
        g = _silu(x_sel @ w_gate)
        u = x_sel @ w_up
        y = g * u @ w_down
        r_sel = _sigmoid(jnp.take_along_axis(r, idx, axis=1))
        y = y * r_sel.reshape(B, C, 1)
        b_off = (jnp.arange(B) * S).reshape(B, 1)
        flat_idx = (idx + b_off).reshape(B * C)
        zero = (x * 0.0).reshape(B * S, D)
        upd = _scatter_add(zero, flat_idx, y.reshape(B * C, D), axis=0)
        return x + upd.reshape(B, S, D)
    x = A_x
    xn = _layernorm(x, axis=-1)
    return x + _A_ref(xn, A_wq, A_wk, A_wv, A_wo, A_beta) + _B_ref(xn, B_w_r, B_w_gate, B_w_up, B_w_down)
```

```python
import functools

import jax
import jax.numpy as jnp
from jax import lax
import jax.experimental.pallas as pl
import jax.experimental.pallas.tpu as pltpu

F32 = jnp.float32
BF16 = jnp.bfloat16
U32 = jnp.uint32
I32 = jnp.int32

S = 2048
D = 576
H = 32
DH = 18
NSEG = 4
L = 512
FF = 4608
HPG = 7
NG = 5
DP = NG * 128
QT = L // 128
VROWS = D + 16
ZROW = 144
MROWS = 160
LOG2E = 1.4426950408889634
QSCALE = (DH ** -0.5) * LOG2E
SAFE_LOG2_RANGE = 60.0
NEG_BIG = -1e30

NT_DIMS = (((1,), (1,)), ((), ()))
TN_DIMS = (((0,), (0,)), ((), ()))


def _heads_in_group(g):
    return min(HPG, H - HPG * g)


def _group_row_start(g):
    return (HPG * g * DH // 16) * 16


def _group_rows(g):
    last = (HPG * g + _heads_in_group(g)) * DH
    return -(-(last - _group_row_start(g)) // 16) * 16


def _round_bf16(x):
    return x.astype(BF16).astype(F32)


def _pad_heads(w):
    rows = w.shape[0]
    parts = []
    for g in range(NG):
        n = _heads_in_group(g) * DH
        parts.append(w[:, HPG * DH * g:HPG * DH * g + n])
        parts.append(jnp.zeros((rows, 128 - n), w.dtype))
    return jnp.concatenate(parts, axis=1)


def _phi(t):
    return jnp.where(t > 0, t + 1.0, jnp.exp(t))


def _kernel(x_hbm, wq_hbm, wk_hbm, wv_hbm, wo_hbm, beta_ref, wr_ref, wg_hbm, wu_hbm, wd_hbm,
            out_hbm,
            x_buf, wq_raw, wk_raw, wv_raw, wo_buf, wg_buf, wu_buf, wd_buf,
            wqk, wvt, xn_buf, base, qs_buf, pq_buf, k_buf, pk_buf, vt_buf, r_buf, zs_buf,
            gate_buf, mt_buf, num_buf, p_buf, ot_buf, out_buf, in_sems, out_sems):
    def x_copy(c):
        return pltpu.make_async_copy(x_hbm.at[0, pl.ds(c * L, L), :], x_buf.at[pl.ds(c * L, L), :],
                                     in_sems.at[c])

    cp_wv = pltpu.make_async_copy(wv_hbm, wv_raw, in_sems.at[4])
    cp_wq = pltpu.make_async_copy(wq_hbm, wq_raw, in_sems.at[5])
    cp_wk = pltpu.make_async_copy(wk_hbm, wk_raw, in_sems.at[6])
    cp_wo = pltpu.make_async_copy(wo_hbm, wo_buf, in_sems.at[7])
    cp_wg = pltpu.make_async_copy(wg_hbm, wg_buf, in_sems.at[8])
    cp_wu = pltpu.make_async_copy(wu_hbm, wu_buf, in_sems.at[9])
    cp_wd = pltpu.make_async_copy(wd_hbm, wd_buf, in_sems.at[10])

    def out_copy(s):
        return pltpu.make_async_copy(out_buf.at[pl.ds(s * L, L), :], out_hbm.at[0, pl.ds(s * L, L), :],
                                     out_sems.at[s])

    x_copy(0).start()
    cp_wv.start()
    cp_wq.start()
    cp_wk.start()
    for c in range(1, NSEG):
        x_copy(c).start()
    cp_wo.start()
    cp_wg.start()
    cp_wu.start()
    cp_wd.start()

    lane128 = lax.broadcasted_iota(I32, (128, 128), 1)
    row128 = lax.broadcasted_iota(I32, (128, 128), 0)
    causal = row128 <= lane128

    beta_row = beta_ref[...].reshape(1, H).astype(F32)
    beta_row = jnp.concatenate([beta_row, jnp.zeros((1, 128 - H), F32)], axis=1)
    e_row = lax.broadcasted_iota(I32, (D, 128), 0)
    e_lane = lax.broadcasted_iota(I32, (D, 128), 1)
    in_head = (e_row >= e_lane * DH) & (e_row < e_lane * DH + DH)
    beta_col = jnp.sum(jnp.where(in_head, beta_row, 0.0), axis=1, keepdims=True)
    gate_buf[...] = jnp.broadcast_to(jax.nn.sigmoid(beta_col), (D, 128))

    mt_buf[...] = jnp.zeros(mt_buf.shape, F32)

    def layernorm(c):
        x = x_buf[pl.ds(c * L, L), :].astype(F32)
        mean = jnp.sum(x, axis=1, keepdims=True) * (1.0 / D)
        cen = x - mean
        var = jnp.sum(cen * cen, axis=1, keepdims=True) * (1.0 / D)
        d = _round_bf16(x - _round_bf16(mean))
        den = _round_bf16(jnp.sqrt(_round_bf16(_round_bf16(var) + 1e-5)))
        xn = (d / den).astype(BF16)
        xn_buf[pl.ds(c * L, L), :] = xn
        base[pl.ds(c * L, L), :] = x + xn.astype(F32)

    x_copy(0).wait()
    layernorm(0)
    cp_wv.wait()
    wvt[0:D, :] = wv_raw[...].T
    wr_row = wr_ref[...].reshape(1, D).astype(F32)
    r16 = lax.broadcasted_iota(I32, (16, D), 0)
    wvt[D:VROWS, :] = jnp.where(r16 == 0, wr_row, 0.0).astype(BF16)
    cp_wq.wait()
    cp_wk.wait()
    wqk[:, 0:DP] = _pad_heads(wq_raw[...].astype(F32)).astype(BF16)
    wqk[:, DP:2 * DP] = _pad_heads(wk_raw[...].astype(F32)).astype(BF16)

    aq = jnp.zeros((8, DP), F32)
    ak = jnp.zeros((8, DP), F32)
    for c in range(NSEG):
        rows = pl.ds(c * L, L)
        xn = xn_buf[rows, :]
        vt = lax.dot_general(wvt[...], xn, NT_DIMS, preferred_element_type=F32)
        vt_buf[c] = vt[0:D].astype(BF16)
        r_buf[:, pl.ds(c * L, L)] = vt[D:D + 8]
        qk = jnp.dot(xn, wqk[...], preferred_element_type=F32)
        q = qk[:, 0:DP]
        k = qk[:, DP:2 * DP]
        qsc = q * QSCALE
        qs_buf[rows, :] = qsc.astype(BF16)
        pq_buf[rows, :] = _phi(q).astype(BF16)
        k_buf[rows, :] = k.astype(BF16)
        pk = _phi(k)
        pk_buf[rows, :] = pk.astype(BF16)
        zs_buf[c] = jnp.sum(pk.reshape(L // 8, 8, DP), axis=0)
        aq = jnp.maximum(aq, jnp.max(jnp.abs(qsc).reshape(L // 8, 8, DP), axis=0))
        ak = jnp.maximum(ak, jnp.max(jnp.abs(k).reshape(L // 8, 8, DP), axis=0))
        if c + 1 < NSEG:
            x_copy(c + 1).wait()
            layernorm(c + 1)

    colmax = jnp.max(aq, axis=0, keepdims=True) * jnp.max(ak, axis=0, keepdims=True)
    logit_bound = jnp.max(colmax) * (DH * 1.02)
    safe = logit_bound <= SAFE_LOG2_RANGE

    r = _round_bf16(r_buf[0:1, :])
    tok = lax.broadcasted_iota(I32, (1, S), 1).astype(F32)
    m1 = jnp.max(r)
    i1 = jnp.min(jnp.where(r == m1, tok, float(S)))
    r_rest = jnp.where(tok == i1, -jnp.inf, r)
    m2 = jnp.max(r_rest)
    i2 = jnp.min(jnp.where(r_rest == m2, tok, float(S)))
    i1 = jnp.clip(i1.astype(I32), 0, S - 1)
    i2 = jnp.clip(i2.astype(I32), 0, S - 1)

    def pick_row(i):
        blk = xn_buf[pl.ds(pl.multiple_of((i // 16) * 16, 16), 16), :].astype(F32)
        return jnp.sum(jnp.where(r16 == i % 16, blk, 0.0), axis=0, keepdims=True)

    xs = jnp.where(r16 == 0, pick_row(i1), jnp.where(r16 == 1, pick_row(i2), 0.0)).astype(BF16)
    cp_wg.wait()
    cp_wu.wait()
    hg = jnp.dot(xs, wg_buf[...], preferred_element_type=F32)
    hu = jnp.dot(xs, wu_buf[...], preferred_element_type=F32)
    hh = (jax.nn.silu(hg) * hu).astype(BF16)
    cp_wd.wait()
    y = jnp.dot(hh, wd_buf[...], preferred_element_type=F32)
    y0 = y[0:1] * jax.nn.sigmoid(jnp.full((1, D), m1, F32))
    y1 = y[1:2] * jax.nn.sigmoid(jnp.full((1, D), m2, F32))
    base[pl.ds(i1, 1), :] = base[pl.ds(i1, 1), :] + y0
    base[pl.ds(i2, 1), :] = base[pl.ds(i2, 1), :] + y1
    cp_wo.wait()

    def memory_read(s, g):
        rg = _group_rows(g)
        rows = pl.ds(pl.multiple_of(s * L, L), L)
        lhs = jnp.concatenate([mt_buf[g, 0:rg, :], mt_buf[g, ZROW:MROWS, :]], axis=0).astype(BF16)
        res = lax.dot_general(lhs, pq_buf[rows, 128 * g:128 * (g + 1)], NT_DIMS,
                              preferred_element_type=F32)
        num_buf[g, 0:rg, :] = res[0:rg]
        num_buf[g, ZROW:MROWS, :] = res[rg:rg + 16]

    def memory_update(s, g):
        rg = _group_rows(g)
        a_g = _group_row_start(g)
        rows = pl.ds(pl.multiple_of(s * L, L), L)
        upd = jnp.dot(vt_buf[s, a_g:a_g + rg, :], pk_buf[rows, 128 * g:128 * (g + 1)],
                      preferred_element_type=F32)
        er = lax.broadcasted_iota(I32, (rg, 128), 0) + (a_g - HPG * DH * g)
        el = lax.broadcasted_iota(I32, (rg, 128), 1)
        same_head = None
        for i in range(_heads_in_group(g)):
            t = ((er >= DH * i) & (er < DH * (i + 1)) & (el >= DH * i) & (el < DH * (i + 1)))
            same_head = t if same_head is None else (same_head | t)
        mt_buf[g, 0:rg, :] = mt_buf[g, 0:rg, :] + jnp.where(same_head, upd, 0.0)
        zr = lax.broadcasted_iota(I32, (8, 128), 0)
        zl = lax.broadcasted_iota(I32, (8, 128), 1)
        zmask = (zl >= zr * DH) & (zl < zr * DH + DH) & (zr < _heads_in_group(g))
        zs = jnp.sum(zs_buf[s, :, 128 * g:128 * (g + 1)], axis=0, keepdims=True)
        mt_buf[g, ZROW:ZROW + 8, :] = mt_buf[g, ZROW:ZROW + 8, :] + jnp.where(zmask, zs, 0.0)

    def project_out(s):
        rows = pl.ds(pl.multiple_of(s * L, L), L)
        attn = lax.dot_general(ot_buf[...].astype(BF16), wo_buf[...], TN_DIMS,
                               preferred_element_type=F32)
        out_buf[rows, :] = (base[rows, :] + attn).astype(BF16)
        out_copy(s).start()

    def fast_segment(s, carry):
        row0 = pl.multiple_of(s * L, L)
        for g in range(NG):
            nh = _heads_in_group(g)
            a_g = _group_row_start(g)
            memory_read(s, g)
            offs = [0, 128, 384, 768]
            lsum = {}
            for j in range(QT - 1, -1, -1):
                n = 128 * (j + 1)
                q = qs_buf[pl.ds(row0 + 128 * j, 128), 128 * g:128 * (g + 1)].astype(F32)
                qm = jnp.concatenate(
                    [jnp.where((lane128 >= DH * i) & (lane128 < DH * (i + 1)), q, 0.0) for i in range(nh)],
                    axis=0).astype(BF16)
                st = lax.dot_general(k_buf[pl.ds(row0, n), 128 * g:128 * (g + 1)], qm, NT_DIMS,
                                     preferred_element_type=F32)
                p = jnp.exp2(st)
                causal_w = jnp.concatenate([causal] * nh, axis=1)
                p_diag = jnp.where(causal_w, p[n - 128:], 0.0)
                p = jnp.concatenate([p[:n - 128], p_diag], axis=0) if j > 0 else p_diag
                lsum[j] = jnp.sum(p, axis=0, keepdims=True)
                p_buf[offs[j] // 2:(offs[j] + n) // 2, 0:nh * 128] = pltpu.bitcast(p.astype(BF16), U32)
            for j in range(QT - 1, -1, -1):
                n = 128 * (j + 1)
                cols = slice(128 * j, 128 * (j + 1))
                for i in range(nh):
                    h = HPG * g + i
                    a = (h * DH // 16) * 16
                    off = h * DH - a
                    p = pltpu.bitcast(p_buf[offs[j] // 2:(offs[j] + n) // 2, 128 * i:128 * (i + 1)], BF16)
                    o = jnp.dot(vt_buf[s, a:a + 32, 0:n], p, preferred_element_type=F32)
                    lo = (off // 8) * 8
                    hi = -(-(off + DH) // 8) * 8
                    gate = gate_buf[a + lo:a + hi, :]
                    rl = 1.0 / lsum[j][:, 128 * i:128 * (i + 1)]
                    rden = 1.0 / (num_buf[g, ZROW + i:ZROW + i + 1, cols] + 1e-6)
                    num = num_buf[g, a - a_g + lo:a - a_g + hi, cols]
                    val = gate * (num * rden) + (1.0 - gate) * (o[lo:hi] * rl)
                    ot_buf[a + off:a + off + DH, cols] = val[off - lo:off - lo + DH]
            memory_update(s, g)
        project_out(s)
        return carry

    def slow_segment(s, carry):
        row0 = pl.multiple_of(s * L, L)
        for g in range(NG):
            memory_read(s, g)
        key_i = lax.broadcasted_iota(I32, (L, L), 0)
        qry_i = lax.broadcasted_iota(I32, (L, L), 1)
        lane_l = lax.broadcasted_iota(I32, (L, 128), 1)
        r32 = lax.broadcasted_iota(I32, (32, L), 0)

        def head(h, c):
            g = jnp.minimum(h // HPG, NG - 1)
            i = h - HPG * g
            a = pl.multiple_of((h * DH // 16) * 16, 16)
            off = h * DH - a
            a_g = (HPG * g * DH // 16) * 16
            win = pl.ds(pl.multiple_of(g * 128, 128), 128)
            q = qs_buf[pl.ds(row0, L), win].astype(F32)
            qm = jnp.where((lane_l >= DH * i) & (lane_l < DH * (i + 1)), q, 0.0).astype(BF16)
            st = lax.dot_general(k_buf[pl.ds(row0, L), win], qm, NT_DIMS, preferred_element_type=F32)
            st = jnp.where(key_i <= qry_i, st, NEG_BIG)
            p = jnp.exp2(st - jnp.max(st, axis=0, keepdims=True))
            rl = 1.0 / jnp.sum(p, axis=0, keepdims=True)
            o = jnp.dot(vt_buf[s, pl.ds(a, 32), :], p.astype(BF16), preferred_element_type=F32)
            gate = jnp.concatenate([gate_buf[pl.ds(a, 32), :]] * QT, axis=1)
            rden = 1.0 / (num_buf[g, pl.ds(ZROW + i, 1), :] + 1e-6)
            num = num_buf[g, pl.ds(pl.multiple_of(a - a_g, 16), 32), :]
            val = gate * (num * rden) + (1.0 - gate) * (o * rl)
            keep = (r32 >= off) & (r32 < off + DH)
            pltpu.store(ot_buf.at[pl.ds(a, 32), :], val, mask=keep)
            return c

        lax.fori_loop(0, H, head, 0)
        for g in range(NG):
            memory_update(s, g)
        project_out(s)
        return carry

    @pl.when(safe)
    def _():
        lax.fori_loop(0, NSEG, fast_segment, 0)

    @pl.when(jnp.logical_not(safe))
    def _():
        lax.fori_loop(0, NSEG, slow_segment, 0)

    for s in range(NSEG):
        out_copy(s).wait()


@jax.jit
def pallas_parallel_sum__memory_aug_infini_attn__moe_arch_mod__prompt_kernel(
    A_x: jax.Array,
    A_wq: jax.Array,
    A_wk: jax.Array,
    A_wv: jax.Array,
    A_wo: jax.Array,
    A_beta: jax.Array,
    B_x: jax.Array,
    B_w_r: jax.Array,
    B_w_gate: jax.Array,
    B_w_up: jax.Array,
    B_w_down: jax.Array,
):
    del B_x
    hbm = pl.BlockSpec(memory_space=pltpu.HBM)
    vmem = pl.BlockSpec(memory_space=pltpu.VMEM)
    scratch = [
        pltpu.VMEM((S, D), BF16),
        pltpu.VMEM((D, D), BF16),
        pltpu.VMEM((D, D), BF16),
        pltpu.VMEM((D, D), BF16),
        pltpu.VMEM((D, D), BF16),
        pltpu.VMEM((D, FF), BF16),
        pltpu.VMEM((D, FF), BF16),
        pltpu.VMEM((FF, D), BF16),
        pltpu.VMEM((D, 2 * DP), BF16),
        pltpu.VMEM((VROWS, D), BF16),
        pltpu.VMEM((S, D), BF16),
        pltpu.VMEM((S, D), F32),
        pltpu.VMEM((S, DP), BF16),
        pltpu.VMEM((S, DP), BF16),
        pltpu.VMEM((S, DP), BF16),
        pltpu.VMEM((S, DP), BF16),
        pltpu.VMEM((NSEG, D, L), BF16),
        pltpu.VMEM((8, S), F32),
        pltpu.VMEM((NSEG, 8, DP), F32),
        pltpu.VMEM((D, 128), F32),
        pltpu.VMEM((NG, MROWS, 128), F32),
        pltpu.VMEM((NG, MROWS, L), F32),
        pltpu.VMEM((640, HPG * 128), U32),
        pltpu.VMEM((D, L), F32),
        pltpu.VMEM((S, D), BF16),
        pltpu.SemaphoreType.DMA((11,)),
        pltpu.SemaphoreType.DMA((NSEG,)),
    ]
    return pl.pallas_call(
        _kernel,
        out_shape=jax.ShapeDtypeStruct((1, S, D), BF16),
        in_specs=[hbm, hbm, hbm, hbm, hbm, vmem, vmem, hbm, hbm, hbm],
        out_specs=hbm,
        scratch_shapes=scratch,
        compiler_params=pltpu.CompilerParams(vmem_limit_bytes=128 * 1024 * 1024),
        name="infini_attn_moe",
    )(A_x, A_wq, A_wk, A_wv, A_wo, A_beta, B_w_r, B_w_gate, B_w_up, B_w_down)
```

```python
import jax
import jax.numpy as jnp
from jax import lax
import jax.experimental.pallas as pl
import jax.experimental.pallas.tpu as pltpu

F32 = jnp.float32
BF16 = jnp.bfloat16
U32 = jnp.uint32
I32 = jnp.int32

S = 2048
D = 576
H = 32
DH = 18
NSEG = 4
L = 512
FF = 4608
HPG = 7
NG = 5
QT = L // 128
GW = (128, 128, 128, 128, 80)
PR = sum(GW)
VROWS = D + 16
ZROW = 144
MROWS = 160
LOG2E = 1.4426950408889634
QSCALE = (DH ** -0.5) * LOG2E
SAFE_LOG2_RANGE = 60.0
NEG_BIG = -1e30

NT_DIMS = (((1,), (1,)), ((), ()))


def _heads_in_group(g):
    return min(HPG, H - HPG * g)


def _group_row_start(g):
    return (HPG * g * DH // 16) * 16


def _group_rows(g):
    last = (HPG * g + _heads_in_group(g)) * DH
    return -(-(last - _group_row_start(g)) // 16) * 16


def _round_bf16(x):
    return x.astype(BF16).astype(F32)


def _pad_heads_t(w):
    parts = []
    for g in range(NG):
        n = _heads_in_group(g) * DH
        parts.append(w[:, HPG * DH * g:HPG * DH * g + n])
        parts.append(jnp.zeros((D, 128 - n), w.dtype))
    return jnp.concatenate(parts, axis=1).T[0:PR]


def _phi(t):
    return jnp.where(t > 0, t + 1.0, jnp.exp(t))


def _kernel(x_hbm, wq_hbm, wk_hbm, wv_hbm, wo_hbm, beta_hbm, wr_hbm, wg_hbm, wu_hbm, wd_hbm,
            out_hbm,
            x_buf, wq_raw, wk_raw, wv_raw, wo_raw, beta_buf, wr_buf, wg_buf, wu_buf, wd_buf,
            wqt, wkt, wvt, wot, xn_buf, base, qs_buf, pq_buf, k_buf, pk_buf, vt_buf, r_buf,
            gate_buf, mt_buf, num_buf, p_buf, ot_buf, out_buf, in_sems, out_sems):
    def x_copy(c):
        return pltpu.make_async_copy(x_hbm.at[0, :, pl.ds(c * L, L)], x_buf.at[c], in_sems.at[c])

    cp_wv = pltpu.make_async_copy(wv_hbm, wv_raw, in_sems.at[4])
    cp_wq = pltpu.make_async_copy(wq_hbm, wq_raw, in_sems.at[5])
    cp_wk = pltpu.make_async_copy(wk_hbm, wk_raw, in_sems.at[6])
    cp_wo = pltpu.make_async_copy(wo_hbm, wo_raw, in_sems.at[7])
    cp_wg = pltpu.make_async_copy(wg_hbm, wg_buf, in_sems.at[8])
    cp_wu = pltpu.make_async_copy(wu_hbm, wu_buf, in_sems.at[9])
    cp_wd = pltpu.make_async_copy(wd_hbm, wd_buf, in_sems.at[10])
    cp_beta = pltpu.make_async_copy(beta_hbm, beta_buf, in_sems.at[11])
    cp_wr = pltpu.make_async_copy(wr_hbm, wr_buf, in_sems.at[12])

    def out_copy(s):
        cols = pl.ds(pl.multiple_of(s * L, L), L)
        return pltpu.make_async_copy(out_buf.at[s], out_hbm.at[0, :, cols], out_sems.at[s])

    x_copy(0).start()
    cp_wv.start()
    cp_wr.start()
    cp_beta.start()
    cp_wq.start()
    cp_wk.start()
    for c in range(1, NSEG):
        x_copy(c).start()
    cp_wo.start()
    cp_wg.start()
    cp_wu.start()
    cp_wd.start()

    lane128 = lax.broadcasted_iota(I32, (128, 128), 1)
    row128 = lax.broadcasted_iota(I32, (128, 128), 0)
    causal = row128 <= lane128
    r16 = lax.broadcasted_iota(I32, (16, D), 0)

    mt_buf[...] = jnp.zeros(mt_buf.shape, F32)

    def layernorm(c):
        x = x_buf[c].astype(F32)
        mean = jnp.sum(x, axis=0, keepdims=True) * (1.0 / D)
        cen = x - mean
        var = jnp.sum(cen * cen, axis=0, keepdims=True) * (1.0 / D)
        d = _round_bf16(x - _round_bf16(mean))
        den = _round_bf16(jnp.sqrt(_round_bf16(_round_bf16(var) + 1e-5)))
        xn = (d / den).astype(BF16)
        xn_buf[c] = xn
        base[c] = x + xn.astype(F32)

    x_copy(0).wait()
    layernorm(0)
    cp_wv.wait()
    cp_wr.wait()
    wvt[0:D, :] = wv_raw[...].T
    wr_row = wr_buf[...].reshape(1, D).astype(F32)
    wvt[D:VROWS, :] = jnp.where(r16 == 0, wr_row, 0.0).astype(BF16)
    cp_wq.wait()
    wqt[...] = _pad_heads_t(wq_raw[...].astype(F32)).astype(BF16)
    cp_wk.wait()
    wkt[...] = _pad_heads_t(wk_raw[...].astype(F32)).astype(BF16)

    cp_beta.wait()
    beta_row = beta_buf[...].reshape(1, H).astype(F32)
    beta_row = jnp.concatenate([beta_row, jnp.zeros((1, 128 - H), F32)], axis=1)
    e_row = lax.broadcasted_iota(I32, (D, 128), 0)
    e_lane = lax.broadcasted_iota(I32, (D, 128), 1)
    in_head = (e_row >= e_lane * DH) & (e_row < e_lane * DH + DH)
    beta_col = jnp.sum(jnp.where(in_head, beta_row, 0.0), axis=1, keepdims=True)
    gate_buf[...] = jnp.broadcast_to(jax.nn.sigmoid(beta_col), (D, 128))

    aq = jnp.zeros((8, L), F32)
    ak = jnp.zeros((8, L), F32)
    r16l = lax.broadcasted_iota(I32, (16, L), 0)
    for c in range(NSEG):
        xn = xn_buf[c]
        vt = jnp.dot(wvt[...], xn, preferred_element_type=F32)
        vt_buf[c, 0:D, :] = vt[0:D].astype(BF16)
        tail = vt[D:VROWS]
        vt_buf[c, D:VROWS, :] = jnp.where(r16l == 1, 1.0, 0.0).astype(BF16)
        r_buf[:, c * L:(c + 1) * L] = tail[0:8]
        qt = jnp.dot(wqt[...], xn, preferred_element_type=F32)
        qsc = qt * QSCALE
        qs_buf[c] = qsc.astype(BF16)
        pq_buf[c] = _phi(qt).astype(BF16)
        kt = jnp.dot(wkt[...], xn, preferred_element_type=F32)
        pk_buf[c] = _phi(kt).astype(BF16)
        for g in range(NG):
            ktg = kt[128 * g:128 * g + GW[g]]
            if GW[g] < 128:
                ktg = jnp.concatenate([ktg, jnp.zeros((128 - GW[g], L), F32)], axis=0)
            k_buf[c, g] = ktg.T.astype(BF16)
        aq = jnp.maximum(aq, jnp.max(jnp.abs(qsc).reshape(PR // 8, 8, L), axis=0))
        ak = jnp.maximum(ak, jnp.max(jnp.abs(kt).reshape(PR // 8, 8, L), axis=0))
        if c + 1 < NSEG:
            x_copy(c + 1).wait()
            layernorm(c + 1)

    logit_bound = jnp.max(aq) * jnp.max(ak) * (DH * 1.02)
    safe = logit_bound <= SAFE_LOG2_RANGE

    cp_wo.wait()
    wot[...] = wo_raw[...].T

    r = _round_bf16(r_buf[0:1, :])
    tok = lax.broadcasted_iota(I32, (1, S), 1).astype(F32)
    m1 = jnp.max(r)
    i1 = jnp.min(jnp.where(r == m1, tok, float(S)))
    r_rest = jnp.where(tok == i1, -jnp.inf, r)
    m2 = jnp.max(r_rest)
    i2 = jnp.min(jnp.where(r_rest == m2, tok, float(S)))
    i1 = jnp.clip(i1.astype(I32), 0, S - 1)
    i2 = jnp.clip(i2.astype(I32), 0, S - 1)

    sel_row = lax.broadcasted_iota(I32, (16, 128), 0)
    sel_lane = lax.broadcasted_iota(I32, (16, 128), 1)

    def token_tile(i):
        return i // L, pl.ds(pl.multiple_of(((i % L) // 128) * 128, 128), 128)

    def pick(i, slot):
        seg, cols = token_tile(i)
        onehot = jnp.where((sel_row == slot) & (sel_lane == i % 128), 1.0, 0.0).astype(BF16)
        return lax.dot_general(onehot, xn_buf[seg, :, cols], NT_DIMS, preferred_element_type=F32)

    xs = (pick(i1, 0) + pick(i2, 1)).astype(BF16)
    cp_wg.wait()
    cp_wu.wait()
    hg = jnp.dot(xs, wg_buf[...], preferred_element_type=F32)
    hu = jnp.dot(xs, wu_buf[...], preferred_element_type=F32)
    hh = (jax.nn.silu(hg) * hu).astype(BF16)
    cp_wd.wait()
    y = lax.dot_general(hh, wd_buf[...], NT_DIMS, preferred_element_type=F32)
    r_sel = jnp.where(r16 == 0, m1, m2)
    y = y * jax.nn.sigmoid(r_sel)
    yt = jnp.concatenate([y, jnp.zeros((128 - 16, D), F32)], axis=0).T
    lane_d = lax.broadcasted_iota(I32, (D, 128), 1)
    for slot, i in ((0, i1), (1, i2)):
        seg, cols = token_tile(i)
        col = jnp.sum(jnp.where(lane_d == slot, yt, 0.0), axis=1, keepdims=True)
        base[seg, :, cols] = base[seg, :, cols] + jnp.where(lane_d == i % 128, col, 0.0)

    def memory_read(s, g):
        rg = _group_rows(g)
        gw = GW[g]
        lhs = jnp.concatenate([mt_buf[g, 0:rg, 0:gw], mt_buf[g, ZROW:MROWS, 0:gw]], axis=0).astype(BF16)
        res = jnp.dot(lhs, pq_buf[s, 128 * g:128 * g + gw, :], preferred_element_type=F32)
        num_buf[g, 0:rg, :] = res[0:rg]
        num_buf[g, ZROW:MROWS, :] = res[rg:rg + 16]

    def memory_update(s, g):
        rg = _group_rows(g)
        a_g = _group_row_start(g)
        gw = GW[g]
        lhs = jnp.concatenate([vt_buf[s, a_g:a_g + rg, :], vt_buf[s, D:VROWS, :]], axis=0)
        upd = lax.dot_general(lhs, pk_buf[s, 128 * g:128 * g + gw, :], NT_DIMS,
                              preferred_element_type=F32)
        er = lax.broadcasted_iota(I32, (rg, gw), 0) + (a_g - HPG * DH * g)
        el = lax.broadcasted_iota(I32, (rg, gw), 1)
        same_head = None
        for i in range(_heads_in_group(g)):
            t = ((er >= DH * i) & (er < DH * (i + 1)) & (el >= DH * i) & (el < DH * (i + 1)))
            same_head = t if same_head is None else (same_head | t)
        mt_buf[g, 0:rg, 0:gw] = mt_buf[g, 0:rg, 0:gw] + jnp.where(same_head, upd[0:rg], 0.0)
        zr = lax.broadcasted_iota(I32, (8, gw), 0)
        zl = lax.broadcasted_iota(I32, (8, gw), 1)
        zmask = (zl >= zr * DH) & (zl < zr * DH + DH) & (zr < _heads_in_group(g))
        zs = upd[rg + 1:rg + 2]
        mt_buf[g, ZROW:ZROW + 8, 0:gw] = mt_buf[g, ZROW:ZROW + 8, 0:gw] + jnp.where(zmask, zs, 0.0)

    def project_out(s):
        attn = jnp.dot(wot[...], ot_buf[...].astype(BF16), preferred_element_type=F32)
        out_buf[s] = (base[s] + attn).astype(BF16)
        out_copy(s).start()

    def fast_segment(s, carry):
        for g in range(NG):
            nh = _heads_in_group(g)
            gw = GW[g]
            a_g = _group_row_start(g)
            memory_read(s, g)
            offs = [0, 128, 384, 768]
            lsum = {}
            rowg = lax.broadcasted_iota(I32, (gw, 128), 0)
            for j in range(QT - 1, -1, -1):
                n = 128 * (j + 1)
                q = qs_buf[s, 128 * g:128 * g + gw, 128 * j:128 * (j + 1)].astype(F32)
                qm = jnp.concatenate(
                    [jnp.where((rowg >= DH * i) & (rowg < DH * (i + 1)), q, 0.0) for i in range(nh)],
                    axis=1).astype(BF16)
                st = jnp.dot(k_buf[s, g, 0:n, 0:gw], qm, preferred_element_type=F32)
                p = jnp.exp2(st)
                causal_w = jnp.concatenate([causal] * nh, axis=1)
                p_diag = jnp.where(causal_w, p[n - 128:], 0.0)
                p = jnp.concatenate([p[:n - 128], p_diag], axis=0) if j > 0 else p_diag
                lsum[j] = jnp.sum(p, axis=0, keepdims=True)
                p_buf[offs[j] // 2:(offs[j] + n) // 2, 0:nh * 128] = pltpu.bitcast(p.astype(BF16), U32)
            for j in range(QT - 1, -1, -1):
                n = 128 * (j + 1)
                cols = slice(128 * j, 128 * (j + 1))
                for i in range(nh):
                    h = HPG * g + i
                    a = (h * DH // 16) * 16
                    off = h * DH - a
                    p = pltpu.bitcast(p_buf[offs[j] // 2:(offs[j] + n) // 2, 128 * i:128 * (i + 1)], BF16)
                    o = jnp.dot(vt_buf[s, a:a + 32, 0:n], p, preferred_element_type=F32)
                    lo = (off // 8) * 8
                    hi = -(-(off + DH) // 8) * 8
                    gate = gate_buf[a + lo:a + hi, :]
                    rl = 1.0 / lsum[j][:, 128 * i:128 * (i + 1)]
                    rden = 1.0 / (num_buf[g, ZROW + i:ZROW + i + 1, cols] + 1e-6)
                    num = num_buf[g, a - a_g + lo:a - a_g + hi, cols]
                    val = gate * (num * rden) + (1.0 - gate) * (o[lo:hi] * rl)
                    ot_buf[a + off:a + off + DH, cols] = val[off - lo:off - lo + DH]
            memory_update(s, g)
        project_out(s)
        return carry

    def slow_segment(s, carry):
        for g in range(NG):
            memory_read(s, g)
        key_i = lax.broadcasted_iota(I32, (L, L), 0)
        qry_i = lax.broadcasted_iota(I32, (L, L), 1)
        r32 = lax.broadcasted_iota(I32, (32, L), 0)
        for g in range(NG):
            gw = GW[g]
            a_g = _group_row_start(g)
            rowg = lax.broadcasted_iota(I32, (gw, L), 0)

            def head(i, c, g=g, gw=gw, a_g=a_g, rowg=rowg):
                h = HPG * g + i
                a = pl.multiple_of((h * DH // 16) * 16, 16)
                off = h * DH - a
                q = qs_buf[s, 128 * g:128 * g + gw, :].astype(F32)
                qm = jnp.where((rowg >= DH * i) & (rowg < DH * (i + 1)), q, 0.0).astype(BF16)
                st = jnp.dot(k_buf[s, g, :, 0:gw], qm, preferred_element_type=F32)
                st = jnp.where(key_i <= qry_i, st, NEG_BIG)
                p = jnp.exp2(st - jnp.max(st, axis=0, keepdims=True))
                rl = 1.0 / jnp.sum(p, axis=0, keepdims=True)
                o = jnp.dot(vt_buf[s, pl.ds(a, 32), :], p.astype(BF16), preferred_element_type=F32)
                gate = jnp.concatenate([gate_buf[pl.ds(a, 32), :]] * QT, axis=1)
                rden = 1.0 / (num_buf[g, pl.ds(ZROW + i, 1), :] + 1e-6)
                num = num_buf[g, pl.ds(pl.multiple_of(a - a_g, 16), 32), :]
                val = gate * (num * rden) + (1.0 - gate) * (o * rl)
                keep = (r32 >= off) & (r32 < off + DH)
                pltpu.store(ot_buf.at[pl.ds(a, 32), :], val, mask=keep)
                return c

            lax.fori_loop(0, _heads_in_group(g), head, 0)
        for g in range(NG):
            memory_update(s, g)
        project_out(s)
        return carry

    @pl.when(safe)
    def _():
        lax.fori_loop(0, NSEG, fast_segment, 0)

    @pl.when(jnp.logical_not(safe))
    def _():
        lax.fori_loop(0, NSEG, slow_segment, 0)

    for s in range(NSEG):
        out_copy(s).wait()


@jax.jit
def pallas_parallel_sum__memory_aug_infini_attn__moe_arch_mod__prompt_kernel(
    A_x: jax.Array,
    A_wq: jax.Array,
    A_wk: jax.Array,
    A_wv: jax.Array,
    A_wo: jax.Array,
    A_beta: jax.Array,
    B_x: jax.Array,
    B_w_r: jax.Array,
    B_w_gate: jax.Array,
    B_w_up: jax.Array,
    B_w_down: jax.Array,
):
    del B_x
    hbm = pl.BlockSpec(memory_space=pl.ANY)
    scratch = [
        pltpu.VMEM((NSEG, D, L), BF16),
        pltpu.VMEM((D, D), BF16),
        pltpu.VMEM((D, D), BF16),
        pltpu.VMEM((D, D), BF16),
        pltpu.VMEM((D, D), BF16),
        pltpu.VMEM((H,), BF16),
        pltpu.VMEM((D,), BF16),
        pltpu.VMEM((D, FF), BF16),
        pltpu.VMEM((D, FF), BF16),
        pltpu.VMEM((D, FF), BF16),
        pltpu.VMEM((PR, D), BF16),
        pltpu.VMEM((PR, D), BF16),
        pltpu.VMEM((VROWS, D), BF16),
        pltpu.VMEM((D, D), BF16),
        pltpu.VMEM((NSEG, D, L), BF16),
        pltpu.VMEM((NSEG, D, L), F32),
        pltpu.VMEM((NSEG, PR, L), BF16),
        pltpu.VMEM((NSEG, PR, L), BF16),
        pltpu.VMEM((NSEG, NG, L, 128), BF16),
        pltpu.VMEM((NSEG, PR, L), BF16),
        pltpu.VMEM((NSEG, VROWS, L), BF16),
        pltpu.VMEM((8, S), F32),
        pltpu.VMEM((D, 128), F32),
        pltpu.VMEM((NG, MROWS, 128), F32),
        pltpu.VMEM((NG, MROWS, L), F32),
        pltpu.VMEM((640, HPG * 128), U32),
        pltpu.VMEM((D, L), F32),
        pltpu.VMEM((NSEG, D, L), BF16),
        pltpu.SemaphoreType.DMA((13,)),
        pltpu.SemaphoreType.DMA((NSEG,)),
    ]
    out_t = pl.pallas_call(
        _kernel,
        out_shape=jax.ShapeDtypeStruct((1, D, S), BF16),
        in_specs=[hbm] * 10,
        out_specs=hbm,
        scratch_shapes=scratch,
        compiler_params=pltpu.CompilerParams(vmem_limit_bytes=128 * 1024 * 1024),
        name="infini_attn_moe",
    )(jnp.transpose(A_x, (0, 2, 1)), A_wq, A_wk, A_wv, A_wo, A_beta, B_w_r, B_w_gate, B_w_up,
      B_w_down.T)
    return jnp.transpose(out_t, (0, 2, 1))
```

```python
import jax
import jax.numpy as jnp
from jax import lax
import jax.experimental.pallas as pl
import jax.experimental.pallas.tpu as pltpu

F32 = jnp.float32
BF16 = jnp.bfloat16
U32 = jnp.uint32
I32 = jnp.int32

S = 2048
D = 576
H = 32
DH = 18
NSEG = 4
L = 512
FF = 4608
HPG = 7
NG = 5
QT = L // 128
GW = (128, 128, 128, 128, 80)
PR = sum(GW)
VROWS = D + 16
ZROW = 144
MROWS = 160
LOG2E = 1.4426950408889634
QSCALE = (DH ** -0.5) * LOG2E
SAFE_LOG2_RANGE = 60.0
NEG_BIG = -1e30

NT_DIMS = (((1,), (1,)), ((), ()))


def _heads_in_group(g):
    return min(HPG, H - HPG * g)


def _group_row_start(g):
    return (HPG * g * DH // 16) * 16


def _group_rows(g):
    last = (HPG * g + _heads_in_group(g)) * DH
    return -(-(last - _group_row_start(g)) // 16) * 16


def _round_bf16(x):
    return x.astype(BF16).astype(F32)


def _pad_heads_t(w):
    parts = []
    for g in range(NG):
        n = _heads_in_group(g) * DH
        parts.append(w[:, HPG * DH * g:HPG * DH * g + n])
        parts.append(jnp.zeros((D, 128 - n), w.dtype))
    return jnp.concatenate(parts, axis=1).T[0:PR]


def _phi(t):
    return jnp.where(t > 0, t + 1.0, jnp.exp(t))


def _kernel(x_hbm, wq_hbm, wk_hbm, wv_hbm, wo_hbm, beta_hbm, wr_hbm, wg_hbm, wu_hbm, wd_hbm,
            out_hbm,
            x_buf, wq_raw, wk_raw, wv_raw, wo_raw, beta_buf, wr_buf, wg_buf, wu_buf, wd_buf,
            wqt, wkt, wvt, wot, xn_buf, base, qs_buf, pq_buf, k_buf, pk_buf, vt_buf, r_buf,
            gate_buf, mt_buf, num_buf, p_buf0, p_buf1, ot_buf, out_buf, in_sems, out_sems):
    def x_copy(c):
        return pltpu.make_async_copy(x_hbm.at[0, :, pl.ds(c * L, L)], x_buf.at[c], in_sems.at[c])

    cp_wv = pltpu.make_async_copy(wv_hbm, wv_raw, in_sems.at[4])
    cp_wq = pltpu.make_async_copy(wq_hbm, wq_raw, in_sems.at[5])
    cp_wk = pltpu.make_async_copy(wk_hbm, wk_raw, in_sems.at[6])
    cp_wo = pltpu.make_async_copy(wo_hbm, wo_raw, in_sems.at[7])
    cp_wg = pltpu.make_async_copy(wg_hbm, wg_buf, in_sems.at[8])
    cp_wu = pltpu.make_async_copy(wu_hbm, wu_buf, in_sems.at[9])
    cp_wd = pltpu.make_async_copy(wd_hbm, wd_buf, in_sems.at[10])
    cp_beta = pltpu.make_async_copy(beta_hbm, beta_buf, in_sems.at[11])
    cp_wr = pltpu.make_async_copy(wr_hbm, wr_buf, in_sems.at[12])

    def out_copy(s):
        cols = pl.ds(pl.multiple_of(s * L, L), L)
        return pltpu.make_async_copy(out_buf.at[s], out_hbm.at[0, :, cols], out_sems.at[s])


    for cp in (x_copy(0), cp_wv, cp_wr, cp_wq, cp_wk, x_copy(1), x_copy(2), x_copy(3), cp_wo, cp_beta,
               cp_wg, cp_wu, cp_wd):
        cp.start()

    lane128 = lax.broadcasted_iota(I32, (128, 128), 1)
    row128 = lax.broadcasted_iota(I32, (128, 128), 0)
    causal = row128 <= lane128
    r16 = lax.broadcasted_iota(I32, (16, D), 0)

    mt_buf[...] = jnp.zeros(mt_buf.shape, F32)

    def layernorm(c):
        x = x_buf[c].astype(F32)
        mean = jnp.sum(x, axis=0, keepdims=True) * (1.0 / D)
        cen = x - mean
        var = jnp.sum(cen * cen, axis=0, keepdims=True) * (1.0 / D)
        d = _round_bf16(x - _round_bf16(mean))
        den = _round_bf16(jnp.sqrt(_round_bf16(_round_bf16(var) + 1e-5)))
        xn = (d / den).astype(BF16)
        xn_buf[c] = xn
        base[c] = x + xn.astype(F32)

    x_copy(0).wait()
    layernorm(0)
    cp_wv.wait()
    cp_wr.wait()
    wvt[0:D, :] = wv_raw[...].T
    wr_row = wr_buf[...].reshape(1, D).astype(F32)
    wvt[D:VROWS, :] = jnp.where(r16 == 0, wr_row, 0.0).astype(BF16)
    cp_wq.wait()

    def project_v(c):
        vt = jnp.dot(wvt[...], xn_buf[c], preferred_element_type=F32)
        vt_buf[c, 0:D, :] = vt[0:D].astype(BF16)
        r16l = lax.broadcasted_iota(I32, (16, L), 0)
        vt_buf[c, D:VROWS, :] = jnp.where(r16l == 1, 1.0, 0.0).astype(BF16)
        r_buf[:, c * L:(c + 1) * L] = vt[D:D + 8]

    def project_q(c):
        qt = jnp.dot(wqt[...], xn_buf[c], preferred_element_type=F32)
        qsc = qt * QSCALE
        qs_buf[c] = qsc.astype(BF16)
        pq_buf[c] = _phi(qt).astype(BF16)
        return jnp.max(jnp.abs(qsc).reshape(PR // 8, 8, L), axis=0)

    def project_k(c):
        kt = jnp.dot(wkt[...], xn_buf[c], preferred_element_type=F32)
        pk_buf[c] = _phi(kt).astype(BF16)
        for g in range(NG):
            ktg = kt[128 * g:128 * g + GW[g]]
            if GW[g] < 128:
                ktg = jnp.concatenate([ktg, jnp.zeros((128 - GW[g], L), F32)], axis=0)
            k_buf[c, g] = ktg.T.astype(BF16)
        return jnp.max(jnp.abs(kt).reshape(PR // 8, 8, L), axis=0)

    wqt[...] = _pad_heads_t(wq_raw[...].astype(F32)).astype(BF16)
    project_v(0)
    cp_wk.wait()
    x_copy(1).wait()
    wkt[...] = _pad_heads_t(wk_raw[...].astype(F32)).astype(BF16)

    aq = project_q(0)
    layernorm(1)
    ak = project_k(0)
    project_v(1)
    x_copy(2).wait()
    x_copy(3).wait()
    for c in range(1, NSEG):
        aq = jnp.maximum(aq, project_q(c))
        if c + 1 < NSEG:
            layernorm(c + 1)
        ak = jnp.maximum(ak, project_k(c))
        if c + 1 < NSEG:
            project_v(c + 1)

    logit_bound = jnp.max(aq) * jnp.max(ak) * (DH * 1.02)
    safe = logit_bound <= SAFE_LOG2_RANGE

    cp_wo.wait()
    cp_beta.wait()
    wot[...] = wo_raw[...].T
    beta_row = beta_buf[...].reshape(1, H).astype(F32)
    beta_row = jnp.concatenate([beta_row, jnp.zeros((1, 128 - H), F32)], axis=1)
    e_row = lax.broadcasted_iota(I32, (D, 128), 0)
    e_lane = lax.broadcasted_iota(I32, (D, 128), 1)
    in_head = (e_row >= e_lane * DH) & (e_row < e_lane * DH + DH)
    beta_col = jnp.sum(jnp.where(in_head, beta_row, 0.0), axis=1, keepdims=True)
    gate_buf[...] = jnp.broadcast_to(jax.nn.sigmoid(beta_col), (D, 128))


    r = _round_bf16(r_buf[0:1, :])
    tok = lax.broadcasted_iota(I32, (1, S), 1).astype(F32)
    m1 = jnp.max(r)
    i1 = jnp.min(jnp.where(r == m1, tok, float(S)))
    r_rest = jnp.where(tok == i1, -jnp.inf, r)
    m2 = jnp.max(r_rest)
    i2 = jnp.min(jnp.where(r_rest == m2, tok, float(S)))
    i1 = jnp.clip(i1.astype(I32), 0, S - 1)
    i2 = jnp.clip(i2.astype(I32), 0, S - 1)

    sel_row = lax.broadcasted_iota(I32, (16, 128), 0)
    sel_lane = lax.broadcasted_iota(I32, (16, 128), 1)

    def token_tile(i):
        return i // L, pl.ds(pl.multiple_of(((i % L) // 128) * 128, 128), 128)

    def pick(i, slot):
        seg, cols = token_tile(i)
        onehot = jnp.where((sel_row == slot) & (sel_lane == i % 128), 1.0, 0.0).astype(BF16)
        return lax.dot_general(onehot, xn_buf[seg, :, cols], NT_DIMS, preferred_element_type=F32)

    xs = (pick(i1, 0) + pick(i2, 1)).astype(BF16)
    cp_wg.wait()
    cp_wu.wait()
    cp_wd.wait()

    def expert_chunk(lo, hi):
        hg = jnp.dot(xs, wg_buf[:, lo:hi], preferred_element_type=F32)
        hu = jnp.dot(xs, wu_buf[:, lo:hi], preferred_element_type=F32)
        hh = (jax.nn.silu(hg) * hu).astype(BF16)
        return lax.dot_general(hh, wd_buf[:, lo:hi], NT_DIMS, preferred_element_type=F32)

    def expert_scatter(y):
        y = y * jax.nn.sigmoid(jnp.where(r16 == 0, m1, m2))
        yt = jnp.concatenate([y, jnp.zeros((128 - 16, D), F32)], axis=0).T
        lane_d = lax.broadcasted_iota(I32, (D, 128), 1)
        for slot, i in ((0, i1), (1, i2)):
            seg, cols = token_tile(i)
            col = jnp.sum(jnp.where(lane_d == slot, yt, 0.0), axis=1, keepdims=True)
            base[seg, :, cols] = base[seg, :, cols] + jnp.where(lane_d == i % 128, col, 0.0)

    def memory_read(s, g):
        rg = _group_rows(g)
        gw = GW[g]
        lhs = jnp.concatenate([mt_buf[g, 0:rg, 0:gw], mt_buf[g, ZROW:MROWS, 0:gw]], axis=0).astype(BF16)
        res = jnp.dot(lhs, pq_buf[s, 128 * g:128 * g + gw, :], preferred_element_type=F32)
        num_buf[g, 0:rg, :] = res[0:rg]
        num_buf[g, ZROW:MROWS, :] = res[rg:rg + 16]

    def memory_update(s, g):
        rg = _group_rows(g)
        a_g = _group_row_start(g)
        gw = GW[g]
        lhs = jnp.concatenate([vt_buf[s, a_g:a_g + rg, :], vt_buf[s, D:VROWS, :]], axis=0)
        upd = lax.dot_general(lhs, pk_buf[s, 128 * g:128 * g + gw, :], NT_DIMS,
                              preferred_element_type=F32)
        er = lax.broadcasted_iota(I32, (rg, gw), 0) + (a_g - HPG * DH * g)
        el = lax.broadcasted_iota(I32, (rg, gw), 1)
        same_head = None
        for i in range(_heads_in_group(g)):
            t = ((er >= DH * i) & (er < DH * (i + 1)) & (el >= DH * i) & (el < DH * (i + 1)))
            same_head = t if same_head is None else (same_head | t)
        mt_buf[g, 0:rg, 0:gw] = mt_buf[g, 0:rg, 0:gw] + jnp.where(same_head, upd[0:rg], 0.0)
        zr = lax.broadcasted_iota(I32, (8, gw), 0)
        zl = lax.broadcasted_iota(I32, (8, gw), 1)
        zmask = (zl >= zr * DH) & (zl < zr * DH + DH) & (zr < _heads_in_group(g))
        zs = upd[rg + 1:rg + 2]
        mt_buf[g, ZROW:ZROW + 8, 0:gw] = mt_buf[g, ZROW:ZROW + 8, 0:gw] + jnp.where(zmask, zs, 0.0)

    def project_out(s):
        attn = jnp.dot(wot[...], ot_buf[...].astype(BF16), preferred_element_type=F32)
        return base[s] + attn

    def emit(s, val):
        out_buf[s] = val.astype(BF16)
        out_copy(s).start()

    zero = lax.shift_right_logical(i1, 16)

    def prow(start, size):
        return pl.ds(pl.multiple_of(zero + start, 8), size)

    P_OFFS = (0, 128, 384, 768)

    def fast_scores(s, g):
        nh = _heads_in_group(g)
        gw = GW[g]
        pb = (p_buf0, p_buf1)[(s * NG + g) % 2]
        rowg = lax.broadcasted_iota(I32, (gw, 128), 0)
        for j in range(QT - 1, -1, -1):
            n = 128 * (j + 1)
            q = qs_buf[s, 128 * g:128 * g + gw, 128 * j:128 * (j + 1)].astype(F32)
            qm = jnp.concatenate(
                [jnp.where((rowg >= DH * i) & (rowg < DH * (i + 1)), q, 0.0) for i in range(nh)],
                axis=1).astype(BF16)
            st = jnp.dot(k_buf[s, g, 0:n, 0:gw], qm, preferred_element_type=F32)
            p = jnp.exp2(st)
            causal_w = jnp.concatenate([causal] * nh, axis=1)
            p_diag = jnp.where(causal_w, p[n - 128:], 0.0)
            p = jnp.concatenate([p[:n - 128], p_diag], axis=0) if j > 0 else p_diag
            pb[P_OFFS[j] // 2:(P_OFFS[j] + n) // 2, 0:nh * 128] = pltpu.bitcast(p.astype(BF16), U32)

    def fast_values(s, g):
        nh = _heads_in_group(g)
        a_g = _group_row_start(g)
        pb = (p_buf0, p_buf1)[(s * NG + g) % 2]
        for j in range(QT - 1, -1, -1):
            n = 128 * (j + 1)
            cols = slice(128 * j, 128 * (j + 1))
            for i in range(nh):
                h = HPG * g + i
                a = (h * DH // 16) * 16
                off = h * DH - a
                p = pltpu.bitcast(pb[prow(P_OFFS[j] // 2, n // 2), 128 * i:128 * (i + 1)], BF16)
                ones_row = 0 if off > 0 else 31
                r32n = lax.broadcasted_iota(I32, (32, n), 0)
                lhs = jnp.where(r32n == ones_row, 1.0, vt_buf[s, a:a + 32, 0:n].astype(F32)).astype(BF16)
                o = jnp.dot(lhs, p, preferred_element_type=F32)
                lo = (off // 8) * 8
                hi = -(-(off + DH) // 8) * 8
                gate = gate_buf[a + lo:a + hi, :]
                rl = 1.0 / o[ones_row:ones_row + 1]
                val = (1.0 - gate) * (o[lo:hi] * rl)
                if s > 0:
                    rden = 1.0 / (num_buf[g, ZROW + i:ZROW + i + 1, cols] + 1e-6)
                    num = num_buf[g, a - a_g + lo:a - a_g + hi, cols]
                    val = gate * (num * rden) + val
                ot_buf[a + off:a + off + DH, cols] = val[off - lo:off - lo + DH]

    def fast_path():
        nchunk = 12
        cw = FF // nchunk
        y = None
        steps = [(s, g) for s in range(NSEG) for g in range(NG)]
        fast_scores(0, 0)
        for t, (s, g) in enumerate(steps):
            if t + 1 < len(steps):
                fast_scores(*steps[t + 1])
            if s > 0:
                memory_read(s, g)
            fast_values(s, g)
            if s + 1 < NSEG:
                memory_update(s, g)
            if s < NSEG - 1 and g < NG - 1:
                ci = s * (NG - 1) + g
                yc = expert_chunk(ci * cw, (ci + 1) * cw)
                y = yc if y is None else y + yc
            if g == NG - 1:
                if s < NSEG - 1:
                    base[s] = project_out(s)
                if s == NSEG - 2:
                    expert_scatter(y)
                    for u in range(NSEG - 1):
                        emit(u, base[u])
        emit(NSEG - 1, project_out(NSEG - 1))

    def slow_segment(s, carry):
        for g in range(NG):
            memory_read(s, g)
        key_i = lax.broadcasted_iota(I32, (L, L), 0)
        qry_i = lax.broadcasted_iota(I32, (L, L), 1)
        r32 = lax.broadcasted_iota(I32, (32, L), 0)
        for g in range(NG):
            gw = GW[g]
            a_g = _group_row_start(g)
            rowg = lax.broadcasted_iota(I32, (gw, L), 0)

            def head(i, c, g=g, gw=gw, a_g=a_g, rowg=rowg):
                h = HPG * g + i
                a = pl.multiple_of((h * DH // 16) * 16, 16)
                off = h * DH - a
                q = qs_buf[s, 128 * g:128 * g + gw, :].astype(F32)
                qm = jnp.where((rowg >= DH * i) & (rowg < DH * (i + 1)), q, 0.0).astype(BF16)
                st = jnp.dot(k_buf[s, g, :, 0:gw], qm, preferred_element_type=F32)
                st = jnp.where(key_i <= qry_i, st, NEG_BIG)
                p = jnp.exp2(st - jnp.max(st, axis=0, keepdims=True))
                rl = 1.0 / jnp.sum(p, axis=0, keepdims=True)
                o = jnp.dot(vt_buf[s, pl.ds(a, 32), :], p.astype(BF16), preferred_element_type=F32)
                gate = jnp.concatenate([gate_buf[pl.ds(a, 32), :]] * QT, axis=1)
                rden = 1.0 / (num_buf[g, pl.ds(ZROW + i, 1), :] + 1e-6)
                num = num_buf[g, pl.ds(pl.multiple_of(a - a_g, 16), 32), :]
                val = gate * (num * rden) + (1.0 - gate) * (o * rl)
                keep = (r32 >= off) & (r32 < off + DH)
                pltpu.store(ot_buf.at[pl.ds(a, 32), :], val, mask=keep)
                return c

            lax.fori_loop(0, _heads_in_group(g), head, 0)
        for g in range(NG):
            memory_update(s, g)
        emit(s, project_out(s))
        return carry

    @pl.when(safe)
    def _():
        fast_path()

    @pl.when(jnp.logical_not(safe))
    def _():
        expert_scatter(expert_chunk(0, FF))
        lax.fori_loop(0, NSEG, slow_segment, 0)

    for s in range(NSEG):
        out_copy(s).wait()


@jax.jit
def pallas_parallel_sum__memory_aug_infini_attn__moe_arch_mod__prompt_kernel(
    A_x: jax.Array,
    A_wq: jax.Array,
    A_wk: jax.Array,
    A_wv: jax.Array,
    A_wo: jax.Array,
    A_beta: jax.Array,
    B_x: jax.Array,
    B_w_r: jax.Array,
    B_w_gate: jax.Array,
    B_w_up: jax.Array,
    B_w_down: jax.Array,
):
    del B_x
    hbm = pl.BlockSpec(memory_space=pl.ANY)
    scratch = [
        pltpu.VMEM((NSEG, D, L), BF16),
        pltpu.VMEM((D, D), BF16),
        pltpu.VMEM((D, D), BF16),
        pltpu.VMEM((D, D), BF16),
        pltpu.VMEM((D, D), BF16),
        pltpu.VMEM((H,), BF16),
        pltpu.VMEM((D,), BF16),
        pltpu.VMEM((D, FF), BF16),
        pltpu.VMEM((D, FF), BF16),
        pltpu.VMEM((D, FF), BF16),
        pltpu.VMEM((PR, D), BF16),
        pltpu.VMEM((PR, D), BF16),
        pltpu.VMEM((VROWS, D), BF16),
        pltpu.VMEM((D, D), BF16),
        pltpu.VMEM((NSEG, D, L), BF16),
        pltpu.VMEM((NSEG, D, L), F32),
        pltpu.VMEM((NSEG, PR, L), BF16),
        pltpu.VMEM((NSEG, PR, L), BF16),
        pltpu.VMEM((NSEG, NG, L, 128), BF16),
        pltpu.VMEM((NSEG, PR, L), BF16),
        pltpu.VMEM((NSEG, VROWS, L), BF16),
        pltpu.VMEM((8, S), F32),
        pltpu.VMEM((D, 128), F32),
        pltpu.VMEM((NG, MROWS, 128), F32),
        pltpu.VMEM((NG, MROWS, L), F32),
        pltpu.VMEM((640, HPG * 128), U32),
        pltpu.VMEM((640, HPG * 128), U32),
        pltpu.VMEM((D, L), F32),
        pltpu.VMEM((NSEG, D, L), BF16),
        pltpu.SemaphoreType.DMA((13,)),
        pltpu.SemaphoreType.DMA((NSEG,)),
    ]
    out_t = pl.pallas_call(
        _kernel,
        out_shape=jax.ShapeDtypeStruct((1, D, S), BF16),
        in_specs=[hbm] * 10,
        out_specs=hbm,
        scratch_shapes=scratch,
        compiler_params=pltpu.CompilerParams(vmem_limit_bytes=128 * 1024 * 1024),
        name="infini_attn_moe",
    )(jnp.transpose(A_x, (0, 2, 1)), A_wq, A_wk, A_wv, A_wo, A_beta, B_w_r, B_w_gate, B_w_up,
      B_w_down.T)
    return jnp.transpose(out_t, (0, 2, 1))
```

```python
import jax
import jax.numpy as jnp
from jax import lax
import jax.experimental.pallas as pl
import jax.experimental.pallas.tpu as pltpu

F32 = jnp.float32
BF16 = jnp.bfloat16
U32 = jnp.uint32
I32 = jnp.int32

S = 2048
D = 576
H = 32
DH = 18
NSEG = 4
L = 512
FF = 4608
HPG = 7
NG = 5
QT = L // 128
GW = (128, 128, 128, 128, 80)
PR = sum(GW)
VROWS = D + 16
ZROW = 144
MROWS = 160
LOG2E = 1.4426950408889634
QSCALE = (DH ** -0.5) * LOG2E
SAFE_LOG2_RANGE = 60.0
NEG_BIG = -1e30

NT_DIMS = (((1,), (1,)), ((), ()))


def _heads_in_group(g):
    return min(HPG, H - HPG * g)


def _group_row_start(g):
    return (HPG * g * DH // 16) * 16


def _group_rows(g):
    last = (HPG * g + _heads_in_group(g)) * DH
    return -(-(last - _group_row_start(g)) // 16) * 16


def _round_bf16(x):
    return x.astype(BF16).astype(F32)


def _pad_heads_t(w):
    parts = []
    for g in range(NG):
        n = _heads_in_group(g) * DH
        parts.append(w[:, HPG * DH * g:HPG * DH * g + n])
        parts.append(jnp.zeros((D, 128 - n), w.dtype))
    return jnp.concatenate(parts, axis=1).T[0:PR]


def _phi(t):
    return jnp.where(t > 0, t + 1.0, jnp.exp(t))


def _kernel(x_hbm, wq_hbm, wk_hbm, wv_hbm, wo_hbm, beta_hbm, wr_hbm, wg_hbm, wu_hbm, wd_hbm,
            out_hbm,
            x_buf, wq_raw, wk_raw, wv_raw, wo_raw, beta_buf, wr_buf, wg_buf, wu_buf, wd_buf,
            wqt, wkt, wvt, wot, xn_buf, base, qs_buf, pq_buf, k_buf, pk_buf, vt_buf, r_buf,
            gate_buf, mt_buf, num_buf, p_buf0, p_buf1, ot_buf, out_buf, in_sems, out_sems):
    def x_copy(c):
        return pltpu.make_async_copy(x_hbm.at[0, :, pl.ds(c * L, L)], x_buf.at[c], in_sems.at[c])

    cp_wv = pltpu.make_async_copy(wv_hbm, wv_raw, in_sems.at[4])
    cp_wq = pltpu.make_async_copy(wq_hbm, wq_raw, in_sems.at[5])
    cp_wk = pltpu.make_async_copy(wk_hbm, wk_raw, in_sems.at[6])
    cp_wo = pltpu.make_async_copy(wo_hbm, wo_raw, in_sems.at[7])
    cp_wg = pltpu.make_async_copy(wg_hbm, wg_buf, in_sems.at[8])
    cp_wu = pltpu.make_async_copy(wu_hbm, wu_buf, in_sems.at[9])
    cp_wd = pltpu.make_async_copy(wd_hbm, wd_buf, in_sems.at[10])
    cp_beta = pltpu.make_async_copy(beta_hbm, beta_buf, in_sems.at[11])
    cp_wr = pltpu.make_async_copy(wr_hbm, wr_buf, in_sems.at[12])

    def out_copy(s):
        cols = pl.ds(pl.multiple_of(s * L, L), L)
        return pltpu.make_async_copy(out_buf.at[s], out_hbm.at[0, :, cols], out_sems.at[s])


    for cp in (x_copy(0), cp_wv, cp_wr, cp_wq, cp_wk, x_copy(1), x_copy(2), x_copy(3), cp_wo, cp_beta,
               cp_wg, cp_wu, cp_wd):
        cp.start()

    lane128 = lax.broadcasted_iota(I32, (128, 128), 1)
    row128 = lax.broadcasted_iota(I32, (128, 128), 0)
    causal = row128 <= lane128
    r16 = lax.broadcasted_iota(I32, (16, D), 0)

    mt_buf[...] = jnp.zeros(mt_buf.shape, F32)

    def layernorm(c):
        x = x_buf[c].astype(F32)
        mean = jnp.sum(x, axis=0, keepdims=True) * (1.0 / D)
        cen = x - mean
        var = jnp.sum(cen * cen, axis=0, keepdims=True) * (1.0 / D)
        d = _round_bf16(x - _round_bf16(mean))
        den = _round_bf16(jnp.sqrt(_round_bf16(_round_bf16(var) + 1e-5)))
        xn = (d / den).astype(BF16)
        xn_buf[c] = xn
        base[c] = x + xn.astype(F32)

    x_copy(0).wait()
    layernorm(0)
    cp_wv.wait()
    cp_wr.wait()
    wvt[0:D, :] = wv_raw[...].T
    wr_row = wr_buf[...].reshape(1, D).astype(F32)
    wvt[D:VROWS, :] = jnp.where(r16 == 0, wr_row, 0.0).astype(BF16)
    cp_wq.wait()

    def project_v(c):
        vt = jnp.dot(wvt[...], xn_buf[c], preferred_element_type=F32)
        vt_buf[c, 0:D, :] = vt[0:D].astype(BF16)
        r16l = lax.broadcasted_iota(I32, (16, L), 0)
        vt_buf[c, D:VROWS, :] = jnp.where(r16l == 1, 1.0, 0.0).astype(BF16)
        r_buf[:, c * L:(c + 1) * L] = vt[D:D + 8]

    def project_q(c):
        qt = jnp.dot(wqt[...], xn_buf[c], preferred_element_type=F32)
        qsc = qt * QSCALE
        qs_buf[c] = qsc.astype(BF16)
        pq_buf[c] = _phi(qt).astype(BF16)
        return jnp.max(jnp.abs(qsc).reshape(PR // 8, 8, L), axis=0)

    def project_k(c):
        kt = jnp.dot(wkt[...], xn_buf[c], preferred_element_type=F32)
        pk_buf[c] = _phi(kt).astype(BF16)
        for g in range(NG):
            ktg = kt[128 * g:128 * g + GW[g]]
            if GW[g] < 128:
                ktg = jnp.concatenate([ktg, jnp.zeros((128 - GW[g], L), F32)], axis=0)
            k_buf[c, g] = ktg.T.astype(BF16)
        return jnp.max(jnp.abs(kt).reshape(PR // 8, 8, L), axis=0)

    wqt[...] = _pad_heads_t(wq_raw[...].astype(F32)).astype(BF16)
    project_v(0)
    cp_wk.wait()
    x_copy(1).wait()
    wkt[...] = _pad_heads_t(wk_raw[...].astype(F32)).astype(BF16)

    aq = project_q(0)
    layernorm(1)
    ak = project_k(0)
    project_v(1)
    x_copy(2).wait()
    x_copy(3).wait()
    for c in range(1, NSEG):
        aq = jnp.maximum(aq, project_q(c))
        if c + 1 < NSEG:
            layernorm(c + 1)
        ak = jnp.maximum(ak, project_k(c))
        if c + 1 < NSEG:
            project_v(c + 1)

    logit_bound = jnp.max(aq) * jnp.max(ak) * (DH * 1.02)
    safe = logit_bound <= SAFE_LOG2_RANGE

    cp_wo.wait()
    cp_beta.wait()
    wot[...] = wo_raw[...].T
    beta_row = beta_buf[...].reshape(1, H).astype(F32)
    beta_row = jnp.concatenate([beta_row, jnp.zeros((1, 128 - H), F32)], axis=1)
    e_row = lax.broadcasted_iota(I32, (D, 128), 0)
    e_lane = lax.broadcasted_iota(I32, (D, 128), 1)
    in_head = (e_row >= e_lane * DH) & (e_row < e_lane * DH + DH)
    beta_col = jnp.sum(jnp.where(in_head, beta_row, 0.0), axis=1, keepdims=True)
    gate_buf[...] = jnp.broadcast_to(jax.nn.sigmoid(beta_col), (D, 128))


    r = _round_bf16(r_buf[0:1, :])
    tok = lax.broadcasted_iota(I32, (1, S), 1).astype(F32)
    m1 = jnp.max(r)
    i1 = jnp.min(jnp.where(r == m1, tok, float(S)))
    r_rest = jnp.where(tok == i1, -jnp.inf, r)
    m2 = jnp.max(r_rest)
    i2 = jnp.min(jnp.where(r_rest == m2, tok, float(S)))
    i1 = jnp.clip(i1.astype(I32), 0, S - 1)
    i2 = jnp.clip(i2.astype(I32), 0, S - 1)

    sel_row = lax.broadcasted_iota(I32, (16, 128), 0)
    sel_lane = lax.broadcasted_iota(I32, (16, 128), 1)

    def token_tile(i):
        return i // L, pl.ds(pl.multiple_of(((i % L) // 128) * 128, 128), 128)

    def pick(i, slot):
        seg, cols = token_tile(i)
        onehot = jnp.where((sel_row == slot) & (sel_lane == i % 128), 1.0, 0.0).astype(BF16)
        return lax.dot_general(onehot, xn_buf[seg, :, cols], NT_DIMS, preferred_element_type=F32)

    xs = (pick(i1, 0) + pick(i2, 1)).astype(BF16)
    cp_wg.wait()
    cp_wu.wait()
    cp_wd.wait()

    def expert_chunk(lo, hi):
        hg = jnp.dot(xs, wg_buf[:, lo:hi], preferred_element_type=F32)
        hu = jnp.dot(xs, wu_buf[:, lo:hi], preferred_element_type=F32)
        hh = (jax.nn.silu(hg) * hu).astype(BF16)
        return lax.dot_general(hh, wd_buf[:, lo:hi], NT_DIMS, preferred_element_type=F32)

    def expert_stream(result):
        kmain = 512
        y_tiles = [None] * 5
        for c0 in range(0, FF, 512):
            rem = []
            for w_ref in (wg_buf, wu_buf):
                rem.append(jnp.dot(xs[:, kmain:D], w_ref[kmain:D, c0:c0 + 512], preferred_element_type=F32))
                yield
            hs = []
            for f0 in range(c0, c0 + 512, 128):
                pre = []
                for w_ref, r in zip((wg_buf, wu_buf), rem):
                    pre.append(jnp.dot(xs[:, 0:kmain], w_ref[0:kmain, f0:f0 + 128], preferred_element_type=F32)
                               + r[:, f0 - c0:f0 - c0 + 128])
                    yield
                hs.append(jax.nn.silu(pre[0]) * pre[1])
            hh = jnp.concatenate(hs, axis=1).astype(BF16)
            for e in range(5):
                e_hi = min(128 * (e + 1), D)
                part = lax.dot_general(hh, wd_buf[128 * e:e_hi, c0:c0 + 512], NT_DIMS,
                                       preferred_element_type=F32)
                y_tiles[e] = part if y_tiles[e] is None else y_tiles[e] + part
                yield
        result.append(jnp.concatenate(y_tiles, axis=1))

    def expert_scatter(y):
        y = y * jax.nn.sigmoid(jnp.where(r16 == 0, m1, m2))
        yt = jnp.concatenate([y, jnp.zeros((128 - 16, D), F32)], axis=0).T
        lane_d = lax.broadcasted_iota(I32, (D, 128), 1)
        for slot, i in ((0, i1), (1, i2)):
            seg, cols = token_tile(i)
            col = jnp.sum(jnp.where(lane_d == slot, yt, 0.0), axis=1, keepdims=True)
            base[seg, :, cols] = base[seg, :, cols] + jnp.where(lane_d == i % 128, col, 0.0)

    def memory_read(s, g):
        rg = _group_rows(g)
        gw = GW[g]
        lhs = jnp.concatenate([mt_buf[g, 0:rg, 0:gw], mt_buf[g, ZROW:MROWS, 0:gw]], axis=0).astype(BF16)
        res = jnp.dot(lhs, pq_buf[s, 128 * g:128 * g + gw, :], preferred_element_type=F32)
        num_buf[g, 0:rg, :] = res[0:rg]
        num_buf[g, ZROW:MROWS, :] = res[rg:rg + 16]

    def memory_update(s, g):
        rg = _group_rows(g)
        a_g = _group_row_start(g)
        gw = GW[g]
        lhs = jnp.concatenate([vt_buf[s, a_g:a_g + rg, :], vt_buf[s, D:VROWS, :]], axis=0)
        upd = lax.dot_general(lhs, pk_buf[s, 128 * g:128 * g + gw, :], NT_DIMS,
                              preferred_element_type=F32)
        er = lax.broadcasted_iota(I32, (rg, gw), 0) + (a_g - HPG * DH * g)
        el = lax.broadcasted_iota(I32, (rg, gw), 1)
        same_head = None
        for i in range(_heads_in_group(g)):
            t = ((er >= DH * i) & (er < DH * (i + 1)) & (el >= DH * i) & (el < DH * (i + 1)))
            same_head = t if same_head is None else (same_head | t)
        mt_buf[g, 0:rg, 0:gw] = mt_buf[g, 0:rg, 0:gw] + jnp.where(same_head, upd[0:rg], 0.0)
        zr = lax.broadcasted_iota(I32, (8, gw), 0)
        zl = lax.broadcasted_iota(I32, (8, gw), 1)
        zmask = (zl >= zr * DH) & (zl < zr * DH + DH) & (zr < _heads_in_group(g))
        zs = upd[rg + 1:rg + 2]
        mt_buf[g, ZROW:ZROW + 8, 0:gw] = mt_buf[g, ZROW:ZROW + 8, 0:gw] + jnp.where(zmask, zs, 0.0)

    def project_out(s):
        attn = jnp.dot(wot[...], ot_buf[...].astype(BF16), preferred_element_type=F32)
        return base[s] + attn

    def emit(s, val):
        out_buf[s] = val.astype(BF16)
        out_copy(s).start()

    zero = lax.shift_right_logical(i1, 16)

    def prow(start, size):
        return pl.ds(pl.multiple_of(zero + start, 8), size)

    P_OFFS = (0, 128, 384, 768)

    def fast_scores(s, g, hook):
        nh = _heads_in_group(g)
        gw = GW[g]
        pb = (p_buf0, p_buf1)[(s * NG + g) % 2]
        rowg = lax.broadcasted_iota(I32, (gw, 128), 0)
        for j in range(QT - 1, -1, -1):
            n = 128 * (j + 1)
            q = qs_buf[s, 128 * g:128 * g + gw, 128 * j:128 * (j + 1)].astype(F32)
            for h0, h1 in ((0, 4), (4, nh)):
                if h1 <= h0:
                    continue
                qm = jnp.concatenate(
                    [jnp.where((rowg >= DH * i) & (rowg < DH * (i + 1)), q, 0.0) for i in range(h0, h1)],
                    axis=1).astype(BF16)
                st = jnp.dot(k_buf[s, g, 0:n, 0:gw], qm, preferred_element_type=F32)
                p = jnp.exp2(st)
                causal_w = jnp.concatenate([causal] * (h1 - h0), axis=1)
                p_diag = jnp.where(causal_w, p[n - 128:], 0.0)
                p = jnp.concatenate([p[:n - 128], p_diag], axis=0) if j > 0 else p_diag
                pb[P_OFFS[j] // 2:(P_OFFS[j] + n) // 2, h0 * 128:h1 * 128] = pltpu.bitcast(p.astype(BF16), U32)
                hook()

    def fast_values(s, g):
        nh = _heads_in_group(g)
        a_g = _group_row_start(g)
        pb = (p_buf0, p_buf1)[(s * NG + g) % 2]
        for j in range(QT - 1, -1, -1):
            n = 128 * (j + 1)
            cols = slice(128 * j, 128 * (j + 1))
            for i in range(nh):
                h = HPG * g + i
                a = (h * DH // 16) * 16
                off = h * DH - a
                p = pltpu.bitcast(pb[prow(P_OFFS[j] // 2, n // 2), 128 * i:128 * (i + 1)], BF16)
                ones_row = 0 if off > 0 else 31
                r32n = lax.broadcasted_iota(I32, (32, n), 0)
                lhs = jnp.where(r32n == ones_row, 1.0, vt_buf[s, a:a + 32, 0:n].astype(F32)).astype(BF16)
                o = jnp.dot(lhs, p, preferred_element_type=F32)
                lo = (off // 8) * 8
                hi = -(-(off + DH) // 8) * 8
                gate = gate_buf[a + lo:a + hi, :]
                rl = 1.0 / o[ones_row:ones_row + 1]
                val = (1.0 - gate) * (o[lo:hi] * rl)
                if s > 0:
                    rden = 1.0 / (num_buf[g, ZROW + i:ZROW + i + 1, cols] + 1e-6)
                    num = num_buf[g, a - a_g + lo:a - a_g + hi, cols]
                    val = gate * (num * rden) + val
                ot_buf[a + off:a + off + DH, cols] = val[off - lo:off - lo + DH]

    def fast_path():
        result = []
        stream = expert_stream(result)

        def hook():
            next(stream, None)

        steps = [(s, g) for s in range(NSEG) for g in range(NG)]
        fast_scores(0, 0, hook)
        for t, (s, g) in enumerate(steps):
            if t + 1 < len(steps):
                fast_scores(*steps[t + 1], hook)
            if s > 0:
                memory_read(s, g)
                hook()
            fast_values(s, g)
            if s + 1 < NSEG:
                memory_update(s, g)
                hook()
            if g == NG - 1:
                if s < NSEG - 1:
                    base[s] = project_out(s)
                    hook()
                if s == NSEG - 2:
                    for _ in stream:
                        pass
                    expert_scatter(result[0])
                    for u in range(NSEG - 1):
                        emit(u, base[u])
        emit(NSEG - 1, project_out(NSEG - 1))

    def slow_segment(s, carry):
        for g in range(NG):
            memory_read(s, g)
        key_i = lax.broadcasted_iota(I32, (L, L), 0)
        qry_i = lax.broadcasted_iota(I32, (L, L), 1)
        r32 = lax.broadcasted_iota(I32, (32, L), 0)
        for g in range(NG):
            gw = GW[g]
            a_g = _group_row_start(g)
            rowg = lax.broadcasted_iota(I32, (gw, L), 0)

            def head(i, c, g=g, gw=gw, a_g=a_g, rowg=rowg):
                h = HPG * g + i
                a = pl.multiple_of((h * DH // 16) * 16, 16)
                off = h * DH - a
                q = qs_buf[s, 128 * g:128 * g + gw, :].astype(F32)
                qm = jnp.where((rowg >= DH * i) & (rowg < DH * (i + 1)), q, 0.0).astype(BF16)
                st = jnp.dot(k_buf[s, g, :, 0:gw], qm, preferred_element_type=F32)
                st = jnp.where(key_i <= qry_i, st, NEG_BIG)
                p = jnp.exp2(st - jnp.max(st, axis=0, keepdims=True))
                rl = 1.0 / jnp.sum(p, axis=0, keepdims=True)
                o = jnp.dot(vt_buf[s, pl.ds(a, 32), :], p.astype(BF16), preferred_element_type=F32)
                gate = jnp.concatenate([gate_buf[pl.ds(a, 32), :]] * QT, axis=1)
                rden = 1.0 / (num_buf[g, pl.ds(ZROW + i, 1), :] + 1e-6)
                num = num_buf[g, pl.ds(pl.multiple_of(a - a_g, 16), 32), :]
                val = gate * (num * rden) + (1.0 - gate) * (o * rl)
                keep = (r32 >= off) & (r32 < off + DH)
                pltpu.store(ot_buf.at[pl.ds(a, 32), :], val, mask=keep)
                return c

            lax.fori_loop(0, _heads_in_group(g), head, 0)
        for g in range(NG):
            memory_update(s, g)
        emit(s, project_out(s))
        return carry

    @pl.when(safe)
    def _():
        fast_path()

    @pl.when(jnp.logical_not(safe))
    def _():
        expert_scatter(expert_chunk(0, FF))
        lax.fori_loop(0, NSEG, slow_segment, 0)

    for s in range(NSEG):
        out_copy(s).wait()


@jax.jit
def pallas_parallel_sum__memory_aug_infini_attn__moe_arch_mod__prompt_kernel(
    A_x: jax.Array,
    A_wq: jax.Array,
    A_wk: jax.Array,
    A_wv: jax.Array,
    A_wo: jax.Array,
    A_beta: jax.Array,
    B_x: jax.Array,
    B_w_r: jax.Array,
    B_w_gate: jax.Array,
    B_w_up: jax.Array,
    B_w_down: jax.Array,
):
    del B_x
    hbm = pl.BlockSpec(memory_space=pl.ANY)
    scratch = [
        pltpu.VMEM((NSEG, D, L), BF16),
        pltpu.VMEM((D, D), BF16),
        pltpu.VMEM((D, D), BF16),
        pltpu.VMEM((D, D), BF16),
        pltpu.VMEM((D, D), BF16),
        pltpu.VMEM((H,), BF16),
        pltpu.VMEM((D,), BF16),
        pltpu.VMEM((D, FF), BF16),
        pltpu.VMEM((D, FF), BF16),
        pltpu.VMEM((D, FF), BF16),
        pltpu.VMEM((PR, D), BF16),
        pltpu.VMEM((PR, D), BF16),
        pltpu.VMEM((VROWS, D), BF16),
        pltpu.VMEM((D, D), BF16),
        pltpu.VMEM((NSEG, D, L), BF16),
        pltpu.VMEM((NSEG, D, L), F32),
        pltpu.VMEM((NSEG, PR, L), BF16),
        pltpu.VMEM((NSEG, PR, L), BF16),
        pltpu.VMEM((NSEG, NG, L, 128), BF16),
        pltpu.VMEM((NSEG, PR, L), BF16),
        pltpu.VMEM((NSEG, VROWS, L), BF16),
        pltpu.VMEM((8, S), F32),
        pltpu.VMEM((D, 128), F32),
        pltpu.VMEM((NG, MROWS, 128), F32),
        pltpu.VMEM((NG, MROWS, L), F32),
        pltpu.VMEM((640, HPG * 128), U32),
        pltpu.VMEM((640, HPG * 128), U32),
        pltpu.VMEM((D, L), F32),
        pltpu.VMEM((NSEG, D, L), BF16),
        pltpu.SemaphoreType.DMA((13,)),
        pltpu.SemaphoreType.DMA((NSEG,)),
    ]
    out_t = pl.pallas_call(
        _kernel,
        out_shape=jax.ShapeDtypeStruct((1, D, S), BF16),
        in_specs=[hbm] * 10,
        out_specs=hbm,
        scratch_shapes=scratch,
        compiler_params=pltpu.CompilerParams(vmem_limit_bytes=128 * 1024 * 1024),
        name="infini_attn_moe",
    )(jnp.transpose(A_x, (0, 2, 1)), A_wq, A_wk, A_wv, A_wo, A_beta, B_w_r, B_w_gate, B_w_up,
      B_w_down.T)
    return jnp.transpose(out_t, (0, 2, 1))
```

```python
import jax
import jax.numpy as jnp
from jax import lax
import jax.experimental.pallas as pl
import jax.experimental.pallas.tpu as pltpu

F32 = jnp.float32
BF16 = jnp.bfloat16
U32 = jnp.uint32
I32 = jnp.int32

S = 2048
D = 576
H = 32
DH = 18
NSEG = 4
L = 512
FF = 4608
HPG = 7
NG = 5
QT = L // 128
GW = (128, 128, 128, 128, 80)
PR = sum(GW)
VROWS = D + 16
ZROW = 144
MROWS = 160
LOG2E = 1.4426950408889634
QSCALE = (DH ** -0.5) * LOG2E
SAFE_LOG2_RANGE = 60.0
NEG_BIG = -1e30

NT_DIMS = (((1,), (1,)), ((), ()))


def _heads_in_group(g):
    return min(HPG, H - HPG * g)


def _group_row_start(g):
    return (HPG * g * DH // 16) * 16


def _group_rows(g):
    last = (HPG * g + _heads_in_group(g)) * DH
    return -(-(last - _group_row_start(g)) // 16) * 16


def _round_bf16(x):
    return x.astype(BF16).astype(F32)


def _pad_heads_t(w):
    parts = []
    for g in range(NG):
        n = _heads_in_group(g) * DH
        parts.append(w[:, HPG * DH * g:HPG * DH * g + n])
        parts.append(jnp.zeros((D, 128 - n), w.dtype))
    return jnp.concatenate(parts, axis=1).T[0:PR]


def _phi(t):
    return jnp.where(t > 0, t + 1.0, jnp.exp(t))


def _kernel(x_hbm, wq_hbm, wk_hbm, wv_hbm, wo_hbm, beta_hbm, wr_hbm, wg_hbm, wu_hbm, wd_hbm,
            out_hbm,
            x_buf, wq_raw, wk_raw, wv_raw, wo_raw, beta_buf, wr_buf, wg_buf, wu_buf, wd_buf,
            wqt, wkt, wvt, wot, xn_buf, base, qs_buf, pq_buf, k_buf, pk_buf, vt_buf, r_buf,
            gate_buf, mt_buf, num_buf, p_buf0, p_buf1, ot_buf, out_buf, in_sems, out_sems):
    def x_copy(c):
        return pltpu.make_async_copy(x_hbm.at[0, :, pl.ds(c * L, L)], x_buf.at[c], in_sems.at[c])

    cp_wv = pltpu.make_async_copy(wv_hbm, wv_raw, in_sems.at[4])
    cp_wq = pltpu.make_async_copy(wq_hbm, wq_raw, in_sems.at[5])
    cp_wk = pltpu.make_async_copy(wk_hbm, wk_raw, in_sems.at[6])
    cp_wo = pltpu.make_async_copy(wo_hbm, wo_raw, in_sems.at[7])
    cp_wg = pltpu.make_async_copy(wg_hbm, wg_buf, in_sems.at[8])
    cp_wu = pltpu.make_async_copy(wu_hbm, wu_buf, in_sems.at[9])
    cp_wd = pltpu.make_async_copy(wd_hbm, wd_buf, in_sems.at[10])
    cp_beta = pltpu.make_async_copy(beta_hbm, beta_buf, in_sems.at[11])
    cp_wr = pltpu.make_async_copy(wr_hbm, wr_buf, in_sems.at[12])

    def out_copy(s):
        cols = pl.ds(pl.multiple_of(s * L, L), L)
        return pltpu.make_async_copy(out_buf.at[s], out_hbm.at[0, :, cols], out_sems.at[s])

    def out_tile_copy(j):
        s = NSEG - 1
        return pltpu.make_async_copy(out_buf.at[s, :, pl.ds(128 * j, 128)],
                                     out_hbm.at[0, :, pl.ds(s * L + 128 * j, 128)], out_sems.at[NSEG + j])


    for cp in (x_copy(0), cp_wv, cp_wr, cp_wq, cp_wk, x_copy(1), x_copy(2), x_copy(3), cp_wo, cp_beta,
               cp_wg, cp_wu, cp_wd):
        cp.start()

    lane128 = lax.broadcasted_iota(I32, (128, 128), 1)
    row128 = lax.broadcasted_iota(I32, (128, 128), 0)
    causal = row128 <= lane128
    r16 = lax.broadcasted_iota(I32, (16, D), 0)

    mt_buf[...] = jnp.zeros(mt_buf.shape, F32)

    def layernorm(c):
        x = x_buf[c].astype(F32)
        mean = jnp.sum(x, axis=0, keepdims=True) * (1.0 / D)
        cen = x - mean
        var = jnp.sum(cen * cen, axis=0, keepdims=True) * (1.0 / D)
        d = _round_bf16(x - _round_bf16(mean))
        den = _round_bf16(jnp.sqrt(_round_bf16(_round_bf16(var) + 1e-5)))
        xn = (d / den).astype(BF16)
        xn_buf[c] = xn
        base[c] = x + xn.astype(F32)

    x_copy(0).wait()
    layernorm(0)
    cp_wv.wait()
    cp_wr.wait()
    wvt[0:D, :] = wv_raw[...].T
    wr_row = wr_buf[...].reshape(1, D).astype(F32)
    wvt[D:VROWS, :] = jnp.where(r16 == 0, wr_row, 0.0).astype(BF16)
    cp_wq.wait()

    def project_v(c):
        vt = jnp.dot(wvt[...], xn_buf[c], preferred_element_type=F32)
        vt_buf[c, 0:D, :] = vt[0:D].astype(BF16)
        r16l = lax.broadcasted_iota(I32, (16, L), 0)
        vt_buf[c, D:VROWS, :] = jnp.where(r16l == 1, 1.0, 0.0).astype(BF16)
        r_buf[:, c * L:(c + 1) * L] = vt[D:D + 8]

    def project_q(c):
        qt = jnp.dot(wqt[...], xn_buf[c], preferred_element_type=F32)
        qsc = qt * QSCALE
        qs_buf[c] = qsc.astype(BF16)
        pq_buf[c] = _phi(qt).astype(BF16)
        return jnp.max(jnp.abs(qsc).reshape(PR // 8, 8, L), axis=0)

    def project_k(c):
        kt = jnp.dot(wkt[...], xn_buf[c], preferred_element_type=F32)
        pk_buf[c] = _phi(kt).astype(BF16)
        for g in range(NG):
            ktg = kt[128 * g:128 * g + GW[g]]
            if GW[g] < 128:
                ktg = jnp.concatenate([ktg, jnp.zeros((128 - GW[g], L), F32)], axis=0)
            k_buf[c, g] = ktg.T.astype(BF16)
        return jnp.max(jnp.abs(kt).reshape(PR // 8, 8, L), axis=0)

    wqt[...] = _pad_heads_t(wq_raw[...].astype(F32)).astype(BF16)
    project_v(0)
    cp_wk.wait()
    x_copy(1).wait()
    wkt[...] = _pad_heads_t(wk_raw[...].astype(F32)).astype(BF16)

    aq = project_q(0)
    layernorm(1)
    ak = project_k(0)
    project_v(1)
    x_copy(2).wait()
    x_copy(3).wait()
    cp_wo.wait()
    cp_beta.wait()
    aq = jnp.maximum(aq, project_q(1))
    layernorm(2)
    ak = jnp.maximum(ak, project_k(1))
    wot[...] = wo_raw[...].T
    beta_row = beta_buf[...].reshape(1, H).astype(F32)
    beta_row = jnp.concatenate([beta_row, jnp.zeros((1, 128 - H), F32)], axis=1)
    e_row = lax.broadcasted_iota(I32, (D, 128), 0)
    e_lane = lax.broadcasted_iota(I32, (D, 128), 1)
    in_head = (e_row >= e_lane * DH) & (e_row < e_lane * DH + DH)
    beta_col = jnp.sum(jnp.where(in_head, beta_row, 0.0), axis=1, keepdims=True)
    gate_buf[...] = jnp.broadcast_to(jax.nn.sigmoid(beta_col), (D, 128))


    project_v(2)
    aq = jnp.maximum(aq, project_q(2))
    layernorm(3)
    ak = jnp.maximum(ak, project_k(2))
    project_v(3)

    r = _round_bf16(r_buf[0:1, :])
    tok = lax.broadcasted_iota(I32, (1, S), 1).astype(F32)
    m1 = jnp.max(r)
    i1 = jnp.min(jnp.where(r == m1, tok, float(S)))
    r_rest = jnp.where(tok == i1, -jnp.inf, r)
    m2 = jnp.max(r_rest)
    i2 = jnp.min(jnp.where(r_rest == m2, tok, float(S)))
    i1 = jnp.clip(i1.astype(I32), 0, S - 1)
    i2 = jnp.clip(i2.astype(I32), 0, S - 1)

    sel_row = lax.broadcasted_iota(I32, (16, 128), 0)
    sel_lane = lax.broadcasted_iota(I32, (16, 128), 1)

    def token_tile(i):
        return i // L, pl.ds(pl.multiple_of(((i % L) // 128) * 128, 128), 128)

    def pick(i, slot):
        seg, cols = token_tile(i)
        onehot = jnp.where((sel_row == slot) & (sel_lane == i % 128), 1.0, 0.0).astype(BF16)
        return lax.dot_general(onehot, xn_buf[seg, :, cols], NT_DIMS, preferred_element_type=F32)

    ak = jnp.maximum(ak, project_k(3))
    aq = jnp.maximum(aq, project_q(3))
    xs = (pick(i1, 0) + pick(i2, 1)).astype(BF16)

    logit_bound = jnp.max(aq) * jnp.max(ak) * (DH * 1.02)
    safe = logit_bound <= SAFE_LOG2_RANGE

    cp_wg.wait()
    cp_wu.wait()

    def expert_chunk(lo, hi):
        hg = jnp.dot(xs, wg_buf[:, lo:hi], preferred_element_type=F32)
        hu = jnp.dot(xs, wu_buf[:, lo:hi], preferred_element_type=F32)
        hh = (jax.nn.silu(hg) * hu).astype(BF16)
        return lax.dot_general(hh, wd_buf[:, lo:hi], NT_DIMS, preferred_element_type=F32)

    def expert_stream(result):
        kmain = 512
        hidden = []
        for c0 in range(0, FF, 512):
            rem = []
            for w_ref in (wg_buf, wu_buf):
                rem.append(jnp.dot(xs[:, kmain:D], w_ref[kmain:D, c0:c0 + 512], preferred_element_type=F32))
                yield
            hs = []
            for f0 in range(c0, c0 + 512, 128):
                pre = []
                for w_ref, r in zip((wg_buf, wu_buf), rem):
                    pre.append(jnp.dot(xs[:, 0:kmain], w_ref[0:kmain, f0:f0 + 128], preferred_element_type=F32)
                               + r[:, f0 - c0:f0 - c0 + 128])
                    yield
                hs.append(jax.nn.silu(pre[0]) * pre[1])
            hidden.append(jnp.concatenate(hs, axis=1).astype(BF16))
        y_tiles = [None] * 5
        for ci, hh in enumerate(hidden):
            for e in range(5):
                e_hi = min(128 * (e + 1), D)
                part = lax.dot_general(hh, wd_buf[128 * e:e_hi, 512 * ci:512 * (ci + 1)], NT_DIMS,
                                       preferred_element_type=F32)
                y_tiles[e] = part if y_tiles[e] is None else y_tiles[e] + part
                yield
        result.append(jnp.concatenate(y_tiles, axis=1))

    def expert_scatter(y):
        y = y * jax.nn.sigmoid(jnp.where(r16 == 0, m1, m2))
        yt = jnp.concatenate([y, jnp.zeros((128 - 16, D), F32)], axis=0).T
        lane_d = lax.broadcasted_iota(I32, (D, 128), 1)
        for slot, i in ((0, i1), (1, i2)):
            seg, cols = token_tile(i)
            col = jnp.sum(jnp.where(lane_d == slot, yt, 0.0), axis=1, keepdims=True)
            base[seg, :, cols] = base[seg, :, cols] + jnp.where(lane_d == i % 128, col, 0.0)

    def memory_read(s, g):
        rg = _group_rows(g)
        gw = GW[g]
        lhs = jnp.concatenate([mt_buf[g, 0:rg, 0:gw], mt_buf[g, ZROW:MROWS, 0:gw]], axis=0).astype(BF16)
        res = jnp.dot(lhs, pq_buf[s, 128 * g:128 * g + gw, :], preferred_element_type=F32)
        num_buf[g, 0:rg, :] = res[0:rg]
        num_buf[g, ZROW:MROWS, :] = res[rg:rg + 16]

    def memory_update(s, g):
        rg = _group_rows(g)
        a_g = _group_row_start(g)
        gw = GW[g]
        lhs = jnp.concatenate([vt_buf[s, a_g:a_g + rg, :], vt_buf[s, D:VROWS, :]], axis=0)
        upd = lax.dot_general(lhs, pk_buf[s, 128 * g:128 * g + gw, :], NT_DIMS,
                              preferred_element_type=F32)
        er = lax.broadcasted_iota(I32, (rg, gw), 0) + (a_g - HPG * DH * g)
        el = lax.broadcasted_iota(I32, (rg, gw), 1)
        same_head = None
        for i in range(_heads_in_group(g)):
            t = ((er >= DH * i) & (er < DH * (i + 1)) & (el >= DH * i) & (el < DH * (i + 1)))
            same_head = t if same_head is None else (same_head | t)
        mt_buf[g, 0:rg, 0:gw] = mt_buf[g, 0:rg, 0:gw] + jnp.where(same_head, upd[0:rg], 0.0)
        zr = lax.broadcasted_iota(I32, (8, gw), 0)
        zl = lax.broadcasted_iota(I32, (8, gw), 1)
        zmask = (zl >= zr * DH) & (zl < zr * DH + DH) & (zr < _heads_in_group(g))
        zs = upd[rg + 1:rg + 2]
        mt_buf[g, ZROW:ZROW + 8, 0:gw] = mt_buf[g, ZROW:ZROW + 8, 0:gw] + jnp.where(zmask, zs, 0.0)

    def project_out(s):
        attn = jnp.dot(wot[...], ot_buf[...].astype(BF16), preferred_element_type=F32)
        return base[s] + attn

    def emit(s, val):
        out_buf[s] = val.astype(BF16)
        out_copy(s).start()

    zero = lax.shift_right_logical(i1, 16)

    def prow(start, size):
        return pl.ds(pl.multiple_of(zero + start, 8), size)

    P_OFFS = (0, 128, 384, 768)

    def fast_scores(s, g, hook):
        nh = _heads_in_group(g)
        gw = GW[g]
        pb = (p_buf0, p_buf1)[(s * NG + g) % 2]
        rowg = lax.broadcasted_iota(I32, (gw, 128), 0)
        for j in range(QT - 1, -1, -1):
            n = 128 * (j + 1)
            q = qs_buf[s, 128 * g:128 * g + gw, 128 * j:128 * (j + 1)].astype(F32)
            for h0, h1 in ((0, 4), (4, nh)):
                if h1 <= h0:
                    continue
                qm = jnp.concatenate(
                    [jnp.where((rowg >= DH * i) & (rowg < DH * (i + 1)), q, 0.0) for i in range(h0, h1)],
                    axis=1).astype(BF16)
                st = jnp.dot(k_buf[s, g, 0:n, 0:gw], qm, preferred_element_type=F32)
                p = jnp.exp2(st)
                causal_w = jnp.concatenate([causal] * (h1 - h0), axis=1)
                p_diag = jnp.where(causal_w, p[n - 128:], 0.0)
                p = jnp.concatenate([p[:n - 128], p_diag], axis=0) if j > 0 else p_diag
                pb[P_OFFS[j] // 2:(P_OFFS[j] + n) // 2, h0 * 128:h1 * 128] = pltpu.bitcast(p.astype(BF16), U32)
                hook()

    def fast_values(s, g):
        nh = _heads_in_group(g)
        a_g = _group_row_start(g)
        pb = (p_buf0, p_buf1)[(s * NG + g) % 2]
        for j in range(QT - 1, -1, -1):
            n = 128 * (j + 1)
            cols = slice(128 * j, 128 * (j + 1))
            for i in range(nh):
                h = HPG * g + i
                a = (h * DH // 16) * 16
                off = h * DH - a
                p = pltpu.bitcast(pb[prow(P_OFFS[j] // 2, n // 2), 128 * i:128 * (i + 1)], BF16)
                ones_row = 0 if off > 0 else 31
                r32n = lax.broadcasted_iota(I32, (32, n), 0)
                lhs = jnp.where(r32n == ones_row, 1.0, vt_buf[s, a:a + 32, 0:n].astype(F32)).astype(BF16)
                o = jnp.dot(lhs, p, preferred_element_type=F32)
                lo = (off // 8) * 8
                hi = -(-(off + DH) // 8) * 8
                gate = gate_buf[a + lo:a + hi, :]
                rl = 1.0 / o[ones_row:ones_row + 1]
                val = (1.0 - gate) * (o[lo:hi] * rl)
                if s > 0:
                    rden = 1.0 / (num_buf[g, ZROW + i:ZROW + i + 1, cols] + 1e-6)
                    num = num_buf[g, a - a_g + lo:a - a_g + hi, cols]
                    val = gate * (num * rden) + val
                ot_buf[a + off:a + off + DH, cols] = val[off - lo:off - lo + DH]

    def side_work():
        result = []
        yield from expert_stream(result)
        expert_scatter(result[0])
        yield
        for u in range(NSEG - 1):
            for j in range(QT):
                cols = slice(128 * j, 128 * (j + 1))
                out_buf[u, :, cols] = base[u, :, cols].astype(BF16)
                if j == QT - 1:
                    out_copy(u).start()
                yield

    def fast_path():
        stream = side_work()

        def hook():
            next(stream, None)

        steps = [(s, g) for s in range(NSEG) for g in range(NG)]
        fast_scores(0, 0, hook)
        for t, (s, g) in enumerate(steps):
            if t + 1 < len(steps):
                fast_scores(*steps[t + 1], hook)
            if s > 0:
                memory_read(s, g)
                hook()
            fast_values(s, g)
            if s + 1 < NSEG:
                memory_update(s, g)
                hook()
            if g == NG - 1 and s < NSEG - 1:
                base[s] = project_out(s)
                if s == 0:
                    cp_wd.wait()
                hook()
        for _ in stream:
            pass
        s = NSEG - 1
        for j in range(QT):
            cols = slice(128 * j, 128 * (j + 1))
            attn = jnp.dot(wot[...], ot_buf[:, cols].astype(BF16), preferred_element_type=F32)
            out_buf[s, :, cols] = (base[s, :, cols] + attn).astype(BF16)
            out_tile_copy(j).start()
        for u in range(NSEG - 1):
            out_copy(u).wait()
        for j in range(QT):
            out_tile_copy(j).wait()

    def slow_segment(s, carry):
        for g in range(NG):
            memory_read(s, g)
        key_i = lax.broadcasted_iota(I32, (L, L), 0)
        qry_i = lax.broadcasted_iota(I32, (L, L), 1)
        r32 = lax.broadcasted_iota(I32, (32, L), 0)
        for g in range(NG):
            gw = GW[g]
            a_g = _group_row_start(g)
            rowg = lax.broadcasted_iota(I32, (gw, L), 0)

            def head(i, c, g=g, gw=gw, a_g=a_g, rowg=rowg):
                h = HPG * g + i
                a = pl.multiple_of((h * DH // 16) * 16, 16)
                off = h * DH - a
                q = qs_buf[s, 128 * g:128 * g + gw, :].astype(F32)
                qm = jnp.where((rowg >= DH * i) & (rowg < DH * (i + 1)), q, 0.0).astype(BF16)
                st = jnp.dot(k_buf[s, g, :, 0:gw], qm, preferred_element_type=F32)
                st = jnp.where(key_i <= qry_i, st, NEG_BIG)
                p = jnp.exp2(st - jnp.max(st, axis=0, keepdims=True))
                rl = 1.0 / jnp.sum(p, axis=0, keepdims=True)
                o = jnp.dot(vt_buf[s, pl.ds(a, 32), :], p.astype(BF16), preferred_element_type=F32)
                gate = jnp.concatenate([gate_buf[pl.ds(a, 32), :]] * QT, axis=1)
                rden = 1.0 / (num_buf[g, pl.ds(ZROW + i, 1), :] + 1e-6)
                num = num_buf[g, pl.ds(pl.multiple_of(a - a_g, 16), 32), :]
                val = gate * (num * rden) + (1.0 - gate) * (o * rl)
                keep = (r32 >= off) & (r32 < off + DH)
                pltpu.store(ot_buf.at[pl.ds(a, 32), :], val, mask=keep)
                return c

            lax.fori_loop(0, _heads_in_group(g), head, 0)
        for g in range(NG):
            memory_update(s, g)
        emit(s, project_out(s))
        return carry

    @pl.when(safe)
    def _():
        fast_path()

    @pl.when(jnp.logical_not(safe))
    def _():
        cp_wd.wait()
        expert_scatter(expert_chunk(0, FF))
        lax.fori_loop(0, NSEG, slow_segment, 0)
        for u in range(NSEG):
            out_copy(u).wait()


@jax.jit
def pallas_parallel_sum__memory_aug_infini_attn__moe_arch_mod__prompt_kernel(
    A_x: jax.Array,
    A_wq: jax.Array,
    A_wk: jax.Array,
    A_wv: jax.Array,
    A_wo: jax.Array,
    A_beta: jax.Array,
    B_x: jax.Array,
    B_w_r: jax.Array,
    B_w_gate: jax.Array,
    B_w_up: jax.Array,
    B_w_down: jax.Array,
):
    del B_x
    hbm = pl.BlockSpec(memory_space=pl.ANY)
    scratch = [
        pltpu.VMEM((NSEG, D, L), BF16),
        pltpu.VMEM((D, D), BF16),
        pltpu.VMEM((D, D), BF16),
        pltpu.VMEM((D, D), BF16),
        pltpu.VMEM((D, D), BF16),
        pltpu.VMEM((H,), BF16),
        pltpu.VMEM((D,), BF16),
        pltpu.VMEM((D, FF), BF16),
        pltpu.VMEM((D, FF), BF16),
        pltpu.VMEM((D, FF), BF16),
        pltpu.VMEM((PR, D), BF16),
        pltpu.VMEM((PR, D), BF16),
        pltpu.VMEM((VROWS, D), BF16),
        pltpu.VMEM((D, D), BF16),
        pltpu.VMEM((NSEG, D, L), BF16),
        pltpu.VMEM((NSEG, D, L), F32),
        pltpu.VMEM((NSEG, PR, L), BF16),
        pltpu.VMEM((NSEG, PR, L), BF16),
        pltpu.VMEM((NSEG, NG, L, 128), BF16),
        pltpu.VMEM((NSEG, PR, L), BF16),
        pltpu.VMEM((NSEG, VROWS, L), BF16),
        pltpu.VMEM((8, S), F32),
        pltpu.VMEM((D, 128), F32),
        pltpu.VMEM((NG, MROWS, 128), F32),
        pltpu.VMEM((NG, MROWS, L), F32),
        pltpu.VMEM((640, HPG * 128), U32),
        pltpu.VMEM((640, HPG * 128), U32),
        pltpu.VMEM((D, L), F32),
        pltpu.VMEM((NSEG, D, L), BF16),
        pltpu.SemaphoreType.DMA((13,)),
        pltpu.SemaphoreType.DMA((NSEG + QT,)),
    ]
    out_t = pl.pallas_call(
        _kernel,
        out_shape=jax.ShapeDtypeStruct((1, D, S), BF16),
        in_specs=[hbm] * 10,
        out_specs=hbm,
        scratch_shapes=scratch,
        compiler_params=pltpu.CompilerParams(vmem_limit_bytes=128 * 1024 * 1024),
        name="infini_attn_moe",
    )(jnp.transpose(A_x, (0, 2, 1)), A_wq, A_wk, A_wv, A_wo, A_beta, B_w_r, B_w_gate, B_w_up,
      B_w_down.T)
    return jnp.transpose(out_t, (0, 2, 1))
```

```python
import jax
import jax.numpy as jnp
from jax import lax
import jax.experimental.pallas as pl
import jax.experimental.pallas.tpu as pltpu

F32 = jnp.float32
BF16 = jnp.bfloat16
U32 = jnp.uint32
I32 = jnp.int32

S = 2048
D = 576
H = 32
DH = 18
NSEG = 4
L = 512
FF = 4608
HPG = 7
NG = 5
QT = L // 128
GW = (128, 128, 128, 128, 80)
PR = sum(GW)
VROWS = D + 16
ZROW = 144
MROWS = 160
LOG2E = 1.4426950408889634
QSCALE = (DH ** -0.5) * LOG2E
SAFE_LOG2_RANGE = 60.0
NEG_BIG = -1e30

NT_DIMS = (((1,), (1,)), ((), ()))


def _heads_in_group(g):
    return min(HPG, H - HPG * g)


def _group_row_start(g):
    return (HPG * g * DH // 16) * 16


def _group_rows(g):
    last = (HPG * g + _heads_in_group(g)) * DH
    return -(-(last - _group_row_start(g)) // 16) * 16


def _round_bf16(x):
    return x.astype(BF16).astype(F32)


def _pad_heads_t(w):
    parts = []
    for g in range(NG):
        n = _heads_in_group(g) * DH
        parts.append(w[:, HPG * DH * g:HPG * DH * g + n])
        parts.append(jnp.zeros((D, 128 - n), w.dtype))
    return jnp.concatenate(parts, axis=1).T[0:PR]


def _phi(t):
    return jnp.where(t > 0, t + 1.0, jnp.exp(t))


def _kernel(x_hbm, wq_hbm, wk_hbm, wv_hbm, wo_hbm, beta_hbm, wr_hbm, wg_hbm, wu_hbm, wd_hbm,
            out_hbm,
            x_buf, wq_raw, wk_raw, wv_raw, wo_raw, beta_buf, wr_buf, wg_buf, wu_buf, wd_buf,
            wqt, wkt, wvt, wot, xn_buf, base, qs_buf, pq_buf, k_buf, pk_buf, vt_buf, r_buf,
            gate_buf, mt_buf, num_buf, p_buf0, p_buf1, ot_buf, out_buf, in_sems, out_sems):
    def x_copy(c):
        return pltpu.make_async_copy(x_hbm.at[0, :, pl.ds(c * L, L)], x_buf.at[c], in_sems.at[c])

    cp_wv = pltpu.make_async_copy(wv_hbm, wv_raw, in_sems.at[4])
    cp_wq = pltpu.make_async_copy(wq_hbm, wq_raw, in_sems.at[5])
    cp_wk = pltpu.make_async_copy(wk_hbm, wk_raw, in_sems.at[6])
    cp_wo = pltpu.make_async_copy(wo_hbm, wo_raw, in_sems.at[7])
    cp_wg = pltpu.make_async_copy(wg_hbm, wg_buf, in_sems.at[8])
    cp_wu = pltpu.make_async_copy(wu_hbm, wu_buf, in_sems.at[9])
    cp_wd = pltpu.make_async_copy(wd_hbm, wd_buf, in_sems.at[10])
    cp_beta = pltpu.make_async_copy(beta_hbm, beta_buf, in_sems.at[11])
    cp_wr = pltpu.make_async_copy(wr_hbm, wr_buf, in_sems.at[12])

    def out_copy(s):
        cols = pl.ds(pl.multiple_of(s * L, L), L)
        return pltpu.make_async_copy(out_buf.at[s], out_hbm.at[0, :, cols], out_sems.at[s])

    def out_tile_copy(j):
        s = NSEG - 1
        return pltpu.make_async_copy(out_buf.at[s, :, pl.ds(128 * j, 128)],
                                     out_hbm.at[0, :, pl.ds(s * L + 128 * j, 128)], out_sems.at[NSEG + j])


    for cp in (x_copy(0), cp_wv, cp_wr, cp_wq, cp_wk, x_copy(1), x_copy(2), x_copy(3), cp_wo, cp_beta,
               cp_wg, cp_wu, cp_wd):
        cp.start()

    lane128 = lax.broadcasted_iota(I32, (128, 128), 1)
    row128 = lax.broadcasted_iota(I32, (128, 128), 0)
    causal = row128 <= lane128
    r16 = lax.broadcasted_iota(I32, (16, D), 0)

    mt_buf[...] = jnp.zeros(mt_buf.shape, F32)

    always = []

    def pace(x, y):
        return x if y is None else jnp.where(always[0], x, y[0:D])

    def ln_mean(c, y):
        return jnp.sum(pace(x_buf[c].astype(F32), y), axis=0, keepdims=True) * (1.0 / D)

    def ln_scale(c, mean, y):
        mean_b = _round_bf16(mean)
        d = pace(x_buf[c].astype(F32), y) - mean_b
        msq = jnp.sum(d * d, axis=0, keepdims=True) * (1.0 / D)
        off = mean - mean_b
        var = jnp.maximum(msq - off * off, 0.0)
        return mean_b, 1.0 / _round_bf16(jnp.sqrt(_round_bf16(_round_bf16(var) + 1e-5)))

    def ln_apply(c, mean_b, inv):
        x = x_buf[c].astype(F32)
        xn = (x - mean_b) * inv
        xn_buf[c] = xn.astype(BF16)
        base[c] = x + xn

    def project_v(c):
        vt = jnp.dot(wvt[...], xn_buf[c], preferred_element_type=F32)
        vt_buf[c, 0:D, :] = vt[0:D].astype(BF16)
        r16l = lax.broadcasted_iota(I32, (16, L), 0)
        vt_buf[c, D:VROWS, :] = jnp.where(r16l == 1, 1.0, 0.0).astype(BF16)
        r_buf[:, c * L:(c + 1) * L] = vt[D:D + 8]
        return vt

    def project(w_ref, c, split):
        if not split:
            return jnp.dot(w_ref[...], xn_buf[c], preferred_element_type=F32), None
        head = jnp.dot(w_ref[:, 0:256], xn_buf[c, 0:256, :], preferred_element_type=F32)
        tail = jnp.dot(w_ref[:, 256:D], xn_buf[c, 256:D, :], preferred_element_type=F32)
        return head + tail, head

    def project_q(c, mid=None):
        qt, head = project(wqt, c, mid is not None)
        if mid is not None:
            mid(head)
        qsc = qt * QSCALE
        qs_buf[c] = qsc.astype(BF16)
        pq_buf[c] = _phi(qt).astype(BF16)
        return qt, jnp.max(jnp.abs(qsc).reshape(PR // 8, 8, L), axis=0)

    def project_k(c, mid=None):
        kt, head = project(wkt, c, mid is not None)
        if mid is not None:
            mid(head)
        pk_buf[c] = _phi(kt).astype(BF16)
        for g in range(NG):
            ktg = kt[128 * g:128 * g + GW[g]]
            if GW[g] < 128:
                ktg = jnp.concatenate([ktg, jnp.zeros((128 - GW[g], L), F32)], axis=0)
            k_buf[c, g] = ktg.T.astype(BF16)
        return jnp.max(jnp.abs(kt).reshape(PR // 8, 8, L), axis=0)

    x_copy(0).wait()
    mean = ln_mean(0, None)
    always.append(jnp.logical_not(jnp.abs(mean) < 0.0))
    ln_apply(0, *ln_scale(0, mean, None))
    cp_wv.wait()
    cp_wr.wait()
    wvt[0:D, :] = wv_raw[...].T
    wr_row = wr_buf[...].reshape(1, D).astype(F32)
    wvt[D:VROWS, :] = jnp.where(r16 == 0, wr_row, 0.0).astype(BF16)
    cp_wq.wait()
    wqt[...] = _pad_heads_t(wq_raw[...].astype(F32)).astype(BF16)
    project_v(0)
    cp_wk.wait()
    x_copy(1).wait()

    def prep_wk(y):
        wk = wk_raw[...].astype(F32)
        wk = jnp.concatenate([jnp.where(always[0], wk[:, 0:L], y[0:D]), wk[:, L:D]], axis=1)
        wkt[...] = _pad_heads_t(wk).astype(BF16)

    qt, aq = project_q(0, prep_wk)
    mean = ln_mean(1, qt)
    stats = []
    ak = project_k(0, lambda y: stats.extend(ln_scale(1, mean, y)))
    ln_apply(1, *stats)
    x_copy(2).wait()
    x_copy(3).wait()
    cp_wo.wait()
    cp_beta.wait()

    beta_row = beta_buf[...].reshape(1, H).astype(F32)
    beta_row = jnp.concatenate([beta_row, jnp.zeros((1, 128 - H), F32)], axis=1)
    h_row = lax.broadcasted_iota(I32, (H, 128), 0)
    h_lane = lax.broadcasted_iota(I32, (H, 128), 1)
    beta_col = jnp.sum(jnp.where(h_row == h_lane, beta_row, 0.0), axis=1, keepdims=True)
    gate_buf[...] = jnp.broadcast_to(jax.nn.sigmoid(beta_col), (H, 128))

    def route():
        r = _round_bf16(r_buf[0:1, :])
        tok = lax.broadcasted_iota(I32, (1, S), 1).astype(F32)
        m1 = jnp.max(r)
        i1 = jnp.min(jnp.where(r == m1, tok, float(S)))
        r_rest = jnp.where(tok == i1, -jnp.inf, r)
        m2 = jnp.max(r_rest)
        i2 = jnp.min(jnp.where(r_rest == m2, tok, float(S)))
        i1 = jnp.clip(i1.astype(I32), 0, S - 1)
        i2 = jnp.clip(i2.astype(I32), 0, S - 1)
        return m1, m2, i1, i2

    for c in range(1, NSEG):
        vt = project_v(c)
        if c + 1 < NSEG:
            mean = ln_mean(c + 1, vt)
        else:
            m1, m2, i1, i2 = route()
        qt, a = project_q(c)
        aq = jnp.maximum(aq, a)
        if c + 1 < NSEG:
            mean_b, inv = ln_scale(c + 1, mean, qt)
        ak = jnp.maximum(ak, project_k(c))
        if c + 1 < NSEG:
            ln_apply(c + 1, mean_b, inv)

    logit_bound = jnp.max(aq) * jnp.max(ak) * (DH * 1.02)
    safe = logit_bound <= SAFE_LOG2_RANGE

    sel_row = lax.broadcasted_iota(I32, (16, 128), 0)
    sel_lane = lax.broadcasted_iota(I32, (16, 128), 1)

    def token_tile(i):
        return i // L, pl.ds(pl.multiple_of(((i % L) // 128) * 128, 128), 128)

    def pick(i, slot):
        seg, cols = token_tile(i)
        onehot = jnp.where((sel_row == slot) & (sel_lane == i % 128), 1.0, 0.0).astype(BF16)
        return lax.dot_general(onehot, xn_buf[seg, :, cols], NT_DIMS, preferred_element_type=F32)

    xs = (pick(i1, 0) + pick(i2, 1)).astype(BF16)

    cp_wg.wait()
    cp_wu.wait()

    def expert_chunk(lo, hi):
        hg = jnp.dot(xs, wg_buf[:, lo:hi], preferred_element_type=F32)
        hu = jnp.dot(xs, wu_buf[:, lo:hi], preferred_element_type=F32)
        hh = (jax.nn.silu(hg) * hu).astype(BF16)
        return lax.dot_general(hh, wd_buf[:, lo:hi], NT_DIMS, preferred_element_type=F32)

    def expert_stream(result):
        kmain = 512
        hidden = []
        for c0 in range(0, FF, 512):
            rem = []
            for w_ref in (wg_buf, wu_buf):
                rem.append(jnp.dot(xs[:, kmain:D], w_ref[kmain:D, c0:c0 + 512], preferred_element_type=F32))
                yield
            hs = []
            for f0 in range(c0, c0 + 512, 128):
                pre = []
                for w_ref, r in zip((wg_buf, wu_buf), rem):
                    pre.append(jnp.dot(xs[:, 0:kmain], w_ref[0:kmain, f0:f0 + 128], preferred_element_type=F32)
                               + r[:, f0 - c0:f0 - c0 + 128])
                    yield
                hs.append(jax.nn.silu(pre[0]) * pre[1])
            hidden.append(jnp.concatenate(hs, axis=1).astype(BF16))
        y_tiles = [None] * 5
        for ci, hh in enumerate(hidden):
            for e in range(5):
                e_hi = min(128 * (e + 1), D)
                part = lax.dot_general(hh, wd_buf[128 * e:e_hi, 512 * ci:512 * (ci + 1)], NT_DIMS,
                                       preferred_element_type=F32)
                y_tiles[e] = part if y_tiles[e] is None else y_tiles[e] + part
                yield
        result.append(jnp.concatenate(y_tiles, axis=1))

    def expert_scatter(y):
        y = y * jax.nn.sigmoid(jnp.where(r16 == 0, m1, m2))
        yt = jnp.concatenate([y, jnp.zeros((128 - 16, D), F32)], axis=0).T
        lane_d = lax.broadcasted_iota(I32, (D, 128), 1)
        for slot, i in ((0, i1), (1, i2)):
            seg, cols = token_tile(i)
            col = jnp.sum(jnp.where(lane_d == slot, yt, 0.0), axis=1, keepdims=True)
            base[seg, :, cols] = base[seg, :, cols] + jnp.where(lane_d == i % 128, col, 0.0)

    def memory_read(s, g):
        rg = _group_rows(g)
        gw = GW[g]
        lhs = jnp.concatenate([mt_buf[g, 0:rg, 0:gw], mt_buf[g, ZROW:MROWS, 0:gw]], axis=0).astype(BF16)
        res = jnp.dot(lhs, pq_buf[s, 128 * g:128 * g + gw, :], preferred_element_type=F32)
        num_buf[g, 0:rg, :] = res[0:rg]
        num_buf[g, ZROW:MROWS, :] = res[rg:rg + 16]

    def memory_update(s, g):
        rg = _group_rows(g)
        a_g = _group_row_start(g)
        gw = GW[g]
        lhs = jnp.concatenate([vt_buf[s, a_g:a_g + rg, :], vt_buf[s, D:VROWS, :]], axis=0)
        upd = lax.dot_general(lhs, pk_buf[s, 128 * g:128 * g + gw, :], NT_DIMS,
                              preferred_element_type=F32)
        er = lax.broadcasted_iota(I32, (rg, gw), 0) + (a_g - HPG * DH * g)
        el = lax.broadcasted_iota(I32, (rg, gw), 1)
        same_head = None
        for i in range(_heads_in_group(g)):
            t = ((er >= DH * i) & (er < DH * (i + 1)) & (el >= DH * i) & (el < DH * (i + 1)))
            same_head = t if same_head is None else (same_head | t)
        mt_buf[g, 0:rg, 0:gw] = mt_buf[g, 0:rg, 0:gw] + jnp.where(same_head, upd[0:rg], 0.0)
        zr = lax.broadcasted_iota(I32, (8, gw), 0)
        zl = lax.broadcasted_iota(I32, (8, gw), 1)
        zmask = (zl >= zr * DH) & (zl < zr * DH + DH) & (zr < _heads_in_group(g))
        zs = upd[rg + 1:rg + 2]
        mt_buf[g, ZROW:ZROW + 8, 0:gw] = mt_buf[g, ZROW:ZROW + 8, 0:gw] + jnp.where(zmask, zs, 0.0)

    def transpose_wo(g):
        hi = min(128 * (g + 1), D)
        wot[128 * g:hi, :] = wo_raw[:, 128 * g:hi].T

    def project_out(s):
        attn = jnp.dot(wot[...], ot_buf[...].astype(BF16), preferred_element_type=F32)
        return base[s] + attn

    def emit(s, val):
        out_buf[s] = val.astype(BF16)
        out_copy(s).start()

    zero = lax.shift_right_logical(i1, 16)

    def prow(start, size):
        return pl.ds(pl.multiple_of(zero + start, 8), size)

    P_OFFS = (0, 128, 384, 768)

    def fast_scores(s, g, hook):
        nh = _heads_in_group(g)
        gw = GW[g]
        pb = (p_buf0, p_buf1)[(s * NG + g) % 2]
        rowg = lax.broadcasted_iota(I32, (gw, 128), 0)
        for j in range(QT - 1, -1, -1):
            n = 128 * (j + 1)
            q = qs_buf[s, 128 * g:128 * g + gw, 128 * j:128 * (j + 1)].astype(F32)
            for h0, h1 in ((0, 4), (4, nh)):
                if h1 <= h0:
                    continue
                qm = jnp.concatenate(
                    [jnp.where((rowg >= DH * i) & (rowg < DH * (i + 1)), q, 0.0) for i in range(h0, h1)],
                    axis=1).astype(BF16)
                st = jnp.dot(k_buf[s, g, 0:n, 0:gw], qm, preferred_element_type=F32)
                p = jnp.exp2(st)
                causal_w = jnp.concatenate([causal] * (h1 - h0), axis=1)
                p_diag = jnp.where(causal_w, p[n - 128:], 0.0)
                p = jnp.concatenate([p[:n - 128], p_diag], axis=0) if j > 0 else p_diag
                pb[P_OFFS[j] // 2:(P_OFFS[j] + n) // 2, h0 * 128:h1 * 128] = pltpu.bitcast(p.astype(BF16), U32)
                hook()

    def fast_values(s, g):
        nh = _heads_in_group(g)
        a_g = _group_row_start(g)
        pb = (p_buf0, p_buf1)[(s * NG + g) % 2]
        for j in range(QT - 1, -1, -1):
            n = 128 * (j + 1)
            cols = slice(128 * j, 128 * (j + 1))
            for i in range(nh):
                h = HPG * g + i
                a = (h * DH // 16) * 16
                off = h * DH - a
                p = pltpu.bitcast(pb[prow(P_OFFS[j] // 2, n // 2), 128 * i:128 * (i + 1)], BF16)
                ones_row = 0 if off > 0 else 31
                r32n = lax.broadcasted_iota(I32, (32, n), 0)
                lhs = jnp.where(r32n == ones_row, 1.0, vt_buf[s, a:a + 32, 0:n].astype(F32)).astype(BF16)
                o = jnp.dot(lhs, p, preferred_element_type=F32)
                lo = (off // 8) * 8
                hi = -(-(off + DH) // 8) * 8
                gate = gate_buf[h:h + 1, :]
                rl = 1.0 / o[ones_row:ones_row + 1]
                val = (1.0 - gate) * (o[lo:hi] * rl)
                if s > 0:
                    rden = 1.0 / (num_buf[g, ZROW + i:ZROW + i + 1, cols] + 1e-6)
                    num = num_buf[g, a - a_g + lo:a - a_g + hi, cols]
                    val = gate * (num * rden) + val
                ot_buf[a + off:a + off + DH, cols] = val[off - lo:off - lo + DH]

    def side_work():
        result = []
        yield from expert_stream(result)
        expert_scatter(result[0])
        yield
        for u in range(NSEG - 1):
            for j in range(QT):
                cols = slice(128 * j, 128 * (j + 1))
                out_buf[u, :, cols] = base[u, :, cols].astype(BF16)
                if j == QT - 1:
                    out_copy(u).start()
                yield

    def fast_path():
        stream = side_work()

        def hook():
            next(stream, None)

        steps = [(s, g) for s in range(NSEG) for g in range(NG)]
        fast_scores(0, 0, hook)
        for t, (s, g) in enumerate(steps):
            if t + 1 < len(steps):
                fast_scores(*steps[t + 1], hook)
            if s > 0:
                memory_read(s, g)
                hook()
            fast_values(s, g)
            if s == 0:
                transpose_wo(g)
            if s + 1 < NSEG:
                memory_update(s, g)
                hook()
            if g == NG - 1 and s < NSEG - 1:
                base[s] = project_out(s)
                if s == 0:
                    cp_wd.wait()
                hook()
        for _ in stream:
            pass
        s = NSEG - 1
        for j in range(QT):
            cols = slice(128 * j, 128 * (j + 1))
            attn = jnp.dot(wot[...], ot_buf[:, cols].astype(BF16), preferred_element_type=F32)
            out_buf[s, :, cols] = (base[s, :, cols] + attn).astype(BF16)
            out_tile_copy(j).start()
        for u in range(NSEG - 1):
            out_copy(u).wait()
        for j in range(QT):
            out_tile_copy(j).wait()

    def slow_segment(s, carry):
        for g in range(NG):
            memory_read(s, g)
        key_i = lax.broadcasted_iota(I32, (L, L), 0)
        qry_i = lax.broadcasted_iota(I32, (L, L), 1)
        r32 = lax.broadcasted_iota(I32, (32, L), 0)
        for g in range(NG):
            gw = GW[g]
            a_g = _group_row_start(g)
            rowg = lax.broadcasted_iota(I32, (gw, L), 0)

            def head(i, c, g=g, gw=gw, a_g=a_g, rowg=rowg):
                h = HPG * g + i
                a = pl.multiple_of((h * DH // 16) * 16, 16)
                off = h * DH - a
                q = qs_buf[s, 128 * g:128 * g + gw, :].astype(F32)
                qm = jnp.where((rowg >= DH * i) & (rowg < DH * (i + 1)), q, 0.0).astype(BF16)
                st = jnp.dot(k_buf[s, g, :, 0:gw], qm, preferred_element_type=F32)
                st = jnp.where(key_i <= qry_i, st, NEG_BIG)
                p = jnp.exp2(st - jnp.max(st, axis=0, keepdims=True))
                rl = 1.0 / jnp.sum(p, axis=0, keepdims=True)
                o = jnp.dot(vt_buf[s, pl.ds(a, 32), :], p.astype(BF16), preferred_element_type=F32)
                gate = jnp.concatenate([gate_buf[pl.ds(h, 1), :]] * QT, axis=1)
                rden = 1.0 / (num_buf[g, pl.ds(ZROW + i, 1), :] + 1e-6)
                num = num_buf[g, pl.ds(pl.multiple_of(a - a_g, 16), 32), :]
                val = gate * (num * rden) + (1.0 - gate) * (o * rl)
                keep = (r32 >= off) & (r32 < off + DH)
                pltpu.store(ot_buf.at[pl.ds(a, 32), :], val, mask=keep)
                return c

            lax.fori_loop(0, _heads_in_group(g), head, 0)
        for g in range(NG):
            memory_update(s, g)
        emit(s, project_out(s))
        return carry

    @pl.when(safe)
    def _():
        fast_path()

    @pl.when(jnp.logical_not(safe))
    def _():
        cp_wd.wait()
        for g in range(NG):
            transpose_wo(g)
        expert_scatter(expert_chunk(0, FF))
        lax.fori_loop(0, NSEG, slow_segment, 0)
        for u in range(NSEG):
            out_copy(u).wait()


@jax.jit
def pallas_parallel_sum__memory_aug_infini_attn__moe_arch_mod__prompt_kernel(
    A_x: jax.Array,
    A_wq: jax.Array,
    A_wk: jax.Array,
    A_wv: jax.Array,
    A_wo: jax.Array,
    A_beta: jax.Array,
    B_x: jax.Array,
    B_w_r: jax.Array,
    B_w_gate: jax.Array,
    B_w_up: jax.Array,
    B_w_down: jax.Array,
):
    del B_x
    hbm = pl.BlockSpec(memory_space=pl.ANY)
    scratch = [
        pltpu.VMEM((NSEG, D, L), BF16),
        pltpu.VMEM((D, D), BF16),
        pltpu.VMEM((D, D), BF16),
        pltpu.VMEM((D, D), BF16),
        pltpu.VMEM((D, D), BF16),
        pltpu.VMEM((H,), BF16),
        pltpu.VMEM((D,), BF16),
        pltpu.VMEM((D, FF), BF16),
        pltpu.VMEM((D, FF), BF16),
        pltpu.VMEM((D, FF), BF16),
        pltpu.VMEM((PR, D), BF16),
        pltpu.VMEM((PR, D), BF16),
        pltpu.VMEM((VROWS, D), BF16),
        pltpu.VMEM((D, D), BF16),
        pltpu.VMEM((NSEG, D, L), BF16),
        pltpu.VMEM((NSEG, D, L), F32),
        pltpu.VMEM((NSEG, PR, L), BF16),
        pltpu.VMEM((NSEG, PR, L), BF16),
        pltpu.VMEM((NSEG, NG, L, 128), BF16),
        pltpu.VMEM((NSEG, PR, L), BF16),
        pltpu.VMEM((NSEG, VROWS, L), BF16),
        pltpu.VMEM((8, S), F32),
        pltpu.VMEM((H, 128), F32),
        pltpu.VMEM((NG, MROWS, 128), F32),
        pltpu.VMEM((NG, MROWS, L), F32),
        pltpu.VMEM((640, HPG * 128), U32),
        pltpu.VMEM((640, HPG * 128), U32),
        pltpu.VMEM((D, L), F32),
        pltpu.VMEM((NSEG, D, L), BF16),
        pltpu.SemaphoreType.DMA((13,)),
        pltpu.SemaphoreType.DMA((NSEG + QT,)),
    ]
    out_t = pl.pallas_call(
        _kernel,
        out_shape=jax.ShapeDtypeStruct((1, D, S), BF16),
        in_specs=[hbm] * 10,
        out_specs=hbm,
        scratch_shapes=scratch,
        compiler_params=pltpu.CompilerParams(vmem_limit_bytes=128 * 1024 * 1024),
        name="infini_attn_moe",
    )(jnp.transpose(A_x, (0, 2, 1)), A_wq, A_wk, A_wv, A_wo, A_beta, B_w_r, B_w_gate, B_w_up,
      B_w_down.T)
    return jnp.transpose(out_t, (0, 2, 1))
```

```python
import jax
import jax.numpy as jnp
from jax import lax
import jax.experimental.pallas as pl
import jax.experimental.pallas.tpu as pltpu

F32 = jnp.float32
BF16 = jnp.bfloat16
U32 = jnp.uint32
I32 = jnp.int32

S = 2048
D = 576
H = 32
DH = 18
NSEG = 4
L = 512
FF = 4608
HPG = 7
NG = 5
QT = L // 128
GW = (128, 128, 128, 128, 80)
PR = sum(GW)
VROWS = D + 16
ZROW = 144
MROWS = 160
LOG2E = 1.4426950408889634
QSCALE = (DH ** -0.5) * LOG2E
SAFE_LOG2_RANGE = 60.0
NEG_BIG = -1e30

NT_DIMS = (((1,), (1,)), ((), ()))


def _heads_in_group(g):
    return min(HPG, H - HPG * g)


def _group_row_start(g):
    return (HPG * g * DH // 16) * 16


def _group_rows(g):
    last = (HPG * g + _heads_in_group(g)) * DH
    return -(-(last - _group_row_start(g)) // 16) * 16


def _round_bf16(x):
    return x.astype(BF16).astype(F32)


def _pad_heads_t(w):
    parts = []
    for g in range(NG):
        n = _heads_in_group(g) * DH
        parts.append(w[:, HPG * DH * g:HPG * DH * g + n])
        parts.append(jnp.zeros((D, 128 - n), w.dtype))
    return jnp.concatenate(parts, axis=1).T[0:PR]


def _phi(t):
    return jnp.where(t > 0, t + 1.0, jnp.exp(t))


def _kernel(x_hbm, wq_hbm, wk_hbm, wv_hbm, wo_hbm, beta_hbm, wr_hbm, wg_hbm, wu_hbm, wd_hbm,
            out_hbm,
            x_buf, wq_raw, wk_raw, wv_raw, wo_raw, beta_buf, wr_buf, wg_buf, wu_buf, wd_buf,
            wqt, wkt, wvt, wot, xn_buf, base, qs_buf, pq_buf, k_buf, pk_buf, vt_buf, r_buf,
            gate_buf, mt_buf, num_buf, p_buf0, p_buf1, ot_buf, out_buf, in_sems, out_sems):
    def x_copy(c):
        return pltpu.make_async_copy(x_hbm.at[0, :, pl.ds(c * L, L)], x_buf.at[c], in_sems.at[c])

    cp_wv = pltpu.make_async_copy(wv_hbm, wv_raw, in_sems.at[4])
    cp_wq = pltpu.make_async_copy(wq_hbm, wq_raw, in_sems.at[5])
    cp_wk = pltpu.make_async_copy(wk_hbm, wk_raw, in_sems.at[6])
    cp_wo = pltpu.make_async_copy(wo_hbm, wo_raw, in_sems.at[7])
    cp_wg = pltpu.make_async_copy(wg_hbm, wg_buf, in_sems.at[8])
    cp_wu = pltpu.make_async_copy(wu_hbm, wu_buf, in_sems.at[9])
    cp_wd = pltpu.make_async_copy(wd_hbm, wd_buf, in_sems.at[10])
    cp_beta = pltpu.make_async_copy(beta_hbm, beta_buf, in_sems.at[11])
    cp_wr = pltpu.make_async_copy(wr_hbm, wr_buf, in_sems.at[12])

    def out_copy(s):
        cols = pl.ds(pl.multiple_of(s * L, L), L)
        return pltpu.make_async_copy(out_buf.at[s], out_hbm.at[0, :, cols], out_sems.at[s])

    def out_tile_copy(j):
        s = NSEG - 1
        return pltpu.make_async_copy(out_buf.at[s, :, pl.ds(128 * j, 128)],
                                     out_hbm.at[0, :, pl.ds(s * L + 128 * j, 128)], out_sems.at[NSEG + j])


    for cp in (cp_wv, cp_wr, x_copy(0), x_copy(1), cp_wq, x_copy(2), cp_wk, x_copy(3), cp_wo, cp_beta,
               cp_wg, cp_wu, cp_wd):
        cp.start()

    lane128 = lax.broadcasted_iota(I32, (128, 128), 1)
    row128 = lax.broadcasted_iota(I32, (128, 128), 0)
    causal = row128 <= lane128
    r16 = lax.broadcasted_iota(I32, (16, D), 0)

    mt_buf[...] = jnp.zeros(mt_buf.shape, F32)

    always = []

    def pace(x, y):
        return x if y is None else jnp.where(always[0], x, y[0:D])

    def ln_mean(c, y):
        return jnp.sum(pace(x_buf[c].astype(F32), y), axis=0, keepdims=True) * (1.0 / D)

    def ln_scale(c, mean, y):
        mean_b = _round_bf16(mean)
        d = pace(x_buf[c].astype(F32), y) - mean_b
        msq = jnp.sum(d * d, axis=0, keepdims=True) * (1.0 / D)
        off = mean - mean_b
        var = jnp.maximum(msq - off * off, 0.0)
        return mean_b, 1.0 / _round_bf16(jnp.sqrt(_round_bf16(_round_bf16(var) + 1e-5)))

    def ln_apply(c, mean_b, inv):
        x = x_buf[c].astype(F32)
        xn = (x - mean_b) * inv
        xn_buf[c] = xn.astype(BF16)
        base[c] = x + xn

    def project(w_ref, c, split):
        if not split:
            return jnp.dot(w_ref[...], xn_buf[c], preferred_element_type=F32), None
        head = jnp.dot(w_ref[:, 0:256], xn_buf[c, 0:256, :], preferred_element_type=F32)
        tail = jnp.dot(w_ref[:, 256:D], xn_buf[c, 256:D, :], preferred_element_type=F32)
        return head + tail, head

    def project_v(c, mid=None):
        vt, head = project(wvt, c, mid is not None)
        if mid is not None:
            mid(head)
        vt_buf[c, 0:D, :] = vt[0:D].astype(BF16)
        r16l = lax.broadcasted_iota(I32, (16, L), 0)
        vt_buf[c, D:VROWS, :] = jnp.where(r16l == 1, 1.0, 0.0).astype(BF16)
        r_buf[:, c * L:(c + 1) * L] = vt[D:D + 8]
        return vt

    def project_q(c, mid=None):
        qt, head = project(wqt, c, mid is not None)
        if mid is not None:
            mid(head)
        qsc = qt * QSCALE
        qs_buf[c] = qsc.astype(BF16)
        pq_buf[c] = _phi(qt).astype(BF16)
        return qt, jnp.max(jnp.abs(qsc).reshape(PR // 8, 8, L), axis=0)

    def project_k(c, mid=None, keep=False):
        kt, head = project(wkt, c, mid is not None)
        if mid is not None:
            mid(head)
        pk_buf[c] = _phi(kt).astype(BF16)
        for g in range(NG):
            ktg = kt[128 * g:128 * g + GW[g]]
            if GW[g] < 128:
                ktg = jnp.concatenate([ktg, jnp.zeros((128 - GW[g], L), F32)], axis=0)
            k_buf[c, g] = ktg.T.astype(BF16)
        top = jnp.max(jnp.abs(kt).reshape(PR // 8, 8, L), axis=0)
        return (kt, top) if keep else top

    cp_wv.wait()
    cp_wr.wait()
    wvt[0:D, :] = wv_raw[...].T
    wr_row = wr_buf[...].reshape(1, D).astype(F32)
    wvt[D:VROWS, :] = jnp.where(r16 == 0, wr_row, 0.0).astype(BF16)
    x_copy(0).wait()
    mean = ln_mean(0, None)
    always.append(jnp.logical_not(jnp.abs(mean) < 0.0))
    ln_apply(0, *ln_scale(0, mean, None))
    x_copy(1).wait()
    mean = ln_mean(1, None)
    stats = []
    project_v(0, lambda y: stats.extend(ln_scale(1, mean, y)))
    ln_apply(1, *stats)
    cp_wq.wait()
    wqt[...] = _pad_heads_t(wq_raw[...].astype(F32)).astype(BF16)
    project_v(1)
    cp_wk.wait()
    x_copy(2).wait()
    x_copy(3).wait()

    def prep_wk(y):
        wk = wk_raw[...].astype(F32)
        wk = jnp.concatenate([jnp.where(always[0], wk[:, 0:L], y[0:D]), wk[:, L:D]], axis=1)
        wkt[...] = _pad_heads_t(wk).astype(BF16)

    def route():
        r = _round_bf16(r_buf[0:1, :])
        tok = lax.broadcasted_iota(I32, (1, S), 1).astype(F32)
        m1 = jnp.max(r)
        i1 = jnp.min(jnp.where(r == m1, tok, float(S)))
        r_rest = jnp.where(tok == i1, -jnp.inf, r)
        m2 = jnp.max(r_rest)
        i2 = jnp.min(jnp.where(r_rest == m2, tok, float(S)))
        i1 = jnp.clip(i1.astype(I32), 0, S - 1)
        i2 = jnp.clip(i2.astype(I32), 0, S - 1)
        return m1, m2, i1, i2

    qt, aq = project_q(0, prep_wk)
    mean = ln_mean(2, qt)
    qt, a = project_q(1)
    aq = jnp.maximum(aq, a)
    mean_b, inv = ln_scale(2, mean, qt)
    ak = project_k(0)
    ln_apply(2, mean_b, inv)
    kt_max = project_k(1, keep=True)
    ak = jnp.maximum(ak, kt_max[1])
    mean = ln_mean(3, kt_max[0])
    vt = project_v(2)
    mean_b, inv = ln_scale(3, mean, vt)
    qt, a = project_q(2)
    aq = jnp.maximum(aq, a)
    ln_apply(3, mean_b, inv)
    ak = jnp.maximum(ak, project_k(2))
    project_v(3)
    m1, m2, i1, i2 = route()
    ak = jnp.maximum(ak, project_k(3))
    qt, a = project_q(3)
    aq = jnp.maximum(aq, a)

    logit_bound = jnp.max(aq) * jnp.max(ak) * (DH * 1.02)
    safe = logit_bound <= SAFE_LOG2_RANGE

    sel_row = lax.broadcasted_iota(I32, (16, 128), 0)
    sel_lane = lax.broadcasted_iota(I32, (16, 128), 1)

    def token_tile(i):
        return i // L, pl.ds(pl.multiple_of(((i % L) // 128) * 128, 128), 128)

    def pick(i, slot):
        seg, cols = token_tile(i)
        onehot = jnp.where((sel_row == slot) & (sel_lane == i % 128), 1.0, 0.0).astype(BF16)
        return lax.dot_general(onehot, xn_buf[seg, :, cols], NT_DIMS, preferred_element_type=F32)

    xs = (pick(i1, 0) + pick(i2, 1)).astype(BF16)

    cp_wo.wait()
    cp_beta.wait()
    cp_wg.wait()
    cp_wu.wait()

    beta_row = beta_buf[...].reshape(1, H).astype(F32)
    beta_row = jnp.concatenate([beta_row, jnp.zeros((1, 128 - H), F32)], axis=1)
    h_row = lax.broadcasted_iota(I32, (H, 128), 0)
    h_lane = lax.broadcasted_iota(I32, (H, 128), 1)
    beta_col = jnp.sum(jnp.where(h_row == h_lane, beta_row, 0.0), axis=1, keepdims=True)
    gate_buf[...] = jnp.broadcast_to(jax.nn.sigmoid(beta_col), (H, 128))


    def expert_chunk(lo, hi):
        hg = jnp.dot(xs, wg_buf[:, lo:hi], preferred_element_type=F32)
        hu = jnp.dot(xs, wu_buf[:, lo:hi], preferred_element_type=F32)
        hh = (jax.nn.silu(hg) * hu).astype(BF16)
        return lax.dot_general(hh, wd_buf[:, lo:hi], NT_DIMS, preferred_element_type=F32)

    def expert_stream(result):
        kmain = 512
        hidden = []
        for c0 in range(0, FF, 512):
            rem = []
            for w_ref in (wg_buf, wu_buf):
                rem.append(jnp.dot(xs[:, kmain:D], w_ref[kmain:D, c0:c0 + 512], preferred_element_type=F32))
                yield
            hs = []
            for f0 in range(c0, c0 + 512, 128):
                pre = []
                for w_ref, r in zip((wg_buf, wu_buf), rem):
                    pre.append(jnp.dot(xs[:, 0:kmain], w_ref[0:kmain, f0:f0 + 128], preferred_element_type=F32)
                               + r[:, f0 - c0:f0 - c0 + 128])
                    yield
                hs.append(jax.nn.silu(pre[0]) * pre[1])
            hidden.append(jnp.concatenate(hs, axis=1).astype(BF16))
        y_tiles = [None] * 5
        for ci, hh in enumerate(hidden):
            for e in range(5):
                e_hi = min(128 * (e + 1), D)
                part = lax.dot_general(hh, wd_buf[128 * e:e_hi, 512 * ci:512 * (ci + 1)], NT_DIMS,
                                       preferred_element_type=F32)
                y_tiles[e] = part if y_tiles[e] is None else y_tiles[e] + part
                yield
        result.append(jnp.concatenate(y_tiles, axis=1))

    def expert_scatter(y):
        y = y * jax.nn.sigmoid(jnp.where(r16 == 0, m1, m2))
        yt = jnp.concatenate([y, jnp.zeros((128 - 16, D), F32)], axis=0).T
        lane_d = lax.broadcasted_iota(I32, (D, 128), 1)
        for slot, i in ((0, i1), (1, i2)):
            seg, cols = token_tile(i)
            col = jnp.sum(jnp.where(lane_d == slot, yt, 0.0), axis=1, keepdims=True)
            base[seg, :, cols] = base[seg, :, cols] + jnp.where(lane_d == i % 128, col, 0.0)

    def memory_read(s, g):
        rg = _group_rows(g)
        gw = GW[g]
        lhs = jnp.concatenate([mt_buf[g, 0:rg, 0:gw], mt_buf[g, ZROW:MROWS, 0:gw]], axis=0).astype(BF16)
        res = jnp.dot(lhs, pq_buf[s, 128 * g:128 * g + gw, :], preferred_element_type=F32)
        num_buf[g, 0:rg, :] = res[0:rg]
        num_buf[g, ZROW:MROWS, :] = res[rg:rg + 16]

    def memory_update(s, g):
        rg = _group_rows(g)
        a_g = _group_row_start(g)
        gw = GW[g]
        lhs = jnp.concatenate([vt_buf[s, a_g:a_g + rg, :], vt_buf[s, D:VROWS, :]], axis=0)
        upd = lax.dot_general(lhs, pk_buf[s, 128 * g:128 * g + gw, :], NT_DIMS,
                              preferred_element_type=F32)
        er = lax.broadcasted_iota(I32, (rg, gw), 0) + (a_g - HPG * DH * g)
        el = lax.broadcasted_iota(I32, (rg, gw), 1)
        same_head = None
        for i in range(_heads_in_group(g)):
            t = ((er >= DH * i) & (er < DH * (i + 1)) & (el >= DH * i) & (el < DH * (i + 1)))
            same_head = t if same_head is None else (same_head | t)
        mt_buf[g, 0:rg, 0:gw] = mt_buf[g, 0:rg, 0:gw] + jnp.where(same_head, upd[0:rg], 0.0)
        zr = lax.broadcasted_iota(I32, (8, gw), 0)
        zl = lax.broadcasted_iota(I32, (8, gw), 1)
        zmask = (zl >= zr * DH) & (zl < zr * DH + DH) & (zr < _heads_in_group(g))
        zs = upd[rg + 1:rg + 2]
        mt_buf[g, ZROW:ZROW + 8, 0:gw] = mt_buf[g, ZROW:ZROW + 8, 0:gw] + jnp.where(zmask, zs, 0.0)

    def transpose_wo(g):
        hi = min(128 * (g + 1), D)
        wot[128 * g:hi, :] = wo_raw[:, 128 * g:hi].T

    def project_out(s):
        attn = jnp.dot(wot[...], ot_buf[...].astype(BF16), preferred_element_type=F32)
        return base[s] + attn

    def emit(s, val):
        out_buf[s] = val.astype(BF16)
        out_copy(s).start()

    zero = lax.shift_right_logical(i1, 16)

    def prow(start, size):
        return pl.ds(pl.multiple_of(zero + start, 8), size)

    P_OFFS = (0, 128, 384, 768)

    def fast_scores(s, g, hook):
        nh = _heads_in_group(g)
        gw = GW[g]
        pb = (p_buf0, p_buf1)[(s * NG + g) % 2]
        rowg = lax.broadcasted_iota(I32, (gw, 128), 0)
        for j in range(QT - 1, -1, -1):
            n = 128 * (j + 1)
            q = qs_buf[s, 128 * g:128 * g + gw, 128 * j:128 * (j + 1)].astype(F32)
            for h0, h1 in ((0, 4), (4, nh)):
                if h1 <= h0:
                    continue
                qm = jnp.concatenate(
                    [jnp.where((rowg >= DH * i) & (rowg < DH * (i + 1)), q, 0.0) for i in range(h0, h1)],
                    axis=1).astype(BF16)
                st = jnp.dot(k_buf[s, g, 0:n, 0:gw], qm, preferred_element_type=F32)
                p = jnp.exp2(st)
                causal_w = jnp.concatenate([causal] * (h1 - h0), axis=1)
                p_diag = jnp.where(causal_w, p[n - 128:], 0.0)
                p = jnp.concatenate([p[:n - 128], p_diag], axis=0) if j > 0 else p_diag
                pb[P_OFFS[j] // 2:(P_OFFS[j] + n) // 2, h0 * 128:h1 * 128] = pltpu.bitcast(p.astype(BF16), U32)
                hook()

    def fast_values(s, g):
        nh = _heads_in_group(g)
        a_g = _group_row_start(g)
        pb = (p_buf0, p_buf1)[(s * NG + g) % 2]
        for j in range(QT - 1, -1, -1):
            n = 128 * (j + 1)
            cols = slice(128 * j, 128 * (j + 1))
            for i in range(nh):
                h = HPG * g + i
                a = (h * DH // 16) * 16
                off = h * DH - a
                p = pltpu.bitcast(pb[prow(P_OFFS[j] // 2, n // 2), 128 * i:128 * (i + 1)], BF16)
                ones_row = 0 if off > 0 else 31
                r32n = lax.broadcasted_iota(I32, (32, n), 0)
                lhs = jnp.where(r32n == ones_row, 1.0, vt_buf[s, a:a + 32, 0:n].astype(F32)).astype(BF16)
                o = jnp.dot(lhs, p, preferred_element_type=F32)
                lo = (off // 8) * 8
                hi = -(-(off + DH) // 8) * 8
                gate = gate_buf[h:h + 1, :]
                rl = 1.0 / o[ones_row:ones_row + 1]
                val = (1.0 - gate) * (o[lo:hi] * rl)
                if s > 0:
                    rden = 1.0 / (num_buf[g, ZROW + i:ZROW + i + 1, cols] + 1e-6)
                    num = num_buf[g, a - a_g + lo:a - a_g + hi, cols]
                    val = gate * (num * rden) + val
                ot_buf[a + off:a + off + DH, cols] = val[off - lo:off - lo + DH]

    def side_work():
        result = []
        yield from expert_stream(result)
        expert_scatter(result[0])
        yield
        for u in range(NSEG - 1):
            for j in range(QT):
                cols = slice(128 * j, 128 * (j + 1))
                out_buf[u, :, cols] = base[u, :, cols].astype(BF16)
                if j == QT - 1:
                    out_copy(u).start()
                yield

    def fast_path():
        stream = side_work()

        def hook():
            next(stream, None)

        steps = [(s, g) for s in range(NSEG) for g in range(NG)]
        fast_scores(0, 0, hook)
        for t, (s, g) in enumerate(steps):
            if t + 1 < len(steps):
                fast_scores(*steps[t + 1], hook)
            if s > 0:
                memory_read(s, g)
                hook()
            fast_values(s, g)
            if s == 0:
                transpose_wo(g)
            if s + 1 < NSEG:
                memory_update(s, g)
                hook()
            if g == NG - 1 and s < NSEG - 1:
                base[s] = project_out(s)
                if s == 0:
                    cp_wd.wait()
                hook()
        for _ in stream:
            pass
        s = NSEG - 1
        for j in range(QT):
            cols = slice(128 * j, 128 * (j + 1))
            attn = jnp.dot(wot[...], ot_buf[:, cols].astype(BF16), preferred_element_type=F32)
            out_buf[s, :, cols] = (base[s, :, cols] + attn).astype(BF16)
            out_tile_copy(j).start()
        for u in range(NSEG - 1):
            out_copy(u).wait()
        for j in range(QT):
            out_tile_copy(j).wait()

    def slow_segment(s, carry):
        for g in range(NG):
            memory_read(s, g)
        key_i = lax.broadcasted_iota(I32, (L, L), 0)
        qry_i = lax.broadcasted_iota(I32, (L, L), 1)
        r32 = lax.broadcasted_iota(I32, (32, L), 0)
        for g in range(NG):
            gw = GW[g]
            a_g = _group_row_start(g)
            rowg = lax.broadcasted_iota(I32, (gw, L), 0)

            def head(i, c, g=g, gw=gw, a_g=a_g, rowg=rowg):
                h = HPG * g + i
                a = pl.multiple_of((h * DH // 16) * 16, 16)
                off = h * DH - a
                q = qs_buf[s, 128 * g:128 * g + gw, :].astype(F32)
                qm = jnp.where((rowg >= DH * i) & (rowg < DH * (i + 1)), q, 0.0).astype(BF16)
                st = jnp.dot(k_buf[s, g, :, 0:gw], qm, preferred_element_type=F32)
                st = jnp.where(key_i <= qry_i, st, NEG_BIG)
                p = jnp.exp2(st - jnp.max(st, axis=0, keepdims=True))
                rl = 1.0 / jnp.sum(p, axis=0, keepdims=True)
                o = jnp.dot(vt_buf[s, pl.ds(a, 32), :], p.astype(BF16), preferred_element_type=F32)
                gate = jnp.concatenate([gate_buf[pl.ds(h, 1), :]] * QT, axis=1)
                rden = 1.0 / (num_buf[g, pl.ds(ZROW + i, 1), :] + 1e-6)
                num = num_buf[g, pl.ds(pl.multiple_of(a - a_g, 16), 32), :]
                val = gate * (num * rden) + (1.0 - gate) * (o * rl)
                keep = (r32 >= off) & (r32 < off + DH)
                pltpu.store(ot_buf.at[pl.ds(a, 32), :], val, mask=keep)
                return c

            lax.fori_loop(0, _heads_in_group(g), head, 0)
        for g in range(NG):
            memory_update(s, g)
        emit(s, project_out(s))
        return carry

    @pl.when(safe)
    def _():
        fast_path()

    @pl.when(jnp.logical_not(safe))
    def _():
        cp_wd.wait()
        for g in range(NG):
            transpose_wo(g)
        expert_scatter(expert_chunk(0, FF))
        lax.fori_loop(0, NSEG, slow_segment, 0)
        for u in range(NSEG):
            out_copy(u).wait()


@jax.jit
def pallas_parallel_sum__memory_aug_infini_attn__moe_arch_mod__prompt_kernel(
    A_x: jax.Array,
    A_wq: jax.Array,
    A_wk: jax.Array,
    A_wv: jax.Array,
    A_wo: jax.Array,
    A_beta: jax.Array,
    B_x: jax.Array,
    B_w_r: jax.Array,
    B_w_gate: jax.Array,
    B_w_up: jax.Array,
    B_w_down: jax.Array,
):
    del B_x
    hbm = pl.BlockSpec(memory_space=pl.ANY)
    scratch = [
        pltpu.VMEM((NSEG, D, L), BF16),
        pltpu.VMEM((D, D), BF16),
        pltpu.VMEM((D, D), BF16),
        pltpu.VMEM((D, D), BF16),
        pltpu.VMEM((D, D), BF16),
        pltpu.VMEM((H,), BF16),
        pltpu.VMEM((D,), BF16),
        pltpu.VMEM((D, FF), BF16),
        pltpu.VMEM((D, FF), BF16),
        pltpu.VMEM((D, FF), BF16),
        pltpu.VMEM((PR, D), BF16),
        pltpu.VMEM((PR, D), BF16),
        pltpu.VMEM((VROWS, D), BF16),
        pltpu.VMEM((D, D), BF16),
        pltpu.VMEM((NSEG, D, L), BF16),
        pltpu.VMEM((NSEG, D, L), F32),
        pltpu.VMEM((NSEG, PR, L), BF16),
        pltpu.VMEM((NSEG, PR, L), BF16),
        pltpu.VMEM((NSEG, NG, L, 128), BF16),
        pltpu.VMEM((NSEG, PR, L), BF16),
        pltpu.VMEM((NSEG, VROWS, L), BF16),
        pltpu.VMEM((8, S), F32),
        pltpu.VMEM((H, 128), F32),
        pltpu.VMEM((NG, MROWS, 128), F32),
        pltpu.VMEM((NG, MROWS, L), F32),
        pltpu.VMEM((640, HPG * 128), U32),
        pltpu.VMEM((640, HPG * 128), U32),
        pltpu.VMEM((D, L), F32),
        pltpu.VMEM((NSEG, D, L), BF16),
        pltpu.SemaphoreType.DMA((13,)),
        pltpu.SemaphoreType.DMA((NSEG + QT,)),
    ]
    out_t = pl.pallas_call(
        _kernel,
        out_shape=jax.ShapeDtypeStruct((1, D, S), BF16),
        in_specs=[hbm] * 10,
        out_specs=hbm,
        scratch_shapes=scratch,
        compiler_params=pltpu.CompilerParams(vmem_limit_bytes=128 * 1024 * 1024),
        name="infini_attn_moe",
    )(jnp.transpose(A_x, (0, 2, 1)), A_wq, A_wk, A_wv, A_wo, A_beta, B_w_r, B_w_gate, B_w_up,
      B_w_down.T)
    return jnp.transpose(out_t, (0, 2, 1))
```

```python
import jax
import jax.numpy as jnp
from jax import lax
import jax.experimental.pallas as pl
import jax.experimental.pallas.tpu as pltpu

F32 = jnp.float32
BF16 = jnp.bfloat16
U32 = jnp.uint32
I32 = jnp.int32

S = 2048
D = 576
H = 32
DH = 18
NSEG = 4
L = 512
FF = 4608
HPG = 7
NG = 5
QT = L // 128
GW = (128, 128, 128, 128, 80)
PR = sum(GW)
VROWS = D + 16
ROUTER_ROW = 126
ZROW = 144
MROWS = 160
LOG2E = 1.4426950408889634
QSCALE = (DH ** -0.5) * LOG2E
SAFE_LOG2_RANGE = 60.0
NEG_BIG = -1e30

NT_DIMS = (((1,), (1,)), ((), ()))


def _heads_in_group(g):
    return min(HPG, H - HPG * g)


def _group_row_start(g):
    return (HPG * g * DH // 16) * 16


def _group_rows(g):
    last = (HPG * g + _heads_in_group(g)) * DH
    return -(-(last - _group_row_start(g)) // 16) * 16


def _round_bf16(x):
    return x.astype(BF16).astype(F32)


def _pad_heads_t(w):
    parts = []
    for g in range(NG):
        n = _heads_in_group(g) * DH
        parts.append(w[:, HPG * DH * g:HPG * DH * g + n])
        parts.append(jnp.zeros((D, 128 - n), w.dtype))
    return jnp.concatenate(parts, axis=1).T[0:PR]


def _phi(t):
    return jnp.where(t > 0, t + 1.0, jnp.exp(t))


def _kernel(x_hbm, wq_hbm, wk_hbm, wv_hbm, wo_hbm, beta_hbm, wr_hbm, wg_hbm, wu_hbm, wd_hbm,
            out_hbm,
            x_buf, wq_raw, wk_raw, wv_raw, wo_raw, beta_buf, wr_buf, wg_buf, wu_buf, wd_buf,
            wqt, wkt, wvt, wot, xn_buf, base, qs_buf, pq_buf, k_buf, pk_buf, vt_buf, r_buf,
            gate_buf, mt_buf, num_buf, p_buf0, p_buf1, ot_buf, out_buf, in_sems, out_sems):
    def x_copy(c):
        return pltpu.make_async_copy(x_hbm.at[0, :, pl.ds(c * L, L)], x_buf.at[c], in_sems.at[c])

    cp_wv = pltpu.make_async_copy(wv_hbm, wv_raw, in_sems.at[4])
    cp_wq = pltpu.make_async_copy(wq_hbm, wq_raw, in_sems.at[5])
    cp_wk = pltpu.make_async_copy(wk_hbm, wk_raw, in_sems.at[6])
    cp_wo = pltpu.make_async_copy(wo_hbm, wo_raw, in_sems.at[7])
    cp_wg = pltpu.make_async_copy(wg_hbm, wg_buf, in_sems.at[8])
    cp_wu = pltpu.make_async_copy(wu_hbm, wu_buf, in_sems.at[9])
    cp_wd = pltpu.make_async_copy(wd_hbm, wd_buf, in_sems.at[10])
    cp_beta = pltpu.make_async_copy(beta_hbm, beta_buf, in_sems.at[11])
    cp_wr = pltpu.make_async_copy(wr_hbm, wr_buf, in_sems.at[12])

    def out_copy(s):
        cols = pl.ds(pl.multiple_of(s * L, L), L)
        return pltpu.make_async_copy(out_buf.at[s], out_hbm.at[0, :, cols], out_sems.at[s])

    def out_tile_copy(j):
        s = NSEG - 1
        return pltpu.make_async_copy(out_buf.at[s, :, pl.ds(128 * j, 128)],
                                     out_hbm.at[0, :, pl.ds(s * L + 128 * j, 128)], out_sems.at[NSEG + j])


    for cp in (cp_wv, x_copy(0), x_copy(1), cp_wq, cp_wr, x_copy(2), cp_wk, x_copy(3), cp_wo, cp_beta,
               cp_wg, cp_wu, cp_wd):
        cp.start()

    lane128 = lax.broadcasted_iota(I32, (128, 128), 1)
    row128 = lax.broadcasted_iota(I32, (128, 128), 0)
    causal = row128 <= lane128
    r16 = lax.broadcasted_iota(I32, (16, D), 0)

    mt_buf[...] = jnp.zeros(mt_buf.shape, F32)

    always = []

    def pace(x, y):
        return x if y is None else jnp.where(always[0], x, y[0:D])

    def ln_mean(c, y):
        return jnp.sum(pace(x_buf[c].astype(F32), y), axis=0, keepdims=True) * (1.0 / D)

    def ln_scale(c, mean, y):
        mean_b = _round_bf16(mean)
        d = pace(x_buf[c].astype(F32), y) - mean_b
        msq = jnp.sum(d * d, axis=0, keepdims=True) * (1.0 / D)
        off = mean - mean_b
        var = jnp.maximum(msq - off * off, 0.0)
        return mean_b, 1.0 / _round_bf16(jnp.sqrt(_round_bf16(_round_bf16(var) + 1e-5)))

    def ln_apply(c, mean_b, inv):
        x = x_buf[c].astype(F32)
        xn = (x - mean_b) * inv
        xn_buf[c] = xn.astype(BF16)
        base[c] = x + xn

    def project(w_ref, c, split):
        if not split:
            return jnp.dot(w_ref[...], xn_buf[c], preferred_element_type=F32), None
        head = jnp.dot(w_ref[:, 0:256], xn_buf[c, 0:256, :], preferred_element_type=F32)
        tail = jnp.dot(w_ref[:, 256:D], xn_buf[c, 256:D, :], preferred_element_type=F32)
        return head + tail, head

    def project_v(c, mid=None):
        vt, head = project(wvt, c, mid is not None)
        if mid is not None:
            mid(head)
        vt_buf[c, 0:D, :] = vt.astype(BF16)
        r16l = lax.broadcasted_iota(I32, (16, L), 0)
        vt_buf[c, D:VROWS, :] = jnp.where(r16l == 1, 1.0, 0.0).astype(BF16)
        return vt

    def project_q(c, mid=None):
        qt, head = project(wqt, c, mid is not None)
        if mid is not None:
            mid(head)
        qsc = qt * QSCALE
        qs_buf[c] = qsc.astype(BF16)
        pq_buf[c] = _phi(qt).astype(BF16)
        r_buf[:, c * L:(c + 1) * L] = qt[120:128]
        mag = jnp.abs(qsc)
        r8 = lax.broadcasted_iota(I32, (8, L), 0)
        mag = jnp.concatenate([mag[0:120], jnp.where(r8 == ROUTER_ROW - 120, 0.0, mag[120:128]), mag[128:]], axis=0)
        return qt, jnp.max(mag.reshape(PR // 8, 8, L), axis=0)

    def project_k(c, mid=None, keep=False):
        kt, head = project(wkt, c, mid is not None)
        if mid is not None:
            mid(head)
        pk_buf[c] = _phi(kt).astype(BF16)
        for g in range(NG):
            ktg = kt[128 * g:128 * g + GW[g]]
            if GW[g] < 128:
                ktg = jnp.concatenate([ktg, jnp.zeros((128 - GW[g], L), F32)], axis=0)
            k_buf[c, g] = ktg.T.astype(BF16)
        top = jnp.max(jnp.abs(kt).reshape(PR // 8, 8, L), axis=0)
        return (kt, top) if keep else top

    cp_wv.wait()
    wvt[...] = wv_raw[...].T
    x_copy(0).wait()
    mean = ln_mean(0, None)
    always.append(jnp.logical_not(jnp.abs(mean) < 0.0))
    ln_apply(0, *ln_scale(0, mean, None))
    x_copy(1).wait()
    mean = ln_mean(1, None)
    stats = []
    project_v(0, lambda y: stats.extend(ln_scale(1, mean, y)))
    ln_apply(1, *stats)
    cp_wq.wait()
    cp_wr.wait()
    wq_t = _pad_heads_t(wq_raw[...].astype(F32))
    wr_row = wr_buf[...].reshape(1, D).astype(F32)
    pr_row = lax.broadcasted_iota(I32, (8, D), 0)
    wq_t = jnp.concatenate([wq_t[0:120], jnp.where(pr_row == ROUTER_ROW - 120, wr_row, wq_t[120:128]), wq_t[128:]],
                           axis=0)
    wqt[...] = wq_t.astype(BF16)
    project_v(1)
    cp_wk.wait()
    x_copy(2).wait()
    x_copy(3).wait()

    def prep_wk(y):
        wk = wk_raw[...].astype(F32)
        wk = jnp.concatenate([jnp.where(always[0], wk[:, 0:L], y[0:D]), wk[:, L:D]], axis=1)
        wkt[...] = _pad_heads_t(wk).astype(BF16)

    def route():
        r = _round_bf16(r_buf[ROUTER_ROW - 120:ROUTER_ROW - 119, :])
        tok = lax.broadcasted_iota(I32, (1, S), 1).astype(F32)
        m1 = jnp.max(r)
        i1 = jnp.min(jnp.where(r == m1, tok, float(S)))
        r_rest = jnp.where(tok == i1, -jnp.inf, r)
        m2 = jnp.max(r_rest)
        i2 = jnp.min(jnp.where(r_rest == m2, tok, float(S)))
        i1 = jnp.clip(i1.astype(I32), 0, S - 1)
        i2 = jnp.clip(i2.astype(I32), 0, S - 1)
        return m1, m2, i1, i2

    qt, aq = project_q(0, prep_wk)
    mean = ln_mean(2, qt)
    qt, a = project_q(1)
    aq = jnp.maximum(aq, a)
    mean_b, inv = ln_scale(2, mean, qt)
    ak = project_k(0)
    ln_apply(2, mean_b, inv)
    kt_max = project_k(1, keep=True)
    ak = jnp.maximum(ak, kt_max[1])
    mean = ln_mean(3, kt_max[0])
    vt = project_v(2)
    mean_b, inv = ln_scale(3, mean, vt)
    qt, a = project_q(2)
    aq = jnp.maximum(aq, a)
    ln_apply(3, mean_b, inv)
    ak = jnp.maximum(ak, project_k(2))
    qt, a = project_q(3)
    aq = jnp.maximum(aq, a)
    m1, m2, i1, i2 = route()
    ak = jnp.maximum(ak, project_k(3))
    project_v(3)

    logit_bound = jnp.max(aq) * jnp.max(ak) * (DH * 1.02)
    safe = logit_bound <= SAFE_LOG2_RANGE

    sel_row = lax.broadcasted_iota(I32, (16, 128), 0)
    sel_lane = lax.broadcasted_iota(I32, (16, 128), 1)

    def token_tile(i):
        return i // L, pl.ds(pl.multiple_of(((i % L) // 128) * 128, 128), 128)

    def pick(i, slot):
        seg, cols = token_tile(i)
        onehot = jnp.where((sel_row == slot) & (sel_lane == i % 128), 1.0, 0.0).astype(BF16)
        return lax.dot_general(onehot, xn_buf[seg, :, cols], NT_DIMS, preferred_element_type=F32)

    xs = (pick(i1, 0) + pick(i2, 1)).astype(BF16)

    cp_wo.wait()
    cp_beta.wait()
    cp_wg.wait()
    cp_wu.wait()

    beta_row = beta_buf[...].reshape(1, H).astype(F32)
    beta_row = jnp.concatenate([beta_row, jnp.zeros((1, 128 - H), F32)], axis=1)
    h_row = lax.broadcasted_iota(I32, (H, 128), 0)
    h_lane = lax.broadcasted_iota(I32, (H, 128), 1)
    beta_col = jnp.sum(jnp.where(h_row == h_lane, beta_row, 0.0), axis=1, keepdims=True)
    gate_buf[...] = jnp.broadcast_to(jax.nn.sigmoid(beta_col), (H, 128))


    def expert_chunk(lo, hi):
        hg = jnp.dot(xs, wg_buf[:, lo:hi], preferred_element_type=F32)
        hu = jnp.dot(xs, wu_buf[:, lo:hi], preferred_element_type=F32)
        hh = (jax.nn.silu(hg) * hu).astype(BF16)
        return lax.dot_general(hh, wd_buf[:, lo:hi], NT_DIMS, preferred_element_type=F32)

    def expert_stream(result):
        kmain = 512
        hidden = []
        for c0 in range(0, FF, 512):
            rem = []
            for w_ref in (wg_buf, wu_buf):
                rem.append(jnp.dot(xs[:, kmain:D], w_ref[kmain:D, c0:c0 + 512], preferred_element_type=F32))
                yield
            hs = []
            for f0 in range(c0, c0 + 512, 128):
                pre = []
                for w_ref, r in zip((wg_buf, wu_buf), rem):
                    pre.append(jnp.dot(xs[:, 0:kmain], w_ref[0:kmain, f0:f0 + 128], preferred_element_type=F32)
                               + r[:, f0 - c0:f0 - c0 + 128])
                    yield
                hs.append(jax.nn.silu(pre[0]) * pre[1])
            hidden.append(jnp.concatenate(hs, axis=1).astype(BF16))
        y_tiles = [None] * 5
        for ci, hh in enumerate(hidden):
            for e in range(5):
                e_hi = min(128 * (e + 1), D)
                part = lax.dot_general(hh, wd_buf[128 * e:e_hi, 512 * ci:512 * (ci + 1)], NT_DIMS,
                                       preferred_element_type=F32)
                y_tiles[e] = part if y_tiles[e] is None else y_tiles[e] + part
                yield
        result.append(jnp.concatenate(y_tiles, axis=1))

    def expert_scatter(y):
        y = y * jax.nn.sigmoid(jnp.where(r16 == 0, m1, m2))
        yt = jnp.concatenate([y, jnp.zeros((128 - 16, D), F32)], axis=0).T
        lane_d = lax.broadcasted_iota(I32, (D, 128), 1)
        for slot, i in ((0, i1), (1, i2)):
            seg, cols = token_tile(i)
            col = jnp.sum(jnp.where(lane_d == slot, yt, 0.0), axis=1, keepdims=True)
            base[seg, :, cols] = base[seg, :, cols] + jnp.where(lane_d == i % 128, col, 0.0)

    def memory_read(s, g):
        rg = _group_rows(g)
        gw = GW[g]
        lhs = jnp.concatenate([mt_buf[g, 0:rg, 0:gw], mt_buf[g, ZROW:MROWS, 0:gw]], axis=0).astype(BF16)
        res = jnp.dot(lhs, pq_buf[s, 128 * g:128 * g + gw, :], preferred_element_type=F32)
        num_buf[g, 0:rg, :] = res[0:rg]
        num_buf[g, ZROW:MROWS, :] = res[rg:rg + 16]

    def memory_update(s, g):
        rg = _group_rows(g)
        a_g = _group_row_start(g)
        gw = GW[g]
        lhs = jnp.concatenate([vt_buf[s, a_g:a_g + rg, :], vt_buf[s, D:VROWS, :]], axis=0)
        upd = lax.dot_general(lhs, pk_buf[s, 128 * g:128 * g + gw, :], NT_DIMS,
                              preferred_element_type=F32)
        er = lax.broadcasted_iota(I32, (rg, gw), 0) + (a_g - HPG * DH * g)
        el = lax.broadcasted_iota(I32, (rg, gw), 1)
        same_head = None
        for i in range(_heads_in_group(g)):
            t = ((er >= DH * i) & (er < DH * (i + 1)) & (el >= DH * i) & (el < DH * (i + 1)))
            same_head = t if same_head is None else (same_head | t)
        mt_buf[g, 0:rg, 0:gw] = mt_buf[g, 0:rg, 0:gw] + jnp.where(same_head, upd[0:rg], 0.0)
        zr = lax.broadcasted_iota(I32, (8, gw), 0)
        zl = lax.broadcasted_iota(I32, (8, gw), 1)
        zmask = (zl >= zr * DH) & (zl < zr * DH + DH) & (zr < _heads_in_group(g))
        zs = upd[rg + 1:rg + 2]
        mt_buf[g, ZROW:ZROW + 8, 0:gw] = mt_buf[g, ZROW:ZROW + 8, 0:gw] + jnp.where(zmask, zs, 0.0)

    def transpose_wo(g):
        hi = min(128 * (g + 1), D)
        wot[128 * g:hi, :] = wo_raw[:, 128 * g:hi].T

    def project_out(s):
        attn = jnp.dot(wot[...], ot_buf[...].astype(BF16), preferred_element_type=F32)
        return base[s] + attn

    def emit(s, val):
        out_buf[s] = val.astype(BF16)
        out_copy(s).start()

    zero = lax.shift_right_logical(i1, 16)

    def prow(start, size):
        return pl.ds(pl.multiple_of(zero + start, 8), size)

    P_OFFS = (0, 128, 384, 768)

    def fast_scores(s, g, hook):
        nh = _heads_in_group(g)
        gw = GW[g]
        pb = (p_buf0, p_buf1)[(s * NG + g) % 2]
        rowg = lax.broadcasted_iota(I32, (gw, 128), 0)
        for j in range(QT - 1, -1, -1):
            n = 128 * (j + 1)
            q = qs_buf[s, 128 * g:128 * g + gw, 128 * j:128 * (j + 1)].astype(F32)
            for h0, h1 in ((0, 4), (4, nh)):
                if h1 <= h0:
                    continue
                qm = jnp.concatenate(
                    [jnp.where((rowg >= DH * i) & (rowg < DH * (i + 1)), q, 0.0) for i in range(h0, h1)],
                    axis=1).astype(BF16)
                st = jnp.dot(k_buf[s, g, 0:n, 0:gw], qm, preferred_element_type=F32)
                p = jnp.exp2(st)
                causal_w = jnp.concatenate([causal] * (h1 - h0), axis=1)
                p_diag = jnp.where(causal_w, p[n - 128:], 0.0)
                p = jnp.concatenate([p[:n - 128], p_diag], axis=0) if j > 0 else p_diag
                pb[P_OFFS[j] // 2:(P_OFFS[j] + n) // 2, h0 * 128:h1 * 128] = pltpu.bitcast(p.astype(BF16), U32)
                hook()

    def fast_values(s, g):
        nh = _heads_in_group(g)
        a_g = _group_row_start(g)
        pb = (p_buf0, p_buf1)[(s * NG + g) % 2]
        for j in range(QT - 1, -1, -1):
            n = 128 * (j + 1)
            cols = slice(128 * j, 128 * (j + 1))
            for i in range(nh):
                h = HPG * g + i
                a = (h * DH // 16) * 16
                off = h * DH - a
                p = pltpu.bitcast(pb[prow(P_OFFS[j] // 2, n // 2), 128 * i:128 * (i + 1)], BF16)
                ones_row = 0 if off > 0 else 31
                r32n = lax.broadcasted_iota(I32, (32, n), 0)
                lhs = jnp.where(r32n == ones_row, 1.0, vt_buf[s, a:a + 32, 0:n].astype(F32)).astype(BF16)
                o = jnp.dot(lhs, p, preferred_element_type=F32)
                lo = (off // 8) * 8
                hi = -(-(off + DH) // 8) * 8
                gate = gate_buf[h:h + 1, :]
                rl = 1.0 / o[ones_row:ones_row + 1]
                val = (1.0 - gate) * (o[lo:hi] * rl)
                if s > 0:
                    rden = 1.0 / (num_buf[g, ZROW + i:ZROW + i + 1, cols] + 1e-6)
                    num = num_buf[g, a - a_g + lo:a - a_g + hi, cols]
                    val = gate * (num * rden) + val
                ot_buf[a + off:a + off + DH, cols] = val[off - lo:off - lo + DH]

    def side_work():
        result = []
        yield from expert_stream(result)
        expert_scatter(result[0])
        yield
        for u in range(NSEG - 1):
            for j in range(QT):
                cols = slice(128 * j, 128 * (j + 1))
                out_buf[u, :, cols] = base[u, :, cols].astype(BF16)
                if j == QT - 1:
                    out_copy(u).start()
                yield

    def fast_path():
        stream = side_work()

        def hook():
            next(stream, None)

        steps = [(s, g) for s in range(NSEG) for g in range(NG)]
        fast_scores(0, 0, hook)
        for t, (s, g) in enumerate(steps):
            if t + 1 < len(steps):
                fast_scores(*steps[t + 1], hook)
            if s > 0:
                memory_read(s, g)
                hook()
            fast_values(s, g)
            if s == 0:
                transpose_wo(g)
            if s + 1 < NSEG:
                memory_update(s, g)
                hook()
            if g == NG - 1 and s < NSEG - 1:
                base[s] = project_out(s)
                if s == 0:
                    cp_wd.wait()
                hook()
        for _ in stream:
            pass
        s = NSEG - 1
        for j in range(QT):
            cols = slice(128 * j, 128 * (j + 1))
            attn = jnp.dot(wot[...], ot_buf[:, cols].astype(BF16), preferred_element_type=F32)
            out_buf[s, :, cols] = (base[s, :, cols] + attn).astype(BF16)
            out_tile_copy(j).start()
        for u in range(NSEG - 1):
            out_copy(u).wait()
        for j in range(QT):
            out_tile_copy(j).wait()

    def slow_segment(s, carry):
        for g in range(NG):
            memory_read(s, g)
        key_i = lax.broadcasted_iota(I32, (L, L), 0)
        qry_i = lax.broadcasted_iota(I32, (L, L), 1)
        r32 = lax.broadcasted_iota(I32, (32, L), 0)
        for g in range(NG):
            gw = GW[g]
            a_g = _group_row_start(g)
            rowg = lax.broadcasted_iota(I32, (gw, L), 0)

            def head(i, c, g=g, gw=gw, a_g=a_g, rowg=rowg):
                h = HPG * g + i
                a = pl.multiple_of((h * DH // 16) * 16, 16)
                off = h * DH - a
                q = qs_buf[s, 128 * g:128 * g + gw, :].astype(F32)
                qm = jnp.where((rowg >= DH * i) & (rowg < DH * (i + 1)), q, 0.0).astype(BF16)
                st = jnp.dot(k_buf[s, g, :, 0:gw], qm, preferred_element_type=F32)
                st = jnp.where(key_i <= qry_i, st, NEG_BIG)
                p = jnp.exp2(st - jnp.max(st, axis=0, keepdims=True))
                rl = 1.0 / jnp.sum(p, axis=0, keepdims=True)
                o = jnp.dot(vt_buf[s, pl.ds(a, 32), :], p.astype(BF16), preferred_element_type=F32)
                gate = jnp.concatenate([gate_buf[pl.ds(h, 1), :]] * QT, axis=1)
                rden = 1.0 / (num_buf[g, pl.ds(ZROW + i, 1), :] + 1e-6)
                num = num_buf[g, pl.ds(pl.multiple_of(a - a_g, 16), 32), :]
                val = gate * (num * rden) + (1.0 - gate) * (o * rl)
                keep = (r32 >= off) & (r32 < off + DH)
                pltpu.store(ot_buf.at[pl.ds(a, 32), :], val, mask=keep)
                return c

            lax.fori_loop(0, _heads_in_group(g), head, 0)
        for g in range(NG):
            memory_update(s, g)
        emit(s, project_out(s))
        return carry

    @pl.when(safe)
    def _():
        fast_path()

    @pl.when(jnp.logical_not(safe))
    def _():
        cp_wd.wait()
        for g in range(NG):
            transpose_wo(g)
        expert_scatter(expert_chunk(0, FF))
        lax.fori_loop(0, NSEG, slow_segment, 0)
        for u in range(NSEG):
            out_copy(u).wait()


@jax.jit
def pallas_parallel_sum__memory_aug_infini_attn__moe_arch_mod__prompt_kernel(
    A_x: jax.Array,
    A_wq: jax.Array,
    A_wk: jax.Array,
    A_wv: jax.Array,
    A_wo: jax.Array,
    A_beta: jax.Array,
    B_x: jax.Array,
    B_w_r: jax.Array,
    B_w_gate: jax.Array,
    B_w_up: jax.Array,
    B_w_down: jax.Array,
):
    del B_x
    hbm = pl.BlockSpec(memory_space=pl.ANY)
    scratch = [
        pltpu.VMEM((NSEG, D, L), BF16),
        pltpu.VMEM((D, D), BF16),
        pltpu.VMEM((D, D), BF16),
        pltpu.VMEM((D, D), BF16),
        pltpu.VMEM((D, D), BF16),
        pltpu.VMEM((H,), BF16),
        pltpu.VMEM((D,), BF16),
        pltpu.VMEM((D, FF), BF16),
        pltpu.VMEM((D, FF), BF16),
        pltpu.VMEM((D, FF), BF16),
        pltpu.VMEM((PR, D), BF16),
        pltpu.VMEM((PR, D), BF16),
        pltpu.VMEM((D, D), BF16),
        pltpu.VMEM((D, D), BF16),
        pltpu.VMEM((NSEG, D, L), BF16),
        pltpu.VMEM((NSEG, D, L), F32),
        pltpu.VMEM((NSEG, PR, L), BF16),
        pltpu.VMEM((NSEG, PR, L), BF16),
        pltpu.VMEM((NSEG, NG, L, 128), BF16),
        pltpu.VMEM((NSEG, PR, L), BF16),
        pltpu.VMEM((NSEG, VROWS, L), BF16),
        pltpu.VMEM((8, S), F32),
        pltpu.VMEM((H, 128), F32),
        pltpu.VMEM((NG, MROWS, 128), F32),
        pltpu.VMEM((NG, MROWS, L), F32),
        pltpu.VMEM((640, HPG * 128), U32),
        pltpu.VMEM((640, HPG * 128), U32),
        pltpu.VMEM((D, L), F32),
        pltpu.VMEM((NSEG, D, L), BF16),
        pltpu.SemaphoreType.DMA((13,)),
        pltpu.SemaphoreType.DMA((NSEG + QT,)),
    ]
    out_t = pl.pallas_call(
        _kernel,
        out_shape=jax.ShapeDtypeStruct((1, D, S), BF16),
        in_specs=[hbm] * 10,
        out_specs=hbm,
        scratch_shapes=scratch,
        compiler_params=pltpu.CompilerParams(vmem_limit_bytes=128 * 1024 * 1024),
        name="infini_attn_moe",
    )(jnp.transpose(A_x, (0, 2, 1)), A_wq, A_wk, A_wv, A_wo, A_beta, B_w_r, B_w_gate, B_w_up,
      B_w_down.T)
    return jnp.transpose(out_t, (0, 2, 1))
```

```python
import jax
import jax.numpy as jnp
from jax import lax
import jax.experimental.pallas as pl
import jax.experimental.pallas.tpu as pltpu

F32 = jnp.float32
BF16 = jnp.bfloat16
U32 = jnp.uint32
I32 = jnp.int32

S = 2048
D = 576
H = 32
DH = 18
NSEG = 4
L = 512
FF = 4608
HPG = 7
NG = 5
QT = L // 128
GW = (128, 128, 128, 128, 80)
PR = sum(GW)
VROWS = D + 16
ROUTER_ROW = 126
ZROW = 144
MROWS = 160
LOG2E = 1.4426950408889634
QSCALE = (DH ** -0.5) * LOG2E
SAFE_LOG2_RANGE = 60.0
NEG_BIG = -1e30

NT_DIMS = (((1,), (1,)), ((), ()))


def _heads_in_group(g):
    return min(HPG, H - HPG * g)


def _group_row_start(g):
    return (HPG * g * DH // 16) * 16


def _group_rows(g):
    last = (HPG * g + _heads_in_group(g)) * DH
    return -(-(last - _group_row_start(g)) // 16) * 16


def _round_bf16(x):
    return x.astype(BF16).astype(F32)


def _pad_heads_t(w):
    parts = []
    for g in range(NG):
        n = _heads_in_group(g) * DH
        parts.append(w[:, HPG * DH * g:HPG * DH * g + n])
        parts.append(jnp.zeros((D, 128 - n), w.dtype))
    return jnp.concatenate(parts, axis=1).T[0:PR]


def _phi(t):
    return jnp.where(t > 0, t + 1.0, jnp.exp(t))


def _kernel(x_hbm, wq_hbm, wk_hbm, wv_hbm, wo_hbm, beta_hbm, wr_hbm, wg_hbm, wu_hbm, wd_hbm,
            out_hbm,
            x_buf, wq_raw, wk_raw, wv_raw, wo_raw, beta_buf, wr_buf, wg_buf, wu_buf, wd_buf,
            wqt, wkt, wvt, wot, xn_buf, base, qs_buf, pq_buf, k_buf, pk_buf, vt_buf, r_buf,
            gate_buf, mt_buf, num_buf, p_buf0, p_buf1, ot_buf, out_buf, in_sems, out_sems):
    def x_copy(c):
        return pltpu.make_async_copy(x_hbm.at[0, :, pl.ds(c * L, L)], x_buf.at[c], in_sems.at[c])

    cp_wv = pltpu.make_async_copy(wv_hbm, wv_raw, in_sems.at[4])
    cp_wq = pltpu.make_async_copy(wq_hbm, wq_raw, in_sems.at[5])
    cp_wk = pltpu.make_async_copy(wk_hbm, wk_raw, in_sems.at[6])
    cp_wo = pltpu.make_async_copy(wo_hbm, wo_raw, in_sems.at[7])
    cp_wg = pltpu.make_async_copy(wg_hbm, wg_buf, in_sems.at[8])
    cp_wu = pltpu.make_async_copy(wu_hbm, wu_buf, in_sems.at[9])
    cp_wd = pltpu.make_async_copy(wd_hbm, wd_buf, in_sems.at[10])
    cp_beta = pltpu.make_async_copy(beta_hbm, beta_buf, in_sems.at[11])
    cp_wr = pltpu.make_async_copy(wr_hbm, wr_buf, in_sems.at[12])

    def out_copy(s):
        cols = pl.ds(pl.multiple_of(s * L, L), L)
        return pltpu.make_async_copy(out_buf.at[s], out_hbm.at[0, :, cols], out_sems.at[s])

    def out_tile_copy(j):
        s = NSEG - 1
        return pltpu.make_async_copy(out_buf.at[s, :, pl.ds(128 * j, 128)],
                                     out_hbm.at[0, :, pl.ds(s * L + 128 * j, 128)], out_sems.at[NSEG + j])


    for cp in (x_copy(0), cp_wv, x_copy(1), cp_wq, cp_wr, x_copy(2), cp_wk, x_copy(3), cp_wo, cp_beta,
               cp_wg, cp_wu, cp_wd):
        cp.start()

    lane128 = lax.broadcasted_iota(I32, (128, 128), 1)
    row128 = lax.broadcasted_iota(I32, (128, 128), 0)
    causal = row128 <= lane128
    r16 = lax.broadcasted_iota(I32, (16, D), 0)

    mt_buf[...] = jnp.zeros(mt_buf.shape, F32)

    always = []

    def pace(x, y):
        return x if y is None else jnp.where(always[0], x, y[0:D])

    def ln_stats(c, y):
        x = pace(x_buf[c].astype(F32), y)
        shift = x_buf[c, 0:16, :].astype(F32)[0:1]
        d = x - shift
        m1 = jnp.sum(d, axis=0, keepdims=True) * (1.0 / D)
        m2 = jnp.sum(d * d, axis=0, keepdims=True) * (1.0 / D)
        var = jnp.maximum(m2 - m1 * m1, 0.0)
        inv = 1.0 / _round_bf16(jnp.sqrt(_round_bf16(_round_bf16(var) + 1e-5)))
        return _round_bf16(shift + m1), inv

    def ln_apply(c, mean_b, inv):
        x = x_buf[c].astype(F32)
        xn = (x - mean_b) * inv
        xn_buf[c] = xn.astype(BF16)
        base[c] = x + xn

    def project(w_ref, c, split):
        if not split:
            return jnp.dot(w_ref[...], xn_buf[c], preferred_element_type=F32), None
        head = jnp.dot(w_ref[:, 0:256], xn_buf[c, 0:256, :], preferred_element_type=F32)
        tail = jnp.dot(w_ref[:, 256:D], xn_buf[c, 256:D, :], preferred_element_type=F32)
        return head + tail, head

    def project_v(c, mid=None):
        vt, head = project(wvt, c, mid is not None)
        if mid is not None:
            mid(head)
        vt_buf[c, 0:D, :] = vt.astype(BF16)
        r16l = lax.broadcasted_iota(I32, (16, L), 0)
        vt_buf[c, D:VROWS, :] = jnp.where(r16l == 1, 1.0, 0.0).astype(BF16)
        return vt

    def project_q(c, mid=None):
        qt, head = project(wqt, c, mid is not None)
        if mid is not None:
            mid(head)
        qsc = qt * QSCALE
        qs_buf[c] = qsc.astype(BF16)
        pq_buf[c] = _phi(qt).astype(BF16)
        r_buf[:, c * L:(c + 1) * L] = qt[120:128]
        mag = jnp.abs(qsc)
        r8 = lax.broadcasted_iota(I32, (8, L), 0)
        mag = jnp.concatenate([mag[0:120], jnp.where(r8 == ROUTER_ROW - 120, 0.0, mag[120:128]), mag[128:]], axis=0)
        return qt, jnp.max(mag.reshape(PR // 8, 8, L), axis=0)

    def project_k(c, mid=None, keep=False):
        kt, head = project(wkt, c, mid is not None)
        if mid is not None:
            mid(head)
        pk_buf[c] = _phi(kt).astype(BF16)
        for g in range(NG):
            ktg = kt[128 * g:128 * g + GW[g]]
            if GW[g] < 128:
                ktg = jnp.concatenate([ktg, jnp.zeros((128 - GW[g], L), F32)], axis=0)
            k_buf[c, g] = ktg.T.astype(BF16)
        top = jnp.max(jnp.abs(kt).reshape(PR // 8, 8, L), axis=0)
        return (kt, top) if keep else top

    x_copy(0).wait()
    stats = ln_stats(0, None)
    always.append(jnp.logical_not(jnp.abs(stats[0]) < 0.0))
    ln_apply(0, *stats)
    cp_wv.wait()
    wvt[...] = wv_raw[...].T
    project_v(0)
    x_copy(1).wait()
    cp_wq.wait()
    cp_wr.wait()
    ln_apply(1, *ln_stats(1, None))
    wq_t = _pad_heads_t(wq_raw[...].astype(F32))
    wr_row = wr_buf[...].reshape(1, D).astype(F32)
    pr_row = lax.broadcasted_iota(I32, (8, D), 0)
    wq_t = jnp.concatenate([wq_t[0:120], jnp.where(pr_row == ROUTER_ROW - 120, wr_row, wq_t[120:128]), wq_t[128:]],
                           axis=0)
    wqt[...] = wq_t.astype(BF16)
    project_v(1)
    cp_wk.wait()
    x_copy(2).wait()
    x_copy(3).wait()

    def prep_wk(y):
        wk = wk_raw[...].astype(F32)
        wk = jnp.concatenate([jnp.where(always[0], wk[:, 0:L], y[0:D]), wk[:, L:D]], axis=1)
        wkt[...] = _pad_heads_t(wk).astype(BF16)

    def route():
        r = _round_bf16(r_buf[ROUTER_ROW - 120:ROUTER_ROW - 119, :])
        tok = lax.broadcasted_iota(I32, (1, S), 1).astype(F32)
        m1 = jnp.max(r)
        i1 = jnp.min(jnp.where(r == m1, tok, float(S)))
        r_rest = jnp.where(tok == i1, -jnp.inf, r)
        m2 = jnp.max(r_rest)
        i2 = jnp.min(jnp.where(r_rest == m2, tok, float(S)))
        i1 = jnp.clip(i1.astype(I32), 0, S - 1)
        i2 = jnp.clip(i2.astype(I32), 0, S - 1)
        return m1, m2, i1, i2

    qt, aq = project_q(0, prep_wk)
    qt, a = project_q(1)
    aq = jnp.maximum(aq, a)
    stats = ln_stats(2, qt)
    ak = project_k(0)
    ln_apply(2, *stats)
    kt, a = project_k(1, keep=True)
    ak = jnp.maximum(ak, a)
    stats = ln_stats(3, kt)
    project_v(2)
    ln_apply(3, *stats)
    qt, a = project_q(2)
    aq = jnp.maximum(aq, a)
    ak = jnp.maximum(ak, project_k(2))
    qt, a = project_q(3)
    aq = jnp.maximum(aq, a)
    m1, m2, i1, i2 = route()
    ak = jnp.maximum(ak, project_k(3))
    project_v(3)

    logit_bound = jnp.max(aq) * jnp.max(ak) * (DH * 1.02)
    safe = logit_bound <= SAFE_LOG2_RANGE

    sel_row = lax.broadcasted_iota(I32, (16, 128), 0)
    sel_lane = lax.broadcasted_iota(I32, (16, 128), 1)

    def token_tile(i):
        return i // L, pl.ds(pl.multiple_of(((i % L) // 128) * 128, 128), 128)

    def pick(i, slot):
        seg, cols = token_tile(i)
        onehot = jnp.where((sel_row == slot) & (sel_lane == i % 128), 1.0, 0.0).astype(BF16)
        return lax.dot_general(onehot, xn_buf[seg, :, cols], NT_DIMS, preferred_element_type=F32)

    xs = (pick(i1, 0) + pick(i2, 1)).astype(BF16)

    cp_wo.wait()
    cp_beta.wait()
    cp_wg.wait()
    cp_wu.wait()

    beta_row = beta_buf[...].reshape(1, H).astype(F32)
    beta_row = jnp.concatenate([beta_row, jnp.zeros((1, 128 - H), F32)], axis=1)
    h_row = lax.broadcasted_iota(I32, (H, 128), 0)
    h_lane = lax.broadcasted_iota(I32, (H, 128), 1)
    beta_col = jnp.sum(jnp.where(h_row == h_lane, beta_row, 0.0), axis=1, keepdims=True)
    gate_buf[...] = jnp.broadcast_to(jax.nn.sigmoid(beta_col), (H, 128))


    def expert_chunk(lo, hi):
        hg = jnp.dot(xs, wg_buf[:, lo:hi], preferred_element_type=F32)
        hu = jnp.dot(xs, wu_buf[:, lo:hi], preferred_element_type=F32)
        hh = (jax.nn.silu(hg) * hu).astype(BF16)
        return lax.dot_general(hh, wd_buf[:, lo:hi], NT_DIMS, preferred_element_type=F32)

    def expert_stream(result):
        kmain = 512
        hidden = []
        for c0 in range(0, FF, 512):
            rem = []
            for w_ref in (wg_buf, wu_buf):
                rem.append(jnp.dot(xs[:, kmain:D], w_ref[kmain:D, c0:c0 + 512], preferred_element_type=F32))
                yield
            hs = []
            for f0 in range(c0, c0 + 512, 128):
                pre = []
                for w_ref, r in zip((wg_buf, wu_buf), rem):
                    pre.append(jnp.dot(xs[:, 0:kmain], w_ref[0:kmain, f0:f0 + 128], preferred_element_type=F32)
                               + r[:, f0 - c0:f0 - c0 + 128])
                    yield
                hs.append(jax.nn.silu(pre[0]) * pre[1])
            hidden.append(jnp.concatenate(hs, axis=1).astype(BF16))
        y_tiles = [None] * 5
        for ci, hh in enumerate(hidden):
            for e in range(5):
                e_hi = min(128 * (e + 1), D)
                part = lax.dot_general(hh, wd_buf[128 * e:e_hi, 512 * ci:512 * (ci + 1)], NT_DIMS,
                                       preferred_element_type=F32)
                y_tiles[e] = part if y_tiles[e] is None else y_tiles[e] + part
                yield
        result.append(jnp.concatenate(y_tiles, axis=1))

    def expert_scatter(y):
        y = y * jax.nn.sigmoid(jnp.where(r16 == 0, m1, m2))
        yt = jnp.concatenate([y, jnp.zeros((128 - 16, D), F32)], axis=0).T
        lane_d = lax.broadcasted_iota(I32, (D, 128), 1)
        for slot, i in ((0, i1), (1, i2)):
            seg, cols = token_tile(i)
            col = jnp.sum(jnp.where(lane_d == slot, yt, 0.0), axis=1, keepdims=True)
            base[seg, :, cols] = base[seg, :, cols] + jnp.where(lane_d == i % 128, col, 0.0)

    def memory_read(s, g):
        rg = _group_rows(g)
        gw = GW[g]
        lhs = jnp.concatenate([mt_buf[g, 0:rg, 0:gw], mt_buf[g, ZROW:MROWS, 0:gw]], axis=0).astype(BF16)
        res = jnp.dot(lhs, pq_buf[s, 128 * g:128 * g + gw, :], preferred_element_type=F32)
        num_buf[g, 0:rg, :] = res[0:rg]
        num_buf[g, ZROW:MROWS, :] = res[rg:rg + 16]

    def memory_update(s, g):
        rg = _group_rows(g)
        a_g = _group_row_start(g)
        gw = GW[g]
        lhs = jnp.concatenate([vt_buf[s, a_g:a_g + rg, :], vt_buf[s, D:VROWS, :]], axis=0)
        upd = lax.dot_general(lhs, pk_buf[s, 128 * g:128 * g + gw, :], NT_DIMS,
                              preferred_element_type=F32)
        er = lax.broadcasted_iota(I32, (rg, gw), 0) + (a_g - HPG * DH * g)
        el = lax.broadcasted_iota(I32, (rg, gw), 1)
        same_head = None
        for i in range(_heads_in_group(g)):
            t = ((er >= DH * i) & (er < DH * (i + 1)) & (el >= DH * i) & (el < DH * (i + 1)))
            same_head = t if same_head is None else (same_head | t)
        mt_buf[g, 0:rg, 0:gw] = mt_buf[g, 0:rg, 0:gw] + jnp.where(same_head, upd[0:rg], 0.0)
        zr = lax.broadcasted_iota(I32, (8, gw), 0)
        zl = lax.broadcasted_iota(I32, (8, gw), 1)
        zmask = (zl >= zr * DH) & (zl < zr * DH + DH) & (zr < _heads_in_group(g))
        zs = upd[rg + 1:rg + 2]
        mt_buf[g, ZROW:ZROW + 8, 0:gw] = mt_buf[g, ZROW:ZROW + 8, 0:gw] + jnp.where(zmask, zs, 0.0)

    def transpose_wo(g):
        hi = min(128 * (g + 1), D)
        wot[128 * g:hi, :] = wo_raw[:, 128 * g:hi].T

    def project_out(s):
        attn = jnp.dot(wot[...], ot_buf[...].astype(BF16), preferred_element_type=F32)
        return base[s] + attn

    def emit(s, val):
        out_buf[s] = val.astype(BF16)
        out_copy(s).start()

    zero = lax.shift_right_logical(i1, 16)

    def prow(start, size):
        return pl.ds(pl.multiple_of(zero + start, 8), size)

    P_OFFS = (0, 128, 384, 768)

    def fast_scores(s, g, hook):
        nh = _heads_in_group(g)
        gw = GW[g]
        pb = (p_buf0, p_buf1)[(s * NG + g) % 2]
        rowg = lax.broadcasted_iota(I32, (gw, 128), 0)
        for j in range(QT - 1, -1, -1):
            n = 128 * (j + 1)
            q = qs_buf[s, 128 * g:128 * g + gw, 128 * j:128 * (j + 1)].astype(F32)
            for h0, h1 in ((0, 4), (4, nh)):
                if h1 <= h0:
                    continue
                qm = jnp.concatenate(
                    [jnp.where((rowg >= DH * i) & (rowg < DH * (i + 1)), q, 0.0) for i in range(h0, h1)],
                    axis=1).astype(BF16)
                st = jnp.dot(k_buf[s, g, 0:n, 0:gw], qm, preferred_element_type=F32)
                p = jnp.exp2(st)
                causal_w = jnp.concatenate([causal] * (h1 - h0), axis=1)
                p_diag = jnp.where(causal_w, p[n - 128:], 0.0)
                p = jnp.concatenate([p[:n - 128], p_diag], axis=0) if j > 0 else p_diag
                pb[P_OFFS[j] // 2:(P_OFFS[j] + n) // 2, h0 * 128:h1 * 128] = pltpu.bitcast(p.astype(BF16), U32)
                hook()

    def fast_values(s, g):
        nh = _heads_in_group(g)
        a_g = _group_row_start(g)
        pb = (p_buf0, p_buf1)[(s * NG + g) % 2]
        for j in range(QT - 1, -1, -1):
            n = 128 * (j + 1)
            cols = slice(128 * j, 128 * (j + 1))
            for i in range(nh):
                h = HPG * g + i
                a = (h * DH // 16) * 16
                off = h * DH - a
                p = pltpu.bitcast(pb[prow(P_OFFS[j] // 2, n // 2), 128 * i:128 * (i + 1)], BF16)
                ones_row = 0 if off > 0 else 31
                r32n = lax.broadcasted_iota(I32, (32, n), 0)
                lhs = jnp.where(r32n == ones_row, 1.0, vt_buf[s, a:a + 32, 0:n].astype(F32)).astype(BF16)
                o = jnp.dot(lhs, p, preferred_element_type=F32)
                lo = (off // 8) * 8
                hi = -(-(off + DH) // 8) * 8
                gate = gate_buf[h:h + 1, :]
                rl = 1.0 / o[ones_row:ones_row + 1]
                val = (1.0 - gate) * (o[lo:hi] * rl)
                if s > 0:
                    rden = 1.0 / (num_buf[g, ZROW + i:ZROW + i + 1, cols] + 1e-6)
                    num = num_buf[g, a - a_g + lo:a - a_g + hi, cols]
                    val = gate * (num * rden) + val
                ot_buf[a + off:a + off + DH, cols] = val[off - lo:off - lo + DH]

    def side_work():
        result = []
        yield from expert_stream(result)
        expert_scatter(result[0])
        yield
        for u in range(NSEG - 1):
            for j in range(QT):
                cols = slice(128 * j, 128 * (j + 1))
                out_buf[u, :, cols] = base[u, :, cols].astype(BF16)
                if j == QT - 1:
                    out_copy(u).start()
                yield

    def fast_path():
        stream = side_work()

        def hook():
            next(stream, None)

        steps = [(s, g) for s in range(NSEG) for g in range(NG)]
        fast_scores(0, 0, hook)
        for t, (s, g) in enumerate(steps):
            if t + 1 < len(steps):
                fast_scores(*steps[t + 1], hook)
            if s > 0:
                memory_read(s, g)
                hook()
            fast_values(s, g)
            if s == 0:
                transpose_wo(g)
            if s + 1 < NSEG:
                memory_update(s, g)
                hook()
            if g == NG - 1 and s < NSEG - 1:
                base[s] = project_out(s)
                if s == 0:
                    cp_wd.wait()
                hook()
        for _ in stream:
            pass
        s = NSEG - 1
        for j in range(QT):
            cols = slice(128 * j, 128 * (j + 1))
            attn = jnp.dot(wot[...], ot_buf[:, cols].astype(BF16), preferred_element_type=F32)
            out_buf[s, :, cols] = (base[s, :, cols] + attn).astype(BF16)
            out_tile_copy(j).start()
        for u in range(NSEG - 1):
            out_copy(u).wait()
        for j in range(QT):
            out_tile_copy(j).wait()

    def slow_segment(s, carry):
        for g in range(NG):
            memory_read(s, g)
        key_i = lax.broadcasted_iota(I32, (L, L), 0)
        qry_i = lax.broadcasted_iota(I32, (L, L), 1)
        r32 = lax.broadcasted_iota(I32, (32, L), 0)
        for g in range(NG):
            gw = GW[g]
            a_g = _group_row_start(g)
            rowg = lax.broadcasted_iota(I32, (gw, L), 0)

            def head(i, c, g=g, gw=gw, a_g=a_g, rowg=rowg):
                h = HPG * g + i
                a = pl.multiple_of((h * DH // 16) * 16, 16)
                off = h * DH - a
                q = qs_buf[s, 128 * g:128 * g + gw, :].astype(F32)
                qm = jnp.where((rowg >= DH * i) & (rowg < DH * (i + 1)), q, 0.0).astype(BF16)
                st = jnp.dot(k_buf[s, g, :, 0:gw], qm, preferred_element_type=F32)
                st = jnp.where(key_i <= qry_i, st, NEG_BIG)
                p = jnp.exp2(st - jnp.max(st, axis=0, keepdims=True))
                rl = 1.0 / jnp.sum(p, axis=0, keepdims=True)
                o = jnp.dot(vt_buf[s, pl.ds(a, 32), :], p.astype(BF16), preferred_element_type=F32)
                gate = jnp.concatenate([gate_buf[pl.ds(h, 1), :]] * QT, axis=1)
                rden = 1.0 / (num_buf[g, pl.ds(ZROW + i, 1), :] + 1e-6)
                num = num_buf[g, pl.ds(pl.multiple_of(a - a_g, 16), 32), :]
                val = gate * (num * rden) + (1.0 - gate) * (o * rl)
                keep = (r32 >= off) & (r32 < off + DH)
                pltpu.store(ot_buf.at[pl.ds(a, 32), :], val, mask=keep)
                return c

            lax.fori_loop(0, _heads_in_group(g), head, 0)
        for g in range(NG):
            memory_update(s, g)
        emit(s, project_out(s))
        return carry

    @pl.when(safe)
    def _():
        fast_path()

    @pl.when(jnp.logical_not(safe))
    def _():
        cp_wd.wait()
        for g in range(NG):
            transpose_wo(g)
        expert_scatter(expert_chunk(0, FF))
        lax.fori_loop(0, NSEG, slow_segment, 0)
        for u in range(NSEG):
            out_copy(u).wait()


@jax.jit
def pallas_parallel_sum__memory_aug_infini_attn__moe_arch_mod__prompt_kernel(
    A_x: jax.Array,
    A_wq: jax.Array,
    A_wk: jax.Array,
    A_wv: jax.Array,
    A_wo: jax.Array,
    A_beta: jax.Array,
    B_x: jax.Array,
    B_w_r: jax.Array,
    B_w_gate: jax.Array,
    B_w_up: jax.Array,
    B_w_down: jax.Array,
):
    del B_x
    hbm = pl.BlockSpec(memory_space=pl.ANY)
    scratch = [
        pltpu.VMEM((NSEG, D, L), BF16),
        pltpu.VMEM((D, D), BF16),
        pltpu.VMEM((D, D), BF16),
        pltpu.VMEM((D, D), BF16),
        pltpu.VMEM((D, D), BF16),
        pltpu.VMEM((H,), BF16),
        pltpu.VMEM((D,), BF16),
        pltpu.VMEM((D, FF), BF16),
        pltpu.VMEM((D, FF), BF16),
        pltpu.VMEM((D, FF), BF16),
        pltpu.VMEM((PR, D), BF16),
        pltpu.VMEM((PR, D), BF16),
        pltpu.VMEM((D, D), BF16),
        pltpu.VMEM((D, D), BF16),
        pltpu.VMEM((NSEG, D, L), BF16),
        pltpu.VMEM((NSEG, D, L), F32),
        pltpu.VMEM((NSEG, PR, L), BF16),
        pltpu.VMEM((NSEG, PR, L), BF16),
        pltpu.VMEM((NSEG, NG, L, 128), BF16),
        pltpu.VMEM((NSEG, PR, L), BF16),
        pltpu.VMEM((NSEG, VROWS, L), BF16),
        pltpu.VMEM((8, S), F32),
        pltpu.VMEM((H, 128), F32),
        pltpu.VMEM((NG, MROWS, 128), F32),
        pltpu.VMEM((NG, MROWS, L), F32),
        pltpu.VMEM((640, HPG * 128), U32),
        pltpu.VMEM((640, HPG * 128), U32),
        pltpu.VMEM((D, L), F32),
        pltpu.VMEM((NSEG, D, L), BF16),
        pltpu.SemaphoreType.DMA((13,)),
        pltpu.SemaphoreType.DMA((NSEG + QT,)),
    ]
    out_t = pl.pallas_call(
        _kernel,
        out_shape=jax.ShapeDtypeStruct((1, D, S), BF16),
        in_specs=[hbm] * 10,
        out_specs=hbm,
        scratch_shapes=scratch,
        compiler_params=pltpu.CompilerParams(vmem_limit_bytes=128 * 1024 * 1024),
        name="infini_attn_moe",
    )(jnp.transpose(A_x, (0, 2, 1)), A_wq, A_wk, A_wv, A_wo, A_beta, B_w_r, B_w_gate, B_w_up,
      B_w_down.T)
    return jnp.transpose(out_t, (0, 2, 1))
```

```python
import jax
import jax.numpy as jnp
from jax import lax
import jax.experimental.pallas as pl
import jax.experimental.pallas.tpu as pltpu

F32 = jnp.float32
BF16 = jnp.bfloat16
U32 = jnp.uint32
I32 = jnp.int32

S = 2048
D = 576
H = 32
DH = 18
NSEG = 4
L = 512
FF = 4608
HPG = 7
NG = 5
QT = L // 128
GW = (128, 128, 128, 128, 80)
PR = sum(GW)
VROWS = D + 16
ROUTER_ROW = 126
ZROW = 144
MROWS = 160
LOG2E = 1.4426950408889634
QSCALE = (DH ** -0.5) * LOG2E
SAFE_LOG2_RANGE = 60.0
NEG_BIG = -1e30

NT_DIMS = (((1,), (1,)), ((), ()))


def _heads_in_group(g):
    return min(HPG, H - HPG * g)


def _group_row_start(g):
    return (HPG * g * DH // 16) * 16


def _group_rows(g):
    last = (HPG * g + _heads_in_group(g)) * DH
    return -(-(last - _group_row_start(g)) // 16) * 16


def _round_bf16(x):
    return x.astype(BF16).astype(F32)


def _pad_heads_t(w):
    parts = []
    for g in range(NG):
        n = _heads_in_group(g) * DH
        parts.append(w[:, HPG * DH * g:HPG * DH * g + n])
        parts.append(jnp.zeros((D, 128 - n), w.dtype))
    return jnp.concatenate(parts, axis=1).T[0:PR]


def _phi(t):
    return jnp.where(t > 0, t + 1.0, jnp.exp(t))


def _kernel(x_hbm, wq_hbm, wk_hbm, wv_hbm, wo_hbm, beta_hbm, wr_hbm, wg_hbm, wu_hbm, wd_hbm,
            out_hbm,
            x_buf, wq_raw, wk_raw, wv_raw, wo_raw, beta_buf, wr_buf, wg_buf, wu_buf, wd_buf,
            wqt, wkt, wvt, wot, xn_buf, base, qs_buf, pq_buf, k_buf, pk_buf, vt_buf, r_buf,
            gate_buf, mt_buf, num_buf, p_buf0, p_buf1, ot_buf, out_buf, in_sems, out_sems):
    def x_copy(c):
        return pltpu.make_async_copy(x_hbm.at[0, :, pl.ds(c * L, L)], x_buf.at[c], in_sems.at[c])

    cp_wv = pltpu.make_async_copy(wv_hbm, wv_raw, in_sems.at[4])
    cp_wq = pltpu.make_async_copy(wq_hbm, wq_raw, in_sems.at[5])
    cp_wk = pltpu.make_async_copy(wk_hbm, wk_raw, in_sems.at[6])
    cp_wo = pltpu.make_async_copy(wo_hbm, wo_raw, in_sems.at[7])
    cp_wg = pltpu.make_async_copy(wg_hbm, wg_buf, in_sems.at[8])
    cp_wu = pltpu.make_async_copy(wu_hbm, wu_buf, in_sems.at[9])
    cp_wd = pltpu.make_async_copy(wd_hbm, wd_buf, in_sems.at[10])
    cp_beta = pltpu.make_async_copy(beta_hbm, beta_buf, in_sems.at[11])
    cp_wr = pltpu.make_async_copy(wr_hbm, wr_buf, in_sems.at[12])

    def out_copy(s):
        cols = pl.ds(pl.multiple_of(s * L, L), L)
        return pltpu.make_async_copy(out_buf.at[s], out_hbm.at[0, :, cols], out_sems.at[s])

    def out_tile_copy(j):
        s = NSEG - 1
        return pltpu.make_async_copy(out_buf.at[s, :, pl.ds(128 * j, 128)],
                                     out_hbm.at[0, :, pl.ds(s * L + 128 * j, 128)], out_sems.at[NSEG + j])


    for cp in (x_copy(0), cp_wv, x_copy(1), cp_wq, cp_wr, x_copy(2), cp_wk, x_copy(3), cp_wo, cp_beta,
               cp_wg, cp_wu, cp_wd):
        cp.start()

    lane128 = lax.broadcasted_iota(I32, (128, 128), 1)
    row128 = lax.broadcasted_iota(I32, (128, 128), 0)
    causal = row128 <= lane128
    r16 = lax.broadcasted_iota(I32, (16, D), 0)

    mt_buf[...] = jnp.zeros(mt_buf.shape, F32)

    always = []

    def pace(x, y):
        return x if y is None else jnp.where(always[0], x, y[0:D])

    def ln_stats(c, y):
        x = pace(x_buf[c].astype(F32), y)
        shift = x_buf[c, 0:16, :].astype(F32)[0:1]
        d = x - shift
        m1 = jnp.sum(d, axis=0, keepdims=True) * (1.0 / D)
        m2 = jnp.sum(d * d, axis=0, keepdims=True) * (1.0 / D)
        var = jnp.maximum(m2 - m1 * m1, 0.0)
        inv = 1.0 / _round_bf16(jnp.sqrt(_round_bf16(_round_bf16(var) + 1e-5)))
        return _round_bf16(shift + m1), inv

    def ln_apply(c, mean_b, inv):
        x = x_buf[c].astype(F32)
        xn = (x - mean_b) * inv
        xn_buf[c] = xn.astype(BF16)
        base[c] = x + xn

    def project(w_ref, c, split):
        if not split:
            return jnp.dot(w_ref[...], xn_buf[c], preferred_element_type=F32), None
        head = jnp.dot(w_ref[:, 0:256], xn_buf[c, 0:256, :], preferred_element_type=F32)
        tail = jnp.dot(w_ref[:, 256:D], xn_buf[c, 256:D, :], preferred_element_type=F32)
        return head + tail, head

    def project_v(c, mid=None):
        vt, head = project(wvt, c, mid is not None)
        if mid is not None:
            mid(head)
        vt_buf[c, 0:D, :] = vt.astype(BF16)
        r16l = lax.broadcasted_iota(I32, (16, L), 0)
        vt_buf[c, D:VROWS, :] = jnp.where(r16l == 1, 1.0, 0.0).astype(BF16)
        return vt

    def project_q(c, mid=None):
        qt, head = project(wqt, c, mid is not None)
        if mid is not None:
            mid(head)
        qsc = qt * QSCALE
        qs_buf[c] = qsc.astype(BF16)
        pq_buf[c] = _phi(qt).astype(BF16)
        r_buf[:, c * L:(c + 1) * L] = qt[120:128]
        mag = jnp.abs(qsc)
        r8 = lax.broadcasted_iota(I32, (8, L), 0)
        mag = jnp.concatenate([mag[0:120], jnp.where(r8 == ROUTER_ROW - 120, 0.0, mag[120:128]), mag[128:]], axis=0)
        return qt, jnp.max(mag.reshape(PR // 8, 8, L), axis=0)

    def project_k(c, mid=None, keep=False):
        kt, head = project(wkt, c, mid is not None)
        if mid is not None:
            mid(head)
        pk_buf[c] = _phi(kt).astype(BF16)
        for g in range(NG):
            ktg = kt[128 * g:128 * g + GW[g]]
            if GW[g] < 128:
                ktg = jnp.concatenate([ktg, jnp.zeros((128 - GW[g], L), F32)], axis=0)
            k_buf[c, g] = ktg.T.astype(BF16)
        top = jnp.max(jnp.abs(kt).reshape(PR // 8, 8, L), axis=0)
        return (kt, top) if keep else top

    x_copy(0).wait()
    stats = ln_stats(0, None)
    always.append(jnp.logical_not(jnp.abs(stats[0]) < 0.0))
    ln_apply(0, *stats)
    cp_wv.wait()
    wvt[...] = wv_raw[...].T
    project_v(0)
    x_copy(1).wait()
    cp_wq.wait()
    cp_wr.wait()
    ln_apply(1, *ln_stats(1, None))

    def paced_weight(w_ref, y):
        w = w_ref[...].astype(F32)
        return jnp.concatenate([jnp.where(always[0], w[:, 0:L], y[0:D]), w[:, L:D]], axis=1)

    def prep_wq(y):
        wq_t = _pad_heads_t(paced_weight(wq_raw, y))
        wr_row = wr_buf[...].reshape(1, D).astype(F32)
        pr_row = lax.broadcasted_iota(I32, (8, D), 0)
        wq_t = jnp.concatenate(
            [wq_t[0:120], jnp.where(pr_row == ROUTER_ROW - 120, wr_row, wq_t[120:128]), wq_t[128:]], axis=0)
        wqt[...] = wq_t.astype(BF16)

    project_v(1, prep_wq)
    cp_wk.wait()
    x_copy(2).wait()
    x_copy(3).wait()

    def prep_wk(y):
        wkt[...] = _pad_heads_t(paced_weight(wk_raw, y)).astype(BF16)

    def route():
        r = _round_bf16(r_buf[ROUTER_ROW - 120:ROUTER_ROW - 119, :])
        tok = lax.broadcasted_iota(I32, (1, S), 1).astype(F32)
        m1 = jnp.max(r)
        i1 = jnp.min(jnp.where(r == m1, tok, float(S)))
        r_rest = jnp.where(tok == i1, -jnp.inf, r)
        m2 = jnp.max(r_rest)
        i2 = jnp.min(jnp.where(r_rest == m2, tok, float(S)))
        i1 = jnp.clip(i1.astype(I32), 0, S - 1)
        i2 = jnp.clip(i2.astype(I32), 0, S - 1)
        return m1, m2, i1, i2

    qt, aq = project_q(0, prep_wk)
    qt, a = project_q(1)
    aq = jnp.maximum(aq, a)
    stats = ln_stats(2, qt)
    ak = project_k(0)
    ln_apply(2, *stats)
    kt, a = project_k(1, keep=True)
    ak = jnp.maximum(ak, a)
    stats = ln_stats(3, kt)
    project_v(2)
    ln_apply(3, *stats)
    qt, a = project_q(2)
    aq = jnp.maximum(aq, a)
    ak = jnp.maximum(ak, project_k(2))
    qt, a = project_q(3)
    aq = jnp.maximum(aq, a)
    m1, m2, i1, i2 = route()
    ak = jnp.maximum(ak, project_k(3))
    project_v(3)

    logit_bound = jnp.max(aq) * jnp.max(ak) * (DH * 1.02)
    safe = logit_bound <= SAFE_LOG2_RANGE

    sel_row = lax.broadcasted_iota(I32, (16, 128), 0)
    sel_lane = lax.broadcasted_iota(I32, (16, 128), 1)

    def token_tile(i):
        return i // L, pl.ds(pl.multiple_of(((i % L) // 128) * 128, 128), 128)

    def pick(i, slot):
        seg, cols = token_tile(i)
        onehot = jnp.where((sel_row == slot) & (sel_lane == i % 128), 1.0, 0.0).astype(BF16)
        return lax.dot_general(onehot, xn_buf[seg, :, cols], NT_DIMS, preferred_element_type=F32)

    xs = (pick(i1, 0) + pick(i2, 1)).astype(BF16)

    cp_wo.wait()
    cp_beta.wait()
    cp_wg.wait()
    cp_wu.wait()

    beta_row = beta_buf[...].reshape(1, H).astype(F32)
    beta_row = jnp.concatenate([beta_row, jnp.zeros((1, 128 - H), F32)], axis=1)
    h_row = lax.broadcasted_iota(I32, (H, 128), 0)
    h_lane = lax.broadcasted_iota(I32, (H, 128), 1)
    beta_col = jnp.sum(jnp.where(h_row == h_lane, beta_row, 0.0), axis=1, keepdims=True)
    gate_buf[...] = jnp.broadcast_to(jax.nn.sigmoid(beta_col), (H, 128))


    def expert_chunk(lo, hi):
        hg = jnp.dot(xs, wg_buf[:, lo:hi], preferred_element_type=F32)
        hu = jnp.dot(xs, wu_buf[:, lo:hi], preferred_element_type=F32)
        hh = (jax.nn.silu(hg) * hu).astype(BF16)
        return lax.dot_general(hh, wd_buf[:, lo:hi], NT_DIMS, preferred_element_type=F32)

    def expert_stream(result):
        kmain = 512
        hidden = []
        for c0 in range(0, FF, 512):
            rem = []
            for w_ref in (wg_buf, wu_buf):
                rem.append(jnp.dot(xs[:, kmain:D], w_ref[kmain:D, c0:c0 + 512], preferred_element_type=F32))
                yield
            hs = []
            for f0 in range(c0, c0 + 512, 128):
                pre = []
                for w_ref, r in zip((wg_buf, wu_buf), rem):
                    pre.append(jnp.dot(xs[:, 0:kmain], w_ref[0:kmain, f0:f0 + 128], preferred_element_type=F32)
                               + r[:, f0 - c0:f0 - c0 + 128])
                    yield
                hs.append(jax.nn.silu(pre[0]) * pre[1])
            hidden.append(jnp.concatenate(hs, axis=1).astype(BF16))
        y_tiles = [None] * 5
        for ci, hh in enumerate(hidden):
            for e in range(5):
                e_hi = min(128 * (e + 1), D)
                part = lax.dot_general(hh, wd_buf[128 * e:e_hi, 512 * ci:512 * (ci + 1)], NT_DIMS,
                                       preferred_element_type=F32)
                y_tiles[e] = part if y_tiles[e] is None else y_tiles[e] + part
                yield
        result.append(jnp.concatenate(y_tiles, axis=1))

    def expert_scatter(y):
        y = y * jax.nn.sigmoid(jnp.where(r16 == 0, m1, m2))
        yt = jnp.concatenate([y, jnp.zeros((128 - 16, D), F32)], axis=0).T
        lane_d = lax.broadcasted_iota(I32, (D, 128), 1)
        for slot, i in ((0, i1), (1, i2)):
            seg, cols = token_tile(i)
            col = jnp.sum(jnp.where(lane_d == slot, yt, 0.0), axis=1, keepdims=True)
            base[seg, :, cols] = base[seg, :, cols] + jnp.where(lane_d == i % 128, col, 0.0)

    def memory_read(s, g):
        rg = _group_rows(g)
        gw = GW[g]
        lhs = jnp.concatenate([mt_buf[g, 0:rg, 0:gw], mt_buf[g, ZROW:MROWS, 0:gw]], axis=0).astype(BF16)
        res = jnp.dot(lhs, pq_buf[s, 128 * g:128 * g + gw, :], preferred_element_type=F32)
        num_buf[g, 0:rg, :] = res[0:rg]
        num_buf[g, ZROW:MROWS, :] = res[rg:rg + 16]

    def memory_update(s, g):
        rg = _group_rows(g)
        a_g = _group_row_start(g)
        gw = GW[g]
        lhs = jnp.concatenate([vt_buf[s, a_g:a_g + rg, :], vt_buf[s, D:VROWS, :]], axis=0)
        upd = lax.dot_general(lhs, pk_buf[s, 128 * g:128 * g + gw, :], NT_DIMS,
                              preferred_element_type=F32)
        er = lax.broadcasted_iota(I32, (rg, gw), 0) + (a_g - HPG * DH * g)
        el = lax.broadcasted_iota(I32, (rg, gw), 1)
        same_head = None
        for i in range(_heads_in_group(g)):
            t = ((er >= DH * i) & (er < DH * (i + 1)) & (el >= DH * i) & (el < DH * (i + 1)))
            same_head = t if same_head is None else (same_head | t)
        mt_buf[g, 0:rg, 0:gw] = mt_buf[g, 0:rg, 0:gw] + jnp.where(same_head, upd[0:rg], 0.0)
        zr = lax.broadcasted_iota(I32, (8, gw), 0)
        zl = lax.broadcasted_iota(I32, (8, gw), 1)
        zmask = (zl >= zr * DH) & (zl < zr * DH + DH) & (zr < _heads_in_group(g))
        zs = upd[rg + 1:rg + 2]
        mt_buf[g, ZROW:ZROW + 8, 0:gw] = mt_buf[g, ZROW:ZROW + 8, 0:gw] + jnp.where(zmask, zs, 0.0)

    def transpose_wo(g):
        hi = min(128 * (g + 1), D)
        wot[128 * g:hi, :] = wo_raw[:, 128 * g:hi].T

    def project_out(s):
        attn = jnp.dot(wot[...], ot_buf[...].astype(BF16), preferred_element_type=F32)
        return base[s] + attn

    def emit(s, val):
        out_buf[s] = val.astype(BF16)
        out_copy(s).start()

    zero = lax.shift_right_logical(i1, 16)

    def prow(start, size):
        return pl.ds(pl.multiple_of(zero + start, 8), size)

    P_OFFS = (0, 128, 384, 768)

    def fast_scores(s, g, hook):
        nh = _heads_in_group(g)
        gw = GW[g]
        pb = (p_buf0, p_buf1)[(s * NG + g) % 2]
        rowg = lax.broadcasted_iota(I32, (gw, 128), 0)
        for j in range(QT - 1, -1, -1):
            n = 128 * (j + 1)
            q = qs_buf[s, 128 * g:128 * g + gw, 128 * j:128 * (j + 1)].astype(F32)
            for h0, h1 in ((0, 4), (4, nh)):
                if h1 <= h0:
                    continue
                qm = jnp.concatenate(
                    [jnp.where((rowg >= DH * i) & (rowg < DH * (i + 1)), q, 0.0) for i in range(h0, h1)],
                    axis=1).astype(BF16)
                st = jnp.dot(k_buf[s, g, 0:n, 0:gw], qm, preferred_element_type=F32)
                p = jnp.exp2(st)
                causal_w = jnp.concatenate([causal] * (h1 - h0), axis=1)
                p_diag = jnp.where(causal_w, p[n - 128:], 0.0)
                p = jnp.concatenate([p[:n - 128], p_diag], axis=0) if j > 0 else p_diag
                pb[P_OFFS[j] // 2:(P_OFFS[j] + n) // 2, h0 * 128:h1 * 128] = pltpu.bitcast(p.astype(BF16), U32)
                hook()

    def fast_values(s, g):
        nh = _heads_in_group(g)
        a_g = _group_row_start(g)
        pb = (p_buf0, p_buf1)[(s * NG + g) % 2]
        for j in range(QT - 1, -1, -1):
            n = 128 * (j + 1)
            cols = slice(128 * j, 128 * (j + 1))
            for i in range(nh):
                h = HPG * g + i
                a = (h * DH // 16) * 16
                off = h * DH - a
                p = pltpu.bitcast(pb[prow(P_OFFS[j] // 2, n // 2), 128 * i:128 * (i + 1)], BF16)
                ones_row = 0 if off > 0 else 31
                r32n = lax.broadcasted_iota(I32, (32, n), 0)
                lhs = jnp.where(r32n == ones_row, 1.0, vt_buf[s, a:a + 32, 0:n].astype(F32)).astype(BF16)
                o = jnp.dot(lhs, p, preferred_element_type=F32)
                lo = (off // 8) * 8
                hi = -(-(off + DH) // 8) * 8
                gate = gate_buf[h:h + 1, :]
                rl = 1.0 / o[ones_row:ones_row + 1]
                val = (1.0 - gate) * (o[lo:hi] * rl)
                if s > 0:
                    rden = 1.0 / (num_buf[g, ZROW + i:ZROW + i + 1, cols] + 1e-6)
                    num = num_buf[g, a - a_g + lo:a - a_g + hi, cols]
                    val = gate * (num * rden) + val
                ot_buf[a + off:a + off + DH, cols] = val[off - lo:off - lo + DH]

    def side_work():
        result = []
        yield from expert_stream(result)
        expert_scatter(result[0])
        yield
        for u in range(NSEG - 1):
            for j in range(QT):
                cols = slice(128 * j, 128 * (j + 1))
                out_buf[u, :, cols] = base[u, :, cols].astype(BF16)
                if j == QT - 1:
                    out_copy(u).start()
                yield

    def fast_path():
        stream = side_work()

        def hook():
            next(stream, None)

        steps = [(s, g) for s in range(NSEG) for g in range(NG)]
        fast_scores(0, 0, hook)
        for t, (s, g) in enumerate(steps):
            if t + 1 < len(steps):
                fast_scores(*steps[t + 1], hook)
            if s > 0:
                memory_read(s, g)
                hook()
            fast_values(s, g)
            if s == 0:
                transpose_wo(g)
            if s + 1 < NSEG:
                memory_update(s, g)
                hook()
            if g == NG - 1 and s < NSEG - 1:
                base[s] = project_out(s)
                if s == 0:
                    cp_wd.wait()
                hook()
        for _ in stream:
            pass
        s = NSEG - 1
        for j in range(QT):
            cols = slice(128 * j, 128 * (j + 1))
            attn = jnp.dot(wot[...], ot_buf[:, cols].astype(BF16), preferred_element_type=F32)
            out_buf[s, :, cols] = (base[s, :, cols] + attn).astype(BF16)
            out_tile_copy(j).start()
        for u in range(NSEG - 1):
            out_copy(u).wait()
        for j in range(QT):
            out_tile_copy(j).wait()

    def slow_segment(s, carry):
        for g in range(NG):
            memory_read(s, g)
        key_i = lax.broadcasted_iota(I32, (L, L), 0)
        qry_i = lax.broadcasted_iota(I32, (L, L), 1)
        r32 = lax.broadcasted_iota(I32, (32, L), 0)
        for g in range(NG):
            gw = GW[g]
            a_g = _group_row_start(g)
            rowg = lax.broadcasted_iota(I32, (gw, L), 0)

            def head(i, c, g=g, gw=gw, a_g=a_g, rowg=rowg):
                h = HPG * g + i
                a = pl.multiple_of((h * DH // 16) * 16, 16)
                off = h * DH - a
                q = qs_buf[s, 128 * g:128 * g + gw, :].astype(F32)
                qm = jnp.where((rowg >= DH * i) & (rowg < DH * (i + 1)), q, 0.0).astype(BF16)
                st = jnp.dot(k_buf[s, g, :, 0:gw], qm, preferred_element_type=F32)
                st = jnp.where(key_i <= qry_i, st, NEG_BIG)
                p = jnp.exp2(st - jnp.max(st, axis=0, keepdims=True))
                rl = 1.0 / jnp.sum(p, axis=0, keepdims=True)
                o = jnp.dot(vt_buf[s, pl.ds(a, 32), :], p.astype(BF16), preferred_element_type=F32)
                gate = jnp.concatenate([gate_buf[pl.ds(h, 1), :]] * QT, axis=1)
                rden = 1.0 / (num_buf[g, pl.ds(ZROW + i, 1), :] + 1e-6)
                num = num_buf[g, pl.ds(pl.multiple_of(a - a_g, 16), 32), :]
                val = gate * (num * rden) + (1.0 - gate) * (o * rl)
                keep = (r32 >= off) & (r32 < off + DH)
                pltpu.store(ot_buf.at[pl.ds(a, 32), :], val, mask=keep)
                return c

            lax.fori_loop(0, _heads_in_group(g), head, 0)
        for g in range(NG):
            memory_update(s, g)
        emit(s, project_out(s))
        return carry

    @pl.when(safe)
    def _():
        fast_path()

    @pl.when(jnp.logical_not(safe))
    def _():
        cp_wd.wait()
        for g in range(NG):
            transpose_wo(g)
        expert_scatter(expert_chunk(0, FF))
        lax.fori_loop(0, NSEG, slow_segment, 0)
        for u in range(NSEG):
            out_copy(u).wait()


@jax.jit
def pallas_parallel_sum__memory_aug_infini_attn__moe_arch_mod__prompt_kernel(
    A_x: jax.Array,
    A_wq: jax.Array,
    A_wk: jax.Array,
    A_wv: jax.Array,
    A_wo: jax.Array,
    A_beta: jax.Array,
    B_x: jax.Array,
    B_w_r: jax.Array,
    B_w_gate: jax.Array,
    B_w_up: jax.Array,
    B_w_down: jax.Array,
):
    del B_x
    hbm = pl.BlockSpec(memory_space=pl.ANY)
    scratch = [
        pltpu.VMEM((NSEG, D, L), BF16),
        pltpu.VMEM((D, D), BF16),
        pltpu.VMEM((D, D), BF16),
        pltpu.VMEM((D, D), BF16),
        pltpu.VMEM((D, D), BF16),
        pltpu.VMEM((H,), BF16),
        pltpu.VMEM((D,), BF16),
        pltpu.VMEM((D, FF), BF16),
        pltpu.VMEM((D, FF), BF16),
        pltpu.VMEM((D, FF), BF16),
        pltpu.VMEM((PR, D), BF16),
        pltpu.VMEM((PR, D), BF16),
        pltpu.VMEM((D, D), BF16),
        pltpu.VMEM((D, D), BF16),
        pltpu.VMEM((NSEG, D, L), BF16),
        pltpu.VMEM((NSEG, D, L), F32),
        pltpu.VMEM((NSEG, PR, L), BF16),
        pltpu.VMEM((NSEG, PR, L), BF16),
        pltpu.VMEM((NSEG, NG, L, 128), BF16),
        pltpu.VMEM((NSEG, PR, L), BF16),
        pltpu.VMEM((NSEG, VROWS, L), BF16),
        pltpu.VMEM((8, S), F32),
        pltpu.VMEM((H, 128), F32),
        pltpu.VMEM((NG, MROWS, 128), F32),
        pltpu.VMEM((NG, MROWS, L), F32),
        pltpu.VMEM((640, HPG * 128), U32),
        pltpu.VMEM((640, HPG * 128), U32),
        pltpu.VMEM((D, L), F32),
        pltpu.VMEM((NSEG, D, L), BF16),
        pltpu.SemaphoreType.DMA((13,)),
        pltpu.SemaphoreType.DMA((NSEG + QT,)),
    ]
    out_t = pl.pallas_call(
        _kernel,
        out_shape=jax.ShapeDtypeStruct((1, D, S), BF16),
        in_specs=[hbm] * 10,
        out_specs=hbm,
        scratch_shapes=scratch,
        compiler_params=pltpu.CompilerParams(vmem_limit_bytes=128 * 1024 * 1024),
        name="infini_attn_moe",
    )(jnp.transpose(A_x, (0, 2, 1)), A_wq, A_wk, A_wv, A_wo, A_beta, B_w_r, B_w_gate, B_w_up,
      B_w_down.T)
    return jnp.transpose(out_t, (0, 2, 1))
```

```python
import jax
import jax.numpy as jnp
from jax import lax
import jax.experimental.pallas as pl
import jax.experimental.pallas.tpu as pltpu

F32 = jnp.float32
BF16 = jnp.bfloat16
U32 = jnp.uint32
I32 = jnp.int32

S = 2048
D = 576
H = 32
DH = 18
NSEG = 4
L = 512
FF = 4608
HPG = 7
NG = 5
QT = L // 128
GW = (128, 128, 128, 128, 80)
PR = sum(GW)
ROUTER_ROW = 126
MROWS = 144
LOG2E = 1.4426950408889634
QSCALE = (DH ** -0.5) * LOG2E
SAFE_LOG2_RANGE = 60.0
NEG_BIG = -1e30

NT_DIMS = (((1,), (1,)), ((), ()))


def _heads_in_group(g):
    return min(HPG, H - HPG * g)


def _group_row_start(g):
    return (HPG * g * DH // 16) * 16


def _group_rows(g):
    last = (HPG * g + _heads_in_group(g)) * DH
    return -(-(last - _group_row_start(g)) // 16) * 16


def _state_rows(g):
    return MROWS if g == 0 else _group_rows(g)


def _norm_row(g):
    return 128 if g == 0 else 0


def _round_bf16(x):
    return x.astype(BF16).astype(F32)


def _pad_heads_t(w):
    parts = []
    for g in range(NG):
        n = _heads_in_group(g) * DH
        parts.append(w[:, HPG * DH * g:HPG * DH * g + n])
        parts.append(jnp.zeros((D, 128 - n), w.dtype))
    return jnp.concatenate(parts, axis=1).T[0:PR]


def _phi(t):
    return jnp.where(t > 0, t + 1.0, jnp.exp(t))


def _kernel(x_hbm, wq_hbm, wk_hbm, wv_hbm, wo_hbm, beta_hbm, wr_hbm, wg_hbm, wu_hbm, wd_hbm,
            out_hbm,
            x_buf, wq_raw, wk_raw, wv_raw, wo_raw, beta_buf, wr_buf, wg_buf, wu_buf, wd_buf,
            wqt, wkt, wvt, wot, xn_buf, base, qs_buf, pq_buf, k_buf, pk_buf, vt_buf, r_buf,
            gate_buf, mt_buf, num_buf, p_buf0, p_buf1, ot_buf, out_buf, in_sems, out_sems):
    def x_copy(c):
        return pltpu.make_async_copy(x_hbm.at[0, :, pl.ds(c * L, L)], x_buf.at[c], in_sems.at[c])

    cp_wv = pltpu.make_async_copy(wv_hbm, wv_raw, in_sems.at[4])
    cp_wq = pltpu.make_async_copy(wq_hbm, wq_raw, in_sems.at[5])
    cp_wk = pltpu.make_async_copy(wk_hbm, wk_raw, in_sems.at[6])
    cp_wo = pltpu.make_async_copy(wo_hbm, wo_raw, in_sems.at[7])
    cp_wg = pltpu.make_async_copy(wg_hbm, wg_buf, in_sems.at[8])
    cp_wu = pltpu.make_async_copy(wu_hbm, wu_buf, in_sems.at[9])
    cp_wd = pltpu.make_async_copy(wd_hbm, wd_buf, in_sems.at[10])
    cp_beta = pltpu.make_async_copy(beta_hbm, beta_buf, in_sems.at[11])
    cp_wr = pltpu.make_async_copy(wr_hbm, wr_buf, in_sems.at[12])

    def out_copy(s):
        cols = pl.ds(pl.multiple_of(s * L, L), L)
        return pltpu.make_async_copy(out_buf.at[s], out_hbm.at[0, :, cols], out_sems.at[s])

    def out_tile_copy(j):
        s = NSEG - 1
        return pltpu.make_async_copy(out_buf.at[s, :, pl.ds(128 * j, 128)],
                                     out_hbm.at[0, :, pl.ds(s * L + 128 * j, 128)], out_sems.at[NSEG + j])


    for cp in (x_copy(0), cp_wv, x_copy(1), cp_wq, cp_wr, x_copy(2), cp_wk, x_copy(3), cp_wo, cp_beta,
               cp_wg, cp_wu, cp_wd):
        cp.start()

    lane128 = lax.broadcasted_iota(I32, (128, 128), 1)
    row128 = lax.broadcasted_iota(I32, (128, 128), 0)
    causal = row128 <= lane128
    r16 = lax.broadcasted_iota(I32, (16, D), 0)

    mt_buf[...] = jnp.zeros(mt_buf.shape, F32)

    always = []

    def pace(x, y):
        return x if y is None else jnp.where(always[0], x, y[0:D])

    def ln_stats(c, y):
        x = pace(x_buf[c].astype(F32), y)
        shift = x_buf[c, 0:16, :].astype(F32)[0:1]
        d = x - shift
        m1 = jnp.sum(d, axis=0, keepdims=True) * (1.0 / D)
        m2 = jnp.sum(d * d, axis=0, keepdims=True) * (1.0 / D)
        var = jnp.maximum(m2 - m1 * m1, 0.0)
        inv = 1.0 / _round_bf16(jnp.sqrt(_round_bf16(_round_bf16(var) + 1e-5)))
        return _round_bf16(shift + m1), inv

    def ln_apply(c, mean_b, inv):
        x = x_buf[c].astype(F32)
        xn = (x - mean_b) * inv
        xn_buf[c] = xn.astype(BF16)
        base[c] = x + xn

    def project(w_ref, c, split):
        if not split:
            return jnp.dot(w_ref[...], xn_buf[c], preferred_element_type=F32), None
        head = jnp.dot(w_ref[:, 0:256], xn_buf[c, 0:256, :], preferred_element_type=F32)
        tail = jnp.dot(w_ref[:, 256:D], xn_buf[c, 256:D, :], preferred_element_type=F32)
        return head + tail, head

    def project_v(c, mid=None):
        vt, head = project(wvt, c, mid is not None)
        if mid is not None:
            mid(head)
        vt_buf[c] = vt.astype(BF16)
        return vt

    def project_q(c, mid=None):
        qt, head = project(wqt, c, mid is not None)
        if mid is not None:
            mid(head)
        qsc = qt * QSCALE
        qs_buf[c] = qsc.astype(BF16)
        pq_buf[c] = _phi(qt).astype(BF16)
        r_buf[:, c * L:(c + 1) * L] = qt[120:128]
        mag = jnp.abs(qsc)
        r8 = lax.broadcasted_iota(I32, (8, L), 0)
        mag = jnp.concatenate([mag[0:120], jnp.where(r8 == ROUTER_ROW - 120, 0.0, mag[120:128]), mag[128:]], axis=0)
        return qt, jnp.max(mag.reshape(PR // 8, 8, L), axis=0)

    def project_k(c, mid=None, keep=False):
        kt, head = project(wkt, c, mid is not None)
        if mid is not None:
            mid(head)
        pk_buf[c] = _phi(kt).astype(BF16)
        for g in range(NG):
            ktg = kt[128 * g:128 * g + GW[g]]
            if GW[g] < 128:
                ktg = jnp.concatenate([ktg, jnp.zeros((128 - GW[g], L), F32)], axis=0)
            k_buf[c, g] = ktg.T.astype(BF16)
        top = jnp.max(jnp.abs(kt).reshape(PR // 8, 8, L), axis=0)
        return (kt, top) if keep else top

    x_copy(0).wait()
    stats = ln_stats(0, None)
    always.append(jnp.logical_not(jnp.abs(stats[0]) < 0.0))
    ln_apply(0, *stats)
    cp_wv.wait()
    wvt[...] = wv_raw[...].T
    project_v(0)
    x_copy(1).wait()
    cp_wq.wait()
    cp_wr.wait()
    ln_apply(1, *ln_stats(1, None))

    def paced_weight(w_ref, y):
        w = w_ref[...].astype(F32)
        return jnp.concatenate([jnp.where(always[0], w[:, 0:L], y[0:D]), w[:, L:D]], axis=1)

    def prep_wq(y):
        wq_t = _pad_heads_t(paced_weight(wq_raw, y))
        wr_row = wr_buf[...].reshape(1, D).astype(F32)
        pr_row = lax.broadcasted_iota(I32, (8, D), 0)
        wq_t = jnp.concatenate(
            [wq_t[0:120], jnp.where(pr_row == ROUTER_ROW - 120, wr_row, wq_t[120:128]), wq_t[128:]], axis=0)
        wqt[...] = wq_t.astype(BF16)

    project_v(1, prep_wq)
    cp_wk.wait()
    x_copy(2).wait()
    x_copy(3).wait()

    def prep_wk(y):
        wkt[...] = _pad_heads_t(paced_weight(wk_raw, y)).astype(BF16)

    def route():
        r = _round_bf16(r_buf[ROUTER_ROW - 120:ROUTER_ROW - 119, :])
        tok = lax.broadcasted_iota(I32, (1, S), 1).astype(F32)
        m1 = jnp.max(r)
        i1 = jnp.min(jnp.where(r == m1, tok, float(S)))
        r_rest = jnp.where(tok == i1, -jnp.inf, r)
        m2 = jnp.max(r_rest)
        i2 = jnp.min(jnp.where(r_rest == m2, tok, float(S)))
        i1 = jnp.clip(i1.astype(I32), 0, S - 1)
        i2 = jnp.clip(i2.astype(I32), 0, S - 1)
        return m1, m2, i1, i2

    qt, aq = project_q(0, prep_wk)
    qt, a = project_q(1)
    aq = jnp.maximum(aq, a)
    stats = ln_stats(2, qt)
    ak = project_k(0)
    ln_apply(2, *stats)
    kt, a = project_k(1, keep=True)
    ak = jnp.maximum(ak, a)
    stats = ln_stats(3, kt)
    project_v(2)
    ln_apply(3, *stats)
    qt, a = project_q(2)
    aq = jnp.maximum(aq, a)
    ak = jnp.maximum(ak, project_k(2))
    qt, a = project_q(3)
    aq = jnp.maximum(aq, a)
    m1, m2, i1, i2 = route()
    ak = jnp.maximum(ak, project_k(3))
    project_v(3)

    logit_bound = jnp.max(aq) * jnp.max(ak) * (DH * 1.02)
    safe = logit_bound <= SAFE_LOG2_RANGE

    sel_row = lax.broadcasted_iota(I32, (16, 128), 0)
    sel_lane = lax.broadcasted_iota(I32, (16, 128), 1)

    def token_tile(i):
        return i // L, pl.ds(pl.multiple_of(((i % L) // 128) * 128, 128), 128)

    def pick(i, slot):
        seg, cols = token_tile(i)
        onehot = jnp.where((sel_row == slot) & (sel_lane == i % 128), 1.0, 0.0).astype(BF16)
        return lax.dot_general(onehot, xn_buf[seg, :, cols], NT_DIMS, preferred_element_type=F32)

    xs = (pick(i1, 0) + pick(i2, 1)).astype(BF16)

    cp_wo.wait()
    cp_beta.wait()
    cp_wg.wait()
    cp_wu.wait()

    beta_row = beta_buf[...].reshape(1, H).astype(F32)
    beta_row = jnp.concatenate([beta_row, jnp.zeros((1, 128 - H), F32)], axis=1)
    h_row = lax.broadcasted_iota(I32, (H, 128), 0)
    h_lane = lax.broadcasted_iota(I32, (H, 128), 1)
    beta_col = jnp.sum(jnp.where(h_row == h_lane, beta_row, 0.0), axis=1, keepdims=True)
    gate_buf[...] = jnp.broadcast_to(jax.nn.sigmoid(beta_col), (H, 128))


    def expert_chunk(lo, hi):
        hg = jnp.dot(xs, wg_buf[:, lo:hi], preferred_element_type=F32)
        hu = jnp.dot(xs, wu_buf[:, lo:hi], preferred_element_type=F32)
        hh = (jax.nn.silu(hg) * hu).astype(BF16)
        return lax.dot_general(hh, wd_buf[:, lo:hi], NT_DIMS, preferred_element_type=F32)

    def expert_up_stream(hidden):
        kmain = 512
        for c0 in range(0, FF, 512):
            rem = []
            for w_ref in (wg_buf, wu_buf):
                rem.append(jnp.dot(xs[:, kmain:D], w_ref[kmain:D, c0:c0 + 512], preferred_element_type=F32))
                yield
            hs = []
            for f0 in range(c0, c0 + 512, 128):
                pre = []
                for w_ref, r in zip((wg_buf, wu_buf), rem):
                    pre.append(jnp.dot(xs[:, 0:kmain], w_ref[0:kmain, f0:f0 + 128], preferred_element_type=F32)
                               + r[:, f0 - c0:f0 - c0 + 128])
                    if len(pre) == 2:
                        hs.append(jax.nn.silu(pre[0]) * pre[1])
                        if len(hs) == 4:
                            hidden.append(jnp.concatenate(hs, axis=1).astype(BF16))
                    yield

    def expert_down_step(hh, ci, e):
        e_hi = min(128 * (e + 1), D)
        return lax.dot_general(hh, wd_buf[128 * e:e_hi, 512 * ci:512 * (ci + 1)], NT_DIMS,
                               preferred_element_type=F32)

    def expert_scatter_parts(y):
        y = y * jax.nn.sigmoid(jnp.where(r16 == 0, m1, m2))
        yt = jnp.concatenate([y, jnp.zeros((128 - 16, D), F32)], axis=0).T
        lane_d = lax.broadcasted_iota(I32, (D, 128), 1)
        for slot, i in ((0, i1), (1, i2)):
            seg, cols = token_tile(i)
            col = jnp.sum(jnp.where(lane_d == slot, yt, 0.0), axis=1, keepdims=True)
            base[seg, :, cols] = base[seg, :, cols] + jnp.where(lane_d == i % 128, col, 0.0)
            yield

    def expert_scatter(y):
        for _ in expert_scatter_parts(y):
            pass

    def memory_read(s, g):
        sr = _state_rows(g)
        gw = GW[g]
        num_buf[g, 0:sr, :] = jnp.dot(mt_buf[g, 0:sr, 0:gw].astype(BF16), pq_buf[s, 128 * g:128 * g + gw, :],
                                      preferred_element_type=F32)

    def memory_update(s, g):
        rg = _group_rows(g)
        a_g = _group_row_start(g)
        gw = GW[g]
        ones_row = 126 if g == 0 else 0
        lhs = jnp.where(lax.broadcasted_iota(I32, (rg, L), 0) == ones_row, 1.0,
                        vt_buf[s, a_g:a_g + rg, :].astype(F32)).astype(BF16)
        upd = lax.dot_general(lhs, pk_buf[s, 128 * g:128 * g + gw, :], NT_DIMS,
                              preferred_element_type=F32)
        er = lax.broadcasted_iota(I32, (rg, gw), 0) + (a_g - HPG * DH * g)
        el = lax.broadcasted_iota(I32, (rg, gw), 1)
        same_head = None
        for i in range(_heads_in_group(g)):
            t = ((er >= DH * i) & (er < DH * (i + 1)) & (el >= DH * i) & (el < DH * (i + 1)))
            same_head = t if same_head is None else (same_head | t)
        mt_buf[g, 0:rg, 0:gw] = mt_buf[g, 0:rg, 0:gw] + jnp.where(same_head, upd, 0.0)
        zr = lax.broadcasted_iota(I32, (8, gw), 0)
        zl = lax.broadcasted_iota(I32, (8, gw), 1)
        zmask = (zl >= zr * DH) & (zl < zr * DH + DH) & (zr < _heads_in_group(g))
        zs = upd[ones_row:ones_row + 1]
        z0 = _norm_row(g)
        mt_buf[g, z0:z0 + 8, 0:gw] = mt_buf[g, z0:z0 + 8, 0:gw] + jnp.where(zmask, zs, 0.0)

    def transpose_wo(g):
        hi = min(128 * (g + 1), D)
        wot[128 * g:hi, :] = wo_raw[:, 128 * g:hi].T

    def project_out(s):
        attn = jnp.dot(wot[...], ot_buf[...].astype(BF16), preferred_element_type=F32)
        return base[s] + attn

    def emit(s, val):
        out_buf[s] = val.astype(BF16)
        out_copy(s).start()

    zero = lax.shift_right_logical(i1, 16)

    def prow(start, size):
        return pl.ds(pl.multiple_of(zero + start, 8), size)

    P_OFFS = (0, 128, 384, 768)

    def fast_scores(s, g, hook):
        nh = _heads_in_group(g)
        gw = GW[g]
        pb = (p_buf0, p_buf1)[(s * NG + g) % 2]
        rowg = lax.broadcasted_iota(I32, (gw, 128), 0)
        for j in range(QT - 1, -1, -1):
            n = 128 * (j + 1)
            q = qs_buf[s, 128 * g:128 * g + gw, 128 * j:128 * (j + 1)].astype(F32)
            for h0, h1 in ((0, 4), (4, nh)):
                if h1 <= h0:
                    continue
                qm = jnp.concatenate(
                    [jnp.where((rowg >= DH * i) & (rowg < DH * (i + 1)), q, 0.0) for i in range(h0, h1)],
                    axis=1).astype(BF16)
                st = jnp.dot(k_buf[s, g, 0:n, 0:gw], qm, preferred_element_type=F32)
                p = jnp.exp2(st)
                causal_w = jnp.concatenate([causal] * (h1 - h0), axis=1)
                p_diag = jnp.where(causal_w, p[n - 128:], 0.0)
                p = jnp.concatenate([p[:n - 128], p_diag], axis=0) if j > 0 else p_diag
                pb[P_OFFS[j] // 2:(P_OFFS[j] + n) // 2, h0 * 128:h1 * 128] = pltpu.bitcast(p.astype(BF16), U32)
                hook(j >= 2, p)

    def fast_values(s, g, after_tile=None):
        nh = _heads_in_group(g)
        a_g = _group_row_start(g)
        pb = (p_buf0, p_buf1)[(s * NG + g) % 2]
        for j in range(QT - 1, -1, -1):
            n = 128 * (j + 1)
            cols = slice(128 * j, 128 * (j + 1))
            for i in range(nh):
                h = HPG * g + i
                a = (h * DH // 16) * 16
                off = h * DH - a
                p = pltpu.bitcast(pb[prow(P_OFFS[j] // 2, n // 2), 128 * i:128 * (i + 1)], BF16)
                ones_row = 0 if off > 0 else 31
                r32n = lax.broadcasted_iota(I32, (32, n), 0)
                lhs = jnp.where(r32n == ones_row, 1.0, vt_buf[s, a:a + 32, 0:n].astype(F32)).astype(BF16)
                o = jnp.dot(lhs, p, preferred_element_type=F32)
                lo = (off // 8) * 8
                hi = -(-(off + DH) // 8) * 8
                gate = gate_buf[h:h + 1, :]
                rl = 1.0 / o[ones_row:ones_row + 1]
                val = (1.0 - gate) * (o[lo:hi] * rl)
                if s > 0:
                    z = _norm_row(g) + i
                    rden = 1.0 / (num_buf[g, z:z + 1, cols] + 1e-6)
                    num = num_buf[g, a - a_g + lo:a - a_g + hi, cols]
                    val = gate * (num * rden) + val
                ot_buf[a + off:a + off + DH, cols] = val[off - lo:off - lo + DH]
            if after_tile is not None:
                after_tile(j)

    def fast_path():
        hidden = []
        up = expert_up_stream(hidden)
        n_chunks = FF // 512
        state = dict(down=0, wd_ready=False, up_done=False, y=[None] * 5, tail=None)

        def finish():
            yield from expert_scatter_parts(jnp.concatenate(state["y"], axis=1))
            for u in range(NSEG - 1):
                for j in range(QT):
                    cols = slice(128 * j, 128 * (j + 1))
                    val = base[u, :, cols]
                    y = state["pacer"]
                    if y is not None:
                        reps = -(-D // y.shape[0])
                        y = jnp.concatenate([y[:, 128 * r:128 * (r + 1)] for r in range(reps)], axis=0)[0:D]
                        val = jnp.where(always[0][:, 0:128], val, y)
                    out_buf[u, :, cols] = val.astype(BF16)
                    if j == QT - 1:
                        out_copy(u).start()
                    yield

        def down_step():
            ci, e = divmod(state["down"], 5)
            part = expert_down_step(hidden[ci], ci, e)
            state["y"][e] = part if state["y"][e] is None else state["y"][e] + part
            state["down"] += 1

        def hook(long, pacer=None):
            state["pacer"] = pacer if pacer is not None and pacer.shape[0] * (pacer.shape[1] // 128) >= D else None
            can_down = (state["wd_ready"] and state["down"] < 5 * n_chunks
                        and state["down"] // 5 < len(hidden))
            if can_down and (long or state["up_done"]):
                down_step()
            elif not state["up_done"]:
                if next(up, "done") == "done":
                    state["up_done"] = True
                    hook(long, pacer)
            elif state["down"] == 5 * n_chunks and state["out_ready"]:
                if state["tail"] is None:
                    state["tail"] = finish()
                if pacer is not None and state["pacer"] is not None or state["tail_steps"] < 2:
                    state["tail_steps"] += 1
                    next(state["tail"], None)

        state["out_ready"] = False
        state["tail_steps"] = 0
        steps = [(s, g) for s in range(NSEG) for g in range(NG)]
        last = NSEG - 1

        def last_tile(j):
            cols = slice(128 * j, 128 * (j + 1))
            attn = jnp.dot(wot[...], ot_buf[:, cols].astype(BF16), preferred_element_type=F32)
            out_buf[last, :, cols] = (base[last, :, cols] + attn).astype(BF16)
            out_tile_copy(j).start()

        fast_scores(0, 0, hook)
        for t, (s, g) in enumerate(steps):
            if t + 1 < len(steps):
                fast_scores(*steps[t + 1], hook)
            if s > 0:
                memory_read(s, g)
                hook(True)
            if t + 1 == len(steps):
                state["pacer"] = None
                while state["tail"] is None or next(state["tail"], "done") != "done":
                    if state["tail"] is None:
                        hook(True)
                fast_values(s, g, last_tile)
            else:
                fast_values(s, g)
            if s == 0:
                transpose_wo(g)
            if s + 1 < NSEG:
                memory_update(s, g)
                hook(True)
            if g == NG - 1 and s < last:
                base[s] = project_out(s)
                if s == 0:
                    cp_wd.wait()
                    state["wd_ready"] = True
                if s == last - 1:
                    state["out_ready"] = True
                hook(True)
        for u in range(NSEG - 1):
            out_copy(u).wait()
        for j in range(QT):
            out_tile_copy(j).wait()

    def slow_segment(s, carry):
        for g in range(NG):
            memory_read(s, g)
        key_i = lax.broadcasted_iota(I32, (L, L), 0)
        qry_i = lax.broadcasted_iota(I32, (L, L), 1)
        r32 = lax.broadcasted_iota(I32, (32, L), 0)
        for g in range(NG):
            gw = GW[g]
            a_g = _group_row_start(g)
            rowg = lax.broadcasted_iota(I32, (gw, L), 0)

            def head(i, c, g=g, gw=gw, a_g=a_g, rowg=rowg):
                h = HPG * g + i
                a = pl.multiple_of((h * DH // 16) * 16, 16)
                off = h * DH - a
                q = qs_buf[s, 128 * g:128 * g + gw, :].astype(F32)
                qm = jnp.where((rowg >= DH * i) & (rowg < DH * (i + 1)), q, 0.0).astype(BF16)
                st = jnp.dot(k_buf[s, g, :, 0:gw], qm, preferred_element_type=F32)
                st = jnp.where(key_i <= qry_i, st, NEG_BIG)
                p = jnp.exp2(st - jnp.max(st, axis=0, keepdims=True))
                rl = 1.0 / jnp.sum(p, axis=0, keepdims=True)
                o = jnp.dot(vt_buf[s, pl.ds(a, 32), :], p.astype(BF16), preferred_element_type=F32)
                gate = jnp.concatenate([gate_buf[pl.ds(h, 1), :]] * QT, axis=1)
                rden = 1.0 / (num_buf[g, pl.ds(_norm_row(g) + i, 1), :] + 1e-6)
                num = num_buf[g, pl.ds(pl.multiple_of(a - a_g, 16), 32), :]
                val = gate * (num * rden) + (1.0 - gate) * (o * rl)
                keep = (r32 >= off) & (r32 < off + DH)
                pltpu.store(ot_buf.at[pl.ds(a, 32), :], val, mask=keep)
                return c

            lax.fori_loop(0, _heads_in_group(g), head, 0)
        for g in range(NG):
            memory_update(s, g)
        emit(s, project_out(s))
        return carry

    @pl.when(safe)
    def _():
        fast_path()

    @pl.when(jnp.logical_not(safe))
    def _():
        cp_wd.wait()
        for g in range(NG):
            transpose_wo(g)
        expert_scatter(expert_chunk(0, FF))
        lax.fori_loop(0, NSEG, slow_segment, 0)
        for u in range(NSEG):
            out_copy(u).wait()


@jax.jit
def pallas_parallel_sum__memory_aug_infini_attn__moe_arch_mod__prompt_kernel(
    A_x: jax.Array,
    A_wq: jax.Array,
    A_wk: jax.Array,
    A_wv: jax.Array,
    A_wo: jax.Array,
    A_beta: jax.Array,
    B_x: jax.Array,
    B_w_r: jax.Array,
    B_w_gate: jax.Array,
    B_w_up: jax.Array,
    B_w_down: jax.Array,
):
    del B_x
    hbm = pl.BlockSpec(memory_space=pl.ANY)
    scratch = [
        pltpu.VMEM((NSEG, D, L), BF16),
        pltpu.VMEM((D, D), BF16),
        pltpu.VMEM((D, D), BF16),
        pltpu.VMEM((D, D), BF16),
        pltpu.VMEM((D, D), BF16),
        pltpu.VMEM((H,), BF16),
        pltpu.VMEM((D,), BF16),
        pltpu.VMEM((D, FF), BF16),
        pltpu.VMEM((D, FF), BF16),
        pltpu.VMEM((D, FF), BF16),
        pltpu.VMEM((PR, D), BF16),
        pltpu.VMEM((PR, D), BF16),
        pltpu.VMEM((D, D), BF16),
        pltpu.VMEM((D, D), BF16),
        pltpu.VMEM((NSEG, D, L), BF16),
        pltpu.VMEM((NSEG, D, L), F32),
        pltpu.VMEM((NSEG, PR, L), BF16),
        pltpu.VMEM((NSEG, PR, L), BF16),
        pltpu.VMEM((NSEG, NG, L, 128), BF16),
        pltpu.VMEM((NSEG, PR, L), BF16),
        pltpu.VMEM((NSEG, D, L), BF16),
        pltpu.VMEM((8, S), F32),
        pltpu.VMEM((H, 128), F32),
        pltpu.VMEM((NG, MROWS, 128), F32),
        pltpu.VMEM((NG, MROWS, L), F32),
        pltpu.VMEM((640, HPG * 128), U32),
        pltpu.VMEM((640, HPG * 128), U32),
        pltpu.VMEM((D, L), F32),
        pltpu.VMEM((NSEG, D, L), BF16),
        pltpu.SemaphoreType.DMA((13,)),
        pltpu.SemaphoreType.DMA((NSEG + QT,)),
    ]
    out_t = pl.pallas_call(
        _kernel,
        out_shape=jax.ShapeDtypeStruct((1, D, S), BF16),
        in_specs=[hbm] * 10,
        out_specs=hbm,
        scratch_shapes=scratch,
        compiler_params=pltpu.CompilerParams(vmem_limit_bytes=128 * 1024 * 1024),
        name="infini_attn_moe",
    )(jnp.transpose(A_x, (0, 2, 1)), A_wq, A_wk, A_wv, A_wo, A_beta, B_w_r, B_w_gate, B_w_up,
      B_w_down.T)
    return jnp.transpose(out_t, (0, 2, 1))
```

```python
import jax
import jax.numpy as jnp
from jax import lax
import jax.experimental.pallas as pl
import jax.experimental.pallas.tpu as pltpu

F32 = jnp.float32
BF16 = jnp.bfloat16
U32 = jnp.uint32
I32 = jnp.int32

S = 2048
D = 576
H = 32
DH = 18
NSEG = 4
L = 512
FF = 4608
HPG = 7
NG = 5
QT = L // 128
GW = (128, 128, 128, 128, 80)
PR = sum(GW)
ROUTER_ROW = 126
MROWS = 144
LOG2E = 1.4426950408889634
QSCALE = (DH ** -0.5) * LOG2E
SAFE_LOG2_RANGE = 60.0
NEG_BIG = -1e30

NT_DIMS = (((1,), (1,)), ((), ()))


def _heads_in_group(g):
    return min(HPG, H - HPG * g)


def _group_row_start(g):
    return (HPG * g * DH // 16) * 16


def _group_rows(g):
    last = (HPG * g + _heads_in_group(g)) * DH
    return -(-(last - _group_row_start(g)) // 16) * 16


def _state_rows(g):
    return MROWS if g == 0 else _group_rows(g)


def _norm_row(g):
    return 128 if g == 0 else 0


def _round_bf16(x):
    return x.astype(BF16).astype(F32)


def _pad_heads_t(w):
    parts = []
    for g in range(NG):
        n = _heads_in_group(g) * DH
        parts.append(w[:, HPG * DH * g:HPG * DH * g + n])
        parts.append(jnp.zeros((D, 128 - n), w.dtype))
    return jnp.concatenate(parts, axis=1).T[0:PR]


def _phi(t):
    return jnp.where(t > 0, t + 1.0, jnp.exp(t))


class _Packed:
    def __init__(self, ref, rows):
        self.ref = ref
        self.rows = rows

    def _slice(self, item, lo, size):
        start = item * (self.rows // 2) + lo // 2
        size = size // 2
        if isinstance(start, int):
            return slice(start, start + size)
        return pl.ds(pl.multiple_of(start, 8), size)

    def load(self, item=0, lo=0, hi=None, cols=slice(None)):
        size = hi if not isinstance(lo, int) else (self.rows if hi is None else hi) - lo
        return pltpu.bitcast(self.ref[self._slice(item, lo, size), cols], BF16)

    def store(self, val, item=0, lo=0, cols=slice(None)):
        self.ref[self._slice(item, lo, val.shape[0]), cols] = pltpu.bitcast(val.astype(BF16), U32)


def _kernel(x_hbm, wq_hbm, wk_hbm, wv_hbm, wo_hbm, beta_hbm, wr_hbm, wg_hbm, wu_hbm, wd_hbm,
            out_hbm,
            x_buf, wq_raw, wk_raw, wv_raw, wo_raw, beta_buf, wr_buf, wg_buf, wu_buf, wd_buf,
            wqt, wkt, wvt, wot, xn_buf, base, qs_buf, pq_buf, k_buf, pk_buf, vt_buf, r_buf,
            gate_buf, mt_buf, num_buf, p_buf0, p_buf1, ot_buf, out_buf, in_sems, out_sems):
    wqt, wkt = _Packed(wqt, PR), _Packed(wkt, PR)
    wvt, wot = _Packed(wvt, D), _Packed(wot, D)
    xn_buf, vt_buf = _Packed(xn_buf, D), _Packed(vt_buf, D)
    qs_buf, pq_buf, pk_buf = _Packed(qs_buf, PR), _Packed(pq_buf, PR), _Packed(pk_buf, PR)
    k_buf = _Packed(k_buf, L)

    def x_copy(c):
        return pltpu.make_async_copy(x_hbm.at[0, :, pl.ds(c * L, L)], x_buf.at[c], in_sems.at[c])

    cp_wv = pltpu.make_async_copy(wv_hbm, wv_raw, in_sems.at[4])
    cp_wq = pltpu.make_async_copy(wq_hbm, wq_raw, in_sems.at[5])
    cp_wk = pltpu.make_async_copy(wk_hbm, wk_raw, in_sems.at[6])
    cp_wo = pltpu.make_async_copy(wo_hbm, wo_raw, in_sems.at[7])
    cp_wg = pltpu.make_async_copy(wg_hbm, wg_buf, in_sems.at[8])
    cp_wu = pltpu.make_async_copy(wu_hbm, wu_buf, in_sems.at[9])
    cp_wd = pltpu.make_async_copy(wd_hbm, wd_buf, in_sems.at[10])
    cp_beta = pltpu.make_async_copy(beta_hbm, beta_buf, in_sems.at[11])
    cp_wr = pltpu.make_async_copy(wr_hbm, wr_buf, in_sems.at[12])

    def out_copy(s):
        cols = pl.ds(pl.multiple_of(s * L, L), L)
        return pltpu.make_async_copy(out_buf.at[s], out_hbm.at[0, :, cols], out_sems.at[s])

    def out_tile_copy(j):
        s = NSEG - 1
        return pltpu.make_async_copy(out_buf.at[s, :, pl.ds(128 * j, 128)],
                                     out_hbm.at[0, :, pl.ds(s * L + 128 * j, 128)], out_sems.at[NSEG + j])


    for cp in (x_copy(0), cp_wv, x_copy(1), cp_wq, cp_wr, x_copy(2), cp_wk, x_copy(3), cp_wo, cp_beta,
               cp_wg, cp_wu, cp_wd):
        cp.start()

    lane128 = lax.broadcasted_iota(I32, (128, 128), 1)
    row128 = lax.broadcasted_iota(I32, (128, 128), 0)
    causal = row128 <= lane128
    r16 = lax.broadcasted_iota(I32, (16, D), 0)

    mt_buf[...] = jnp.zeros(mt_buf.shape, F32)

    always = []

    def pace(x, y):
        return x if y is None else jnp.where(always[0], x, y[0:D])

    def ln_stats(c, y):
        x = pace(x_buf[c].astype(F32), y)
        shift = x_buf[c, 0:16, :].astype(F32)[0:1]
        d = x - shift
        m1 = jnp.sum(d, axis=0, keepdims=True) * (1.0 / D)
        m2 = jnp.sum(d * d, axis=0, keepdims=True) * (1.0 / D)
        var = jnp.maximum(m2 - m1 * m1, 0.0)
        inv = 1.0 / _round_bf16(jnp.sqrt(_round_bf16(_round_bf16(var) + 1e-5)))
        return _round_bf16(shift + m1), inv

    def ln_apply(c, mean_b, inv):
        x = x_buf[c].astype(F32)
        xn = (x - mean_b) * inv
        xn_buf.store(xn, c)
        base[c] = x + xn

    def project(w_ref, c, split):
        if not split:
            return jnp.dot(w_ref.load(), xn_buf.load(c), preferred_element_type=F32), None
        head = jnp.dot(w_ref.load(cols=slice(0, 256)), xn_buf.load(c, 0, 256), preferred_element_type=F32)
        tail = jnp.dot(w_ref.load(cols=slice(256, D)), xn_buf.load(c, 256, D), preferred_element_type=F32)
        return head + tail, head

    def project_v(c, mid=None):
        vt, head = project(wvt, c, mid is not None)
        if mid is not None:
            mid(head)
        vt_buf.store(vt, c)
        return vt

    def project_q(c, mid=None):
        qt, head = project(wqt, c, mid is not None)
        if mid is not None:
            mid(head)
        qsc = qt * QSCALE
        qs_buf.store(qsc, c)
        pq_buf.store(_phi(qt), c)
        r_buf[:, c * L:(c + 1) * L] = qt[120:128]
        mag = jnp.abs(qsc)
        r8 = lax.broadcasted_iota(I32, (8, L), 0)
        mag = jnp.concatenate([mag[0:120], jnp.where(r8 == ROUTER_ROW - 120, 0.0, mag[120:128]), mag[128:]], axis=0)
        return qt, jnp.max(mag.reshape(PR // 8, 8, L), axis=0)

    def project_k(c, mid=None, keep=False):
        kt, head = project(wkt, c, mid is not None)
        if mid is not None:
            mid(head)
        pk_buf.store(_phi(kt), c)
        for g in range(NG):
            ktg = kt[128 * g:128 * g + GW[g]]
            if GW[g] < 128:
                ktg = jnp.concatenate([ktg, jnp.zeros((128 - GW[g], L), F32)], axis=0)
            k_buf.store(ktg.T, c * NG + g)
        top = jnp.max(jnp.abs(kt).reshape(PR // 8, 8, L), axis=0)
        return (kt, top) if keep else top

    x_copy(0).wait()
    stats = ln_stats(0, None)
    always.append(jnp.logical_not(jnp.abs(stats[0]) < 0.0))
    ln_apply(0, *stats)
    cp_wv.wait()
    wvt.store(wv_raw[...].T)
    project_v(0)
    x_copy(1).wait()
    cp_wq.wait()
    cp_wr.wait()
    ln_apply(1, *ln_stats(1, None))

    def paced_weight(w_ref, y):
        w = w_ref[...].astype(F32)
        return jnp.concatenate([jnp.where(always[0], w[:, 0:L], y[0:D]), w[:, L:D]], axis=1)

    def prep_wq(y):
        wq_t = _pad_heads_t(paced_weight(wq_raw, y))
        wr_row = wr_buf[...].reshape(1, D).astype(F32)
        pr_row = lax.broadcasted_iota(I32, (8, D), 0)
        wq_t = jnp.concatenate(
            [wq_t[0:120], jnp.where(pr_row == ROUTER_ROW - 120, wr_row, wq_t[120:128]), wq_t[128:]], axis=0)
        wqt.store(wq_t)

    project_v(1, prep_wq)
    cp_wk.wait()
    x_copy(2).wait()
    x_copy(3).wait()

    def prep_wk(y):
        wkt.store(_pad_heads_t(paced_weight(wk_raw, y)))

    def route():
        r = _round_bf16(r_buf[ROUTER_ROW - 120:ROUTER_ROW - 119, :])
        tok = lax.broadcasted_iota(I32, (1, S), 1).astype(F32)
        m1 = jnp.max(r)
        i1 = jnp.min(jnp.where(r == m1, tok, float(S)))
        r_rest = jnp.where(tok == i1, -jnp.inf, r)
        m2 = jnp.max(r_rest)
        i2 = jnp.min(jnp.where(r_rest == m2, tok, float(S)))
        i1 = jnp.clip(i1.astype(I32), 0, S - 1)
        i2 = jnp.clip(i2.astype(I32), 0, S - 1)
        return m1, m2, i1, i2

    qt, aq = project_q(0, prep_wk)
    qt, a = project_q(1)
    aq = jnp.maximum(aq, a)
    stats = ln_stats(2, qt)
    ak = project_k(0)
    ln_apply(2, *stats)
    kt, a = project_k(1, keep=True)
    ak = jnp.maximum(ak, a)
    stats = ln_stats(3, kt)
    project_v(2)
    ln_apply(3, *stats)
    qt, a = project_q(2)
    aq = jnp.maximum(aq, a)
    ak = jnp.maximum(ak, project_k(2))
    qt, a = project_q(3)
    aq = jnp.maximum(aq, a)
    m1, m2, i1, i2 = route()
    ak = jnp.maximum(ak, project_k(3))
    project_v(3)

    logit_bound = jnp.max(aq) * jnp.max(ak) * (DH * 1.02)
    safe = logit_bound <= SAFE_LOG2_RANGE

    sel_row = lax.broadcasted_iota(I32, (16, 128), 0)
    sel_lane = lax.broadcasted_iota(I32, (16, 128), 1)

    def token_tile(i):
        return i // L, pl.ds(pl.multiple_of(((i % L) // 128) * 128, 128), 128)

    def pick(i, slot):
        seg, cols = token_tile(i)
        onehot = jnp.where((sel_row == slot) & (sel_lane == i % 128), 1.0, 0.0).astype(BF16)
        return lax.dot_general(onehot, xn_buf.load(seg, cols=cols), NT_DIMS, preferred_element_type=F32)

    xs = (pick(i1, 0) + pick(i2, 1)).astype(BF16)

    cp_wo.wait()
    cp_beta.wait()
    cp_wg.wait()
    cp_wu.wait()

    beta_row = beta_buf[...].reshape(1, H).astype(F32)
    beta_row = jnp.concatenate([beta_row, jnp.zeros((1, 128 - H), F32)], axis=1)
    h_row = lax.broadcasted_iota(I32, (H, 128), 0)
    h_lane = lax.broadcasted_iota(I32, (H, 128), 1)
    beta_col = jnp.sum(jnp.where(h_row == h_lane, beta_row, 0.0), axis=1, keepdims=True)
    gate_buf[...] = jnp.broadcast_to(jax.nn.sigmoid(beta_col), (H, 128))


    def expert_chunk(lo, hi):
        hg = jnp.dot(xs, wg_buf[:, lo:hi], preferred_element_type=F32)
        hu = jnp.dot(xs, wu_buf[:, lo:hi], preferred_element_type=F32)
        hh = (jax.nn.silu(hg) * hu).astype(BF16)
        return lax.dot_general(hh, wd_buf[:, lo:hi], NT_DIMS, preferred_element_type=F32)

    def expert_up_stream(hidden):
        kmain = 512
        for c0 in range(0, FF, 512):
            rem = []
            for w_ref in (wg_buf, wu_buf):
                rem.append(jnp.dot(xs[:, kmain:D], w_ref[kmain:D, c0:c0 + 512], preferred_element_type=F32))
                yield
            hs = []
            for f0 in range(c0, c0 + 512, 128):
                pre = []
                for w_ref, r in zip((wg_buf, wu_buf), rem):
                    pre.append(jnp.dot(xs[:, 0:kmain], w_ref[0:kmain, f0:f0 + 128], preferred_element_type=F32)
                               + r[:, f0 - c0:f0 - c0 + 128])
                    if len(pre) == 2:
                        hs.append(jax.nn.silu(pre[0]) * pre[1])
                        if len(hs) == 4:
                            hidden.append(jnp.concatenate(hs, axis=1).astype(BF16))
                    yield

    def expert_down_step(hh, ci, e):
        e_hi = min(128 * (e + 1), D)
        return lax.dot_general(hh, wd_buf[128 * e:e_hi, 512 * ci:512 * (ci + 1)], NT_DIMS,
                               preferred_element_type=F32)

    def expert_scatter_parts(y):
        y = y * jax.nn.sigmoid(jnp.where(r16 == 0, m1, m2))
        yt = jnp.concatenate([y, jnp.zeros((128 - 16, D), F32)], axis=0).T
        lane_d = lax.broadcasted_iota(I32, (D, 128), 1)
        for slot, i in ((0, i1), (1, i2)):
            seg, cols = token_tile(i)
            col = jnp.sum(jnp.where(lane_d == slot, yt, 0.0), axis=1, keepdims=True)
            base[seg, :, cols] = base[seg, :, cols] + jnp.where(lane_d == i % 128, col, 0.0)
            yield

    def expert_scatter(y):
        for _ in expert_scatter_parts(y):
            pass

    def memory_read(s, g):
        sr = _state_rows(g)
        gw = GW[g]
        num_buf[g, 0:sr, :] = jnp.dot(mt_buf[g, 0:sr, 0:gw].astype(BF16), pq_buf.load(s, 128 * g, 128 * g + gw),
                                      preferred_element_type=F32)

    def memory_update(s, g):
        rg = _group_rows(g)
        a_g = _group_row_start(g)
        gw = GW[g]
        ones_row = 126 if g == 0 else 0
        lhs = jnp.where(lax.broadcasted_iota(I32, (rg, L), 0) == ones_row, 1.0,
                        vt_buf.load(s, a_g, a_g + rg).astype(F32)).astype(BF16)
        upd = lax.dot_general(lhs, pk_buf.load(s, 128 * g, 128 * g + gw), NT_DIMS,
                              preferred_element_type=F32)
        er = lax.broadcasted_iota(I32, (rg, gw), 0) + (a_g - HPG * DH * g)
        el = lax.broadcasted_iota(I32, (rg, gw), 1)
        same_head = None
        for i in range(_heads_in_group(g)):
            t = ((er >= DH * i) & (er < DH * (i + 1)) & (el >= DH * i) & (el < DH * (i + 1)))
            same_head = t if same_head is None else (same_head | t)
        mt_buf[g, 0:rg, 0:gw] = mt_buf[g, 0:rg, 0:gw] + jnp.where(same_head, upd, 0.0)
        zr = lax.broadcasted_iota(I32, (8, gw), 0)
        zl = lax.broadcasted_iota(I32, (8, gw), 1)
        zmask = (zl >= zr * DH) & (zl < zr * DH + DH) & (zr < _heads_in_group(g))
        zs = upd[ones_row:ones_row + 1]
        z0 = _norm_row(g)
        mt_buf[g, z0:z0 + 8, 0:gw] = mt_buf[g, z0:z0 + 8, 0:gw] + jnp.where(zmask, zs, 0.0)

    def transpose_wo(g):
        hi = min(128 * (g + 1), D)
        wot.store(wo_raw[:, 128 * g:hi].T, lo=128 * g)

    def project_out(s):
        attn = jnp.dot(wot.load(), ot_buf[...].astype(BF16), preferred_element_type=F32)
        return base[s] + attn

    def emit(s, val):
        out_buf[s] = val.astype(BF16)
        out_copy(s).start()

    zero = lax.shift_right_logical(i1, 16)

    def prow(start, size):
        return pl.ds(pl.multiple_of(zero + start, 8), size)

    P_OFFS = (0, 128, 384, 768)

    def fast_scores(s, g, hook):
        nh = _heads_in_group(g)
        gw = GW[g]
        pb = (p_buf0, p_buf1)[(s * NG + g) % 2]
        rowg = lax.broadcasted_iota(I32, (gw, 128), 0)
        for j in range(QT - 1, -1, -1):
            n = 128 * (j + 1)
            q = qs_buf.load(s, 128 * g, 128 * g + gw, slice(128 * j, 128 * (j + 1))).astype(F32)
            for h0, h1 in ((0, 4), (4, nh)):
                if h1 <= h0:
                    continue
                qm = jnp.concatenate(
                    [jnp.where((rowg >= DH * i) & (rowg < DH * (i + 1)), q, 0.0) for i in range(h0, h1)],
                    axis=1).astype(BF16)
                st = jnp.dot(k_buf.load(s * NG + g, 0, n, slice(0, gw)), qm, preferred_element_type=F32)
                p = jnp.exp2(st)
                causal_w = jnp.concatenate([causal] * (h1 - h0), axis=1)
                p_diag = jnp.where(causal_w, p[n - 128:], 0.0)
                p = jnp.concatenate([p[:n - 128], p_diag], axis=0) if j > 0 else p_diag
                pb[P_OFFS[j] // 2:(P_OFFS[j] + n) // 2, h0 * 128:h1 * 128] = pltpu.bitcast(p.astype(BF16), U32)
                hook(j >= 2, p)

    def fast_values(s, g, after_tile=None):
        nh = _heads_in_group(g)
        a_g = _group_row_start(g)
        pb = (p_buf0, p_buf1)[(s * NG + g) % 2]
        for j in range(QT - 1, -1, -1):
            n = 128 * (j + 1)
            cols = slice(128 * j, 128 * (j + 1))
            for i in range(nh):
                h = HPG * g + i
                a = (h * DH // 16) * 16
                off = h * DH - a
                p = pltpu.bitcast(pb[prow(P_OFFS[j] // 2, n // 2), 128 * i:128 * (i + 1)], BF16)
                ones_row = 0 if off > 0 else 31
                r32n = lax.broadcasted_iota(I32, (32, n), 0)
                lhs = jnp.where(r32n == ones_row, 1.0, vt_buf.load(s, a, a + 32, slice(0, n)).astype(F32)).astype(BF16)
                o = jnp.dot(lhs, p, preferred_element_type=F32)
                lo = (off // 8) * 8
                hi = -(-(off + DH) // 8) * 8
                gate = gate_buf[h:h + 1, :]
                rl = 1.0 / o[ones_row:ones_row + 1]
                val = (1.0 - gate) * (o[lo:hi] * rl)
                if s > 0:
                    z = _norm_row(g) + i
                    rden = 1.0 / (num_buf[g, z:z + 1, cols] + 1e-6)
                    num = num_buf[g, a - a_g + lo:a - a_g + hi, cols]
                    val = gate * (num * rden) + val
                ot_buf[a + off:a + off + DH, cols] = val[off - lo:off - lo + DH]
            if after_tile is not None:
                after_tile(j)

    def fast_path():
        hidden = []
        up = expert_up_stream(hidden)
        n_chunks = FF // 512
        state = dict(down=0, wd_ready=False, up_done=False, y=[None] * 5, tail=None)

        def finish():
            yield from expert_scatter_parts(jnp.concatenate(state["y"], axis=1))
            for u in range(NSEG - 1):
                for j in range(QT):
                    cols = slice(128 * j, 128 * (j + 1))
                    val = base[u, :, cols]
                    y = state["pacer"]
                    if y is not None:
                        reps = -(-D // y.shape[0])
                        y = jnp.concatenate([y[:, 128 * r:128 * (r + 1)] for r in range(reps)], axis=0)[0:D]
                        val = jnp.where(always[0][:, 0:128], val, y)
                    out_buf[u, :, cols] = val.astype(BF16)
                    if j == QT - 1:
                        out_copy(u).start()
                    yield

        def down_step():
            ci, e = divmod(state["down"], 5)
            part = expert_down_step(hidden[ci], ci, e)
            state["y"][e] = part if state["y"][e] is None else state["y"][e] + part
            state["down"] += 1

        def hook(long, pacer=None):
            state["pacer"] = pacer if pacer is not None and pacer.shape[0] * (pacer.shape[1] // 128) >= D else None
            can_down = (state["wd_ready"] and state["down"] < 5 * n_chunks
                        and state["down"] // 5 < len(hidden))
            if can_down and (long or state["up_done"]):
                down_step()
            elif not state["up_done"]:
                if next(up, "done") == "done":
                    state["up_done"] = True
                    hook(long, pacer)
            elif state["down"] == 5 * n_chunks and state["out_ready"]:
                if state["tail"] is None:
                    state["tail"] = finish()
                if pacer is not None and state["pacer"] is not None or state["tail_steps"] < 2:
                    state["tail_steps"] += 1
                    next(state["tail"], None)

        state["out_ready"] = False
        state["tail_steps"] = 0
        steps = [(s, g) for s in range(NSEG) for g in range(NG)]
        last = NSEG - 1

        def last_tile(j):
            cols = slice(128 * j, 128 * (j + 1))
            attn = jnp.dot(wot.load(), ot_buf[:, cols].astype(BF16), preferred_element_type=F32)
            out_buf[last, :, cols] = (base[last, :, cols] + attn).astype(BF16)
            out_tile_copy(j).start()

        fast_scores(0, 0, hook)
        for t, (s, g) in enumerate(steps):
            if t + 1 < len(steps):
                fast_scores(*steps[t + 1], hook)
            if s > 0:
                memory_read(s, g)
                hook(True)
            if t + 1 == len(steps):
                state["pacer"] = None
                while state["tail"] is None or next(state["tail"], "done") != "done":
                    if state["tail"] is None:
                        hook(True)
                fast_values(s, g, last_tile)
            else:
                fast_values(s, g)
            if s == 0:
                transpose_wo(g)
            if s + 1 < NSEG:
                memory_update(s, g)
                hook(True)
            if g == NG - 1 and s < last:
                base[s] = project_out(s)
                if s == 0:
                    cp_wd.wait()
                    state["wd_ready"] = True
                if s == last - 1:
                    state["out_ready"] = True
                hook(True)
        for u in range(NSEG - 1):
            out_copy(u).wait()
        for j in range(QT):
            out_tile_copy(j).wait()

    def slow_segment(s, carry):
        for g in range(NG):
            memory_read(s, g)
        key_i = lax.broadcasted_iota(I32, (L, L), 0)
        qry_i = lax.broadcasted_iota(I32, (L, L), 1)
        r32 = lax.broadcasted_iota(I32, (32, L), 0)
        for g in range(NG):
            gw = GW[g]
            a_g = _group_row_start(g)
            rowg = lax.broadcasted_iota(I32, (gw, L), 0)

            def head(i, c, g=g, gw=gw, a_g=a_g, rowg=rowg):
                h = HPG * g + i
                a = pl.multiple_of((h * DH // 16) * 16, 16)
                off = h * DH - a
                q = qs_buf.load(s, 128 * g, 128 * g + gw).astype(F32)
                qm = jnp.where((rowg >= DH * i) & (rowg < DH * (i + 1)), q, 0.0).astype(BF16)
                st = jnp.dot(k_buf.load(s * NG + g, cols=slice(0, gw)), qm, preferred_element_type=F32)
                st = jnp.where(key_i <= qry_i, st, NEG_BIG)
                p = jnp.exp2(st - jnp.max(st, axis=0, keepdims=True))
                rl = 1.0 / jnp.sum(p, axis=0, keepdims=True)
                o = jnp.dot(vt_buf.load(s, a, 32), p.astype(BF16), preferred_element_type=F32)
                gate = jnp.concatenate([gate_buf[pl.ds(h, 1), :]] * QT, axis=1)
                rden = 1.0 / (num_buf[g, pl.ds(_norm_row(g) + i, 1), :] + 1e-6)
                num = num_buf[g, pl.ds(pl.multiple_of(a - a_g, 16), 32), :]
                val = gate * (num * rden) + (1.0 - gate) * (o * rl)
                keep = (r32 >= off) & (r32 < off + DH)
                pltpu.store(ot_buf.at[pl.ds(a, 32), :], val, mask=keep)
                return c

            lax.fori_loop(0, _heads_in_group(g), head, 0)
        for g in range(NG):
            memory_update(s, g)
        emit(s, project_out(s))
        return carry

    @pl.when(safe)
    def _():
        fast_path()

    @pl.when(jnp.logical_not(safe))
    def _():
        cp_wd.wait()
        for g in range(NG):
            transpose_wo(g)
        expert_scatter(expert_chunk(0, FF))
        lax.fori_loop(0, NSEG, slow_segment, 0)
        for u in range(NSEG):
            out_copy(u).wait()


@jax.jit
def pallas_parallel_sum__memory_aug_infini_attn__moe_arch_mod__prompt_kernel(
    A_x: jax.Array,
    A_wq: jax.Array,
    A_wk: jax.Array,
    A_wv: jax.Array,
    A_wo: jax.Array,
    A_beta: jax.Array,
    B_x: jax.Array,
    B_w_r: jax.Array,
    B_w_gate: jax.Array,
    B_w_up: jax.Array,
    B_w_down: jax.Array,
):
    del B_x
    hbm = pl.BlockSpec(memory_space=pl.ANY)
    scratch = [
        pltpu.VMEM((NSEG, D, L), BF16),
        pltpu.VMEM((D, D), BF16),
        pltpu.VMEM((D, D), BF16),
        pltpu.VMEM((D, D), BF16),
        pltpu.VMEM((D, D), BF16),
        pltpu.VMEM((H,), BF16),
        pltpu.VMEM((D,), BF16),
        pltpu.VMEM((D, FF), BF16),
        pltpu.VMEM((D, FF), BF16),
        pltpu.VMEM((D, FF), BF16),
        pltpu.VMEM((PR // 2, D), U32),
        pltpu.VMEM((PR // 2, D), U32),
        pltpu.VMEM((D // 2, D), U32),
        pltpu.VMEM((D // 2, D), U32),
        pltpu.VMEM((NSEG * D // 2, L), U32),
        pltpu.VMEM((NSEG, D, L), F32),
        pltpu.VMEM((NSEG * PR // 2, L), U32),
        pltpu.VMEM((NSEG * PR // 2, L), U32),
        pltpu.VMEM((NSEG * NG * L // 2, 128), U32),
        pltpu.VMEM((NSEG * PR // 2, L), U32),
        pltpu.VMEM((NSEG * D // 2, L), U32),
        pltpu.VMEM((8, S), F32),
        pltpu.VMEM((H, 128), F32),
        pltpu.VMEM((NG, MROWS, 128), F32),
        pltpu.VMEM((NG, MROWS, L), F32),
        pltpu.VMEM((640, HPG * 128), U32),
        pltpu.VMEM((640, HPG * 128), U32),
        pltpu.VMEM((D, L), F32),
        pltpu.VMEM((NSEG, D, L), BF16),
        pltpu.SemaphoreType.DMA((13,)),
        pltpu.SemaphoreType.DMA((NSEG + QT,)),
    ]
    out_t = pl.pallas_call(
        _kernel,
        out_shape=jax.ShapeDtypeStruct((1, D, S), BF16),
        in_specs=[hbm] * 10,
        out_specs=hbm,
        scratch_shapes=scratch,
        compiler_params=pltpu.CompilerParams(vmem_limit_bytes=128 * 1024 * 1024),
        name="infini_attn_moe",
    )(jnp.transpose(A_x, (0, 2, 1)), A_wq, A_wk, A_wv, A_wo, A_beta, B_w_r, B_w_gate, B_w_up,
      B_w_down.T)
    return jnp.transpose(out_t, (0, 2, 1))
```

```python
import jax
import jax.numpy as jnp
from jax import lax
import jax.experimental.pallas as pl
import jax.experimental.pallas.tpu as pltpu

F32 = jnp.float32
BF16 = jnp.bfloat16
U32 = jnp.uint32
I32 = jnp.int32

S = 2048
D = 576
H = 32
DH = 18
NSEG = 4
L = 512
FF = 4608
HPG = 7
NG = 5
QT = L // 128
GW = (128, 128, 128, 128, 80)
PR = sum(GW)
ROUTER_ROW = 126
MROWS = 144
LOG2E = 1.4426950408889634
QSCALE = (DH ** -0.5) * LOG2E
SAFE_LOG2_RANGE = 60.0
NEG_BIG = -1e30

NT_DIMS = (((1,), (1,)), ((), ()))


def _heads_in_group(g):
    return min(HPG, H - HPG * g)


def _group_row_start(g):
    return (HPG * g * DH // 16) * 16


def _group_rows(g):
    last = (HPG * g + _heads_in_group(g)) * DH
    return -(-(last - _group_row_start(g)) // 16) * 16


def _state_rows(g):
    return MROWS if g == 0 else _group_rows(g)


def _norm_row(g):
    return 128 if g == 0 else 0


def _round_bf16(x):
    return x.astype(BF16).astype(F32)


def _pad_heads_t(w):
    parts = []
    for g in range(NG):
        n = _heads_in_group(g) * DH
        parts.append(w[:, HPG * DH * g:HPG * DH * g + n])
        parts.append(jnp.zeros((D, 128 - n), w.dtype))
    return jnp.concatenate(parts, axis=1).T[0:PR]


def _phi(t):
    return jnp.where(t > 0, t + 1.0, jnp.exp(t))


class _Packed:
    def __init__(self, ref, rows):
        self.ref = ref
        self.rows = rows

    def _slice(self, item, lo, size):
        start = item * (self.rows // 2) + lo // 2
        size = size // 2
        if isinstance(start, int):
            return slice(start, start + size)
        return pl.ds(pl.multiple_of(start, 8), size)

    def load(self, item=0, lo=0, hi=None, cols=slice(None)):
        size = hi if not isinstance(lo, int) else (self.rows if hi is None else hi) - lo
        return pltpu.bitcast(self.ref[self._slice(item, lo, size), cols], BF16)

    def store(self, val, item=0, lo=0, cols=slice(None)):
        self.ref[self._slice(item, lo, val.shape[0]), cols] = pltpu.bitcast(val.astype(BF16), U32)


def _kernel(x_hbm, wq_hbm, wk_hbm, wv_hbm, wo_hbm, beta_hbm, wr_hbm, wg_hbm, wu_hbm, wd_hbm,
            out_hbm,
            x_buf, wq_raw, wk_raw, wv_raw, wo_raw, beta_buf, wr_buf, wg_buf, wu_buf, wd_buf,
            wqt, wkt, wvt, wot, xn_buf, base, qs_buf, pq_buf, k_buf, pk_buf, vt_buf, r_buf,
            gate_buf, mt_buf, num_buf, p_buf0, p_buf1, ot_buf, out_buf, in_sems, out_sems):
    wqt, wkt = _Packed(wqt, PR), _Packed(wkt, PR)
    wvt, wot = _Packed(wvt, D), _Packed(wot, D)
    xn_buf, vt_buf = _Packed(xn_buf, D), _Packed(vt_buf, D)
    qs_buf, pq_buf, pk_buf = _Packed(qs_buf, PR), _Packed(pq_buf, PR), _Packed(pk_buf, PR)
    k_buf = _Packed(k_buf, L)

    def x_copy(c):
        return pltpu.make_async_copy(x_hbm.at[0, :, pl.ds(c * L, L)], x_buf.at[c], in_sems.at[c])

    cp_wv = pltpu.make_async_copy(wv_hbm, wv_raw, in_sems.at[4])
    cp_wq = pltpu.make_async_copy(wq_hbm, wq_raw, in_sems.at[5])
    cp_wk = pltpu.make_async_copy(wk_hbm, wk_raw, in_sems.at[6])
    cp_wo = pltpu.make_async_copy(wo_hbm, wo_raw, in_sems.at[7])
    cp_wg = pltpu.make_async_copy(wg_hbm, wg_buf, in_sems.at[8])
    cp_wu = pltpu.make_async_copy(wu_hbm, wu_buf, in_sems.at[9])
    cp_wd = pltpu.make_async_copy(wd_hbm, wd_buf, in_sems.at[10])
    cp_beta = pltpu.make_async_copy(beta_hbm, beta_buf, in_sems.at[11])
    cp_wr = pltpu.make_async_copy(wr_hbm, wr_buf, in_sems.at[12])

    def out_copy(s):
        cols = pl.ds(pl.multiple_of(s * L, L), L)
        return pltpu.make_async_copy(out_buf.at[s], out_hbm.at[0, :, cols], out_sems.at[s])

    def out_tile_copy(j):
        s = NSEG - 1
        return pltpu.make_async_copy(out_buf.at[s, :, pl.ds(128 * j, 128)],
                                     out_hbm.at[0, :, pl.ds(s * L + 128 * j, 128)], out_sems.at[NSEG + j])


    for cp in (x_copy(0), cp_wv, x_copy(1), cp_wq, cp_wr, x_copy(2), cp_wk, x_copy(3), cp_wo, cp_beta,
               cp_wg, cp_wu, cp_wd):
        cp.start()

    lane128 = lax.broadcasted_iota(I32, (128, 128), 1)
    row128 = lax.broadcasted_iota(I32, (128, 128), 0)
    causal = row128 <= lane128
    r16 = lax.broadcasted_iota(I32, (16, D), 0)

    mt_buf[...] = jnp.zeros(mt_buf.shape, F32)

    always = []

    def pace(x, y):
        return x if y is None else jnp.where(always[0], x, y[0:D])

    def ln_stats(c, y):
        shift = x_buf[c, 0:16, :].astype(F32)[0:1]
        d = pace(x_buf[c].astype(F32), y) - shift
        m1 = jnp.sum(d, axis=0, keepdims=True) * (1.0 / D)
        m2 = jnp.sum(d * d, axis=0, keepdims=True) * (1.0 / D)
        var = jnp.maximum(m2 - m1 * m1, 0.0)
        inv = 1.0 / _round_bf16(jnp.sqrt(_round_bf16(_round_bf16(var) + 1e-5)))
        return _round_bf16(shift + m1), inv

    def ln_apply(c, mean_b, inv):
        x = x_buf[c].astype(F32)
        xn = (x - mean_b) * inv
        xn_buf.store(xn, c)
        base[c] = x + xn

    def project(w_ref, c, split):
        if not split:
            return jnp.dot(w_ref.load(), xn_buf.load(c), preferred_element_type=F32), None
        head = jnp.dot(w_ref.load(cols=slice(0, 256)), xn_buf.load(c, 0, 256), preferred_element_type=F32)
        tail = jnp.dot(w_ref.load(cols=slice(256, D)), xn_buf.load(c, 256, D), preferred_element_type=F32)
        return head + tail, head

    def project_v(c, mid=None):
        vt, head = project(wvt, c, mid is not None)
        if mid is not None:
            mid(head)
        vt_buf.store(vt, c)
        return vt

    def project_q(c, mid=None):
        qt, head = project(wqt, c, mid is not None)
        if mid is not None:
            mid(head)
        qsc = qt * QSCALE
        qs_buf.store(qsc, c)
        pq_buf.store(_phi(qt), c)
        r_buf[:, c * L:(c + 1) * L] = qt[120:128]
        mag = jnp.abs(qsc)
        r8 = lax.broadcasted_iota(I32, (8, L), 0)
        mag = jnp.concatenate([mag[0:120], jnp.where(r8 == ROUTER_ROW - 120, 0.0, mag[120:128]), mag[128:]], axis=0)
        return qt, jnp.max(mag.reshape(PR // 8, 8, L), axis=0)

    def project_k(c, mid=None, keep=False):
        kt, head = project(wkt, c, mid is not None)
        if mid is not None:
            mid(head)
        pk_buf.store(_phi(kt), c)
        for g in range(NG):
            ktg = kt[128 * g:128 * g + GW[g]]
            if GW[g] < 128:
                ktg = jnp.concatenate([ktg, jnp.zeros((128 - GW[g], L), F32)], axis=0)
            k_buf.store(ktg.T, c * NG + g)
        top = jnp.max(jnp.abs(kt).reshape(PR // 8, 8, L), axis=0)
        return (kt, top) if keep else top

    x_copy(0).wait()
    stats = ln_stats(0, None)
    always.append(jnp.logical_not(jnp.abs(stats[0]) < 0.0))
    ln_apply(0, *stats)
    cp_wv.wait()
    wvt.store(wv_raw[...].T)
    project_v(0)
    x_copy(1).wait()
    cp_wq.wait()
    cp_wr.wait()
    ln_apply(1, *ln_stats(1, None))

    def paced_weight(w_ref, y):
        w = w_ref[...].astype(F32)
        return jnp.concatenate([jnp.where(always[0], w[:, 0:L], y[0:D]), w[:, L:D]], axis=1)

    def prep_wq(y):
        wq_t = _pad_heads_t(paced_weight(wq_raw, y))
        wr_row = wr_buf[...].reshape(1, D).astype(F32)
        pr_row = lax.broadcasted_iota(I32, (8, D), 0)
        wq_t = jnp.concatenate(
            [wq_t[0:120], jnp.where(pr_row == ROUTER_ROW - 120, wr_row, wq_t[120:128]), wq_t[128:]], axis=0)
        wqt.store(wq_t)

    project_v(1, prep_wq)
    cp_wk.wait()
    x_copy(2).wait()
    x_copy(3).wait()

    def prep_wk(y):
        wkt.store(_pad_heads_t(paced_weight(wk_raw, y)))

    def route():
        r = _round_bf16(r_buf[ROUTER_ROW - 120:ROUTER_ROW - 119, :])
        tok = lax.broadcasted_iota(I32, (1, S), 1).astype(F32)
        m1 = jnp.max(r)
        i1 = jnp.min(jnp.where(r == m1, tok, float(S)))
        r_rest = jnp.where(tok == i1, -jnp.inf, r)
        m2 = jnp.max(r_rest)
        i2 = jnp.min(jnp.where(r_rest == m2, tok, float(S)))
        i1 = jnp.clip(i1.astype(I32), 0, S - 1)
        i2 = jnp.clip(i2.astype(I32), 0, S - 1)
        return m1, m2, i1, i2

    qt, aq = project_q(0, prep_wk)
    qt, a = project_q(1)
    aq = jnp.maximum(aq, a)
    stats = ln_stats(2, qt)
    ak = project_k(0)
    ln_apply(2, *stats)
    kt, a = project_k(1, keep=True)
    ak = jnp.maximum(ak, a)
    stats = ln_stats(3, kt)
    project_v(2)
    ln_apply(3, *stats)
    qt, a = project_q(2)
    aq = jnp.maximum(aq, a)
    ak = jnp.maximum(ak, project_k(2))
    qt, a = project_q(3)
    aq = jnp.maximum(aq, a)
    m1, m2, i1, i2 = route()
    ak = jnp.maximum(ak, project_k(3))
    project_v(3)

    logit_bound = jnp.max(aq) * jnp.max(ak) * (DH * 1.02)
    safe = logit_bound <= SAFE_LOG2_RANGE

    sel_row = lax.broadcasted_iota(I32, (16, 128), 0)
    sel_lane = lax.broadcasted_iota(I32, (16, 128), 1)

    def token_tile(i):
        return i // L, pl.ds(pl.multiple_of(((i % L) // 128) * 128, 128), 128)

    def pick(i, slot):
        seg, cols = token_tile(i)
        onehot = jnp.where((sel_row == slot) & (sel_lane == i % 128), 1.0, 0.0).astype(BF16)
        return lax.dot_general(onehot, xn_buf.load(seg, cols=cols), NT_DIMS, preferred_element_type=F32)

    def routed_rows():
        return (pick(i1, 0) + pick(i2, 1)).astype(BF16)

    cp_wo.wait()
    cp_beta.wait()
    cp_wg.wait()
    cp_wu.wait()

    beta_row = beta_buf[...].reshape(1, H).astype(F32)
    beta_row = jnp.concatenate([beta_row, jnp.zeros((1, 128 - H), F32)], axis=1)
    h_row = lax.broadcasted_iota(I32, (H, 128), 0)
    h_lane = lax.broadcasted_iota(I32, (H, 128), 1)
    beta_col = jnp.sum(jnp.where(h_row == h_lane, beta_row, 0.0), axis=1, keepdims=True)
    gate_buf[...] = jnp.broadcast_to(jax.nn.sigmoid(beta_col), (H, 128))


    def expert_chunk(lo, hi):
        xs = routed_rows()
        hg = jnp.dot(xs, wg_buf[:, lo:hi], preferred_element_type=F32)
        hu = jnp.dot(xs, wu_buf[:, lo:hi], preferred_element_type=F32)
        hh = (jax.nn.silu(hg) * hu).astype(BF16)
        return lax.dot_general(hh, wd_buf[:, lo:hi], NT_DIMS, preferred_element_type=F32)

    def expert_up_stream(hidden):
        kmain = 512
        xs = routed_rows()
        yield
        for c0 in range(0, FF, 512):
            rem = []
            for w_ref in (wg_buf, wu_buf):
                rem.append(jnp.dot(xs[:, kmain:D], w_ref[kmain:D, c0:c0 + 512], preferred_element_type=F32))
                yield
            hs = []
            for f0 in range(c0, c0 + 512, 128):
                pre = []
                for w_ref, r in zip((wg_buf, wu_buf), rem):
                    pre.append(jnp.dot(xs[:, 0:kmain], w_ref[0:kmain, f0:f0 + 128], preferred_element_type=F32)
                               + r[:, f0 - c0:f0 - c0 + 128])
                    if len(pre) == 2:
                        hs.append(jax.nn.silu(pre[0]) * pre[1])
                        if len(hs) == 4:
                            hidden.append(jnp.concatenate(hs, axis=1).astype(BF16))
                    yield

    def expert_down_step(hh, ci, e):
        e_hi = min(128 * (e + 1), D)
        return lax.dot_general(hh, wd_buf[128 * e:e_hi, 512 * ci:512 * (ci + 1)], NT_DIMS,
                               preferred_element_type=F32)

    def expert_scatter_parts(y):
        y = y * jax.nn.sigmoid(jnp.where(r16 == 0, m1, m2))
        yt = jnp.concatenate([y, jnp.zeros((128 - 16, D), F32)], axis=0).T
        lane_d = lax.broadcasted_iota(I32, (D, 128), 1)
        for slot, i in ((0, i1), (1, i2)):
            seg, cols = token_tile(i)
            col = jnp.sum(jnp.where(lane_d == slot, yt, 0.0), axis=1, keepdims=True)
            base[seg, :, cols] = base[seg, :, cols] + jnp.where(lane_d == i % 128, col, 0.0)
            yield

    def expert_scatter(y):
        for _ in expert_scatter_parts(y):
            pass

    def memory_read(s, g):
        sr = _state_rows(g)
        gw = GW[g]
        num_buf[g, 0:sr, :] = jnp.dot(mt_buf[g, 0:sr, 0:gw].astype(BF16), pq_buf.load(s, 128 * g, 128 * g + gw),
                                      preferred_element_type=F32)

    def memory_update(s, g):
        rg = _group_rows(g)
        a_g = _group_row_start(g)
        gw = GW[g]
        ones_row = 126 if g == 0 else 0
        lhs = jnp.where(lax.broadcasted_iota(I32, (rg, L), 0) == ones_row, 1.0,
                        vt_buf.load(s, a_g, a_g + rg).astype(F32)).astype(BF16)
        upd = lax.dot_general(lhs, pk_buf.load(s, 128 * g, 128 * g + gw), NT_DIMS,
                              preferred_element_type=F32)
        er = lax.broadcasted_iota(I32, (rg, gw), 0) + (a_g - HPG * DH * g)
        el = lax.broadcasted_iota(I32, (rg, gw), 1)
        same_head = None
        for i in range(_heads_in_group(g)):
            t = ((er >= DH * i) & (er < DH * (i + 1)) & (el >= DH * i) & (el < DH * (i + 1)))
            same_head = t if same_head is None else (same_head | t)
        mt_buf[g, 0:rg, 0:gw] = mt_buf[g, 0:rg, 0:gw] + jnp.where(same_head, upd, 0.0)
        zr = lax.broadcasted_iota(I32, (8, gw), 0)
        zl = lax.broadcasted_iota(I32, (8, gw), 1)
        zmask = (zl >= zr * DH) & (zl < zr * DH + DH) & (zr < _heads_in_group(g))
        zs = upd[ones_row:ones_row + 1]
        z0 = _norm_row(g)
        mt_buf[g, z0:z0 + 8, 0:gw] = mt_buf[g, z0:z0 + 8, 0:gw] + jnp.where(zmask, zs, 0.0)

    def transpose_wo(g):
        hi = min(128 * (g + 1), D)
        wot.store(wo_raw[:, 128 * g:hi].T, lo=128 * g)

    def project_out(s):
        attn = jnp.dot(wot.load(), ot_buf[...].astype(BF16), preferred_element_type=F32)
        return base[s] + attn

    def emit(s, val):
        out_buf[s] = val.astype(BF16)
        out_copy(s).start()

    zero = lax.shift_right_logical(i1, 16)

    def prow(start, size):
        return pl.ds(pl.multiple_of(zero + start, 8), size)

    P_OFFS = (0, 128, 384, 768)

    def fast_scores(s, g, hook):
        nh = _heads_in_group(g)
        gw = GW[g]
        pb = (p_buf0, p_buf1)[(s * NG + g) % 2]
        rowg = lax.broadcasted_iota(I32, (gw, 128), 0)
        for j in range(QT - 1, -1, -1):
            n = 128 * (j + 1)
            q = qs_buf.load(s, 128 * g, 128 * g + gw, slice(128 * j, 128 * (j + 1))).astype(F32)
            for h0, h1 in ((0, 4), (4, nh)):
                if h1 <= h0:
                    continue
                qm = jnp.concatenate(
                    [jnp.where((rowg >= DH * i) & (rowg < DH * (i + 1)), q, 0.0) for i in range(h0, h1)],
                    axis=1).astype(BF16)
                st = jnp.dot(k_buf.load(s * NG + g, 0, n, slice(0, gw)), qm, preferred_element_type=F32)
                p = jnp.exp2(st)
                causal_w = jnp.concatenate([causal] * (h1 - h0), axis=1)
                p_diag = jnp.where(causal_w, p[n - 128:], 0.0)
                p = jnp.concatenate([p[:n - 128], p_diag], axis=0) if j > 0 else p_diag
                pb[P_OFFS[j] // 2:(P_OFFS[j] + n) // 2, h0 * 128:h1 * 128] = pltpu.bitcast(p.astype(BF16), U32)
                hook(j >= 2, p)

    def fast_values(s, g, after_tile=None):
        nh = _heads_in_group(g)
        a_g = _group_row_start(g)
        pb = (p_buf0, p_buf1)[(s * NG + g) % 2]
        for j in range(QT - 1, -1, -1):
            n = 128 * (j + 1)
            cols = slice(128 * j, 128 * (j + 1))
            for i in range(nh):
                h = HPG * g + i
                a = (h * DH // 16) * 16
                off = h * DH - a
                p = pltpu.bitcast(pb[prow(P_OFFS[j] // 2, n // 2), 128 * i:128 * (i + 1)], BF16)
                ones_row = 0 if off > 0 else 31
                r32n = lax.broadcasted_iota(I32, (32, n), 0)
                lhs = jnp.where(r32n == ones_row, 1.0, vt_buf.load(s, a, a + 32, slice(0, n)).astype(F32)).astype(BF16)
                o = jnp.dot(lhs, p, preferred_element_type=F32)
                lo = (off // 8) * 8
                hi = -(-(off + DH) // 8) * 8
                gate = gate_buf[h:h + 1, :]
                rl = 1.0 / o[ones_row:ones_row + 1]
                val = (1.0 - gate) * (o[lo:hi] * rl)
                if s > 0:
                    z = _norm_row(g) + i
                    rden = 1.0 / (num_buf[g, z:z + 1, cols] + 1e-6)
                    num = num_buf[g, a - a_g + lo:a - a_g + hi, cols]
                    val = gate * (num * rden) + val
                ot_buf[a + off:a + off + DH, cols] = val[off - lo:off - lo + DH]
            if after_tile is not None:
                after_tile(j)

    def fast_path():
        hidden = []
        up = expert_up_stream(hidden)
        n_chunks = FF // 512
        state = dict(down=0, wd_ready=False, up_done=False, y=[None] * 5, tail=None)

        def finish():
            yield from expert_scatter_parts(jnp.concatenate(state["y"], axis=1))
            for u in range(NSEG - 1):
                for j in range(QT):
                    cols = slice(128 * j, 128 * (j + 1))
                    val = base[u, :, cols]
                    y = state["pacer"]
                    if y is not None:
                        reps = -(-D // y.shape[0])
                        y = jnp.concatenate([y[:, 128 * r:128 * (r + 1)] for r in range(reps)], axis=0)[0:D]
                        val = jnp.where(always[0][:, 0:128], val, y)
                    out_buf[u, :, cols] = val.astype(BF16)
                    if j == QT - 1:
                        out_copy(u).start()
                    yield

        def down_step():
            ci, e = divmod(state["down"], 5)
            part = expert_down_step(hidden[ci], ci, e)
            state["y"][e] = part if state["y"][e] is None else state["y"][e] + part
            state["down"] += 1

        def hook(long, pacer=None):
            state["pacer"] = pacer if pacer is not None and pacer.shape[0] * (pacer.shape[1] // 128) >= D else None
            can_down = (state["wd_ready"] and state["down"] < 5 * n_chunks
                        and state["down"] // 5 < len(hidden))
            if can_down and (long or state["up_done"]):
                down_step()
            elif not state["up_done"]:
                if next(up, "done") == "done":
                    state["up_done"] = True
                    hook(long, pacer)
            elif state["down"] == 5 * n_chunks and state["out_ready"]:
                if state["tail"] is None:
                    state["tail"] = finish()
                if pacer is not None and state["pacer"] is not None or state["tail_steps"] < 2:
                    state["tail_steps"] += 1
                    next(state["tail"], None)

        state["out_ready"] = False
        state["tail_steps"] = 0
        steps = [(s, g) for s in range(NSEG) for g in range(NG)]
        last = NSEG - 1

        def last_tile(j):
            cols = slice(128 * j, 128 * (j + 1))
            attn = jnp.dot(wot.load(), ot_buf[:, cols].astype(BF16), preferred_element_type=F32)
            out_buf[last, :, cols] = (base[last, :, cols] + attn).astype(BF16)
            out_tile_copy(j).start()

        fast_scores(0, 0, hook)
        for t, (s, g) in enumerate(steps):
            if t + 1 < len(steps):
                fast_scores(*steps[t + 1], hook)
            if s > 0:
                memory_read(s, g)
                hook(True)
            if t + 1 == len(steps):
                state["pacer"] = None
                while state["tail"] is None or next(state["tail"], "done") != "done":
                    if state["tail"] is None:
                        hook(True)
                pending = []

                def after_tile(j):
                    if pending:
                        last_tile(pending.pop())
                    pending.append(j)

                fast_values(s, g, after_tile)
                last_tile(pending.pop())
            else:
                fast_values(s, g)
            if s == 0:
                transpose_wo(g)
            if s + 1 < NSEG:
                memory_update(s, g)
                hook(True)
            if g == NG - 1 and s < last:
                base[s] = project_out(s)
                if s == 0:
                    cp_wd.wait()
                    state["wd_ready"] = True
                if s == last - 1:
                    state["out_ready"] = True
                hook(True)
        for u in range(NSEG - 1):
            out_copy(u).wait()
        for j in range(QT):
            out_tile_copy(j).wait()

    def slow_segment(s, carry):
        for g in range(NG):
            memory_read(s, g)
        key_i = lax.broadcasted_iota(I32, (L, L), 0)
        qry_i = lax.broadcasted_iota(I32, (L, L), 1)
        r32 = lax.broadcasted_iota(I32, (32, L), 0)
        for g in range(NG):
            gw = GW[g]
            a_g = _group_row_start(g)
            rowg = lax.broadcasted_iota(I32, (gw, L), 0)

            def head(i, c, g=g, gw=gw, a_g=a_g, rowg=rowg):
                h = HPG * g + i
                a = pl.multiple_of((h * DH // 16) * 16, 16)
                off = h * DH - a
                q = qs_buf.load(s, 128 * g, 128 * g + gw).astype(F32)
                qm = jnp.where((rowg >= DH * i) & (rowg < DH * (i + 1)), q, 0.0).astype(BF16)
                st = jnp.dot(k_buf.load(s * NG + g, cols=slice(0, gw)), qm, preferred_element_type=F32)
                st = jnp.where(key_i <= qry_i, st, NEG_BIG)
                p = jnp.exp2(st - jnp.max(st, axis=0, keepdims=True))
                rl = 1.0 / jnp.sum(p, axis=0, keepdims=True)
                o = jnp.dot(vt_buf.load(s, a, 32), p.astype(BF16), preferred_element_type=F32)
                gate = jnp.concatenate([gate_buf[pl.ds(h, 1), :]] * QT, axis=1)
                rden = 1.0 / (num_buf[g, pl.ds(_norm_row(g) + i, 1), :] + 1e-6)
                num = num_buf[g, pl.ds(pl.multiple_of(a - a_g, 16), 32), :]
                val = gate * (num * rden) + (1.0 - gate) * (o * rl)
                keep = (r32 >= off) & (r32 < off + DH)
                pltpu.store(ot_buf.at[pl.ds(a, 32), :], val, mask=keep)
                return c

            lax.fori_loop(0, _heads_in_group(g), head, 0)
        for g in range(NG):
            memory_update(s, g)
        emit(s, project_out(s))
        return carry

    @pl.when(safe)
    def _():
        fast_path()

    @pl.when(jnp.logical_not(safe))
    def _():
        cp_wd.wait()
        for g in range(NG):
            transpose_wo(g)
        expert_scatter(expert_chunk(0, FF))
        lax.fori_loop(0, NSEG, slow_segment, 0)
        for u in range(NSEG):
            out_copy(u).wait()


@jax.jit
def pallas_parallel_sum__memory_aug_infini_attn__moe_arch_mod__prompt_kernel(
    A_x: jax.Array,
    A_wq: jax.Array,
    A_wk: jax.Array,
    A_wv: jax.Array,
    A_wo: jax.Array,
    A_beta: jax.Array,
    B_x: jax.Array,
    B_w_r: jax.Array,
    B_w_gate: jax.Array,
    B_w_up: jax.Array,
    B_w_down: jax.Array,
):
    del B_x
    hbm = pl.BlockSpec(memory_space=pl.ANY)
    scratch = [
        pltpu.VMEM((NSEG, D, L), BF16),
        pltpu.VMEM((D, D), BF16),
        pltpu.VMEM((D, D), BF16),
        pltpu.VMEM((D, D), BF16),
        pltpu.VMEM((D, D), BF16),
        pltpu.VMEM((H,), BF16),
        pltpu.VMEM((D,), BF16),
        pltpu.VMEM((D, FF), BF16),
        pltpu.VMEM((D, FF), BF16),
        pltpu.VMEM((D, FF), BF16),
        pltpu.VMEM((PR // 2, D), U32),
        pltpu.VMEM((PR // 2, D), U32),
        pltpu.VMEM((D // 2, D), U32),
        pltpu.VMEM((D // 2, D), U32),
        pltpu.VMEM((NSEG * D // 2, L), U32),
        pltpu.VMEM((NSEG, D, L), F32),
        pltpu.VMEM((NSEG * PR // 2, L), U32),
        pltpu.VMEM((NSEG * PR // 2, L), U32),
        pltpu.VMEM((NSEG * NG * L // 2, 128), U32),
        pltpu.VMEM((NSEG * PR // 2, L), U32),
        pltpu.VMEM((NSEG * D // 2, L), U32),
        pltpu.VMEM((8, S), F32),
        pltpu.VMEM((H, 128), F32),
        pltpu.VMEM((NG, MROWS, 128), F32),
        pltpu.VMEM((NG, MROWS, L), F32),
        pltpu.VMEM((640, HPG * 128), U32),
        pltpu.VMEM((640, HPG * 128), U32),
        pltpu.VMEM((D, L), F32),
        pltpu.VMEM((NSEG, D, L), BF16),
        pltpu.SemaphoreType.DMA((13,)),
        pltpu.SemaphoreType.DMA((NSEG + QT,)),
    ]
    out_t = pl.pallas_call(
        _kernel,
        out_shape=jax.ShapeDtypeStruct((1, D, S), BF16),
        in_specs=[hbm] * 10,
        out_specs=hbm,
        scratch_shapes=scratch,
        compiler_params=pltpu.CompilerParams(vmem_limit_bytes=128 * 1024 * 1024),
        name="infini_attn_moe",
    )(jnp.transpose(A_x, (0, 2, 1)), A_wq, A_wk, A_wv, A_wo, A_beta, B_w_r, B_w_gate, B_w_up,
      B_w_down.T)
    return jnp.transpose(out_t, (0, 2, 1))
```

```python
import jax
import jax.numpy as jnp
from jax import lax
import jax.experimental.pallas as pl
import jax.experimental.pallas.tpu as pltpu

F32 = jnp.float32
BF16 = jnp.bfloat16
U32 = jnp.uint32
I32 = jnp.int32

S = 2048
D = 576
H = 32
DH = 18
NSEG = 4
L = 512
FF = 4608
HPG = 7
NG = 5
QT = L // 128
GW = (128, 128, 128, 128, 80)
PR = sum(GW)
ROUTER_ROW = 126
MROWS = 144
LOG2E = 1.4426950408889634
QSCALE = (DH ** -0.5) * LOG2E
SAFE_LOG2_RANGE = 60.0
NEG_BIG = -1e30

NT_DIMS = (((1,), (1,)), ((), ()))


def _heads_in_group(g):
    return min(HPG, H - HPG * g)


def _group_row_start(g):
    return (HPG * g * DH // 16) * 16


def _group_rows(g):
    last = (HPG * g + _heads_in_group(g)) * DH
    return -(-(last - _group_row_start(g)) // 16) * 16


def _state_rows(g):
    return MROWS if g == 0 else _group_rows(g)


def _norm_row(g):
    return 128 if g == 0 else 0


def _round_bf16(x):
    return x.astype(BF16).astype(F32)


def _pad_heads_t(w):
    parts = []
    for g in range(NG):
        n = _heads_in_group(g) * DH
        parts.append(w[:, HPG * DH * g:HPG * DH * g + n])
        parts.append(jnp.zeros((D, 128 - n), w.dtype))
    return jnp.concatenate(parts, axis=1).T[0:PR]


def _phi(t):
    return jnp.where(t > 0, t + 1.0, jnp.exp(t))


class _Packed:
    def __init__(self, ref, rows):
        self.ref = ref
        self.rows = rows

    def _slice(self, item, lo, size):
        start = item * (self.rows // 2) + lo // 2
        size = size // 2
        if isinstance(start, int):
            return slice(start, start + size)
        return pl.ds(pl.multiple_of(start, 8), size)

    def load(self, item=0, lo=0, hi=None, cols=slice(None)):
        size = hi if not isinstance(lo, int) else (self.rows if hi is None else hi) - lo
        return pltpu.bitcast(self.ref[self._slice(item, lo, size), cols], BF16)

    def store(self, val, item=0, lo=0, cols=slice(None)):
        self.ref[self._slice(item, lo, val.shape[0]), cols] = pltpu.bitcast(val.astype(BF16), U32)


def _kernel(x_hbm, wq_hbm, wk_hbm, wv_hbm, wo_hbm, beta_hbm, wr_hbm, wg_hbm, wu_hbm, wd_hbm,
            out_hbm,
            x_buf, wq_raw, wk_raw, wv_raw, wo_raw, beta_buf, wr_buf, wg_buf, wu_buf, wd_buf,
            wqt, wkt, wvt, wot, xn_buf, base, qs_buf, pq_buf, k_buf, pk_buf, vt_buf, r_buf,
            gate_buf, mt_buf, num_buf, p_buf0, p_buf1, ot_buf, out_buf, in_sems, out_sems):
    wqt, wkt = _Packed(wqt, PR), _Packed(wkt, PR)
    wvt, wot = _Packed(wvt, D), _Packed(wot, D)
    xn_buf, vt_buf = _Packed(xn_buf, D), _Packed(vt_buf, D)
    qs_buf, pq_buf, pk_buf = _Packed(qs_buf, PR), _Packed(pq_buf, PR), _Packed(pk_buf, PR)
    k_buf = _Packed(k_buf, L)

    def x_copy(c):
        return pltpu.make_async_copy(x_hbm.at[0, :, pl.ds(c * L, L)], x_buf.at[c], in_sems.at[c])

    cp_wv = pltpu.make_async_copy(wv_hbm, wv_raw, in_sems.at[4])
    cp_wq = pltpu.make_async_copy(wq_hbm, wq_raw, in_sems.at[5])
    cp_wk = pltpu.make_async_copy(wk_hbm, wk_raw, in_sems.at[6])
    cp_wo = pltpu.make_async_copy(wo_hbm, wo_raw, in_sems.at[7])
    cp_wg = pltpu.make_async_copy(wg_hbm, wg_buf, in_sems.at[8])
    cp_wu = pltpu.make_async_copy(wu_hbm, wu_buf, in_sems.at[9])
    cp_wd = pltpu.make_async_copy(wd_hbm, wd_buf, in_sems.at[10])
    cp_beta = pltpu.make_async_copy(beta_hbm, beta_buf, in_sems.at[11])
    cp_wr = pltpu.make_async_copy(wr_hbm, wr_buf, in_sems.at[12])

    def out_copy(s):
        cols = pl.ds(pl.multiple_of(s * L, L), L)
        return pltpu.make_async_copy(out_buf.at[s], out_hbm.at[0, :, cols], out_sems.at[s])

    def out_tile_copy(j):
        s = NSEG - 1
        return pltpu.make_async_copy(out_buf.at[s, :, pl.ds(128 * j, 128)],
                                     out_hbm.at[0, :, pl.ds(s * L + 128 * j, 128)], out_sems.at[NSEG + j])


    for cp in (x_copy(0), cp_wv, x_copy(1), cp_wq, cp_wr, cp_beta, x_copy(2), cp_wk, x_copy(3), cp_wo,
               cp_wg, cp_wu, cp_wd):
        cp.start()

    lane128 = lax.broadcasted_iota(I32, (128, 128), 1)
    row128 = lax.broadcasted_iota(I32, (128, 128), 0)
    causal = row128 <= lane128
    r16 = lax.broadcasted_iota(I32, (16, D), 0)

    mt_buf[...] = jnp.zeros(mt_buf.shape, F32)

    always = []

    def pace(x, y):
        return x if y is None else jnp.where(always[0], x, y[0:D])

    def ln_stats(c, y):
        shift = x_buf[c, 0:16, :].astype(F32)[0:1]
        d = pace(x_buf[c].astype(F32), y) - shift
        m1 = jnp.sum(d, axis=0, keepdims=True) * (1.0 / D)
        m2 = jnp.sum(d * d, axis=0, keepdims=True) * (1.0 / D)
        var = jnp.maximum(m2 - m1 * m1, 0.0)
        inv = 1.0 / _round_bf16(jnp.sqrt(_round_bf16(_round_bf16(var) + 1e-5)))
        return _round_bf16(shift + m1), inv

    def ln_apply(c, mean_b, inv):
        x = x_buf[c].astype(F32)
        xn = (x - mean_b) * inv
        xn_buf.store(xn, c)
        if c == NSEG - 1:
            base[c] = jnp.zeros((D, L), F32)

    def project(w_ref, c, split):
        if not split:
            return jnp.dot(w_ref.load(), xn_buf.load(c), preferred_element_type=F32), None
        head = jnp.dot(w_ref.load(cols=slice(0, 256)), xn_buf.load(c, 0, 256), preferred_element_type=F32)
        tail = jnp.dot(w_ref.load(cols=slice(256, D)), xn_buf.load(c, 256, D), preferred_element_type=F32)
        return head + tail, head

    def project_v(c, mid=None):
        vt, head = project(wvt, c, mid is not None)
        if mid is not None:
            mid(head)
        vt_buf.store(vt, c)
        return vt

    def project_q(c, mid=None):
        qt, head = project(wqt, c, mid is not None)
        if mid is not None:
            mid(head)
        qsc = qt * QSCALE
        qs_buf.store(qsc, c)
        pq_buf.store(_phi(qt), c)
        r_buf[:, c * L:(c + 1) * L] = qt[120:128]
        mag = jnp.abs(qsc)
        r8 = lax.broadcasted_iota(I32, (8, L), 0)
        mag = jnp.concatenate([mag[0:120], jnp.where(r8 == ROUTER_ROW - 120, 0.0, mag[120:128]), mag[128:]], axis=0)
        return qt, jnp.max(mag.reshape(PR // 8, 8, L), axis=0)

    def project_k(c, mid=None, keep=False):
        kt, head = project(wkt, c, mid is not None)
        if mid is not None:
            mid(head)
        pk_buf.store(_phi(kt), c)
        for g in range(NG):
            ktg = kt[128 * g:128 * g + GW[g]]
            if GW[g] < 128:
                ktg = jnp.concatenate([ktg, jnp.zeros((128 - GW[g], L), F32)], axis=0)
            k_buf.store(ktg.T, c * NG + g)
        top = jnp.max(jnp.abs(kt).reshape(PR // 8, 8, L), axis=0)
        return (kt, top) if keep else top

    x_copy(0).wait()
    stats = ln_stats(0, None)
    always.append(jnp.logical_not(jnp.abs(stats[0]) < 0.0))
    ln_apply(0, *stats)
    cp_wv.wait()
    wvt.store(wv_raw[...].T)
    project_v(0)
    x_copy(1).wait()
    cp_wq.wait()
    cp_wr.wait()
    ln_apply(1, *ln_stats(1, None))

    def paced_weight(w_ref, y):
        w = w_ref[...].astype(F32)
        return jnp.concatenate([jnp.where(always[0], w[:, 0:L], y[0:D]), w[:, L:D]], axis=1)

    def prep_wq(y):
        wq_t = _pad_heads_t(paced_weight(wq_raw, y))
        wr_row = wr_buf[...].reshape(1, D).astype(F32)
        pr_row = lax.broadcasted_iota(I32, (8, D), 0)
        wq_t = jnp.concatenate(
            [wq_t[0:120], jnp.where(pr_row == ROUTER_ROW - 120, wr_row, wq_t[120:128]), wq_t[128:]], axis=0)
        wqt.store(wq_t)

    project_v(1, prep_wq)
    cp_wk.wait()
    cp_beta.wait()
    x_copy(2).wait()
    x_copy(3).wait()

    beta_row = beta_buf[...].reshape(1, H).astype(F32)
    beta_row = jnp.concatenate([beta_row, jnp.zeros((1, 128 - H), F32)], axis=1)
    h_row = lax.broadcasted_iota(I32, (H, 128), 0)
    h_lane = lax.broadcasted_iota(I32, (H, 128), 1)
    beta_col = jnp.sum(jnp.where(h_row == h_lane, beta_row, 0.0), axis=1, keepdims=True)
    gate_buf[...] = jnp.broadcast_to(jax.nn.sigmoid(beta_col), (H, 128))

    def prep_wk(y):
        wkt.store(_pad_heads_t(paced_weight(wk_raw, y)))

    def route():
        r = _round_bf16(r_buf[ROUTER_ROW - 120:ROUTER_ROW - 119, :])
        tok = lax.broadcasted_iota(I32, (1, S), 1).astype(F32)
        m1 = jnp.max(r)
        i1 = jnp.min(jnp.where(r == m1, tok, float(S)))
        r_rest = jnp.where(tok == i1, -jnp.inf, r)
        m2 = jnp.max(r_rest)
        i2 = jnp.min(jnp.where(r_rest == m2, tok, float(S)))
        i1 = jnp.clip(i1.astype(I32), 0, S - 1)
        i2 = jnp.clip(i2.astype(I32), 0, S - 1)
        return m1, m2, i1, i2

    qt, aq = project_q(0, prep_wk)
    qt, a = project_q(1)
    aq = jnp.maximum(aq, a)
    stats = ln_stats(2, qt)
    ak = project_k(0)
    ln_apply(2, *stats)
    kt, a = project_k(1, keep=True)
    ak = jnp.maximum(ak, a)
    stats = ln_stats(3, kt)
    project_v(2)
    ln_apply(3, *stats)
    qt, a = project_q(2)
    aq = jnp.maximum(aq, a)
    ak = jnp.maximum(ak, project_k(2))
    qt, a = project_q(3)
    aq = jnp.maximum(aq, a)
    m1, m2, i1, i2 = route()
    ak = jnp.maximum(ak, project_k(3))
    project_v(3)

    logit_bound = jnp.max(aq) * jnp.max(ak) * (DH * 1.02)
    safe = logit_bound <= SAFE_LOG2_RANGE

    sel_row = lax.broadcasted_iota(I32, (16, 128), 0)
    sel_lane = lax.broadcasted_iota(I32, (16, 128), 1)

    def token_tile(i):
        return i // L, pl.ds(pl.multiple_of(((i % L) // 128) * 128, 128), 128)

    def pick(i, slot):
        seg, cols = token_tile(i)
        onehot = jnp.where((sel_row == slot) & (sel_lane == i % 128), 1.0, 0.0).astype(BF16)
        return lax.dot_general(onehot, xn_buf.load(seg, cols=cols), NT_DIMS, preferred_element_type=F32)

    def routed_rows():
        return (pick(i1, 0) + pick(i2, 1)).astype(BF16)

    cp_wo.wait()
    cp_wg.wait()
    cp_wu.wait()


    def expert_chunk(lo, hi):
        xs = routed_rows()
        hg = jnp.dot(xs, wg_buf[:, lo:hi], preferred_element_type=F32)
        hu = jnp.dot(xs, wu_buf[:, lo:hi], preferred_element_type=F32)
        hh = (jax.nn.silu(hg) * hu).astype(BF16)
        return lax.dot_general(hh, wd_buf[:, lo:hi], NT_DIMS, preferred_element_type=F32)

    def expert_up_stream(hidden):
        kmain = 512
        xs = routed_rows()
        yield
        for c0 in range(0, FF, 512):
            rem = []
            for w_ref in (wg_buf, wu_buf):
                rem.append(jnp.dot(xs[:, kmain:D], w_ref[kmain:D, c0:c0 + 512], preferred_element_type=F32))
                yield
            hs = []
            for f0 in range(c0, c0 + 512, 128):
                pre = []
                for w_ref, r in zip((wg_buf, wu_buf), rem):
                    pre.append(jnp.dot(xs[:, 0:kmain], w_ref[0:kmain, f0:f0 + 128], preferred_element_type=F32)
                               + r[:, f0 - c0:f0 - c0 + 128])
                    if len(pre) == 2:
                        hs.append(jax.nn.silu(pre[0]) * pre[1])
                        if len(hs) == 4:
                            hidden.append(jnp.concatenate(hs, axis=1).astype(BF16))
                    yield

    def expert_down_step(hh, ci, e):
        e_hi = min(128 * (e + 1), D)
        return lax.dot_general(hh, wd_buf[128 * e:e_hi, 512 * ci:512 * (ci + 1)], NT_DIMS,
                               preferred_element_type=F32)

    def expert_scatter_parts(y):
        y = y * jax.nn.sigmoid(jnp.where(r16 == 0, m1, m2))
        yt = jnp.concatenate([y, jnp.zeros((128 - 16, D), F32)], axis=0).T
        lane_d = lax.broadcasted_iota(I32, (D, 128), 1)
        for slot, i in ((0, i1), (1, i2)):
            seg, cols = token_tile(i)
            col = jnp.sum(jnp.where(lane_d == slot, yt, 0.0), axis=1, keepdims=True)
            base[seg, :, cols] = base[seg, :, cols] + jnp.where(lane_d == i % 128, col, 0.0)
            yield

    def expert_scatter(y):
        for _ in expert_scatter_parts(y):
            pass

    def memory_read(s, g):
        sr = _state_rows(g)
        gw = GW[g]
        num_buf[g, 0:sr, :] = jnp.dot(mt_buf[g, 0:sr, 0:gw].astype(BF16), pq_buf.load(s, 128 * g, 128 * g + gw),
                                      preferred_element_type=F32)

    def memory_update(s, g):
        rg = _group_rows(g)
        a_g = _group_row_start(g)
        gw = GW[g]
        ones_row = 126 if g == 0 else 0
        lhs = jnp.where(lax.broadcasted_iota(I32, (rg, L), 0) == ones_row, 1.0,
                        vt_buf.load(s, a_g, a_g + rg).astype(F32)).astype(BF16)
        upd = lax.dot_general(lhs, pk_buf.load(s, 128 * g, 128 * g + gw), NT_DIMS,
                              preferred_element_type=F32)
        er = lax.broadcasted_iota(I32, (rg, gw), 0) + (a_g - HPG * DH * g)
        el = lax.broadcasted_iota(I32, (rg, gw), 1)
        same_head = None
        for i in range(_heads_in_group(g)):
            t = ((er >= DH * i) & (er < DH * (i + 1)) & (el >= DH * i) & (el < DH * (i + 1)))
            same_head = t if same_head is None else (same_head | t)
        mt_buf[g, 0:rg, 0:gw] = mt_buf[g, 0:rg, 0:gw] + jnp.where(same_head, upd, 0.0)
        zr = lax.broadcasted_iota(I32, (8, gw), 0)
        zl = lax.broadcasted_iota(I32, (8, gw), 1)
        zmask = (zl >= zr * DH) & (zl < zr * DH + DH) & (zr < _heads_in_group(g))
        zs = upd[ones_row:ones_row + 1]
        z0 = _norm_row(g)
        mt_buf[g, z0:z0 + 8, 0:gw] = mt_buf[g, z0:z0 + 8, 0:gw] + jnp.where(zmask, zs, 0.0)

    def transpose_wo(g):
        hi = min(128 * (g + 1), D)
        wot.store(wo_raw[:, 128 * g:hi].T, lo=128 * g)

    def project_out(s):
        return jnp.dot(wot.load(), ot_buf[...].astype(BF16), preferred_element_type=F32)

    def residual(s, cols=slice(None)):
        return x_buf[s, :, cols].astype(F32) + xn_buf.load(s, cols=cols).astype(F32)

    def emit(s, val):
        out_buf[s] = val.astype(BF16)
        out_copy(s).start()

    zero = lax.shift_right_logical(i1, 16)

    def prow(start, size):
        return pl.ds(pl.multiple_of(zero + start, 8), size)

    P_OFFS = (0, 128, 384, 768)

    def fast_scores(s, g, hook):
        nh = _heads_in_group(g)
        gw = GW[g]
        pb = (p_buf0, p_buf1)[(s * NG + g) % 2]
        rowg = lax.broadcasted_iota(I32, (gw, 128), 0)
        for j in range(QT - 1, -1, -1):
            n = 128 * (j + 1)
            q = qs_buf.load(s, 128 * g, 128 * g + gw, slice(128 * j, 128 * (j + 1))).astype(F32)
            for h0, h1 in ((0, 4), (4, nh)):
                if h1 <= h0:
                    continue
                qm = jnp.concatenate(
                    [jnp.where((rowg >= DH * i) & (rowg < DH * (i + 1)), q, 0.0) for i in range(h0, h1)],
                    axis=1).astype(BF16)
                st = jnp.dot(k_buf.load(s * NG + g, 0, n, slice(0, gw)), qm, preferred_element_type=F32)
                p = jnp.exp2(st)
                causal_w = jnp.concatenate([causal] * (h1 - h0), axis=1)
                p_diag = jnp.where(causal_w, p[n - 128:], 0.0)
                p = jnp.concatenate([p[:n - 128], p_diag], axis=0) if j > 0 else p_diag
                pb[P_OFFS[j] // 2:(P_OFFS[j] + n) // 2, h0 * 128:h1 * 128] = pltpu.bitcast(p.astype(BF16), U32)
                hook(j >= 2, p)

    def fast_values(s, g, after_tile=None):
        nh = _heads_in_group(g)
        a_g = _group_row_start(g)
        pb = (p_buf0, p_buf1)[(s * NG + g) % 2]
        for j in range(QT - 1, -1, -1):
            n = 128 * (j + 1)
            cols = slice(128 * j, 128 * (j + 1))
            for i in range(nh):
                h = HPG * g + i
                a = (h * DH // 16) * 16
                off = h * DH - a
                p = pltpu.bitcast(pb[prow(P_OFFS[j] // 2, n // 2), 128 * i:128 * (i + 1)], BF16)
                ones_row = 0 if off > 0 else 31
                r32n = lax.broadcasted_iota(I32, (32, n), 0)
                lhs = jnp.where(r32n == ones_row, 1.0, vt_buf.load(s, a, a + 32, slice(0, n)).astype(F32)).astype(BF16)
                o = jnp.dot(lhs, p, preferred_element_type=F32)
                lo = (off // 8) * 8
                hi = -(-(off + DH) // 8) * 8
                gate = gate_buf[h:h + 1, :]
                rl = 1.0 / o[ones_row:ones_row + 1]
                val = (1.0 - gate) * (o[lo:hi] * rl)
                if s > 0:
                    z = _norm_row(g) + i
                    rden = 1.0 / (num_buf[g, z:z + 1, cols] + 1e-6)
                    num = num_buf[g, a - a_g + lo:a - a_g + hi, cols]
                    val = gate * (num * rden) + val
                ot_buf[a + off:a + off + DH, cols] = val[off - lo:off - lo + DH]
            if after_tile is not None:
                after_tile(j)

    def fast_path():
        hidden = []
        up = expert_up_stream(hidden)
        n_chunks = FF // 512
        state = dict(down=0, wd_ready=False, up_done=False, y=[None] * 5, tail=None)

        def finish():
            yield from expert_scatter_parts(jnp.concatenate(state["y"], axis=1))
            for u in range(NSEG - 1):
                for j in range(QT):
                    cols = slice(128 * j, 128 * (j + 1))
                    val = base[u, :, cols]
                    y = state["pacer"]
                    if y is not None:
                        reps = -(-D // y.shape[0])
                        y = jnp.concatenate([y[:, 128 * r:128 * (r + 1)] for r in range(reps)], axis=0)[0:D]
                        val = jnp.where(always[0][:, 0:128], val, y)
                    val = (val + x_buf[u, :, cols].astype(F32)) + xn_buf.load(u, cols=cols).astype(F32)
                    out_buf[u, :, cols] = val.astype(BF16)
                    if j == QT - 1:
                        out_copy(u).start()
                    yield

        def down_step():
            ci, e = divmod(state["down"], 5)
            part = expert_down_step(hidden[ci], ci, e)
            state["y"][e] = part if state["y"][e] is None else state["y"][e] + part
            state["down"] += 1

        def hook(long, pacer=None):
            state["pacer"] = pacer if pacer is not None and pacer.shape[0] * (pacer.shape[1] // 128) >= D else None
            can_down = (state["wd_ready"] and state["down"] < 5 * n_chunks
                        and state["down"] // 5 < len(hidden))
            if can_down and (long or state["up_done"]):
                down_step()
            elif not state["up_done"]:
                if next(up, "done") == "done":
                    state["up_done"] = True
                    hook(long, pacer)
            elif state["down"] == 5 * n_chunks and state["out_ready"]:
                if state["tail"] is None:
                    state["tail"] = finish()
                if pacer is not None and state["pacer"] is not None or state["tail_steps"] < 2:
                    state["tail_steps"] += 1
                    next(state["tail"], None)

        state["out_ready"] = False
        state["tail_steps"] = 0
        steps = [(s, g) for s in range(NSEG) for g in range(NG)]
        last = NSEG - 1

        def last_tile(j):
            cols = slice(128 * j, 128 * (j + 1))
            attn = jnp.dot(wot.load(), ot_buf[:, cols].astype(BF16), preferred_element_type=F32)
            out_buf[last, :, cols] = (base[last, :, cols] + residual(last, cols) + attn).astype(BF16)
            out_tile_copy(j).start()

        fast_scores(0, 0, hook)
        for t, (s, g) in enumerate(steps):
            if t + 1 < len(steps):
                fast_scores(*steps[t + 1], hook)
            if s > 0:
                memory_read(s, g)
                hook(True)
            if t + 1 == len(steps):
                state["pacer"] = None
                while state["tail"] is None or next(state["tail"], "done") != "done":
                    if state["tail"] is None:
                        hook(True)
                pending = []

                def after_tile(j):
                    if pending:
                        last_tile(pending.pop())
                    pending.append(j)

                fast_values(s, g, after_tile)
                last_tile(pending.pop())
            else:
                fast_values(s, g)
            if s == 0:
                transpose_wo(g)
            if s + 1 < NSEG:
                memory_update(s, g)
                hook(True)
            if g == NG - 1 and s < last:
                base[s] = project_out(s)
                if s == 0:
                    cp_wd.wait()
                    state["wd_ready"] = True
                if s == last - 1:
                    state["out_ready"] = True
                hook(True)
        for u in range(NSEG - 1):
            out_copy(u).wait()
        for j in range(QT):
            out_tile_copy(j).wait()

    def slow_segment(s, carry):
        for g in range(NG):
            memory_read(s, g)
        key_i = lax.broadcasted_iota(I32, (L, L), 0)
        qry_i = lax.broadcasted_iota(I32, (L, L), 1)
        r32 = lax.broadcasted_iota(I32, (32, L), 0)
        for g in range(NG):
            gw = GW[g]
            a_g = _group_row_start(g)
            rowg = lax.broadcasted_iota(I32, (gw, L), 0)

            def head(i, c, g=g, gw=gw, a_g=a_g, rowg=rowg):
                h = HPG * g + i
                a = pl.multiple_of((h * DH // 16) * 16, 16)
                off = h * DH - a
                q = qs_buf.load(s, 128 * g, 128 * g + gw).astype(F32)
                qm = jnp.where((rowg >= DH * i) & (rowg < DH * (i + 1)), q, 0.0).astype(BF16)
                st = jnp.dot(k_buf.load(s * NG + g, cols=slice(0, gw)), qm, preferred_element_type=F32)
                st = jnp.where(key_i <= qry_i, st, NEG_BIG)
                p = jnp.exp2(st - jnp.max(st, axis=0, keepdims=True))
                rl = 1.0 / jnp.sum(p, axis=0, keepdims=True)
                o = jnp.dot(vt_buf.load(s, a, 32), p.astype(BF16), preferred_element_type=F32)
                gate = jnp.concatenate([gate_buf[pl.ds(h, 1), :]] * QT, axis=1)
                rden = 1.0 / (num_buf[g, pl.ds(_norm_row(g) + i, 1), :] + 1e-6)
                num = num_buf[g, pl.ds(pl.multiple_of(a - a_g, 16), 32), :]
                val = gate * (num * rden) + (1.0 - gate) * (o * rl)
                keep = (r32 >= off) & (r32 < off + DH)
                pltpu.store(ot_buf.at[pl.ds(a, 32), :], val, mask=keep)
                return c

            lax.fori_loop(0, _heads_in_group(g), head, 0)
        for g in range(NG):
            memory_update(s, g)
        emit(s, base[s] + residual(s) + project_out(s))
        return carry

    @pl.when(safe)
    def _():
        fast_path()

    @pl.when(jnp.logical_not(safe))
    def _():
        cp_wd.wait()
        for u in range(NSEG - 1):
            base[u] = jnp.zeros((D, L), F32)
        for g in range(NG):
            transpose_wo(g)
        expert_scatter(expert_chunk(0, FF))
        lax.fori_loop(0, NSEG, slow_segment, 0)
        for u in range(NSEG):
            out_copy(u).wait()


@jax.jit
def pallas_parallel_sum__memory_aug_infini_attn__moe_arch_mod__prompt_kernel(
    A_x: jax.Array,
    A_wq: jax.Array,
    A_wk: jax.Array,
    A_wv: jax.Array,
    A_wo: jax.Array,
    A_beta: jax.Array,
    B_x: jax.Array,
    B_w_r: jax.Array,
    B_w_gate: jax.Array,
    B_w_up: jax.Array,
    B_w_down: jax.Array,
):
    del B_x
    hbm = pl.BlockSpec(memory_space=pl.ANY)
    scratch = [
        pltpu.VMEM((NSEG, D, L), BF16),
        pltpu.VMEM((D, D), BF16),
        pltpu.VMEM((D, D), BF16),
        pltpu.VMEM((D, D), BF16),
        pltpu.VMEM((D, D), BF16),
        pltpu.VMEM((H,), BF16),
        pltpu.VMEM((D,), BF16),
        pltpu.VMEM((D, FF), BF16),
        pltpu.VMEM((D, FF), BF16),
        pltpu.VMEM((D, FF), BF16),
        pltpu.VMEM((PR // 2, D), U32),
        pltpu.VMEM((PR // 2, D), U32),
        pltpu.VMEM((D // 2, D), U32),
        pltpu.VMEM((D // 2, D), U32),
        pltpu.VMEM((NSEG * D // 2, L), U32),
        pltpu.VMEM((NSEG, D, L), F32),
        pltpu.VMEM((NSEG * PR // 2, L), U32),
        pltpu.VMEM((NSEG * PR // 2, L), U32),
        pltpu.VMEM((NSEG * NG * L // 2, 128), U32),
        pltpu.VMEM((NSEG * PR // 2, L), U32),
        pltpu.VMEM((NSEG * D // 2, L), U32),
        pltpu.VMEM((8, S), F32),
        pltpu.VMEM((H, 128), F32),
        pltpu.VMEM((NG, MROWS, 128), F32),
        pltpu.VMEM((NG, MROWS, L), F32),
        pltpu.VMEM((640, HPG * 128), U32),
        pltpu.VMEM((640, HPG * 128), U32),
        pltpu.VMEM((D, L), F32),
        pltpu.VMEM((NSEG, D, L), BF16),
        pltpu.SemaphoreType.DMA((13,)),
        pltpu.SemaphoreType.DMA((NSEG + QT,)),
    ]
    out_t = pl.pallas_call(
        _kernel,
        out_shape=jax.ShapeDtypeStruct((1, D, S), BF16),
        in_specs=[hbm] * 10,
        out_specs=hbm,
        scratch_shapes=scratch,
        compiler_params=pltpu.CompilerParams(vmem_limit_bytes=128 * 1024 * 1024),
        name="infini_attn_moe",
    )(jnp.transpose(A_x, (0, 2, 1)), A_wq, A_wk, A_wv, A_wo, A_beta, B_w_r, B_w_gate, B_w_up,
      B_w_down.T)
    return jnp.transpose(out_t, (0, 2, 1))
```

```python
import jax
import jax.numpy as jnp
from jax import lax
import jax.experimental.pallas as pl
import jax.experimental.pallas.tpu as pltpu

F32 = jnp.float32
BF16 = jnp.bfloat16
U32 = jnp.uint32
I32 = jnp.int32

S = 2048
D = 576
H = 32
DH = 18
NSEG = 4
L = 512
FF = 4608
HPG = 7
NG = 5
QT = L // 128
GW = (128, 128, 128, 128, 80)
PR = sum(GW)
ROUTER_ROW = 126
MROWS = 144
LOG2E = 1.4426950408889634
QSCALE = (DH ** -0.5) * LOG2E
SAFE_LOG2_RANGE = 60.0
NEG_BIG = -1e30

NT_DIMS = (((1,), (1,)), ((), ()))


def _heads_in_group(g):
    return min(HPG, H - HPG * g)


def _group_row_start(g):
    return (HPG * g * DH // 16) * 16


def _group_rows(g):
    last = (HPG * g + _heads_in_group(g)) * DH
    return -(-(last - _group_row_start(g)) // 16) * 16


def _state_rows(g):
    return MROWS if g == 0 else _group_rows(g)


def _norm_row(g):
    return 128 if g == 0 else 0


def _round_bf16(x):
    return x.astype(BF16).astype(F32)


def _pad_heads_t(w):
    parts = []
    for g in range(NG):
        n = _heads_in_group(g) * DH
        parts.append(w[:, HPG * DH * g:HPG * DH * g + n])
        parts.append(jnp.zeros((D, 128 - n), w.dtype))
    return jnp.concatenate(parts, axis=1).T[0:PR]


def _phi(t):
    return jnp.where(t > 0, t + 1.0, jnp.exp(t))


class _Packed:
    def __init__(self, ref, rows):
        self.ref = ref
        self.rows = rows

    def _slice(self, item, lo, size):
        start = item * (self.rows // 2) + lo // 2
        size = size // 2
        if isinstance(start, int):
            return slice(start, start + size)
        return pl.ds(pl.multiple_of(start, 8), size)

    def load(self, item=0, lo=0, hi=None, cols=slice(None)):
        size = hi if not isinstance(lo, int) else (self.rows if hi is None else hi) - lo
        return pltpu.bitcast(self.ref[self._slice(item, lo, size), cols], BF16)

    def store(self, val, item=0, lo=0, cols=slice(None)):
        self.ref[self._slice(item, lo, val.shape[0]), cols] = pltpu.bitcast(val.astype(BF16), U32)


def _kernel(x_hbm, wq_hbm, wk_hbm, wv_hbm, wo_hbm, beta_hbm, wr_hbm, wg_hbm, wu_hbm, wd_hbm,
            out_hbm,
            x_buf, wq_raw, wk_raw, wv_raw, wo_raw, beta_buf, wr_buf, wg_buf, wu_buf, wd_buf,
            wqt, wkt, wvt, wot, xn_buf, base, qs_buf, pq_buf, k_buf, pk_buf, vt_buf, r_buf,
            gate_buf, mt_buf, num_buf, p_buf0, p_buf1, ot_buf, out_buf, in_sems, out_sems):
    wqt, wkt = _Packed(wqt, PR), _Packed(wkt, PR)
    wvt, wot = _Packed(wvt, D), _Packed(wot, D)
    xn_buf, vt_buf = _Packed(xn_buf, D), _Packed(vt_buf, D)
    qs_buf, pq_buf, pk_buf = _Packed(qs_buf, PR), _Packed(pq_buf, PR), _Packed(pk_buf, PR)
    k_buf = _Packed(k_buf, L)

    def x_copy(c):
        return pltpu.make_async_copy(x_hbm.at[0, :, pl.ds(c * L, L)], x_buf.at[c], in_sems.at[c])

    cp_wv = pltpu.make_async_copy(wv_hbm, wv_raw, in_sems.at[4])
    cp_wq = pltpu.make_async_copy(wq_hbm, wq_raw, in_sems.at[5])
    cp_wk = pltpu.make_async_copy(wk_hbm, wk_raw, in_sems.at[6])
    cp_wo = pltpu.make_async_copy(wo_hbm, wo_raw, in_sems.at[7])
    cp_wg = pltpu.make_async_copy(wg_hbm, wg_buf, in_sems.at[8])
    cp_wu = pltpu.make_async_copy(wu_hbm, wu_buf, in_sems.at[9])
    cp_wd = pltpu.make_async_copy(wd_hbm, wd_buf, in_sems.at[10])
    cp_beta = pltpu.make_async_copy(beta_hbm, beta_buf, in_sems.at[11])
    cp_wr = pltpu.make_async_copy(wr_hbm, wr_buf, in_sems.at[12])

    def out_copy(s):
        cols = pl.ds(pl.multiple_of(s * L, L), L)
        return pltpu.make_async_copy(out_buf.at[s], out_hbm.at[0, :, cols], out_sems.at[s])

    def out_tile_copy(j):
        s = NSEG - 1
        return pltpu.make_async_copy(out_buf.at[s, :, pl.ds(128 * j, 128)],
                                     out_hbm.at[0, :, pl.ds(s * L + 128 * j, 128)], out_sems.at[NSEG + j])


    for cp in (x_copy(0), cp_wv, x_copy(1), cp_wq, cp_wr, cp_beta, x_copy(2), cp_wk, x_copy(3), cp_wo,
               cp_wg, cp_wu, cp_wd):
        cp.start()

    lane128 = lax.broadcasted_iota(I32, (128, 128), 1)
    row128 = lax.broadcasted_iota(I32, (128, 128), 0)
    causal = row128 <= lane128
    r16 = lax.broadcasted_iota(I32, (16, D), 0)

    mt_buf[...] = jnp.zeros(mt_buf.shape, F32)

    always = []

    def pace(x, y):
        return x if y is None else jnp.where(always[0], x, y[0:D])

    def ln_stats(c, y):
        shift = x_buf[c, 0:16, :].astype(F32)[0:1]
        d = pace(x_buf[c].astype(F32), y) - shift
        m1 = jnp.sum(d, axis=0, keepdims=True) * (1.0 / D)
        m2 = jnp.sum(d * d, axis=0, keepdims=True) * (1.0 / D)
        var = jnp.maximum(m2 - m1 * m1, 0.0)
        inv = 1.0 / _round_bf16(jnp.sqrt(_round_bf16(_round_bf16(var) + 1e-5)))
        return _round_bf16(shift + m1), inv

    def ln_apply(c, mean_b, inv):
        x = x_buf[c].astype(F32)
        xn = (x - mean_b) * inv
        xn_buf.store(xn, c)
        if c == NSEG - 1:
            base[c] = jnp.zeros((D, L), F32)

    def project(w_ref, c, split):
        if not split:
            return jnp.dot(w_ref.load(), xn_buf.load(c), preferred_element_type=F32), None
        head = jnp.dot(w_ref.load(cols=slice(0, 256)), xn_buf.load(c, 0, 256), preferred_element_type=F32)
        tail = jnp.dot(w_ref.load(cols=slice(256, D)), xn_buf.load(c, 256, D), preferred_element_type=F32)
        return head + tail, head

    def project_v(c, mid=None):
        vt, head = project(wvt, c, mid is not None)
        if mid is not None:
            mid(head)
        vt_buf.store(vt, c)
        return vt

    def project_q(c, mid=None):
        qt, head = project(wqt, c, mid is not None)
        if mid is not None:
            mid(head)
        qsc = qt * QSCALE
        qs_buf.store(qsc, c)
        pq_buf.store(_phi(qt), c)
        r_buf[:, c * L:(c + 1) * L] = qt[120:128]
        mag = jnp.abs(qsc)
        r8 = lax.broadcasted_iota(I32, (8, L), 0)
        mag = jnp.concatenate([mag[0:120], jnp.where(r8 == ROUTER_ROW - 120, 0.0, mag[120:128]), mag[128:]], axis=0)
        return qt, jnp.max(mag.reshape(PR // 8, 8, L), axis=0)

    def project_k(c, mid=None, keep=False):
        kt, head = project(wkt, c, mid is not None)
        if mid is not None:
            mid(head)
        pk_buf.store(_phi(kt), c)
        for g in range(NG):
            ktg = kt[128 * g:128 * g + GW[g]]
            if GW[g] < 128:
                ktg = jnp.concatenate([ktg, jnp.zeros((128 - GW[g], L), F32)], axis=0)
            k_buf.store(ktg.T, c * NG + g)
        top = jnp.max(jnp.abs(kt).reshape(PR // 8, 8, L), axis=0)
        return (kt, top) if keep else top

    x_copy(0).wait()
    stats = ln_stats(0, None)
    always.append(jnp.logical_not(jnp.abs(stats[0]) < 0.0))
    ln_apply(0, *stats)
    cp_wv.wait()
    wvt.store(wv_raw[...].T)
    project_v(0)
    x_copy(1).wait()
    cp_wq.wait()
    cp_wr.wait()
    ln_apply(1, *ln_stats(1, None))

    def paced_weight(w_ref, y):
        w = w_ref[...].astype(F32)
        return jnp.concatenate([jnp.where(always[0], w[:, 0:L], y[0:D]), w[:, L:D]], axis=1)

    def prep_wq(y):
        wq_t = _pad_heads_t(paced_weight(wq_raw, y))
        wr_row = wr_buf[...].reshape(1, D).astype(F32)
        pr_row = lax.broadcasted_iota(I32, (8, D), 0)
        wq_t = jnp.concatenate(
            [wq_t[0:120], jnp.where(pr_row == ROUTER_ROW - 120, wr_row, wq_t[120:128]), wq_t[128:]], axis=0)
        wqt.store(wq_t)

    project_v(1, prep_wq)
    cp_wk.wait()
    cp_beta.wait()
    x_copy(2).wait()
    x_copy(3).wait()

    beta_row = beta_buf[...].reshape(1, H).astype(F32)
    beta_row = jnp.concatenate([beta_row, jnp.zeros((1, 128 - H), F32)], axis=1)
    h_row = lax.broadcasted_iota(I32, (H, 128), 0)
    h_lane = lax.broadcasted_iota(I32, (H, 128), 1)
    beta_col = jnp.sum(jnp.where(h_row == h_lane, beta_row, 0.0), axis=1, keepdims=True)
    gate_buf[...] = jnp.broadcast_to(jax.nn.sigmoid(beta_col), (H, 128))

    def prep_wk(y):
        wkt.store(_pad_heads_t(paced_weight(wk_raw, y)))

    def route():
        r = _round_bf16(r_buf[ROUTER_ROW - 120:ROUTER_ROW - 119, :])
        tok = lax.broadcasted_iota(I32, (1, S), 1).astype(F32)
        m1 = jnp.max(r)
        i1 = jnp.min(jnp.where(r == m1, tok, float(S)))
        r_rest = jnp.where(tok == i1, -jnp.inf, r)
        m2 = jnp.max(r_rest)
        i2 = jnp.min(jnp.where(r_rest == m2, tok, float(S)))
        i1 = jnp.clip(i1.astype(I32), 0, S - 1)
        i2 = jnp.clip(i2.astype(I32), 0, S - 1)
        return m1, m2, i1, i2

    qt, aq = project_q(0, prep_wk)
    qt, a = project_q(1)
    aq = jnp.maximum(aq, a)
    stats = ln_stats(2, qt)
    ak = project_k(0)
    ln_apply(2, *stats)
    kt, a = project_k(1, keep=True)
    ak = jnp.maximum(ak, a)
    stats = ln_stats(3, kt)
    project_v(2)
    ln_apply(3, *stats)
    qt, a = project_q(2)
    aq = jnp.maximum(aq, a)
    ak = jnp.maximum(ak, project_k(2))
    qt, a = project_q(3)
    aq = jnp.maximum(aq, a)
    m1, m2, i1, i2 = route()
    ak = jnp.maximum(ak, project_k(3))
    project_v(3)

    logit_bound = jnp.max(aq) * jnp.max(ak) * (DH * 1.02)
    safe = logit_bound <= SAFE_LOG2_RANGE

    sel_row = lax.broadcasted_iota(I32, (16, 128), 0)
    sel_lane = lax.broadcasted_iota(I32, (16, 128), 1)

    def token_tile(i):
        return i // L, pl.ds(pl.multiple_of(((i % L) // 128) * 128, 128), 128)

    def pick(i, slot):
        seg, cols = token_tile(i)
        onehot = jnp.where((sel_row == slot) & (sel_lane == i % 128), 1.0, 0.0).astype(BF16)
        return lax.dot_general(onehot, xn_buf.load(seg, cols=cols), NT_DIMS, preferred_element_type=F32)

    def routed_rows():
        return (pick(i1, 0) + pick(i2, 1)).astype(BF16)

    cp_wo.wait()
    cp_wg.wait()
    cp_wu.wait()


    def expert_chunk(lo, hi):
        xs = routed_rows()
        hg = jnp.dot(xs, wg_buf[:, lo:hi], preferred_element_type=F32)
        hu = jnp.dot(xs, wu_buf[:, lo:hi], preferred_element_type=F32)
        hh = (jax.nn.silu(hg) * hu).astype(BF16)
        return lax.dot_general(hh, wd_buf[:, lo:hi], NT_DIMS, preferred_element_type=F32)

    def expert_up_stream(hidden):
        kmain = 512
        xs = routed_rows()
        yield
        for c0 in range(0, FF, 512):
            rem = []
            for w_ref in (wg_buf, wu_buf):
                rem.append(jnp.dot(xs[:, kmain:D], w_ref[kmain:D, c0:c0 + 512], preferred_element_type=F32))
                yield
            hs = []
            for f0 in range(c0, c0 + 512, 128):
                pre = []
                for w_ref, r in zip((wg_buf, wu_buf), rem):
                    pre.append(jnp.dot(xs[:, 0:kmain], w_ref[0:kmain, f0:f0 + 128], preferred_element_type=F32)
                               + r[:, f0 - c0:f0 - c0 + 128])
                    if len(pre) == 2:
                        hs.append(jax.nn.silu(pre[0]) * pre[1])
                        if len(hs) == 4:
                            hidden.append(jnp.concatenate(hs, axis=1).astype(BF16))
                    yield

    def expert_down_step(hh, ci, e):
        e_hi = min(128 * (e + 1), D)
        return lax.dot_general(hh, wd_buf[128 * e:e_hi, 512 * ci:512 * (ci + 1)], NT_DIMS,
                               preferred_element_type=F32)

    def expert_scatter_parts(y):
        y = y * jax.nn.sigmoid(jnp.where(r16 == 0, m1, m2))
        yt = jnp.concatenate([y, jnp.zeros((128 - 16, D), F32)], axis=0).T
        lane_d = lax.broadcasted_iota(I32, (D, 128), 1)
        for slot, i in ((0, i1), (1, i2)):
            seg, cols = token_tile(i)
            col = jnp.sum(jnp.where(lane_d == slot, yt, 0.0), axis=1, keepdims=True)
            base[seg, :, cols] = base[seg, :, cols] + jnp.where(lane_d == i % 128, col, 0.0)
            yield

    def expert_scatter(y):
        for _ in expert_scatter_parts(y):
            pass

    def memory_read(s, g):
        sr = _state_rows(g)
        gw = GW[g]
        num_buf[g, 0:sr, :] = jnp.dot(mt_buf[g, 0:sr, 0:gw].astype(BF16), pq_buf.load(s, 128 * g, 128 * g + gw),
                                      preferred_element_type=F32)

    def memory_update(s, g):
        rg = _group_rows(g)
        a_g = _group_row_start(g)
        gw = GW[g]
        ones_row = 126 if g == 0 else 0
        lhs = jnp.where(lax.broadcasted_iota(I32, (rg, L), 0) == ones_row, 1.0,
                        vt_buf.load(s, a_g, a_g + rg).astype(F32)).astype(BF16)
        upd = lax.dot_general(lhs, pk_buf.load(s, 128 * g, 128 * g + gw), NT_DIMS,
                              preferred_element_type=F32)
        er = lax.broadcasted_iota(I32, (rg, gw), 0) + (a_g - HPG * DH * g)
        el = lax.broadcasted_iota(I32, (rg, gw), 1)
        same_head = None
        for i in range(_heads_in_group(g)):
            t = ((er >= DH * i) & (er < DH * (i + 1)) & (el >= DH * i) & (el < DH * (i + 1)))
            same_head = t if same_head is None else (same_head | t)
        mt_buf[g, 0:rg, 0:gw] = mt_buf[g, 0:rg, 0:gw] + jnp.where(same_head, upd, 0.0)
        zr = lax.broadcasted_iota(I32, (8, gw), 0)
        zl = lax.broadcasted_iota(I32, (8, gw), 1)
        zmask = (zl >= zr * DH) & (zl < zr * DH + DH) & (zr < _heads_in_group(g))
        zs = upd[ones_row:ones_row + 1]
        z0 = _norm_row(g)
        mt_buf[g, z0:z0 + 8, 0:gw] = mt_buf[g, z0:z0 + 8, 0:gw] + jnp.where(zmask, zs, 0.0)

    def transpose_wo(g):
        hi = min(128 * (g + 1), D)
        wot.store(wo_raw[:, 128 * g:hi].T, lo=128 * g)

    def project_out(s):
        return jnp.dot(wot.load(), ot_buf[...].astype(BF16), preferred_element_type=F32)

    def residual(s, cols=slice(None)):
        return x_buf[s, :, cols].astype(F32) + xn_buf.load(s, cols=cols).astype(F32)

    def emit(s, val):
        out_buf[s] = val.astype(BF16)
        out_copy(s).start()

    zero = lax.shift_right_logical(i1, 16)

    def prow(start, size):
        return pl.ds(pl.multiple_of(zero + start, 8), size)

    P_OFFS = (0, 128, 384, 768)

    def fast_scores(s, g, hook, anchor):
        nh = _heads_in_group(g)
        gw = GW[g]
        pb = (p_buf0, p_buf1)[(s * NG + g) % 2]
        rowg = lax.broadcasted_iota(I32, (gw, 128), 0)
        laneg = lax.broadcasted_iota(I32, (gw, 128), 1)
        head_rows = [(rowg >= DH * i) & (rowg < DH * (i + 1)) for i in range(nh)]
        row64 = lax.broadcasted_iota(I32, (64, 128), 0)
        lane64 = lax.broadcasted_iota(I32, (64, 128), 1)
        visible_lo = row64 <= lane64
        visible_hi = row64 <= (lane64 & 63)
        upper = lax.broadcasted_iota(I32, (32, 128), 1) >= 64
        for j in range(QT - 1, -1, -1):
            n = 128 * (j + 1)
            m = n - 64
            q = qs_buf.load(s, 128 * g, 128 * g + gw, slice(128 * j, 128 * (j + 1))).astype(F32)
            for h0, h1 in ((0, 4), (4, nh)):
                if h1 <= h0:
                    continue
                q_in = anchor(q)
                qm = jnp.concatenate([jnp.where(head_rows[i], q_in, 0.0) for i in range(h0, h1)],
                                     axis=1).astype(BF16)
                st = jnp.dot(k_buf.load(s * NG + g, 0, m, slice(0, gw)), qm, preferred_element_type=F32)
                p = jnp.exp2(st)
                p_diag = jnp.where(jnp.concatenate([visible_lo] * (h1 - h0), axis=1), p[m - 64:], 0.0)
                p = jnp.concatenate([p[:m - 64], p_diag], axis=0) if j > 0 else p_diag
                pb[P_OFFS[j] // 2:(P_OFFS[j] + m) // 2, h0 * 128:h1 * 128] = pltpu.bitcast(p.astype(BF16), U32)
                hook(j >= 2, p)
            q_hi = jnp.where(laneg >= 64, q, pltpu.roll(q, 64, 1))
            pairs = [(i, i + 1) if i + 1 < nh else (None, i) for i in range(0, nh, 2)]
            tiles = []
            for a, b in pairs:
                keep = head_rows[b] & (laneg >= 64)
                if a is not None:
                    keep = keep | (head_rows[a] & (laneg < 64))
                tiles.append(jnp.where(keep, q_hi, 0.0))
            st = jnp.dot(k_buf.load(s * NG + g, m, n, slice(0, gw)), jnp.concatenate(tiles, axis=1).astype(BF16),
                         preferred_element_type=F32)
            p = jnp.where(jnp.concatenate([visible_hi] * len(pairs), axis=1), jnp.exp2(st), 0.0)
            p = pltpu.bitcast(p.astype(BF16), U32)
            rows = slice((P_OFFS[j] + m) // 2, (P_OFFS[j] + n) // 2)
            for t, (a, b) in enumerate(pairs):
                both = p[:, 128 * t:128 * (t + 1)]
                pb[rows, 128 * b:128 * (b + 1)] = jnp.where(upper, both, jnp.uint32(0))
                if a is not None:
                    pb[rows, 128 * a:128 * (a + 1)] = jnp.where(upper, pltpu.roll(both, 64, 1), jnp.uint32(0))

    def fast_values(s, g, after_tile=None):
        nh = _heads_in_group(g)
        a_g = _group_row_start(g)
        pb = (p_buf0, p_buf1)[(s * NG + g) % 2]
        for j in range(QT - 1, -1, -1):
            n = 128 * (j + 1)
            cols = slice(128 * j, 128 * (j + 1))
            for i in range(nh):
                h = HPG * g + i
                a = (h * DH // 16) * 16
                off = h * DH - a
                p = pltpu.bitcast(pb[prow(P_OFFS[j] // 2, n // 2), 128 * i:128 * (i + 1)], BF16)
                ones_row = 0 if off > 0 else 31
                r32n = lax.broadcasted_iota(I32, (32, n), 0)
                lhs = jnp.where(r32n == ones_row, 1.0, vt_buf.load(s, a, a + 32, slice(0, n)).astype(F32)).astype(BF16)
                o = jnp.dot(lhs, p, preferred_element_type=F32)
                lo = (off // 8) * 8
                hi = -(-(off + DH) // 8) * 8
                gate = gate_buf[h:h + 1, :]
                rl = 1.0 / o[ones_row:ones_row + 1]
                val = (1.0 - gate) * (o[lo:hi] * rl)
                if s > 0:
                    z = _norm_row(g) + i
                    rden = 1.0 / (num_buf[g, z:z + 1, cols] + 1e-6)
                    num = num_buf[g, a - a_g + lo:a - a_g + hi, cols]
                    val = gate * (num * rden) + val
                ot_buf[a + off:a + off + DH, cols] = val[off - lo:off - lo + DH]
            if after_tile is not None:
                after_tile(j)

    def fast_path():
        hidden = []
        up = expert_up_stream(hidden)
        n_chunks = FF // 512
        state = dict(down=0, wd_ready=False, up_done=False, y=[None] * 5, tail=None)

        def finish():
            yield from expert_scatter_parts(jnp.concatenate(state["y"], axis=1))
            for u in range(NSEG - 1):
                for j in range(QT):
                    cols = slice(128 * j, 128 * (j + 1))
                    val = base[u, :, cols]
                    y = state["pacer"]
                    if y is not None:
                        reps = -(-D // y.shape[0])
                        y = jnp.concatenate([y[:, 128 * r:128 * (r + 1)] for r in range(reps)], axis=0)[0:D]
                        val = jnp.where(always[0][:, 0:128], val, y)
                    val = (val + x_buf[u, :, cols].astype(F32)) + xn_buf.load(u, cols=cols).astype(F32)
                    out_buf[u, :, cols] = val.astype(BF16)
                    state["anchor"] = val
                    if j == QT - 1:
                        out_copy(u).start()
                    yield

        def anchor(q):
            val, state["anchor_next"], state["anchor"] = state["anchor_next"], state["anchor"], None
            return q if val is None else jnp.where(always[0][:, 0:128], q, val[D - q.shape[0]:D])

        def down_step():
            ci, e = divmod(state["down"], 5)
            part = expert_down_step(hidden[ci], ci, e)
            state["y"][e] = part if state["y"][e] is None else state["y"][e] + part
            state["down"] += 1

        def hook(long, pacer=None):
            state["pacer"] = pacer if pacer is not None and pacer.shape[0] * (pacer.shape[1] // 128) >= D else None
            can_down = (state["wd_ready"] and state["down"] < 5 * n_chunks
                        and state["down"] // 5 < len(hidden))
            if can_down and (long or state["up_done"]):
                down_step()
            elif not state["up_done"]:
                if next(up, "done") == "done":
                    state["up_done"] = True
                    hook(long, pacer)
            elif state["down"] == 5 * n_chunks and state["out_ready"]:
                if state["tail"] is None:
                    state["tail"] = finish()
                if pacer is not None and state["pacer"] is not None or state["tail_steps"] < 2:
                    state["tail_steps"] += 1
                    next(state["tail"], None)

        state["out_ready"] = False
        state["tail_steps"] = 0
        state["anchor"] = None
        state["anchor_next"] = None
        steps = [(s, g) for s in range(NSEG) for g in range(NG)]
        last = NSEG - 1

        def last_tile(j):
            cols = slice(128 * j, 128 * (j + 1))
            attn = jnp.dot(wot.load(), ot_buf[:, cols].astype(BF16), preferred_element_type=F32)
            out_buf[last, :, cols] = (base[last, :, cols] + residual(last, cols) + attn).astype(BF16)
            out_tile_copy(j).start()

        fast_scores(0, 0, hook, anchor)
        for t, (s, g) in enumerate(steps):
            if t + 1 < len(steps):
                fast_scores(*steps[t + 1], hook, anchor)
            if s > 0:
                memory_read(s, g)
                hook(True)
            if t + 1 == len(steps):
                state["pacer"] = None
                while state["tail"] is None or next(state["tail"], "done") != "done":
                    if state["tail"] is None:
                        hook(True)
                pending = []

                def after_tile(j):
                    if pending:
                        last_tile(pending.pop())
                    pending.append(j)

                fast_values(s, g, after_tile)
                last_tile(pending.pop())
            else:
                fast_values(s, g)
            if s == 0:
                transpose_wo(g)
            if s + 1 < NSEG:
                memory_update(s, g)
                hook(True)
            if g == NG - 1 and s < last:
                base[s] = project_out(s)
                if s == 0:
                    cp_wd.wait()
                    state["wd_ready"] = True
                if s == last - 1:
                    state["out_ready"] = True
                hook(True)
        for u in range(NSEG - 1):
            out_copy(u).wait()
        for j in range(QT):
            out_tile_copy(j).wait()

    def slow_segment(s, carry):
        for g in range(NG):
            memory_read(s, g)
        key_i = lax.broadcasted_iota(I32, (L, L), 0)
        qry_i = lax.broadcasted_iota(I32, (L, L), 1)
        r32 = lax.broadcasted_iota(I32, (32, L), 0)
        for g in range(NG):
            gw = GW[g]
            a_g = _group_row_start(g)
            rowg = lax.broadcasted_iota(I32, (gw, L), 0)

            def head(i, c, g=g, gw=gw, a_g=a_g, rowg=rowg):
                h = HPG * g + i
                a = pl.multiple_of((h * DH // 16) * 16, 16)
                off = h * DH - a
                q = qs_buf.load(s, 128 * g, 128 * g + gw).astype(F32)
                qm = jnp.where((rowg >= DH * i) & (rowg < DH * (i + 1)), q, 0.0).astype(BF16)
                st = jnp.dot(k_buf.load(s * NG + g, cols=slice(0, gw)), qm, preferred_element_type=F32)
                st = jnp.where(key_i <= qry_i, st, NEG_BIG)
                p = jnp.exp2(st - jnp.max(st, axis=0, keepdims=True))
                rl = 1.0 / jnp.sum(p, axis=0, keepdims=True)
                o = jnp.dot(vt_buf.load(s, a, 32), p.astype(BF16), preferred_element_type=F32)
                gate = jnp.concatenate([gate_buf[pl.ds(h, 1), :]] * QT, axis=1)
                rden = 1.0 / (num_buf[g, pl.ds(_norm_row(g) + i, 1), :] + 1e-6)
                num = num_buf[g, pl.ds(pl.multiple_of(a - a_g, 16), 32), :]
                val = gate * (num * rden) + (1.0 - gate) * (o * rl)
                keep = (r32 >= off) & (r32 < off + DH)
                pltpu.store(ot_buf.at[pl.ds(a, 32), :], val, mask=keep)
                return c

            lax.fori_loop(0, _heads_in_group(g), head, 0)
        for g in range(NG):
            memory_update(s, g)
        emit(s, base[s] + residual(s) + project_out(s))
        return carry

    @pl.when(safe)
    def _():
        fast_path()

    @pl.when(jnp.logical_not(safe))
    def _():
        cp_wd.wait()
        for u in range(NSEG - 1):
            base[u] = jnp.zeros((D, L), F32)
        for g in range(NG):
            transpose_wo(g)
        expert_scatter(expert_chunk(0, FF))
        lax.fori_loop(0, NSEG, slow_segment, 0)
        for u in range(NSEG):
            out_copy(u).wait()


@jax.jit
def pallas_parallel_sum__memory_aug_infini_attn__moe_arch_mod__prompt_kernel(
    A_x: jax.Array,
    A_wq: jax.Array,
    A_wk: jax.Array,
    A_wv: jax.Array,
    A_wo: jax.Array,
    A_beta: jax.Array,
    B_x: jax.Array,
    B_w_r: jax.Array,
    B_w_gate: jax.Array,
    B_w_up: jax.Array,
    B_w_down: jax.Array,
):
    del B_x
    hbm = pl.BlockSpec(memory_space=pl.ANY)
    scratch = [
        pltpu.VMEM((NSEG, D, L), BF16),
        pltpu.VMEM((D, D), BF16),
        pltpu.VMEM((D, D), BF16),
        pltpu.VMEM((D, D), BF16),
        pltpu.VMEM((D, D), BF16),
        pltpu.VMEM((H,), BF16),
        pltpu.VMEM((D,), BF16),
        pltpu.VMEM((D, FF), BF16),
        pltpu.VMEM((D, FF), BF16),
        pltpu.VMEM((D, FF), BF16),
        pltpu.VMEM((PR // 2, D), U32),
        pltpu.VMEM((PR // 2, D), U32),
        pltpu.VMEM((D // 2, D), U32),
        pltpu.VMEM((D // 2, D), U32),
        pltpu.VMEM((NSEG * D // 2, L), U32),
        pltpu.VMEM((NSEG, D, L), F32),
        pltpu.VMEM((NSEG * PR // 2, L), U32),
        pltpu.VMEM((NSEG * PR // 2, L), U32),
        pltpu.VMEM((NSEG * NG * L // 2, 128), U32),
        pltpu.VMEM((NSEG * PR // 2, L), U32),
        pltpu.VMEM((NSEG * D // 2, L), U32),
        pltpu.VMEM((8, S), F32),
        pltpu.VMEM((H, 128), F32),
        pltpu.VMEM((NG, MROWS, 128), F32),
        pltpu.VMEM((NG, MROWS, L), F32),
        pltpu.VMEM((640, HPG * 128), U32),
        pltpu.VMEM((640, HPG * 128), U32),
        pltpu.VMEM((D, L), F32),
        pltpu.VMEM((NSEG, D, L), BF16),
        pltpu.SemaphoreType.DMA((13,)),
        pltpu.SemaphoreType.DMA((NSEG + QT,)),
    ]
    out_t = pl.pallas_call(
        _kernel,
        out_shape=jax.ShapeDtypeStruct((1, D, S), BF16),
        in_specs=[hbm] * 10,
        out_specs=hbm,
        scratch_shapes=scratch,
        compiler_params=pltpu.CompilerParams(vmem_limit_bytes=128 * 1024 * 1024),
        name="infini_attn_moe",
    )(jnp.transpose(A_x, (0, 2, 1)), A_wq, A_wk, A_wv, A_wo, A_beta, B_w_r, B_w_gate, B_w_up,
      B_w_down.T)
    return jnp.transpose(out_t, (0, 2, 1))
```

```python
import jax
import jax.numpy as jnp
from jax import lax
import jax.experimental.pallas as pl
import jax.experimental.pallas.tpu as pltpu

F32 = jnp.float32
BF16 = jnp.bfloat16
U32 = jnp.uint32
I32 = jnp.int32

S = 2048
D = 576
H = 32
DH = 18
NSEG = 4
L = 512
FF = 4608
HPG = 7
NG = 5
QT = L // 128
GW = (128, 128, 128, 128, 80)
PR = sum(GW)
ROUTER_ROW = 126
MROWS = 144
LOG2E = 1.4426950408889634
QSCALE = (DH ** -0.5) * LOG2E
SAFE_LOG2_RANGE = 60.0
NEG_BIG = -1e30

NT_DIMS = (((1,), (1,)), ((), ()))


def _heads_in_group(g):
    return min(HPG, H - HPG * g)


def _group_row_start(g):
    return (HPG * g * DH // 16) * 16


def _group_rows(g):
    last = (HPG * g + _heads_in_group(g)) * DH
    return -(-(last - _group_row_start(g)) // 16) * 16


def _state_rows(g):
    return MROWS if g == 0 else _group_rows(g)


def _norm_row(g):
    return 128 if g == 0 else 0


def _round_bf16(x):
    return x.astype(BF16).astype(F32)


def _pad_heads_t(w):
    parts = []
    for g in range(NG):
        n = _heads_in_group(g) * DH
        parts.append(w[:, HPG * DH * g:HPG * DH * g + n])
        parts.append(jnp.zeros((D, 128 - n), w.dtype))
    return jnp.concatenate(parts, axis=1).T[0:PR]


def _phi(t):
    return jnp.where(t > 0, t + 1.0, jnp.exp(t))


class _Packed:
    def __init__(self, ref, rows):
        self.ref = ref
        self.rows = rows

    def _slice(self, item, lo, size):
        start = item * (self.rows // 2) + lo // 2
        size = size // 2
        if isinstance(start, int):
            return slice(start, start + size)
        return pl.ds(pl.multiple_of(start, 8), size)

    def load(self, item=0, lo=0, hi=None, cols=slice(None)):
        size = hi if not isinstance(lo, int) else (self.rows if hi is None else hi) - lo
        return pltpu.bitcast(self.ref[self._slice(item, lo, size), cols], BF16)

    def store(self, val, item=0, lo=0, cols=slice(None)):
        self.ref[self._slice(item, lo, val.shape[0]), cols] = pltpu.bitcast(val.astype(BF16), U32)


def _kernel(x_hbm, wq_hbm, wk_hbm, wv_hbm, wo_hbm, beta_hbm, wr_hbm, wg_hbm, wu_hbm, wd_hbm,
            out_hbm,
            x_buf, wq_raw, wk_raw, wv_raw, wo_raw, beta_buf, wr_buf, wg_buf, wu_buf, wd_buf,
            wqt, wkt, wvt, wot, xn_buf, base, qs_buf, pq_buf, k_buf, pk_buf, vt_buf, r_buf,
            gate_buf, mt_buf, num_buf, p_buf0, p_buf1, ot_buf, out_buf, in_sems, out_sems):
    wqt, wkt = _Packed(wqt, PR), _Packed(wkt, PR)
    wvt, wot = _Packed(wvt, D), _Packed(wot, D)
    xn_buf, vt_buf = _Packed(xn_buf, D), _Packed(vt_buf, D)
    qs_buf, pq_buf, pk_buf = _Packed(qs_buf, PR), _Packed(pq_buf, PR), _Packed(pk_buf, PR)
    k_buf = _Packed(k_buf, L)

    def x_copy(c):
        return pltpu.make_async_copy(x_hbm.at[0, :, pl.ds(c * L, L)], x_buf.at[c], in_sems.at[c])

    cp_wv = pltpu.make_async_copy(wv_hbm, wv_raw, in_sems.at[4])
    cp_wq = pltpu.make_async_copy(wq_hbm, wq_raw, in_sems.at[5])
    cp_wk = pltpu.make_async_copy(wk_hbm, wk_raw, in_sems.at[6])
    cp_wo = pltpu.make_async_copy(wo_hbm, wo_raw, in_sems.at[7])
    cp_wg = pltpu.make_async_copy(wg_hbm, wg_buf, in_sems.at[8])
    cp_wu = pltpu.make_async_copy(wu_hbm, wu_buf, in_sems.at[9])
    cp_wd = pltpu.make_async_copy(wd_hbm, wd_buf, in_sems.at[10])
    cp_beta = pltpu.make_async_copy(beta_hbm, beta_buf, in_sems.at[11])
    cp_wr = pltpu.make_async_copy(wr_hbm, wr_buf, in_sems.at[12])

    def out_copy(s):
        cols = pl.ds(pl.multiple_of(s * L, L), L)
        return pltpu.make_async_copy(out_buf.at[s], out_hbm.at[0, :, cols], out_sems.at[s])

    def out_tile_copy(j):
        s = NSEG - 1
        return pltpu.make_async_copy(out_buf.at[s, :, pl.ds(128 * j, 128)],
                                     out_hbm.at[0, :, pl.ds(s * L + 128 * j, 128)], out_sems.at[NSEG + j])


    for cp in (x_copy(0), cp_wv, x_copy(1), cp_wq, cp_wr, cp_beta, x_copy(2), cp_wk, x_copy(3), cp_wo,
               cp_wg, cp_wu, cp_wd):
        cp.start()

    lane128 = lax.broadcasted_iota(I32, (128, 128), 1)
    row128 = lax.broadcasted_iota(I32, (128, 128), 0)
    causal = row128 <= lane128
    r16 = lax.broadcasted_iota(I32, (16, D), 0)

    mt_buf[...] = jnp.zeros(mt_buf.shape, F32)

    always = []

    def pace(x, y):
        return x if y is None else jnp.where(always[0], x, y[0:D])

    def ln_stats(c, y):
        shift = x_buf[c, 0:16, :].astype(F32)[0:1]
        d = pace(x_buf[c].astype(F32), y) - shift
        m1 = jnp.sum(d, axis=0, keepdims=True) * (1.0 / D)
        m2 = jnp.sum(d * d, axis=0, keepdims=True) * (1.0 / D)
        var = jnp.maximum(m2 - m1 * m1, 0.0)
        inv = 1.0 / _round_bf16(jnp.sqrt(_round_bf16(_round_bf16(var) + 1e-5)))
        return _round_bf16(shift + m1), inv

    def ln_apply(c, mean_b, inv):
        x = x_buf[c].astype(F32)
        xn = (x - mean_b) * inv
        xn_buf.store(xn, c)
        if c == NSEG - 1:
            base[c] = jnp.zeros((D, L), F32)

    def project(w_ref, c, split):
        if not split:
            return jnp.dot(w_ref.load(), xn_buf.load(c), preferred_element_type=F32), None
        head = jnp.dot(w_ref.load(cols=slice(0, 256)), xn_buf.load(c, 0, 256), preferred_element_type=F32)
        tail = jnp.dot(w_ref.load(cols=slice(256, D)), xn_buf.load(c, 256, D), preferred_element_type=F32)
        return head + tail, head

    def project_v(c, mid=None):
        vt, head = project(wvt, c, mid is not None)
        if mid is not None:
            mid(head)
        vt_buf.store(vt, c)
        return vt

    def project_q(c, mid=None):
        qt, head = project(wqt, c, mid is not None)
        if mid is not None:
            mid(head)
        qsc = qt * QSCALE
        qs_buf.store(qsc, c)
        pq_buf.store(_phi(qt), c)
        r_buf[:, c * L:(c + 1) * L] = qt[120:128]
        mag = jnp.abs(qsc)
        r8 = lax.broadcasted_iota(I32, (8, L), 0)
        mag = jnp.concatenate([mag[0:120], jnp.where(r8 == ROUTER_ROW - 120, 0.0, mag[120:128]), mag[128:]], axis=0)
        return qt, jnp.max(mag.reshape(PR // 8, 8, L), axis=0)

    def project_k(c, mid=None, keep=False):
        kt, head = project(wkt, c, mid is not None)
        if mid is not None:
            mid(head)
        pk_buf.store(_phi(kt), c)
        for g in range(NG):
            ktg = kt[128 * g:128 * g + GW[g]]
            if GW[g] < 128:
                ktg = jnp.concatenate([ktg, jnp.zeros((128 - GW[g], L), F32)], axis=0)
            k_buf.store(ktg.T, c * NG + g)
        top = jnp.max(jnp.abs(kt).reshape(PR // 8, 8, L), axis=0)
        return (kt, top) if keep else top

    x_copy(0).wait()
    stats = ln_stats(0, None)
    always.append(jnp.logical_not(jnp.abs(stats[0]) < 0.0))
    ln_apply(0, *stats)
    cp_wv.wait()
    wvt.store(wv_raw[...].T)
    project_v(0)
    x_copy(1).wait()
    cp_wq.wait()
    cp_wr.wait()
    ln_apply(1, *ln_stats(1, None))

    def paced_weight(w_ref, y):
        w = w_ref[...].astype(F32)
        return jnp.concatenate([jnp.where(always[0], w[:, 0:L], y[0:D]), w[:, L:D]], axis=1)

    def prep_wq(y):
        wq_t = _pad_heads_t(paced_weight(wq_raw, y))
        wr_row = wr_buf[...].reshape(1, D).astype(F32)
        pr_row = lax.broadcasted_iota(I32, (8, D), 0)
        wq_t = jnp.concatenate(
            [wq_t[0:120], jnp.where(pr_row == ROUTER_ROW - 120, wr_row, wq_t[120:128]), wq_t[128:]], axis=0)
        wqt.store(wq_t)

    project_v(1, prep_wq)
    cp_wk.wait()
    cp_beta.wait()
    x_copy(2).wait()
    x_copy(3).wait()

    beta_row = beta_buf[...].reshape(1, H).astype(F32)
    beta_row = jnp.concatenate([beta_row, jnp.zeros((1, 128 - H), F32)], axis=1)
    h_row = lax.broadcasted_iota(I32, (H, 128), 0)
    h_lane = lax.broadcasted_iota(I32, (H, 128), 1)
    beta_col = jnp.sum(jnp.where(h_row == h_lane, beta_row, 0.0), axis=1, keepdims=True)
    gate_buf[...] = jnp.broadcast_to(jax.nn.sigmoid(beta_col), (H, 128))

    def prep_wk(y):
        wkt.store(_pad_heads_t(paced_weight(wk_raw, y)))

    def route():
        r = _round_bf16(r_buf[ROUTER_ROW - 120:ROUTER_ROW - 119, :])
        tok = lax.broadcasted_iota(I32, (1, S), 1).astype(F32)
        m1 = jnp.max(r)
        i1 = jnp.min(jnp.where(r == m1, tok, float(S)))
        r_rest = jnp.where(tok == i1, -jnp.inf, r)
        m2 = jnp.max(r_rest)
        i2 = jnp.min(jnp.where(r_rest == m2, tok, float(S)))
        i1 = jnp.clip(i1.astype(I32), 0, S - 1)
        i2 = jnp.clip(i2.astype(I32), 0, S - 1)
        return m1, m2, i1, i2

    qt, aq = project_q(0, prep_wk)
    qt, a = project_q(1)
    aq = jnp.maximum(aq, a)
    stats = ln_stats(2, qt)
    ak = project_k(0)
    ln_apply(2, *stats)
    kt, a = project_k(1, keep=True)
    ak = jnp.maximum(ak, a)
    stats = ln_stats(3, kt)
    project_v(2)
    ln_apply(3, *stats)
    qt, a = project_q(2)
    aq = jnp.maximum(aq, a)
    ak = jnp.maximum(ak, project_k(2))
    qt, a = project_q(3)
    aq = jnp.maximum(aq, a)
    m1, m2, i1, i2 = route()
    ak = jnp.maximum(ak, project_k(3))
    project_v(3)

    logit_bound = jnp.max(aq) * jnp.max(ak) * (DH * 1.02)
    safe = logit_bound <= SAFE_LOG2_RANGE

    sel_row = lax.broadcasted_iota(I32, (16, 128), 0)
    sel_lane = lax.broadcasted_iota(I32, (16, 128), 1)

    def token_tile(i):
        return i // L, pl.ds(pl.multiple_of(((i % L) // 128) * 128, 128), 128)

    def pick(i, slot):
        seg, cols = token_tile(i)
        onehot = jnp.where((sel_row == slot) & (sel_lane == i % 128), 1.0, 0.0).astype(BF16)
        return lax.dot_general(onehot, xn_buf.load(seg, cols=cols), NT_DIMS, preferred_element_type=F32)

    def routed_rows():
        return (pick(i1, 0) + pick(i2, 1)).astype(BF16)

    cp_wo.wait()
    cp_wg.wait()
    cp_wu.wait()


    def expert_chunk(lo, hi):
        xs = routed_rows()
        hg = jnp.dot(xs, wg_buf[:, lo:hi], preferred_element_type=F32)
        hu = jnp.dot(xs, wu_buf[:, lo:hi], preferred_element_type=F32)
        hh = (jax.nn.silu(hg) * hu).astype(BF16)
        return lax.dot_general(hh, wd_buf[:, lo:hi], NT_DIMS, preferred_element_type=F32)

    def expert_up_stream(hidden):
        kmain = 512
        xs = routed_rows()
        yield
        for c0 in range(0, FF, 512):
            rem = []
            for w_ref in (wg_buf, wu_buf):
                rem.append(jnp.dot(xs[:, kmain:D], w_ref[kmain:D, c0:c0 + 512], preferred_element_type=F32))
                yield
            hs = []
            for f0 in range(c0, c0 + 512, 128):
                pre = []
                for w_ref, r in zip((wg_buf, wu_buf), rem):
                    pre.append(jnp.dot(xs[:, 0:kmain], w_ref[0:kmain, f0:f0 + 128], preferred_element_type=F32)
                               + r[:, f0 - c0:f0 - c0 + 128])
                    if len(pre) == 2:
                        hs.append(jax.nn.silu(pre[0]) * pre[1])
                        if len(hs) == 4:
                            hidden.append(_round_bf16(jnp.concatenate(hs, axis=1)))
                    yield

    lane_d = lax.broadcasted_iota(I32, (D, 128), 1)

    def expert_scatter_parts(columns):
        for col, i, score in zip(columns, (i1, i2), (m1, m2)):
            seg, cols = token_tile(i)
            col = col * jax.nn.sigmoid(jnp.full((D, 1), score, F32))
            base[seg, :, cols] = base[seg, :, cols] + jnp.where(lane_d == i % 128, col, 0.0)
            yield

    def expert_scatter_rows(y):
        yt = jnp.concatenate([y, jnp.zeros((128 - 16, D), F32)], axis=0).T
        columns = [jnp.sum(jnp.where(lane_d == slot, yt, 0.0), axis=1, keepdims=True) for slot in range(2)]
        for _ in expert_scatter_parts(columns):
            pass

    def memory_read(s, g):
        sr = _state_rows(g)
        gw = GW[g]
        num_buf[g, 0:sr, :] = jnp.dot(mt_buf[g, 0:sr, 0:gw].astype(BF16), pq_buf.load(s, 128 * g, 128 * g + gw),
                                      preferred_element_type=F32)

    def memory_update(s, g):
        rg = _group_rows(g)
        a_g = _group_row_start(g)
        gw = GW[g]
        ones_row = 126 if g == 0 else 0
        lhs = jnp.where(lax.broadcasted_iota(I32, (rg, L), 0) == ones_row, 1.0,
                        vt_buf.load(s, a_g, a_g + rg).astype(F32)).astype(BF16)
        upd = lax.dot_general(lhs, pk_buf.load(s, 128 * g, 128 * g + gw), NT_DIMS,
                              preferred_element_type=F32)
        er = lax.broadcasted_iota(I32, (rg, gw), 0) + (a_g - HPG * DH * g)
        el = lax.broadcasted_iota(I32, (rg, gw), 1)
        same_head = None
        for i in range(_heads_in_group(g)):
            t = ((er >= DH * i) & (er < DH * (i + 1)) & (el >= DH * i) & (el < DH * (i + 1)))
            same_head = t if same_head is None else (same_head | t)
        mt_buf[g, 0:rg, 0:gw] = mt_buf[g, 0:rg, 0:gw] + jnp.where(same_head, upd, 0.0)
        zr = lax.broadcasted_iota(I32, (8, gw), 0)
        zl = lax.broadcasted_iota(I32, (8, gw), 1)
        zmask = (zl >= zr * DH) & (zl < zr * DH + DH) & (zr < _heads_in_group(g))
        zs = upd[ones_row:ones_row + 1]
        z0 = _norm_row(g)
        mt_buf[g, z0:z0 + 8, 0:gw] = mt_buf[g, z0:z0 + 8, 0:gw] + jnp.where(zmask, zs, 0.0)

    def transpose_wo(g):
        hi = min(128 * (g + 1), D)
        wot.store(wo_raw[:, 128 * g:hi].T, lo=128 * g)

    def project_out(s):
        return jnp.dot(wot.load(), ot_buf[...].astype(BF16), preferred_element_type=F32)

    def residual(s, cols=slice(None)):
        return x_buf[s, :, cols].astype(F32) + xn_buf.load(s, cols=cols).astype(F32)

    def emit(s, val):
        out_buf[s] = val.astype(BF16)
        out_copy(s).start()

    zero = lax.shift_right_logical(i1, 16)

    def prow(start, size):
        return pl.ds(pl.multiple_of(zero + start, 8), size)

    P_OFFS = (0, 128, 384, 768)

    def fast_scores(s, g, hook, anchor):
        nh = _heads_in_group(g)
        gw = GW[g]
        pb = (p_buf0, p_buf1)[(s * NG + g) % 2]
        rowg = lax.broadcasted_iota(I32, (gw, 128), 0)
        laneg = lax.broadcasted_iota(I32, (gw, 128), 1)
        head_rows = [(rowg >= DH * i) & (rowg < DH * (i + 1)) for i in range(nh)]
        row64 = lax.broadcasted_iota(I32, (64, 128), 0)
        lane64 = lax.broadcasted_iota(I32, (64, 128), 1)
        visible_lo = row64 <= lane64
        row32 = lax.broadcasted_iota(I32, (32, 128), 0)
        lane32 = lax.broadcasted_iota(I32, (32, 128), 1)
        lane16 = lax.broadcasted_iota(I32, (16, 128), 1)
        for j in range(QT - 1, -1, -1):
            n = 128 * (j + 1)
            m = n - 64
            q = qs_buf.load(s, 128 * g, 128 * g + gw, slice(128 * j, 128 * (j + 1))).astype(F32)
            for h0, h1 in ((0, 4), (4, nh)):
                if h1 <= h0:
                    continue
                q_in = anchor(q)
                qm = jnp.concatenate([jnp.where(head_rows[i], q_in, 0.0) for i in range(h0, h1)],
                                     axis=1).astype(BF16)
                st = jnp.dot(k_buf.load(s * NG + g, 0, m, slice(0, gw)), qm, preferred_element_type=F32)
                p = jnp.exp2(st)
                p_diag = jnp.where(jnp.concatenate([visible_lo] * (h1 - h0), axis=1), p[m - 64:], 0.0)
                p = jnp.concatenate([p[:m - 64], p_diag], axis=0) if j > 0 else p_diag
                pb[P_OFFS[j] // 2:(P_OFFS[j] + m) // 2, h0 * 128:h1 * 128] = pltpu.bitcast(p.astype(BF16), U32)
                hook(j >= 2, p)
            for width, k0 in ((64, m), (32, m + 32)):
                per = 128 // width
                q_top = q
                for t in range(per - 1):
                    q_top = jnp.where((laneg >= width * t) & (laneg < width * (t + 1)),
                                      pltpu.roll(q, width * (t + 1), 1), q_top)
                groups = [list(range(i, min(i + per, nh))) for i in range(0, nh, per)]
                tiles = []
                for heads in groups:
                    keep = None
                    for t, i in enumerate(heads):
                        slot = per - len(heads) + t
                        sel = head_rows[i] & (laneg >= width * slot) & (laneg < width * (slot + 1))
                        keep = sel if keep is None else (keep | sel)
                    tiles.append(jnp.where(keep, q_top, 0.0))
                st = jnp.dot(k_buf.load(s * NG + g, k0, k0 + 32, slice(0, gw)),
                             jnp.concatenate(tiles, axis=1).astype(BF16),
                             preferred_element_type=F32)
                visible = row32 + (k0 - m) <= (lane32 & (width - 1)) + (64 - width)
                p = jnp.where(jnp.concatenate([visible] * len(groups), axis=1), jnp.exp2(st), 0.0)
                p = pltpu.bitcast(p.astype(BF16), U32)
                rows = slice((P_OFFS[j] + k0) // 2, (P_OFFS[j] + k0 + 32) // 2)
                top = lane16 >= 128 - width
                for gi, heads in enumerate(groups):
                    shared = p[:, 128 * gi:128 * (gi + 1)]
                    for t, i in enumerate(heads):
                        slot = per - len(heads) + t
                        shift = width * (per - 1 - slot)
                        mine = shared if shift == 0 else pltpu.roll(shared, shift, 1)
                        pb[rows, 128 * i:128 * (i + 1)] = jnp.where(top, mine, jnp.uint32(0))

    def fast_values(s, g, after_tile=None):
        nh = _heads_in_group(g)
        a_g = _group_row_start(g)
        pb = (p_buf0, p_buf1)[(s * NG + g) % 2]
        for j in range(QT - 1, -1, -1):
            n = 128 * (j + 1)
            cols = slice(128 * j, 128 * (j + 1))
            for i in range(nh):
                h = HPG * g + i
                a = (h * DH // 16) * 16
                off = h * DH - a
                p = pltpu.bitcast(pb[prow(P_OFFS[j] // 2, n // 2), 128 * i:128 * (i + 1)], BF16)
                ones_row = 0 if off > 0 else 31
                r32n = lax.broadcasted_iota(I32, (32, n), 0)
                lhs = jnp.where(r32n == ones_row, 1.0, vt_buf.load(s, a, a + 32, slice(0, n)).astype(F32)).astype(BF16)
                o = jnp.dot(lhs, p, preferred_element_type=F32)
                lo = (off // 8) * 8
                hi = -(-(off + DH) // 8) * 8
                gate = gate_buf[h:h + 1, :]
                rl = 1.0 / o[ones_row:ones_row + 1]
                val = (1.0 - gate) * (o[lo:hi] * rl)
                if s > 0:
                    z = _norm_row(g) + i
                    rden = 1.0 / (num_buf[g, z:z + 1, cols] + 1e-6)
                    num = num_buf[g, a - a_g + lo:a - a_g + hi, cols]
                    val = gate * (num * rden) + val
                ot_buf[a + off:a + off + DH, cols] = val[off - lo:off - lo + DH]
            if after_tile is not None:
                after_tile(j)

    def fast_path():
        hidden = []
        up = expert_up_stream(hidden)
        n_down = FF // 128
        state = dict(down=0, wd_ready=False, up_done=False, y=[None] * 2, tail=None)

        def finish():
            yield from expert_scatter_parts([jnp.sum(acc, axis=1, keepdims=True) for acc in state["y"]])
            for u in range(NSEG - 1):
                for j in range(QT):
                    cols = slice(128 * j, 128 * (j + 1))
                    val = base[u, :, cols]
                    val = paced(val)
                    val = (val + x_buf[u, :, cols].astype(F32)) + xn_buf.load(u, cols=cols).astype(F32)
                    out_buf[u, :, cols] = val.astype(BF16)
                    state["anchor"] = val
                    if j == QT - 1:
                        out_copy(u).start()
                    yield

        def anchor(q):
            val, state["anchor_next"], state["anchor"] = state["anchor_next"], state["anchor"], None
            return q if val is None else jnp.where(always[0][:, 0:128], q, val[D - q.shape[0]:D])

        def paced(val):
            y = state["pacer"]
            if y is None:
                return val
            reps = -(-D // y.shape[0])
            y = jnp.concatenate([y[:, 128 * r:128 * (r + 1)] for r in range(reps)], axis=0)[0:D]
            return jnp.where(always[0][:, 0:128], val, y)

        def down_step():
            ft = state["down"]
            w = paced(wd_buf[:, 128 * ft:128 * (ft + 1)].astype(F32))
            hh = hidden[ft // 4][:, 128 * (ft % 4):128 * (ft % 4 + 1)]
            for slot in range(2):
                term = w * hh[slot:slot + 1]
                state["y"][slot] = term if state["y"][slot] is None else state["y"][slot] + term
            if ft % 3 == 2:
                state["anchor"] = state["y"][1]
            state["down"] += 1

        def hook(long, pacer=None):
            state["pacer"] = pacer if pacer is not None and pacer.shape[0] * (pacer.shape[1] // 128) >= D else None
            if not state["up_done"] and next(up, "done") == "done":
                state["up_done"] = True
            if state["down"] < n_down:
                if state["wd_ready"] and state["pacer"] is not None and state["down"] // 4 < len(hidden):
                    down_step()
            elif state["out_ready"]:
                if state["tail"] is None:
                    state["tail"] = finish()
                if state["pacer"] is not None or state["tail_steps"] < 2:
                    state["tail_steps"] += 1
                    next(state["tail"], None)

        state["out_ready"] = False
        state["tail_steps"] = 0
        state["anchor"] = None
        state["anchor_next"] = None
        steps = [(s, g) for s in range(NSEG) for g in range(NG)]
        last = NSEG - 1

        def last_tile(j):
            cols = slice(128 * j, 128 * (j + 1))
            attn = jnp.dot(wot.load(), ot_buf[:, cols].astype(BF16), preferred_element_type=F32)
            out_buf[last, :, cols] = (base[last, :, cols] + residual(last, cols) + attn).astype(BF16)
            out_tile_copy(j).start()

        fast_scores(0, 0, hook, anchor)
        for t, (s, g) in enumerate(steps):
            if t + 1 < len(steps):
                fast_scores(*steps[t + 1], hook, anchor)
            if s > 0:
                memory_read(s, g)
                hook(True)
            if t + 1 == len(steps):
                state["pacer"] = None
                assert state["down"] == n_down and state["tail"] is not None
                while next(state["tail"], "done") != "done":
                    pass
                pending = []

                def after_tile(j):
                    if pending:
                        last_tile(pending.pop())
                    pending.append(j)

                fast_values(s, g, after_tile)
                last_tile(pending.pop())
            else:
                fast_values(s, g)
            if s == 0:
                transpose_wo(g)
            if s + 1 < NSEG:
                memory_update(s, g)
                hook(True)
            if g == NG - 1 and s < last:
                base[s] = project_out(s)
                if s == 0:
                    cp_wd.wait()
                    state["wd_ready"] = True
                if s == last - 1:
                    state["out_ready"] = True
                hook(True)
        for u in range(NSEG - 1):
            out_copy(u).wait()
        for j in range(QT):
            out_tile_copy(j).wait()

    def slow_segment(s, carry):
        for g in range(NG):
            memory_read(s, g)
        key_i = lax.broadcasted_iota(I32, (L, L), 0)
        qry_i = lax.broadcasted_iota(I32, (L, L), 1)
        r32 = lax.broadcasted_iota(I32, (32, L), 0)
        for g in range(NG):
            gw = GW[g]
            a_g = _group_row_start(g)
            rowg = lax.broadcasted_iota(I32, (gw, L), 0)

            def head(i, c, g=g, gw=gw, a_g=a_g, rowg=rowg):
                h = HPG * g + i
                a = pl.multiple_of((h * DH // 16) * 16, 16)
                off = h * DH - a
                q = qs_buf.load(s, 128 * g, 128 * g + gw).astype(F32)
                qm = jnp.where((rowg >= DH * i) & (rowg < DH * (i + 1)), q, 0.0).astype(BF16)
                st = jnp.dot(k_buf.load(s * NG + g, cols=slice(0, gw)), qm, preferred_element_type=F32)
                st = jnp.where(key_i <= qry_i, st, NEG_BIG)
                p = jnp.exp2(st - jnp.max(st, axis=0, keepdims=True))
                rl = 1.0 / jnp.sum(p, axis=0, keepdims=True)
                o = jnp.dot(vt_buf.load(s, a, 32), p.astype(BF16), preferred_element_type=F32)
                gate = jnp.concatenate([gate_buf[pl.ds(h, 1), :]] * QT, axis=1)
                rden = 1.0 / (num_buf[g, pl.ds(_norm_row(g) + i, 1), :] + 1e-6)
                num = num_buf[g, pl.ds(pl.multiple_of(a - a_g, 16), 32), :]
                val = gate * (num * rden) + (1.0 - gate) * (o * rl)
                keep = (r32 >= off) & (r32 < off + DH)
                pltpu.store(ot_buf.at[pl.ds(a, 32), :], val, mask=keep)
                return c

            lax.fori_loop(0, _heads_in_group(g), head, 0)
        for g in range(NG):
            memory_update(s, g)
        emit(s, base[s] + residual(s) + project_out(s))
        return carry

    @pl.when(safe)
    def _():
        fast_path()

    @pl.when(jnp.logical_not(safe))
    def _():
        cp_wd.wait()
        for u in range(NSEG - 1):
            base[u] = jnp.zeros((D, L), F32)
        for g in range(NG):
            transpose_wo(g)
        expert_scatter_rows(expert_chunk(0, FF))
        lax.fori_loop(0, NSEG, slow_segment, 0)
        for u in range(NSEG):
            out_copy(u).wait()


@jax.jit
def pallas_parallel_sum__memory_aug_infini_attn__moe_arch_mod__prompt_kernel(
    A_x: jax.Array,
    A_wq: jax.Array,
    A_wk: jax.Array,
    A_wv: jax.Array,
    A_wo: jax.Array,
    A_beta: jax.Array,
    B_x: jax.Array,
    B_w_r: jax.Array,
    B_w_gate: jax.Array,
    B_w_up: jax.Array,
    B_w_down: jax.Array,
):
    del B_x
    hbm = pl.BlockSpec(memory_space=pl.ANY)
    scratch = [
        pltpu.VMEM((NSEG, D, L), BF16),
        pltpu.VMEM((D, D), BF16),
        pltpu.VMEM((D, D), BF16),
        pltpu.VMEM((D, D), BF16),
        pltpu.VMEM((D, D), BF16),
        pltpu.VMEM((H,), BF16),
        pltpu.VMEM((D,), BF16),
        pltpu.VMEM((D, FF), BF16),
        pltpu.VMEM((D, FF), BF16),
        pltpu.VMEM((D, FF), BF16),
        pltpu.VMEM((PR // 2, D), U32),
        pltpu.VMEM((PR // 2, D), U32),
        pltpu.VMEM((D // 2, D), U32),
        pltpu.VMEM((D // 2, D), U32),
        pltpu.VMEM((NSEG * D // 2, L), U32),
        pltpu.VMEM((NSEG, D, L), F32),
        pltpu.VMEM((NSEG * PR // 2, L), U32),
        pltpu.VMEM((NSEG * PR // 2, L), U32),
        pltpu.VMEM((NSEG * NG * L // 2, 128), U32),
        pltpu.VMEM((NSEG * PR // 2, L), U32),
        pltpu.VMEM((NSEG * D // 2, L), U32),
        pltpu.VMEM((8, S), F32),
        pltpu.VMEM((H, 128), F32),
        pltpu.VMEM((NG, MROWS, 128), F32),
        pltpu.VMEM((NG, MROWS, L), F32),
        pltpu.VMEM((640, HPG * 128), U32),
        pltpu.VMEM((640, HPG * 128), U32),
        pltpu.VMEM((D, L), F32),
        pltpu.VMEM((NSEG, D, L), BF16),
        pltpu.SemaphoreType.DMA((13,)),
        pltpu.SemaphoreType.DMA((NSEG + QT,)),
    ]
    out_t = pl.pallas_call(
        _kernel,
        out_shape=jax.ShapeDtypeStruct((1, D, S), BF16),
        in_specs=[hbm] * 10,
        out_specs=hbm,
        scratch_shapes=scratch,
        compiler_params=pltpu.CompilerParams(vmem_limit_bytes=128 * 1024 * 1024),
        name="infini_attn_moe",
    )(jnp.transpose(A_x, (0, 2, 1)), A_wq, A_wk, A_wv, A_wo, A_beta, B_w_r, B_w_gate, B_w_up,
      B_w_down.T)
    return jnp.transpose(out_t, (0, 2, 1))
```

```python
import jax
import jax.numpy as jnp
from jax import lax
import jax.experimental.pallas as pl
import jax.experimental.pallas.tpu as pltpu

F32 = jnp.float32
BF16 = jnp.bfloat16
U32 = jnp.uint32
I32 = jnp.int32

S = 2048
D = 576
H = 32
DH = 18
NSEG = 4
L = 512
FF = 4608
HPG = 7
NG = 5
QT = L // 128
GW = (128, 128, 128, 128, 80)
PR = sum(GW)
ROUTER_ROW = 126
MROWS = 144
LOG2E = 1.4426950408889634
QSCALE = (DH ** -0.5) * LOG2E
SAFE_LOG2_RANGE = 60.0
NEG_BIG = -1e30

NT_DIMS = (((1,), (1,)), ((), ()))


def _heads_in_group(g):
    return min(HPG, H - HPG * g)


def _group_row_start(g):
    return (HPG * g * DH // 16) * 16


def _group_rows(g):
    last = (HPG * g + _heads_in_group(g)) * DH
    return -(-(last - _group_row_start(g)) // 16) * 16


def _state_rows(g):
    return MROWS if g == 0 else _group_rows(g)


def _norm_row(g):
    return 128 if g == 0 else 0


def _round_bf16(x):
    return x.astype(BF16).astype(F32)


def _pad_heads_t(w):
    parts = []
    for g in range(NG):
        n = _heads_in_group(g) * DH
        parts.append(w[:, HPG * DH * g:HPG * DH * g + n])
        parts.append(jnp.zeros((D, 128 - n), w.dtype))
    return jnp.concatenate(parts, axis=1).T[0:PR]


def _phi(t):
    return jnp.where(t > 0, t + 1.0, jnp.exp(t))


class _Packed:
    def __init__(self, ref, rows):
        self.ref = ref
        self.rows = rows

    def _slice(self, item, lo, size):
        start = item * (self.rows // 2) + lo // 2
        size = size // 2
        if isinstance(start, int):
            return slice(start, start + size)
        return pl.ds(pl.multiple_of(start, 8), size)

    def load(self, item=0, lo=0, hi=None, cols=slice(None)):
        size = hi if not isinstance(lo, int) else (self.rows if hi is None else hi) - lo
        return pltpu.bitcast(self.ref[self._slice(item, lo, size), cols], BF16)

    def store(self, val, item=0, lo=0, cols=slice(None)):
        self.ref[self._slice(item, lo, val.shape[0]), cols] = pltpu.bitcast(val.astype(BF16), U32)


def _kernel(x_hbm, wq_hbm, wk_hbm, wv_hbm, wo_hbm, beta_hbm, wr_hbm, wg_hbm, wu_hbm, wd_hbm,
            out_hbm,
            x_buf, wq_raw, wk_raw, wv_raw, wo_raw, beta_buf, wr_buf, wg_buf, wu_buf, wd_buf,
            wqt, wkt, wvt, wot, xn_buf, base, qs_buf, pq_buf, k_buf, pk_buf, vt_buf, r_buf,
            gate_buf, mt_buf, num_buf, p_buf0, p_buf1, ot_buf, out_buf, in_sems, out_sems):
    wqt, wkt = _Packed(wqt, PR), _Packed(wkt, PR)
    wvt, wot = _Packed(wvt, D), _Packed(wot, D)
    xn_buf, vt_buf = _Packed(xn_buf, D), _Packed(vt_buf, D)
    qs_buf, pq_buf, pk_buf = _Packed(qs_buf, PR), _Packed(pq_buf, PR), _Packed(pk_buf, PR)
    k_buf = _Packed(k_buf, L)

    def x_copy(c):
        return pltpu.make_async_copy(x_hbm.at[0, :, pl.ds(c * L, L)], x_buf.at[c], in_sems.at[c])

    cp_wv = pltpu.make_async_copy(wv_hbm, wv_raw, in_sems.at[4])
    cp_wq = pltpu.make_async_copy(wq_hbm, wq_raw, in_sems.at[5])
    cp_wk = pltpu.make_async_copy(wk_hbm, wk_raw, in_sems.at[6])
    cp_wo = pltpu.make_async_copy(wo_hbm, wo_raw, in_sems.at[7])
    cp_wg = pltpu.make_async_copy(wg_hbm, wg_buf, in_sems.at[8])
    cp_wu = pltpu.make_async_copy(wu_hbm, wu_buf, in_sems.at[9])
    cp_wd = pltpu.make_async_copy(wd_hbm, wd_buf, in_sems.at[10])
    cp_beta = pltpu.make_async_copy(beta_hbm, beta_buf, in_sems.at[11])
    cp_wr = pltpu.make_async_copy(wr_hbm, wr_buf, in_sems.at[12])

    def out_copy(s):
        cols = pl.ds(pl.multiple_of(s * L, L), L)
        return pltpu.make_async_copy(out_buf.at[s], out_hbm.at[0, :, cols], out_sems.at[s])

    def out_tile_copy(j):
        s = NSEG - 1
        return pltpu.make_async_copy(out_buf.at[s, :, pl.ds(128 * j, 128)],
                                     out_hbm.at[0, :, pl.ds(s * L + 128 * j, 128)], out_sems.at[NSEG + j])


    for cp in (x_copy(0), cp_wv, x_copy(1), cp_wq, cp_wr, cp_beta, x_copy(2), cp_wk, x_copy(3), cp_wo,
               cp_wg, cp_wu, cp_wd):
        cp.start()

    lane128 = lax.broadcasted_iota(I32, (128, 128), 1)
    row128 = lax.broadcasted_iota(I32, (128, 128), 0)
    causal = row128 <= lane128
    r16 = lax.broadcasted_iota(I32, (16, D), 0)

    mt_buf[...] = jnp.zeros(mt_buf.shape, F32)

    always = []

    def pace(x, y):
        return x if y is None else jnp.where(always[0], x, y[0:D])

    def ln_stats(c, y):
        shift = x_buf[c, 0:16, :].astype(F32)[0:1]
        d = pace(x_buf[c].astype(F32), y) - shift
        m1 = jnp.sum(d, axis=0, keepdims=True) * (1.0 / D)
        m2 = jnp.sum(d * d, axis=0, keepdims=True) * (1.0 / D)
        var = jnp.maximum(m2 - m1 * m1, 0.0)
        inv = 1.0 / _round_bf16(jnp.sqrt(_round_bf16(_round_bf16(var) + 1e-5)))
        return _round_bf16(shift + m1), inv

    def ln_apply(c, mean_b, inv):
        x = x_buf[c].astype(F32)
        xn = (x - mean_b) * inv
        xn_buf.store(xn, c)
        if c == NSEG - 1:
            base[c] = jnp.zeros((D, L), F32)

    def project(w_ref, c, split):
        if not split:
            return jnp.dot(w_ref.load(), xn_buf.load(c), preferred_element_type=F32), None
        head = jnp.dot(w_ref.load(cols=slice(0, 256)), xn_buf.load(c, 0, 256), preferred_element_type=F32)
        tail = jnp.dot(w_ref.load(cols=slice(256, D)), xn_buf.load(c, 256, D), preferred_element_type=F32)
        return head + tail, head

    def project_v(c, mid=None):
        vt, head = project(wvt, c, mid is not None)
        if mid is not None:
            mid(head)
        vt_buf.store(vt, c)
        return vt

    def project_q(c, mid=None):
        qt, head = project(wqt, c, mid is not None)
        if mid is not None:
            mid(head)
        qsc = qt * QSCALE
        qs_buf.store(qsc, c)
        pq_buf.store(_phi(qt), c)
        r_buf[:, c * L:(c + 1) * L] = qt[120:128]
        mag = jnp.abs(qsc)
        r8 = lax.broadcasted_iota(I32, (8, L), 0)
        mag = jnp.concatenate([mag[0:120], jnp.where(r8 == ROUTER_ROW - 120, 0.0, mag[120:128]), mag[128:]], axis=0)
        return qt, jnp.max(mag.reshape(PR // 8, 8, L), axis=0)

    def project_k(c, mid=None, keep=False):
        kt, head = project(wkt, c, mid is not None)
        if mid is not None:
            mid(head)
        pk_buf.store(_phi(kt), c)
        for g in range(NG):
            ktg = kt[128 * g:128 * g + GW[g]]
            if GW[g] < 128:
                ktg = jnp.concatenate([ktg, jnp.zeros((128 - GW[g], L), F32)], axis=0)
            k_buf.store(ktg.T, c * NG + g)
        top = jnp.max(jnp.abs(kt).reshape(PR // 8, 8, L), axis=0)
        return (kt, top) if keep else top

    x_copy(0).wait()
    stats = ln_stats(0, None)
    always.append(jnp.logical_not(jnp.abs(stats[0]) < 0.0))
    ln_apply(0, *stats)
    cp_wv.wait()
    wvt.store(wv_raw[...].T)
    project_v(0)
    x_copy(1).wait()
    cp_wq.wait()
    cp_wr.wait()
    ln_apply(1, *ln_stats(1, None))

    def paced_weight(w_ref, y):
        w = w_ref[...].astype(F32)
        return jnp.concatenate([jnp.where(always[0], w[:, 0:L], y[0:D]), w[:, L:D]], axis=1)

    def prep_wq(y):
        wq_t = _pad_heads_t(paced_weight(wq_raw, y))
        wr_row = wr_buf[...].reshape(1, D).astype(F32)
        pr_row = lax.broadcasted_iota(I32, (8, D), 0)
        wq_t = jnp.concatenate(
            [wq_t[0:120], jnp.where(pr_row == ROUTER_ROW - 120, wr_row, wq_t[120:128]), wq_t[128:]], axis=0)
        wqt.store(wq_t)

    project_v(1, prep_wq)
    cp_wk.wait()
    cp_beta.wait()
    x_copy(2).wait()
    x_copy(3).wait()

    beta_row = beta_buf[...].reshape(1, H).astype(F32)
    beta_row = jnp.concatenate([beta_row, jnp.zeros((1, 128 - H), F32)], axis=1)
    h_row = lax.broadcasted_iota(I32, (H, 128), 0)
    h_lane = lax.broadcasted_iota(I32, (H, 128), 1)
    beta_col = jnp.sum(jnp.where(h_row == h_lane, beta_row, 0.0), axis=1, keepdims=True)
    gate_buf[...] = jnp.broadcast_to(jax.nn.sigmoid(beta_col), (H, 128))

    def prep_wk(y):
        wkt.store(_pad_heads_t(paced_weight(wk_raw, y)))

    def route():
        r = _round_bf16(r_buf[ROUTER_ROW - 120:ROUTER_ROW - 119, :])
        tok = lax.broadcasted_iota(I32, (1, S), 1).astype(F32)
        m1 = jnp.max(r)
        i1 = jnp.min(jnp.where(r == m1, tok, float(S)))
        r_rest = jnp.where(tok == i1, -jnp.inf, r)
        m2 = jnp.max(r_rest)
        i2 = jnp.min(jnp.where(r_rest == m2, tok, float(S)))
        i1 = jnp.clip(i1.astype(I32), 0, S - 1)
        i2 = jnp.clip(i2.astype(I32), 0, S - 1)
        return m1, m2, i1, i2

    qt, aq = project_q(0, prep_wk)
    qt, a = project_q(1)
    aq = jnp.maximum(aq, a)
    stats = ln_stats(2, qt)
    ak = project_k(0)
    ln_apply(2, *stats)
    kt, a = project_k(1, keep=True)
    ak = jnp.maximum(ak, a)
    stats = ln_stats(3, kt)
    project_v(2)
    ln_apply(3, *stats)
    qt, a = project_q(2)
    aq = jnp.maximum(aq, a)
    ak = jnp.maximum(ak, project_k(2))
    qt, a = project_q(3)
    aq = jnp.maximum(aq, a)
    m1, m2, i1, i2 = route()
    ak = jnp.maximum(ak, project_k(3))
    project_v(3)

    logit_bound = jnp.max(aq) * jnp.max(ak) * (DH * 1.02)
    safe = logit_bound <= SAFE_LOG2_RANGE

    sel_row = lax.broadcasted_iota(I32, (16, 128), 0)
    sel_lane = lax.broadcasted_iota(I32, (16, 128), 1)

    def token_tile(i):
        return i // L, pl.ds(pl.multiple_of(((i % L) // 128) * 128, 128), 128)

    def pick(i, slot):
        seg, cols = token_tile(i)
        onehot = jnp.where((sel_row == slot) & (sel_lane == i % 128), 1.0, 0.0).astype(BF16)
        return lax.dot_general(onehot, xn_buf.load(seg, cols=cols), NT_DIMS, preferred_element_type=F32)

    def routed_rows():
        return (pick(i1, 0) + pick(i2, 1)).astype(BF16)

    cp_wo.wait()
    cp_wg.wait()
    cp_wu.wait()


    def expert_chunk(lo, hi):
        xs = routed_rows()
        hg = jnp.dot(xs, wg_buf[:, lo:hi], preferred_element_type=F32)
        hu = jnp.dot(xs, wu_buf[:, lo:hi], preferred_element_type=F32)
        hh = (jax.nn.silu(hg) * hu).astype(BF16)
        return lax.dot_general(hh, wd_buf[:, lo:hi], NT_DIMS, preferred_element_type=F32)

    def expert_up_stream(hidden):
        kmain = 512
        xs = routed_rows()
        tail = xs[:, kmain:D].astype(F32)
        zero = jnp.zeros_like(tail)
        r16k = lax.broadcasted_iota(I32, (16, 128), 0)
        xs_rem = jnp.where(r16k < 2, jnp.concatenate([tail, zero], axis=1),
                           pltpu.roll(jnp.concatenate([zero, tail], axis=1), 2, 0)).astype(BF16)
        yield
        for c0 in range(0, FF, 512):
            w_rem = jnp.concatenate([wg_buf[kmain:D, c0:c0 + 512], wu_buf[kmain:D, c0:c0 + 512]], axis=0)
            both = jnp.dot(xs_rem, w_rem, preferred_element_type=F32)
            rem = (both, pltpu.roll(both, 14, 0))
            yield
            hs = []
            for f0 in range(c0, c0 + 512, 128):
                pre = []
                for w_ref, r in zip((wg_buf, wu_buf), rem):
                    pre.append(jnp.dot(xs[:, 0:kmain], w_ref[0:kmain, f0:f0 + 128], preferred_element_type=F32)
                               + r[:, f0 - c0:f0 - c0 + 128])
                    if len(pre) == 2:
                        hs.append(jax.nn.silu(pre[0]) * pre[1])
                        if len(hs) == 4:
                            hidden.append(_round_bf16(jnp.concatenate(hs, axis=1)))
                    yield

    lane_d = lax.broadcasted_iota(I32, (D, 128), 1)

    def expert_scatter_parts(columns):
        for col, i, score in zip(columns, (i1, i2), (m1, m2)):
            seg, cols = token_tile(i)
            col = col * jax.nn.sigmoid(jnp.full((D, 1), score, F32))
            base[seg, :, cols] = base[seg, :, cols] + jnp.where(lane_d == i % 128, col, 0.0)
            yield

    def expert_scatter_rows(y):
        yt = jnp.concatenate([y, jnp.zeros((128 - 16, D), F32)], axis=0).T
        columns = [jnp.sum(jnp.where(lane_d == slot, yt, 0.0), axis=1, keepdims=True) for slot in range(2)]
        for _ in expert_scatter_parts(columns):
            pass

    def memory_read(s, g):
        sr = _state_rows(g)
        gw = GW[g]
        num_buf[g, 0:sr, :] = jnp.dot(mt_buf[g, 0:sr, 0:gw].astype(BF16), pq_buf.load(s, 128 * g, 128 * g + gw),
                                      preferred_element_type=F32)

    def memory_update(s, g):
        rg = _group_rows(g)
        a_g = _group_row_start(g)
        gw = GW[g]
        ones_row = 126 if g == 0 else 0
        lhs = jnp.where(lax.broadcasted_iota(I32, (rg, L), 0) == ones_row, 1.0,
                        vt_buf.load(s, a_g, a_g + rg).astype(F32)).astype(BF16)
        upd = lax.dot_general(lhs, pk_buf.load(s, 128 * g, 128 * g + gw), NT_DIMS,
                              preferred_element_type=F32)
        er = lax.broadcasted_iota(I32, (rg, gw), 0) + (a_g - HPG * DH * g)
        el = lax.broadcasted_iota(I32, (rg, gw), 1)
        same_head = None
        for i in range(_heads_in_group(g)):
            t = ((er >= DH * i) & (er < DH * (i + 1)) & (el >= DH * i) & (el < DH * (i + 1)))
            same_head = t if same_head is None else (same_head | t)
        mt_buf[g, 0:rg, 0:gw] = mt_buf[g, 0:rg, 0:gw] + jnp.where(same_head, upd, 0.0)
        zr = lax.broadcasted_iota(I32, (8, gw), 0)
        zl = lax.broadcasted_iota(I32, (8, gw), 1)
        zmask = (zl >= zr * DH) & (zl < zr * DH + DH) & (zr < _heads_in_group(g))
        zs = upd[ones_row:ones_row + 1]
        z0 = _norm_row(g)
        mt_buf[g, z0:z0 + 8, 0:gw] = mt_buf[g, z0:z0 + 8, 0:gw] + jnp.where(zmask, zs, 0.0)

    def transpose_wo(g):
        hi = min(128 * (g + 1), D)
        wot.store(wo_raw[:, 128 * g:hi].T, lo=128 * g)

    def project_out(s):
        return jnp.dot(wot.load(), ot_buf[...].astype(BF16), preferred_element_type=F32)

    def residual(s, cols=slice(None)):
        return x_buf[s, :, cols].astype(F32) + xn_buf.load(s, cols=cols).astype(F32)

    def emit(s, val):
        out_buf[s] = val.astype(BF16)
        out_copy(s).start()

    zero = lax.shift_right_logical(i1, 16)

    def prow(start, size):
        return pl.ds(pl.multiple_of(zero + start, 8), size)

    P_OFFS = (0, 128, 384, 768)

    def fast_scores(s, g, hook, anchor):
        nh = _heads_in_group(g)
        gw = GW[g]
        pb = (p_buf0, p_buf1)[(s * NG + g) % 2]
        rowg = lax.broadcasted_iota(I32, (gw, 128), 0)
        laneg = lax.broadcasted_iota(I32, (gw, 128), 1)
        head_rows = [(rowg >= DH * i) & (rowg < DH * (i + 1)) for i in range(nh)]
        row64 = lax.broadcasted_iota(I32, (64, 128), 0)
        lane64 = lax.broadcasted_iota(I32, (64, 128), 1)
        visible_lo = row64 <= lane64
        row32 = lax.broadcasted_iota(I32, (32, 128), 0)
        lane32 = lax.broadcasted_iota(I32, (32, 128), 1)
        lane16 = lax.broadcasted_iota(I32, (16, 128), 1)
        for j in range(QT - 1, -1, -1):
            n = 128 * (j + 1)
            m = n - 64
            q = qs_buf.load(s, 128 * g, 128 * g + gw, slice(128 * j, 128 * (j + 1))).astype(F32)
            for h0, h1 in (((0, 3), (3, nh)) if nh == 7 else ((0, 4),)):
                if h1 <= h0:
                    continue
                q_in = anchor(q)
                qm = jnp.concatenate([jnp.where(head_rows[i], q_in, 0.0) for i in range(h0, h1)],
                                     axis=1).astype(BF16)
                st = jnp.dot(k_buf.load(s * NG + g, 0, m, slice(0, gw)), qm, preferred_element_type=F32)
                p = jnp.exp2(st)
                p_diag = jnp.where(jnp.concatenate([visible_lo] * (h1 - h0), axis=1), p[m - 64:], 0.0)
                p = jnp.concatenate([p[:m - 64], p_diag], axis=0) if j > 0 else p_diag
                pb[P_OFFS[j] // 2:(P_OFFS[j] + m) // 2, h0 * 128:h1 * 128] = pltpu.bitcast(p.astype(BF16), U32)
                hook(j >= 2, p)
            for width, k0 in ((64, m), (32, m + 32)):
                per = 128 // width
                q_top = q
                for t in range(per - 1):
                    q_top = jnp.where((laneg >= width * t) & (laneg < width * (t + 1)),
                                      pltpu.roll(q, width * (t + 1), 1), q_top)
                groups = [list(range(i, min(i + per, nh))) for i in range(0, nh, per)]
                tiles = []
                for heads in groups:
                    keep = None
                    for t, i in enumerate(heads):
                        slot = per - len(heads) + t
                        sel = head_rows[i] & (laneg >= width * slot) & (laneg < width * (slot + 1))
                        keep = sel if keep is None else (keep | sel)
                    tiles.append(jnp.where(keep, q_top, 0.0))
                st = jnp.dot(k_buf.load(s * NG + g, k0, k0 + 32, slice(0, gw)),
                             jnp.concatenate(tiles, axis=1).astype(BF16),
                             preferred_element_type=F32)
                visible = row32 + (k0 - m) <= (lane32 & (width - 1)) + (64 - width)
                p = jnp.where(jnp.concatenate([visible] * len(groups), axis=1), jnp.exp2(st), 0.0)
                p = pltpu.bitcast(p.astype(BF16), U32)
                rows = slice((P_OFFS[j] + k0) // 2, (P_OFFS[j] + k0 + 32) // 2)
                top = lane16 >= 128 - width
                for gi, heads in enumerate(groups):
                    shared = p[:, 128 * gi:128 * (gi + 1)]
                    for t, i in enumerate(heads):
                        slot = per - len(heads) + t
                        shift = width * (per - 1 - slot)
                        mine = shared if shift == 0 else pltpu.roll(shared, shift, 1)
                        pb[rows, 128 * i:128 * (i + 1)] = jnp.where(top, mine, jnp.uint32(0))

    def fast_values(s, g, after_tile=None):
        nh = _heads_in_group(g)
        a_g = _group_row_start(g)
        pb = (p_buf0, p_buf1)[(s * NG + g) % 2]
        for j in range(QT - 1, -1, -1):
            n = 128 * (j + 1)
            cols = slice(128 * j, 128 * (j + 1))
            for i in range(nh):
                h = HPG * g + i
                a = (h * DH // 16) * 16
                off = h * DH - a
                p = pltpu.bitcast(pb[prow(P_OFFS[j] // 2, n // 2), 128 * i:128 * (i + 1)], BF16)
                ones_row = 0 if off > 0 else 31
                r32n = lax.broadcasted_iota(I32, (32, n), 0)
                lhs = jnp.where(r32n == ones_row, 1.0, vt_buf.load(s, a, a + 32, slice(0, n)).astype(F32)).astype(BF16)
                o = jnp.dot(lhs, p, preferred_element_type=F32)
                lo = (off // 8) * 8
                hi = -(-(off + DH) // 8) * 8
                gate = gate_buf[h:h + 1, :]
                rl = 1.0 / o[ones_row:ones_row + 1]
                val = (1.0 - gate) * (o[lo:hi] * rl)
                if s > 0:
                    z = _norm_row(g) + i
                    rden = 1.0 / (num_buf[g, z:z + 1, cols] + 1e-6)
                    num = num_buf[g, a - a_g + lo:a - a_g + hi, cols]
                    val = gate * (num * rden) + val
                ot_buf[a + off:a + off + DH, cols] = val[off - lo:off - lo + DH]
            if after_tile is not None:
                after_tile(j)

    def fast_path():
        hidden = []
        up = expert_up_stream(hidden)
        n_down = FF // 128
        state = dict(down=0, wd_ready=False, up_done=False, y=[None] * 2, tail=None)

        def finish():
            yield from expert_scatter_parts([jnp.sum(acc, axis=1, keepdims=True) for acc in state["y"]])
            for u in range(NSEG - 1):
                for j in range(QT):
                    cols = slice(128 * j, 128 * (j + 1))
                    val = base[u, :, cols]
                    val = paced(val)
                    val = (val + x_buf[u, :, cols].astype(F32)) + xn_buf.load(u, cols=cols).astype(F32)
                    out_buf[u, :, cols] = val.astype(BF16)
                    state["anchor"] = val
                    if j == QT - 1:
                        out_copy(u).start()
                    yield

        def anchor(q):
            val, state["anchor_next"], state["anchor"] = state["anchor_next"], state["anchor"], None
            return q if val is None else jnp.where(always[0][:, 0:128], q, val[D - q.shape[0]:D])

        def paced(val):
            y = state["pacer"]
            if y is None:
                return val
            reps = -(-D // y.shape[0])
            y = jnp.concatenate([y[:, 128 * r:128 * (r + 1)] for r in range(reps)], axis=0)[0:D]
            return jnp.where(always[0][:, 0:128], val, y)

        def down_step():
            ft = state["down"]
            w = paced(wd_buf[:, 128 * ft:128 * (ft + 1)].astype(F32))
            hh = hidden[ft // 4][:, 128 * (ft % 4):128 * (ft % 4 + 1)]
            for slot in range(2):
                term = w * hh[slot:slot + 1]
                state["y"][slot] = term if state["y"][slot] is None else state["y"][slot] + term
            if ft % 6 == 5:
                state["anchor"] = state["y"][1]
            state["down"] += 1

        def hook(long, pacer=None):
            state["pacer"] = pacer if pacer is not None and pacer.shape[0] * (pacer.shape[1] // 128) >= D else None
            if not state["up_done"] and next(up, "done") == "done":
                state["up_done"] = True
            if state["down"] < n_down:
                if state["wd_ready"] and state["pacer"] is not None and state["down"] // 4 < len(hidden):
                    down_step()
            elif state["out_ready"]:
                if state["tail"] is None:
                    state["tail"] = finish()
                if state["pacer"] is not None or state["tail_steps"] < 2:
                    state["tail_steps"] += 1
                    next(state["tail"], None)

        state["out_ready"] = False
        state["tail_steps"] = 0
        state["anchor"] = None
        state["anchor_next"] = None
        steps = [(s, g) for s in range(NSEG) for g in range(NG)]
        last = NSEG - 1

        def last_tile(j):
            cols = slice(128 * j, 128 * (j + 1))
            attn = jnp.dot(wot.load(), ot_buf[:, cols].astype(BF16), preferred_element_type=F32)
            out_buf[last, :, cols] = (base[last, :, cols] + residual(last, cols) + attn).astype(BF16)
            out_tile_copy(j).start()

        fast_scores(0, 0, hook, anchor)
        for t, (s, g) in enumerate(steps):
            if t + 1 < len(steps):
                fast_scores(*steps[t + 1], hook, anchor)
            if s > 0:
                memory_read(s, g)
                hook(True)
            if t + 1 == len(steps):
                state["pacer"] = None
                assert state["down"] == n_down and state["tail"] is not None
                while next(state["tail"], "done") != "done":
                    pass
                pending = []

                def after_tile(j):
                    if pending:
                        last_tile(pending.pop())
                    pending.append(j)

                fast_values(s, g, after_tile)
                last_tile(pending.pop())
            else:
                fast_values(s, g)
            if s == 0:
                transpose_wo(g)
            if s + 1 < NSEG:
                memory_update(s, g)
                hook(True)
            if g == NG - 1 and s < last:
                base[s] = project_out(s)
                if s == 0:
                    cp_wd.wait()
                    state["wd_ready"] = True
                if s == last - 1:
                    state["out_ready"] = True
                hook(True)
        for u in range(NSEG - 1):
            out_copy(u).wait()
        for j in range(QT):
            out_tile_copy(j).wait()

    def slow_segment(s, carry):
        for g in range(NG):
            memory_read(s, g)
        key_i = lax.broadcasted_iota(I32, (L, L), 0)
        qry_i = lax.broadcasted_iota(I32, (L, L), 1)
        r32 = lax.broadcasted_iota(I32, (32, L), 0)
        for g in range(NG):
            gw = GW[g]
            a_g = _group_row_start(g)
            rowg = lax.broadcasted_iota(I32, (gw, L), 0)

            def head(i, c, g=g, gw=gw, a_g=a_g, rowg=rowg):
                h = HPG * g + i
                a = pl.multiple_of((h * DH // 16) * 16, 16)
                off = h * DH - a
                q = qs_buf.load(s, 128 * g, 128 * g + gw).astype(F32)
                qm = jnp.where((rowg >= DH * i) & (rowg < DH * (i + 1)), q, 0.0).astype(BF16)
                st = jnp.dot(k_buf.load(s * NG + g, cols=slice(0, gw)), qm, preferred_element_type=F32)
                st = jnp.where(key_i <= qry_i, st, NEG_BIG)
                p = jnp.exp2(st - jnp.max(st, axis=0, keepdims=True))
                rl = 1.0 / jnp.sum(p, axis=0, keepdims=True)
                o = jnp.dot(vt_buf.load(s, a, 32), p.astype(BF16), preferred_element_type=F32)
                gate = jnp.concatenate([gate_buf[pl.ds(h, 1), :]] * QT, axis=1)
                rden = 1.0 / (num_buf[g, pl.ds(_norm_row(g) + i, 1), :] + 1e-6)
                num = num_buf[g, pl.ds(pl.multiple_of(a - a_g, 16), 32), :]
                val = gate * (num * rden) + (1.0 - gate) * (o * rl)
                keep = (r32 >= off) & (r32 < off + DH)
                pltpu.store(ot_buf.at[pl.ds(a, 32), :], val, mask=keep)
                return c

            lax.fori_loop(0, _heads_in_group(g), head, 0)
        for g in range(NG):
            memory_update(s, g)
        emit(s, base[s] + residual(s) + project_out(s))
        return carry

    @pl.when(safe)
    def _():
        fast_path()

    @pl.when(jnp.logical_not(safe))
    def _():
        cp_wd.wait()
        for u in range(NSEG - 1):
            base[u] = jnp.zeros((D, L), F32)
        for g in range(NG):
            transpose_wo(g)
        expert_scatter_rows(expert_chunk(0, FF))
        lax.fori_loop(0, NSEG, slow_segment, 0)
        for u in range(NSEG):
            out_copy(u).wait()


@jax.jit
def pallas_parallel_sum__memory_aug_infini_attn__moe_arch_mod__prompt_kernel(
    A_x: jax.Array,
    A_wq: jax.Array,
    A_wk: jax.Array,
    A_wv: jax.Array,
    A_wo: jax.Array,
    A_beta: jax.Array,
    B_x: jax.Array,
    B_w_r: jax.Array,
    B_w_gate: jax.Array,
    B_w_up: jax.Array,
    B_w_down: jax.Array,
):
    del B_x
    hbm = pl.BlockSpec(memory_space=pl.ANY)
    scratch = [
        pltpu.VMEM((NSEG, D, L), BF16),
        pltpu.VMEM((D, D), BF16),
        pltpu.VMEM((D, D), BF16),
        pltpu.VMEM((D, D), BF16),
        pltpu.VMEM((D, D), BF16),
        pltpu.VMEM((H,), BF16),
        pltpu.VMEM((D,), BF16),
        pltpu.VMEM((D, FF), BF16),
        pltpu.VMEM((D, FF), BF16),
        pltpu.VMEM((D, FF), BF16),
        pltpu.VMEM((PR // 2, D), U32),
        pltpu.VMEM((PR // 2, D), U32),
        pltpu.VMEM((D // 2, D), U32),
        pltpu.VMEM((D // 2, D), U32),
        pltpu.VMEM((NSEG * D // 2, L), U32),
        pltpu.VMEM((NSEG, D, L), F32),
        pltpu.VMEM((NSEG * PR // 2, L), U32),
        pltpu.VMEM((NSEG * PR // 2, L), U32),
        pltpu.VMEM((NSEG * NG * L // 2, 128), U32),
        pltpu.VMEM((NSEG * PR // 2, L), U32),
        pltpu.VMEM((NSEG * D // 2, L), U32),
        pltpu.VMEM((8, S), F32),
        pltpu.VMEM((H, 128), F32),
        pltpu.VMEM((NG, MROWS, 128), F32),
        pltpu.VMEM((NG, MROWS, L), F32),
        pltpu.VMEM((640, HPG * 128), U32),
        pltpu.VMEM((640, HPG * 128), U32),
        pltpu.VMEM((D, L), F32),
        pltpu.VMEM((NSEG, D, L), BF16),
        pltpu.SemaphoreType.DMA((13,)),
        pltpu.SemaphoreType.DMA((NSEG + QT,)),
    ]
    out_t = pl.pallas_call(
        _kernel,
        out_shape=jax.ShapeDtypeStruct((1, D, S), BF16),
        in_specs=[hbm] * 10,
        out_specs=hbm,
        scratch_shapes=scratch,
        compiler_params=pltpu.CompilerParams(vmem_limit_bytes=128 * 1024 * 1024),
        name="infini_attn_moe",
    )(jnp.transpose(A_x, (0, 2, 1)), A_wq, A_wk, A_wv, A_wo, A_beta, B_w_r, B_w_gate, B_w_up,
      B_w_down.T)
    return jnp.transpose(out_t, (0, 2, 1))
```

```python
import jax
import jax.numpy as jnp
from jax import lax
import jax.experimental.pallas as pl
import jax.experimental.pallas.tpu as pltpu

F32 = jnp.float32
BF16 = jnp.bfloat16
U32 = jnp.uint32
I32 = jnp.int32

S = 2048
D = 576
H = 32
DH = 18
NSEG = 4
L = 512
FF = 4608
HPG = 7
NG = 5
QT = L // 128
GW = (128, 128, 128, 128, 80)
PR = sum(GW)
ROUTER_ROW = 126
MROWS = 144
LOG2E = 1.4426950408889634
QSCALE = (DH ** -0.5) * LOG2E
SAFE_LOG2_RANGE = 40.0
NEG_BIG = -1e30

NT_DIMS = (((1,), (1,)), ((), ()))


def _heads_in_group(g):
    return min(HPG, H - HPG * g)


def _group_row_start(g):
    return (HPG * g * DH // 16) * 16


def _group_rows(g):
    last = (HPG * g + _heads_in_group(g)) * DH
    return -(-(last - _group_row_start(g)) // 16) * 16


def _state_rows(g):
    return MROWS if g == 0 else _group_rows(g)


def _norm_row(g):
    return 128 if g == 0 else 0


def _round_bf16(x):
    return x.astype(BF16).astype(F32)


def _pad_heads_t(w):
    parts = []
    for g in range(NG):
        n = _heads_in_group(g) * DH
        parts.append(w[:, HPG * DH * g:HPG * DH * g + n])
        parts.append(jnp.zeros((D, 128 - n), w.dtype))
    return jnp.concatenate(parts, axis=1).T[0:PR]


def _phi(t):
    return jnp.where(t > 0, t + 1.0, jnp.exp(t))


class _Packed:
    def __init__(self, ref, rows):
        self.ref = ref
        self.rows = rows

    def _slice(self, item, lo, size):
        start = item * (self.rows // 2) + lo // 2
        size = size // 2
        if isinstance(start, int):
            return slice(start, start + size)
        return pl.ds(pl.multiple_of(start, 8), size)

    def load(self, item=0, lo=0, hi=None, cols=slice(None)):
        size = hi if not isinstance(lo, int) else (self.rows if hi is None else hi) - lo
        return pltpu.bitcast(self.ref[self._slice(item, lo, size), cols], BF16)

    def store(self, val, item=0, lo=0, cols=slice(None)):
        self.ref[self._slice(item, lo, val.shape[0]), cols] = pltpu.bitcast(val.astype(BF16), U32)


def _kernel(x_hbm, wq_hbm, wk_hbm, wv_hbm, wo_hbm, beta_hbm, wr_hbm, wg_hbm, wu_hbm, wd_hbm,
            out_hbm,
            x_buf, wq_raw, wk_raw, wv_raw, wo_raw, beta_buf, wr_buf, wg_buf, wu_buf, wd_buf,
            wqt, wkt, wvt, wot, xn_buf, base, qs_buf, pq_buf, k_buf, pk_buf, vt_buf, r_buf,
            gate_buf, mt_buf, num_buf, p_buf0, p_buf1, ot_buf, out_buf, in_sems, out_sems):
    wqt, wkt = _Packed(wqt, PR), _Packed(wkt, PR)
    wvt, wot = _Packed(wvt, D), _Packed(wot, D)
    xn_buf, vt_buf = _Packed(xn_buf, D), _Packed(vt_buf, D)
    qs_buf, pq_buf, pk_buf = _Packed(qs_buf, PR), _Packed(pq_buf, PR), _Packed(pk_buf, PR)
    k_buf = _Packed(k_buf, L)

    def x_copy(c):
        return pltpu.make_async_copy(x_hbm.at[0, :, pl.ds(c * L, L)], x_buf.at[c], in_sems.at[c])

    cp_wv = pltpu.make_async_copy(wv_hbm, wv_raw, in_sems.at[4])
    cp_wq = pltpu.make_async_copy(wq_hbm, wq_raw, in_sems.at[5])
    cp_wk = pltpu.make_async_copy(wk_hbm, wk_raw, in_sems.at[6])
    cp_wo = pltpu.make_async_copy(wo_hbm, wo_raw, in_sems.at[7])
    cp_wg = pltpu.make_async_copy(wg_hbm, wg_buf, in_sems.at[8])
    cp_wu = pltpu.make_async_copy(wu_hbm, wu_buf, in_sems.at[9])
    cp_wd = pltpu.make_async_copy(wd_hbm, wd_buf, in_sems.at[10])
    cp_beta = pltpu.make_async_copy(beta_hbm, beta_buf, in_sems.at[11])
    cp_wr = pltpu.make_async_copy(wr_hbm, wr_buf, in_sems.at[12])

    def out_copy(s):
        cols = pl.ds(pl.multiple_of(s * L, L), L)
        return pltpu.make_async_copy(out_buf.at[s], out_hbm.at[0, :, cols], out_sems.at[s])

    def out_tile_copy(j):
        s = NSEG - 1
        return pltpu.make_async_copy(out_buf.at[s, :, pl.ds(128 * j, 128)],
                                     out_hbm.at[0, :, pl.ds(s * L + 128 * j, 128)], out_sems.at[NSEG + j])

    for cp in (x_copy(0), cp_wv, x_copy(1), cp_wq, cp_wr, cp_beta, x_copy(2), cp_wk, x_copy(3), cp_wo,
               cp_wg, cp_wu, cp_wd):
        cp.start()

    mt_buf[...] = jnp.zeros(mt_buf.shape, F32)

    always = []

    def pace(x, y):
        return x if y is None else jnp.where(always[0], x, y[0:D])

    def ln_stats(c, y):
        shift = x_buf[c, 0:16, :].astype(F32)[0:1]
        d = pace(x_buf[c].astype(F32), y) - shift
        m1 = jnp.sum(d, axis=0, keepdims=True) * (1.0 / D)
        m2 = jnp.sum(d * d, axis=0, keepdims=True) * (1.0 / D)
        var = jnp.maximum(m2 - m1 * m1, 0.0)
        inv = 1.0 / _round_bf16(jnp.sqrt(_round_bf16(_round_bf16(var) + 1e-5)))
        return _round_bf16(shift + m1), inv

    def ln_apply(c, mean_b, inv):
        x = x_buf[c].astype(F32)
        xn = (x - mean_b) * inv
        xn_buf.store(xn, c)
        if c == NSEG - 1:
            base[c] = jnp.zeros((D, L), F32)

    def project(w_ref, c, split):
        if not split:
            return jnp.dot(w_ref.load(), xn_buf.load(c), preferred_element_type=F32), None
        head = jnp.dot(w_ref.load(cols=slice(0, 256)), xn_buf.load(c, 0, 256), preferred_element_type=F32)
        tail = jnp.dot(w_ref.load(cols=slice(256, D)), xn_buf.load(c, 256, D), preferred_element_type=F32)
        return head + tail, head

    def project_v(c, mid=None):
        vt, head = project(wvt, c, mid is not None)
        if mid is not None:
            mid(head)
        vt_buf.store(vt, c)
        return vt

    def project_q(c, mid=None):
        qt, head = project(wqt, c, mid is not None)
        if mid is not None:
            mid(head)
        qsc = qt * QSCALE
        qs_buf.store(qsc, c)
        pq_buf.store(_phi(qt), c)
        r_buf[:, c * L:(c + 1) * L] = qt[120:128]
        mag = jnp.abs(qsc)
        r8 = lax.broadcasted_iota(I32, (8, L), 0)
        mag = jnp.concatenate([mag[0:120], jnp.where(r8 == ROUTER_ROW - 120, 0.0, mag[120:128]), mag[128:]], axis=0)
        return qt, jnp.max(mag.reshape(PR // 8, 8, L), axis=0)

    def project_k(c, mid=None, keep=False):
        kt, head = project(wkt, c, mid is not None)
        if mid is not None:
            mid(head)
        pk_buf.store(_phi(kt), c)
        for g in range(NG):
            ktg = kt[128 * g:128 * g + GW[g]]
            if GW[g] < 128:
                ktg = jnp.concatenate([ktg, jnp.zeros((128 - GW[g], L), F32)], axis=0)
            k_buf.store(ktg.T, c * NG + g)
        top = jnp.max(jnp.abs(kt).reshape(PR // 8, 8, L), axis=0)
        return (kt, top) if keep else top

    x_copy(0).wait()
    stats = ln_stats(0, None)
    always.append(jnp.logical_not(jnp.abs(stats[0]) < 0.0))
    ln_apply(0, *stats)
    cp_wv.wait()
    wvt.store(wv_raw[...].T)
    project_v(0)
    x_copy(1).wait()
    cp_wq.wait()
    cp_wr.wait()
    ln_apply(1, *ln_stats(1, None))

    def paced_weight(w_ref, y):
        w = w_ref[...].astype(F32)
        return jnp.concatenate([jnp.where(always[0], w[:, 0:L], y[0:D]), w[:, L:D]], axis=1)

    def prep_wq(y):
        wq_t = _pad_heads_t(paced_weight(wq_raw, y))
        wr_row = wr_buf[...].reshape(1, D).astype(F32)
        pr_row = lax.broadcasted_iota(I32, (8, D), 0)
        wq_t = jnp.concatenate(
            [wq_t[0:120], jnp.where(pr_row == ROUTER_ROW - 120, wr_row, wq_t[120:128]), wq_t[128:]], axis=0)
        wqt.store(wq_t)

    project_v(1, prep_wq)
    cp_wk.wait()
    cp_beta.wait()
    x_copy(2).wait()
    x_copy(3).wait()

    beta_row = beta_buf[...].reshape(1, H).astype(F32)
    beta_row = jnp.concatenate([beta_row, jnp.zeros((1, 128 - H), F32)], axis=1)
    h_row = lax.broadcasted_iota(I32, (H, 128), 0)
    h_lane = lax.broadcasted_iota(I32, (H, 128), 1)
    beta_col = jnp.sum(jnp.where(h_row == h_lane, beta_row, 0.0), axis=1, keepdims=True)
    gate_buf[...] = jnp.broadcast_to(jax.nn.sigmoid(beta_col), (H, 128))

    def prep_wk(y):
        wkt.store(_pad_heads_t(paced_weight(wk_raw, y)))

    def route():
        r = _round_bf16(r_buf[ROUTER_ROW - 120:ROUTER_ROW - 119, :])
        tok = lax.broadcasted_iota(I32, (1, S), 1).astype(F32)
        m1 = jnp.max(r)
        i1 = jnp.min(jnp.where(r == m1, tok, float(S)))
        r_rest = jnp.where(tok == i1, -jnp.inf, r)
        m2 = jnp.max(r_rest)
        i2 = jnp.min(jnp.where(r_rest == m2, tok, float(S)))
        i1 = jnp.clip(i1.astype(I32), 0, S - 1)
        i2 = jnp.clip(i2.astype(I32), 0, S - 1)
        return m1, m2, i1, i2

    qt, aq = project_q(0, prep_wk)
    qt, a = project_q(1)
    aq = jnp.maximum(aq, a)
    stats = ln_stats(2, qt)
    ak = project_k(0)
    ln_apply(2, *stats)
    kt, a = project_k(1, keep=True)
    ak = jnp.maximum(ak, a)
    stats = ln_stats(3, kt)
    project_v(2)
    ln_apply(3, *stats)
    qt, a = project_q(2)
    aq = jnp.maximum(aq, a)
    ak = jnp.maximum(ak, project_k(2))
    qt, a = project_q(3)
    aq = jnp.maximum(aq, a)
    m1, m2, i1, i2 = route()
    ak = jnp.maximum(ak, project_k(3))
    project_v(3)

    logit_bound = jnp.max(aq) * jnp.max(ak) * (DH * 1.02)
    safe = logit_bound <= SAFE_LOG2_RANGE

    sel_row = lax.broadcasted_iota(I32, (16, 128), 0)
    sel_lane = lax.broadcasted_iota(I32, (16, 128), 1)

    def token_tile(i):
        return i // L, pl.ds(pl.multiple_of(((i % L) // 128) * 128, 128), 128)

    def pick(i, slot):
        seg, cols = token_tile(i)
        onehot = jnp.where((sel_row == slot) & (sel_lane == i % 128), 1.0, 0.0).astype(BF16)
        return lax.dot_general(onehot, xn_buf.load(seg, cols=cols), NT_DIMS, preferred_element_type=F32)

    def routed_rows():
        return (pick(i1, 0) + pick(i2, 1)).astype(BF16)

    cp_wo.wait()
    cp_wg.wait()
    cp_wu.wait()

    def expert_chunk(lo, hi):
        xs = routed_rows()
        hg = jnp.dot(xs, wg_buf[:, lo:hi], preferred_element_type=F32)
        hu = jnp.dot(xs, wu_buf[:, lo:hi], preferred_element_type=F32)
        hh = (jax.nn.silu(hg) * hu).astype(BF16)
        return lax.dot_general(hh, wd_buf[:, lo:hi], NT_DIMS, preferred_element_type=F32)

    def expert_up_stream(hidden):
        kmain = 512
        xs = routed_rows()
        tail = xs[:, kmain:D].astype(F32)
        zero = jnp.zeros_like(tail)
        r16k = lax.broadcasted_iota(I32, (16, 128), 0)
        xs_rem = jnp.where(r16k < 2, jnp.concatenate([tail, zero], axis=1),
                           pltpu.roll(jnp.concatenate([zero, tail], axis=1), 2, 0)).astype(BF16)
        yield
        for c0 in range(0, FF, 512):
            w_rem = jnp.concatenate([wg_buf[kmain:D, c0:c0 + 512], wu_buf[kmain:D, c0:c0 + 512]], axis=0)
            both = jnp.dot(xs_rem, w_rem, preferred_element_type=F32)
            rem = (both, pltpu.roll(both, 14, 0))
            yield
            hs = []
            for f0 in range(c0, c0 + 512, 128):
                pre = []
                for w_ref, r in zip((wg_buf, wu_buf), rem):
                    pre.append(jnp.dot(xs[:, 0:kmain], w_ref[0:kmain, f0:f0 + 128], preferred_element_type=F32)
                               + r[:, f0 - c0:f0 - c0 + 128])
                    if len(pre) == 2:
                        hs.append(jax.nn.silu(pre[0]) * pre[1])
                        if len(hs) == 4:
                            hidden.append(_round_bf16(jnp.concatenate(hs, axis=1)))
                    yield

    lane_d = lax.broadcasted_iota(I32, (D, 128), 1)

    def expert_scatter_parts(columns):
        for col, i, score in zip(columns, (i1, i2), (m1, m2)):
            seg, cols = token_tile(i)
            col = col * jax.nn.sigmoid(jnp.full((D, 1), score, F32))
            base[seg, :, cols] = base[seg, :, cols] + jnp.where(lane_d == i % 128, col, 0.0)
            yield

    def expert_scatter_rows(y):
        yt = jnp.concatenate([y, jnp.zeros((128 - 16, D), F32)], axis=0).T
        columns = [jnp.sum(jnp.where(lane_d == slot, yt, 0.0), axis=1, keepdims=True) for slot in range(2)]
        for _ in expert_scatter_parts(columns):
            pass

    def memory_read(s, g):
        sr = _state_rows(g)
        gw = GW[g]
        num_buf[g, 0:sr, :] = jnp.dot(mt_buf[g, 0:sr, 0:gw].astype(BF16), pq_buf.load(s, 128 * g, 128 * g + gw),
                                      preferred_element_type=F32)

    def memory_update(s, g):
        rg = _group_rows(g)
        a_g = _group_row_start(g)
        gw = GW[g]
        ones_row = 126 if g == 0 else 0
        lhs = jnp.where(lax.broadcasted_iota(I32, (rg, L), 0) == ones_row, 1.0,
                        vt_buf.load(s, a_g, a_g + rg).astype(F32)).astype(BF16)
        upd = lax.dot_general(lhs, pk_buf.load(s, 128 * g, 128 * g + gw), NT_DIMS,
                              preferred_element_type=F32)
        er = lax.broadcasted_iota(I32, (rg, gw), 0) + (a_g - HPG * DH * g)
        el = lax.broadcasted_iota(I32, (rg, gw), 1)
        same_head = None
        for i in range(_heads_in_group(g)):
            t = ((er >= DH * i) & (er < DH * (i + 1)) & (el >= DH * i) & (el < DH * (i + 1)))
            same_head = t if same_head is None else (same_head | t)
        mt_buf[g, 0:rg, 0:gw] = mt_buf[g, 0:rg, 0:gw] + jnp.where(same_head, upd, 0.0)
        zr = lax.broadcasted_iota(I32, (8, gw), 0)
        zl = lax.broadcasted_iota(I32, (8, gw), 1)
        zmask = (zl >= zr * DH) & (zl < zr * DH + DH) & (zr < _heads_in_group(g))
        zs = upd[ones_row:ones_row + 1]
        z0 = _norm_row(g)
        mt_buf[g, z0:z0 + 8, 0:gw] = mt_buf[g, z0:z0 + 8, 0:gw] + jnp.where(zmask, zs, 0.0)

    def transpose_wo(g):
        hi = min(128 * (g + 1), D)
        wot.store(wo_raw[:, 128 * g:hi].T, lo=128 * g)

    def project_out(s):
        return jnp.dot(wot.load(), ot_buf[...].astype(BF16), preferred_element_type=F32)

    def residual(s, cols=slice(None)):
        return x_buf[s, :, cols].astype(F32) + xn_buf.load(s, cols=cols).astype(F32)

    def emit(s, val):
        out_buf[s] = val.astype(BF16)
        out_copy(s).start()

    zero = lax.shift_right_logical(i1, 16)

    def prow(start, size):
        return pl.ds(pl.multiple_of(zero + start, 8), size)

    P_OFFS = (0, 128, 384, 768)

    def fast_scores(s, g, hook, anchor):
        nh = _heads_in_group(g)
        gw = GW[g]
        pb = (p_buf0, p_buf1)[(s * NG + g) % 2]
        rowg = lax.broadcasted_iota(I32, (gw, 128), 0)
        laneg = lax.broadcasted_iota(I32, (gw, 128), 1)
        head_rows = [(rowg >= DH * i) & (rowg < DH * (i + 1)) for i in range(nh)]
        row64 = lax.broadcasted_iota(I32, (64, 128), 0)
        lane64 = lax.broadcasted_iota(I32, (64, 128), 1)
        visible_lo = row64 <= lane64
        row32 = lax.broadcasted_iota(I32, (32, 128), 0)
        lane32 = lax.broadcasted_iota(I32, (32, 128), 1)
        lane16 = lax.broadcasted_iota(I32, (16, 128), 1)
        for j in range(QT - 1, -1, -1):
            n = 128 * (j + 1)
            m = n - 64
            q = qs_buf.load(s, 128 * g, 128 * g + gw, slice(128 * j, 128 * (j + 1))).astype(F32)
            for h0, h1 in (((0, 3), (3, nh)) if nh == HPG else ((0, nh),)):
                q_in = anchor(q)
                qm = jnp.concatenate([jnp.where(head_rows[i], q_in, 0.0) for i in range(h0, h1)],
                                     axis=1).astype(BF16)
                st = jnp.dot(k_buf.load(s * NG + g, 0, m, slice(0, gw)), qm, preferred_element_type=F32)
                p = jnp.exp2(st)
                p_diag = jnp.where(jnp.concatenate([visible_lo] * (h1 - h0), axis=1), p[m - 64:], 0.0)
                p = jnp.concatenate([p[:m - 64], p_diag], axis=0) if j > 0 else p_diag
                pb[P_OFFS[j] // 2:(P_OFFS[j] + m) // 2, h0 * 128:h1 * 128] = pltpu.bitcast(p.astype(BF16), U32)
                hook(p)
            for width, k0 in ((64, m), (32, m + 32)):
                per = 128 // width
                q_top = q
                for t in range(per - 1):
                    q_top = jnp.where((laneg >= width * t) & (laneg < width * (t + 1)),
                                      pltpu.roll(q, width * (t + 1), 1), q_top)
                groups = [list(range(i, min(i + per, nh))) for i in range(0, nh, per)]
                tiles = []
                for heads in groups:
                    keep = None
                    for t, i in enumerate(heads):
                        slot = per - len(heads) + t
                        sel = head_rows[i] & (laneg >= width * slot) & (laneg < width * (slot + 1))
                        keep = sel if keep is None else (keep | sel)
                    tiles.append(jnp.where(keep, q_top, 0.0))
                st = jnp.dot(k_buf.load(s * NG + g, k0, k0 + 32, slice(0, gw)),
                             jnp.concatenate(tiles, axis=1).astype(BF16),
                             preferred_element_type=F32)
                visible = row32 + (k0 - m) <= (lane32 & (width - 1)) + (64 - width)
                p = jnp.where(jnp.concatenate([visible] * len(groups), axis=1), jnp.exp2(st), 0.0)
                p = pltpu.bitcast(p.astype(BF16), U32)
                rows = slice((P_OFFS[j] + k0) // 2, (P_OFFS[j] + k0 + 32) // 2)
                top = lane16 >= 128 - width
                for gi, heads in enumerate(groups):
                    shared = p[:, 128 * gi:128 * (gi + 1)]
                    for t, i in enumerate(heads):
                        slot = per - len(heads) + t
                        shift = width * (per - 1 - slot)
                        mine = shared if shift == 0 else pltpu.roll(shared, shift, 1)
                        pb[rows, 128 * i:128 * (i + 1)] = jnp.where(top, mine, jnp.uint32(0))

    def fast_values(s, g, after_tile=None):
        nh = _heads_in_group(g)
        a_g = _group_row_start(g)
        pb = (p_buf0, p_buf1)[(s * NG + g) % 2]
        for j in range(QT - 1, -1, -1):
            n = 128 * (j + 1)
            cols = slice(128 * j, 128 * (j + 1))
            for i in range(nh):
                h = HPG * g + i
                a = (h * DH // 16) * 16
                off = h * DH - a
                p = pltpu.bitcast(pb[prow(P_OFFS[j] // 2, n // 2), 128 * i:128 * (i + 1)], BF16)
                ones_row = 0 if off > 0 else 31
                r32n = lax.broadcasted_iota(I32, (32, n), 0)
                lhs = jnp.where(r32n == ones_row, 1.0, vt_buf.load(s, a, a + 32, slice(0, n)).astype(F32)).astype(BF16)
                o = jnp.dot(lhs, p, preferred_element_type=F32)
                lo = (off // 8) * 8
                hi = -(-(off + DH) // 8) * 8
                gate = gate_buf[h:h + 1, :]
                rl = 1.0 / o[ones_row:ones_row + 1]
                val = (1.0 - gate) * (o[lo:hi] * rl)
                if s > 0:
                    z = _norm_row(g) + i
                    rden = 1.0 / (num_buf[g, z:z + 1, cols] + 1e-6)
                    num = num_buf[g, a - a_g + lo:a - a_g + hi, cols]
                    val = gate * (num * rden) + val
                ot_buf[a + off:a + off + DH, cols] = val[off - lo:off - lo + DH]
            if after_tile is not None:
                after_tile(j)

    def fast_path():
        hidden = []
        up = expert_up_stream(hidden)
        n_down = FF // 128
        state = dict(down=0, wd_ready=False, up_done=False, y=[None] * 2, tail=None, tail_steps=0,
                     out_ready=False, pacer=None, anchor=None, anchor_next=None)

        def finish():
            yield from expert_scatter_parts([jnp.sum(acc, axis=1, keepdims=True) for acc in state["y"]])
            for u in range(NSEG - 1):
                for j in range(QT):
                    cols = slice(128 * j, 128 * (j + 1))
                    val = (paced(base[u, :, cols]) + x_buf[u, :, cols].astype(F32)
                           ) + xn_buf.load(u, cols=cols).astype(F32)
                    out_buf[u, :, cols] = val.astype(BF16)
                    state["anchor"] = val
                    if j == QT - 1:
                        out_copy(u).start()
                    yield

        def anchor(q):
            val, state["anchor_next"], state["anchor"] = state["anchor_next"], state["anchor"], None
            return q if val is None else jnp.where(always[0][:, 0:128], q, val[D - q.shape[0]:D])

        def paced(val):
            y = state["pacer"]
            if y is None:
                return val
            reps = -(-D // y.shape[0])
            y = jnp.concatenate([y[:, 128 * r:128 * (r + 1)] for r in range(reps)], axis=0)[0:D]
            return jnp.where(always[0][:, 0:128], val, y)

        def down_step():
            ft = state["down"]
            w = paced(wd_buf[:, 128 * ft:128 * (ft + 1)].astype(F32))
            hh = hidden[ft // 4][:, 128 * (ft % 4):128 * (ft % 4 + 1)]
            for slot in range(2):
                term = w * hh[slot:slot + 1]
                state["y"][slot] = term if state["y"][slot] is None else state["y"][slot] + term
            if ft % 6 == 5:
                state["anchor"] = state["y"][1]
            state["down"] += 1

        def hook(pacer=None):
            state["pacer"] = pacer if pacer is not None and pacer.shape[0] * (pacer.shape[1] // 128) >= D else None
            if not state["up_done"] and next(up, "done") == "done":
                state["up_done"] = True
            if state["down"] < n_down:
                if state["wd_ready"] and state["pacer"] is not None and state["down"] // 4 < len(hidden):
                    down_step()
            elif state["out_ready"]:
                if state["tail"] is None:
                    state["tail"] = finish()
                if state["pacer"] is not None or state["tail_steps"] < 2:
                    state["tail_steps"] += 1
                    next(state["tail"], None)

        steps = [(s, g) for s in range(NSEG) for g in range(NG)]
        last = NSEG - 1

        def last_tile(j):
            cols = slice(128 * j, 128 * (j + 1))
            attn = jnp.dot(wot.load(), ot_buf[:, cols].astype(BF16), preferred_element_type=F32)
            out_buf[last, :, cols] = (base[last, :, cols] + residual(last, cols) + attn).astype(BF16)
            out_tile_copy(j).start()

        fast_scores(0, 0, hook, anchor)
        for t, (s, g) in enumerate(steps):
            if t + 1 < len(steps):
                fast_scores(*steps[t + 1], hook, anchor)
            if s > 0:
                memory_read(s, g)
                hook()
            if t + 1 == len(steps):
                state["pacer"] = None
                assert state["down"] == n_down and state["tail"] is not None
                while next(state["tail"], "done") != "done":
                    pass
                pending = []

                def after_tile(j):
                    if pending:
                        last_tile(pending.pop())
                    pending.append(j)

                fast_values(s, g, after_tile)
                last_tile(pending.pop())
            else:
                fast_values(s, g)
            if s == 0:
                transpose_wo(g)
            if s + 1 < NSEG:
                memory_update(s, g)
                hook()
            if g == NG - 1 and s < last:
                base[s] = project_out(s)
                if s == 0:
                    cp_wd.wait()
                    state["wd_ready"] = True
                if s == last - 1:
                    state["out_ready"] = True
                hook()
        for u in range(NSEG - 1):
            out_copy(u).wait()
        for j in range(QT):
            out_tile_copy(j).wait()

    def slow_segment(s, carry):
        for g in range(NG):
            memory_read(s, g)
        key_i = lax.broadcasted_iota(I32, (L, L), 0)
        qry_i = lax.broadcasted_iota(I32, (L, L), 1)
        r32 = lax.broadcasted_iota(I32, (32, L), 0)
        for g in range(NG):
            gw = GW[g]
            a_g = _group_row_start(g)
            rowg = lax.broadcasted_iota(I32, (gw, L), 0)

            def head(i, c, g=g, gw=gw, a_g=a_g, rowg=rowg):
                h = HPG * g + i
                a = pl.multiple_of((h * DH // 16) * 16, 16)
                off = h * DH - a
                q = qs_buf.load(s, 128 * g, 128 * g + gw).astype(F32)
                qm = jnp.where((rowg >= DH * i) & (rowg < DH * (i + 1)), q, 0.0).astype(BF16)
                st = jnp.dot(k_buf.load(s * NG + g, cols=slice(0, gw)), qm, preferred_element_type=F32)
                st = jnp.where(key_i <= qry_i, st, NEG_BIG)
                p = jnp.exp2(st - jnp.max(st, axis=0, keepdims=True))
                rl = 1.0 / jnp.sum(p, axis=0, keepdims=True)
                o = jnp.dot(vt_buf.load(s, a, 32), p.astype(BF16), preferred_element_type=F32)
                gate = jnp.concatenate([gate_buf[pl.ds(h, 1), :]] * QT, axis=1)
                rden = 1.0 / (num_buf[g, pl.ds(_norm_row(g) + i, 1), :] + 1e-6)
                num = num_buf[g, pl.ds(pl.multiple_of(a - a_g, 16), 32), :]
                val = gate * (num * rden) + (1.0 - gate) * (o * rl)
                keep = (r32 >= off) & (r32 < off + DH)
                pltpu.store(ot_buf.at[pl.ds(a, 32), :], val, mask=keep)
                return c

            lax.fori_loop(0, _heads_in_group(g), head, 0)
        for g in range(NG):
            memory_update(s, g)
        emit(s, base[s] + residual(s) + project_out(s))
        return carry

    @pl.when(safe)
    def _():
        fast_path()

    @pl.when(jnp.logical_not(safe))
    def _():
        cp_wd.wait()
        for u in range(NSEG - 1):
            base[u] = jnp.zeros((D, L), F32)
        for g in range(NG):
            transpose_wo(g)
        expert_scatter_rows(expert_chunk(0, FF))
        lax.fori_loop(0, NSEG, slow_segment, 0)
        for u in range(NSEG):
            out_copy(u).wait()


@jax.jit
def pallas_parallel_sum__memory_aug_infini_attn__moe_arch_mod__prompt_kernel(
    A_x: jax.Array,
    A_wq: jax.Array,
    A_wk: jax.Array,
    A_wv: jax.Array,
    A_wo: jax.Array,
    A_beta: jax.Array,
    B_x: jax.Array,
    B_w_r: jax.Array,
    B_w_gate: jax.Array,
    B_w_up: jax.Array,
    B_w_down: jax.Array,
):
    del B_x
    hbm = pl.BlockSpec(memory_space=pl.ANY)
    scratch = [
        pltpu.VMEM((NSEG, D, L), BF16),
        pltpu.VMEM((D, D), BF16),
        pltpu.VMEM((D, D), BF16),
        pltpu.VMEM((D, D), BF16),
        pltpu.VMEM((D, D), BF16),
        pltpu.VMEM((H,), BF16),
        pltpu.VMEM((D,), BF16),
        pltpu.VMEM((D, FF), BF16),
        pltpu.VMEM((D, FF), BF16),
        pltpu.VMEM((D, FF), BF16),
        pltpu.VMEM((PR // 2, D), U32),
        pltpu.VMEM((PR // 2, D), U32),
        pltpu.VMEM((D // 2, D), U32),
        pltpu.VMEM((D // 2, D), U32),
        pltpu.VMEM((NSEG * D // 2, L), U32),
        pltpu.VMEM((NSEG, D, L), F32),
        pltpu.VMEM((NSEG * PR // 2, L), U32),
        pltpu.VMEM((NSEG * PR // 2, L), U32),
        pltpu.VMEM((NSEG * NG * L // 2, 128), U32),
        pltpu.VMEM((NSEG * PR // 2, L), U32),
        pltpu.VMEM((NSEG * D // 2, L), U32),
        pltpu.VMEM((8, S), F32),
        pltpu.VMEM((H, 128), F32),
        pltpu.VMEM((NG, MROWS, 128), F32),
        pltpu.VMEM((NG, MROWS, L), F32),
        pltpu.VMEM((640, HPG * 128), U32),
        pltpu.VMEM((640, HPG * 128), U32),
        pltpu.VMEM((D, L), F32),
        pltpu.VMEM((NSEG, D, L), BF16),
        pltpu.SemaphoreType.DMA((13,)),
        pltpu.SemaphoreType.DMA((NSEG + QT,)),
    ]
    out_t = pl.pallas_call(
        _kernel,
        out_shape=jax.ShapeDtypeStruct((1, D, S), BF16),
        in_specs=[hbm] * 10,
        out_specs=hbm,
        scratch_shapes=scratch,
        compiler_params=pltpu.CompilerParams(vmem_limit_bytes=128 * 1024 * 1024),
        name="infini_attn_moe",
    )(jnp.transpose(A_x, (0, 2, 1)), A_wq, A_wk, A_wv, A_wo, A_beta, B_w_r, B_w_gate, B_w_up,
      B_w_down.T)
    return jnp.transpose(out_t, (0, 2, 1))
```

```python
import jax
import jax.numpy as jnp
from jax import lax
import jax.experimental.pallas as pl
import jax.experimental.pallas.tpu as pltpu

F32 = jnp.float32
BF16 = jnp.bfloat16
U32 = jnp.uint32
I32 = jnp.int32

S = 2048
D = 576
H = 32
DH = 18
NSEG = 4
L = 512
FF = 4608
HPG = 7
NG = 5
QT = L // 128
GW = (128, 128, 128, 128, 80)
PR = sum(GW)
ROUTER_ROW = 126
MROWS = 144
LOG2E = 1.4426950408889634
QSCALE = (DH ** -0.5) * LOG2E
SAFE_LOG2_RANGE = 40.0
NEG_BIG = -1e30

NT_DIMS = (((1,), (1,)), ((), ()))


def _heads_in_group(g):
    return min(HPG, H - HPG * g)


def _group_row_start(g):
    return (HPG * g * DH // 16) * 16


def _group_rows(g):
    last = (HPG * g + _heads_in_group(g)) * DH
    return -(-(last - _group_row_start(g)) // 16) * 16


def _state_rows(g):
    return MROWS if g == 0 else _group_rows(g)


def _norm_row(g):
    return 128 if g == 0 else 0


def _round_bf16(x):
    return x.astype(BF16).astype(F32)


def _pad_heads_t(w):
    parts = []
    for g in range(NG):
        n = _heads_in_group(g) * DH
        parts.append(w[:, HPG * DH * g:HPG * DH * g + n])
        parts.append(jnp.zeros((D, 128 - n), w.dtype))
    return jnp.concatenate(parts, axis=1).T[0:PR]


def _phi(t):
    return jnp.where(t > 0, t + 1.0, jnp.exp(t))


class _Packed:
    def __init__(self, ref, rows):
        self.ref = ref
        self.rows = rows

    def _slice(self, item, lo, size):
        start = item * (self.rows // 2) + lo // 2
        size = size // 2
        if isinstance(start, int):
            return slice(start, start + size)
        return pl.ds(pl.multiple_of(start, 8), size)

    def load_words(self, item=0, lo=0, hi=None, cols=slice(None)):
        size = hi if not isinstance(lo, int) else (self.rows if hi is None else hi) - lo
        return self.ref[self._slice(item, lo, size), cols]

    def load(self, item=0, lo=0, hi=None, cols=slice(None)):
        return pltpu.bitcast(self.load_words(item, lo, hi, cols), BF16)

    def store(self, val, item=0, lo=0, cols=slice(None)):
        self.ref[self._slice(item, lo, val.shape[0]), cols] = pltpu.bitcast(val.astype(BF16), U32)


def _with_ones_row(words, row):
    r = row // 2
    lo = (r // 8) * 8
    keep, one = (0x0000FFFF, 0x3F800000) if row % 2 else (0xFFFF0000, 0x00003F80)
    blk = words[lo:lo + 8]
    hit = lax.broadcasted_iota(I32, blk.shape, 0) == r - lo
    blk = jnp.where(hit, (blk & jnp.uint32(keep)) | jnp.uint32(one), blk)
    parts = [part for part in (words[0:lo], blk, words[lo + 8:]) if part.shape[0]]
    return pltpu.bitcast(jnp.concatenate(parts, axis=0), BF16)


def _kernel(x_hbm, wq_hbm, wk_hbm, wv_hbm, wo_hbm, beta_hbm, wr_hbm, wg_hbm, wu_hbm, wd_hbm,
            out_hbm,
            x_buf, wq_raw, wk_raw, wv_raw, wo_raw, beta_buf, wr_buf, wg_buf, wu_buf, wd_buf,
            wqt, wkt, wvt, wot, xn_buf, base, qs_buf, pq_buf, k_buf, pk_buf, vt_buf, r_buf,
            gate_buf, mt_buf, num_buf, p_buf0, p_buf1, ot_buf, out_buf, in_sems, out_sems):
    wqt, wkt = _Packed(wqt, PR), _Packed(wkt, PR)
    wvt, wot = _Packed(wvt, D), _Packed(wot, D)
    xn_buf, vt_buf = _Packed(xn_buf, D), _Packed(vt_buf, D)
    qs_buf, pq_buf, pk_buf = _Packed(qs_buf, PR), _Packed(pq_buf, PR), _Packed(pk_buf, PR)
    k_buf = _Packed(k_buf, L)

    def x_copy(c):
        return pltpu.make_async_copy(x_hbm.at[0, :, pl.ds(c * L, L)], x_buf.at[c], in_sems.at[c])

    cp_wv = pltpu.make_async_copy(wv_hbm, wv_raw, in_sems.at[4])
    cp_wq = pltpu.make_async_copy(wq_hbm, wq_raw, in_sems.at[5])
    cp_wk = pltpu.make_async_copy(wk_hbm, wk_raw, in_sems.at[6])
    cp_wo = pltpu.make_async_copy(wo_hbm, wo_raw, in_sems.at[7])
    cp_wg = pltpu.make_async_copy(wg_hbm, wg_buf, in_sems.at[8])
    cp_wu = pltpu.make_async_copy(wu_hbm, wu_buf, in_sems.at[9])
    cp_wd = pltpu.make_async_copy(wd_hbm, wd_buf, in_sems.at[10])
    cp_beta = pltpu.make_async_copy(beta_hbm, beta_buf, in_sems.at[11])
    cp_wr = pltpu.make_async_copy(wr_hbm, wr_buf, in_sems.at[12])

    def out_copy(s):
        cols = pl.ds(pl.multiple_of(s * L, L), L)
        return pltpu.make_async_copy(out_buf.at[s], out_hbm.at[0, :, cols], out_sems.at[s])

    def out_tile_copy(j):
        s = NSEG - 1
        return pltpu.make_async_copy(out_buf.at[s, :, pl.ds(128 * j, 128)],
                                     out_hbm.at[0, :, pl.ds(s * L + 128 * j, 128)], out_sems.at[NSEG + j])

    for cp in (x_copy(0), cp_wv, x_copy(1), cp_wq, cp_wr, cp_beta, x_copy(2), cp_wk, x_copy(3), cp_wo,
               cp_wg, cp_wu, cp_wd):
        cp.start()

    mt_buf[...] = jnp.zeros(mt_buf.shape, F32)

    always = []

    def pace(x, y):
        return x if y is None else jnp.where(always[0], x, y[0:D])

    def ln_stats(c, y):
        shift = x_buf[c, 0:16, :].astype(F32)[0:1]
        d = pace(x_buf[c].astype(F32), y) - shift
        m1 = jnp.sum(d, axis=0, keepdims=True) * (1.0 / D)
        m2 = jnp.sum(d * d, axis=0, keepdims=True) * (1.0 / D)
        var = jnp.maximum(m2 - m1 * m1, 0.0)
        inv = 1.0 / _round_bf16(jnp.sqrt(_round_bf16(_round_bf16(var) + 1e-5)))
        return _round_bf16(shift + m1), inv

    def ln_apply(c, mean_b, inv):
        x = x_buf[c].astype(F32)
        xn = (x - mean_b) * inv
        xn_buf.store(xn, c)
        if c == NSEG - 1:
            base[c] = jnp.zeros((D, L), F32)

    def project(w_ref, c, split):
        if not split:
            return jnp.dot(w_ref.load(), xn_buf.load(c), preferred_element_type=F32), None
        head = jnp.dot(w_ref.load(cols=slice(0, 256)), xn_buf.load(c, 0, 256), preferred_element_type=F32)
        tail = jnp.dot(w_ref.load(cols=slice(256, D)), xn_buf.load(c, 256, D), preferred_element_type=F32)
        return head + tail, head

    def project_v(c, mid=None):
        vt, head = project(wvt, c, mid is not None)
        if mid is not None:
            mid(head)
        vt_buf.store(vt, c)
        return vt

    def project_q(c, mid=None):
        qt, head = project(wqt, c, mid is not None)
        if mid is not None:
            mid(head)
        qsc = qt * QSCALE
        qs_buf.store(qsc, c)
        pq_buf.store(_phi(qt), c)
        r_buf[:, c * L:(c + 1) * L] = qt[120:128]
        mag = jnp.abs(qsc)
        r8 = lax.broadcasted_iota(I32, (8, L), 0)
        mag = jnp.concatenate([mag[0:120], jnp.where(r8 == ROUTER_ROW - 120, 0.0, mag[120:128]), mag[128:]], axis=0)
        return qt, jnp.max(mag.reshape(PR // 8, 8, L), axis=0)

    def project_k(c, mid=None, keep=False):
        kt, head = project(wkt, c, mid is not None)
        if mid is not None:
            mid(head)
        pk_buf.store(_phi(kt), c)
        for g in range(NG):
            ktg = kt[128 * g:128 * g + GW[g]]
            if GW[g] < 128:
                ktg = jnp.concatenate([ktg, jnp.zeros((128 - GW[g], L), F32)], axis=0)
            k_buf.store(ktg.T, c * NG + g)
        top = jnp.max(jnp.abs(kt).reshape(PR // 8, 8, L), axis=0)
        return (kt, top) if keep else top

    x_copy(0).wait()
    stats = ln_stats(0, None)
    always.append(jnp.logical_not(jnp.abs(stats[0]) < 0.0))
    ln_apply(0, *stats)
    cp_wv.wait()
    wvt.store(wv_raw[...].T)
    project_v(0)
    x_copy(1).wait()
    cp_wq.wait()
    cp_wr.wait()
    ln_apply(1, *ln_stats(1, None))

    def paced_weight(w_ref, y):
        w = w_ref[...].astype(F32)
        return jnp.concatenate([jnp.where(always[0], w[:, 0:L], y[0:D]), w[:, L:D]], axis=1)

    def prep_wq(y):
        wq_t = _pad_heads_t(paced_weight(wq_raw, y))
        wr_row = wr_buf[...].reshape(1, D).astype(F32)
        pr_row = lax.broadcasted_iota(I32, (8, D), 0)
        wq_t = jnp.concatenate(
            [wq_t[0:120], jnp.where(pr_row == ROUTER_ROW - 120, wr_row, wq_t[120:128]), wq_t[128:]], axis=0)
        wqt.store(wq_t)

    project_v(1, prep_wq)
    cp_wk.wait()
    cp_beta.wait()
    x_copy(2).wait()
    x_copy(3).wait()

    beta_row = beta_buf[...].reshape(1, H).astype(F32)
    beta_row = jnp.concatenate([beta_row, jnp.zeros((1, 128 - H), F32)], axis=1)
    h_row = lax.broadcasted_iota(I32, (H, 128), 0)
    h_lane = lax.broadcasted_iota(I32, (H, 128), 1)
    beta_col = jnp.sum(jnp.where(h_row == h_lane, beta_row, 0.0), axis=1, keepdims=True)
    gate_buf[...] = jnp.broadcast_to(jax.nn.sigmoid(beta_col), (H, 128))

    def prep_wk(y):
        wkt.store(_pad_heads_t(paced_weight(wk_raw, y)))

    def route():
        r = _round_bf16(r_buf[ROUTER_ROW - 120:ROUTER_ROW - 119, :])
        tok = lax.broadcasted_iota(I32, (1, S), 1).astype(F32)
        m1 = jnp.max(r)
        i1 = jnp.min(jnp.where(r == m1, tok, float(S)))
        r_rest = jnp.where(tok == i1, -jnp.inf, r)
        m2 = jnp.max(r_rest)
        i2 = jnp.min(jnp.where(r_rest == m2, tok, float(S)))
        i1 = jnp.clip(i1.astype(I32), 0, S - 1)
        i2 = jnp.clip(i2.astype(I32), 0, S - 1)
        return m1, m2, i1, i2

    qt, aq = project_q(0, prep_wk)
    qt, a = project_q(1)
    aq = jnp.maximum(aq, a)
    stats = ln_stats(2, qt)
    ak = project_k(0)
    ln_apply(2, *stats)
    kt, a = project_k(1, keep=True)
    ak = jnp.maximum(ak, a)
    stats = ln_stats(3, kt)
    project_v(2)
    ln_apply(3, *stats)
    qt, a = project_q(2)
    aq = jnp.maximum(aq, a)
    ak = jnp.maximum(ak, project_k(2))
    qt, a = project_q(3)
    aq = jnp.maximum(aq, a)
    m1, m2, i1, i2 = route()
    ak = jnp.maximum(ak, project_k(3))
    project_v(3)

    logit_bound = jnp.max(aq) * jnp.max(ak) * (DH * 1.02)
    safe = logit_bound <= SAFE_LOG2_RANGE

    sel_row = lax.broadcasted_iota(I32, (16, 128), 0)
    sel_lane = lax.broadcasted_iota(I32, (16, 128), 1)

    def token_tile(i):
        return i // L, pl.ds(pl.multiple_of(((i % L) // 128) * 128, 128), 128)

    def pick(i, slot):
        seg, cols = token_tile(i)
        onehot = jnp.where((sel_row == slot) & (sel_lane == i % 128), 1.0, 0.0).astype(BF16)
        return lax.dot_general(onehot, xn_buf.load(seg, cols=cols), NT_DIMS, preferred_element_type=F32)

    def routed_rows():
        return (pick(i1, 0) + pick(i2, 1)).astype(BF16)

    cp_wo.wait()
    cp_wg.wait()
    cp_wu.wait()

    def expert_chunk(lo, hi):
        xs = routed_rows()
        hg = jnp.dot(xs, wg_buf[:, lo:hi], preferred_element_type=F32)
        hu = jnp.dot(xs, wu_buf[:, lo:hi], preferred_element_type=F32)
        hh = (jax.nn.silu(hg) * hu).astype(BF16)
        return lax.dot_general(hh, wd_buf[:, lo:hi], NT_DIMS, preferred_element_type=F32)

    def expert_up_stream(hidden):
        kmain = 512
        xs = routed_rows()
        tail = xs[:, kmain:D].astype(F32)
        zero = jnp.zeros_like(tail)
        r16k = lax.broadcasted_iota(I32, (16, 128), 0)
        xs_rem = jnp.where(r16k < 2, jnp.concatenate([tail, zero], axis=1),
                           pltpu.roll(jnp.concatenate([zero, tail], axis=1), 2, 0)).astype(BF16)
        yield
        for c0 in range(0, FF, 512):
            w_rem = jnp.concatenate([wg_buf[kmain:D, c0:c0 + 512], wu_buf[kmain:D, c0:c0 + 512]], axis=0)
            both = jnp.dot(xs_rem, w_rem, preferred_element_type=F32)
            rem = (both, pltpu.roll(both, 14, 0))
            yield
            hs = []
            for f0 in range(c0, c0 + 512, 128):
                pre = []
                for w_ref, r in zip((wg_buf, wu_buf), rem):
                    pre.append(jnp.dot(xs[:, 0:kmain], w_ref[0:kmain, f0:f0 + 128], preferred_element_type=F32)
                               + r[:, f0 - c0:f0 - c0 + 128])
                    if len(pre) == 2:
                        hs.append(jax.nn.silu(pre[0]) * pre[1])
                        if len(hs) == 4:
                            hidden.append(_round_bf16(jnp.concatenate(hs, axis=1)))
                    yield

    lane_d = lax.broadcasted_iota(I32, (D, 128), 1)

    def expert_scatter_parts(columns):
        for col, i, score in zip(columns, (i1, i2), (m1, m2)):
            seg, cols = token_tile(i)
            col = col * jax.nn.sigmoid(jnp.full((D, 1), score, F32))
            base[seg, :, cols] = base[seg, :, cols] + jnp.where(lane_d == i % 128, col, 0.0)
            yield

    def expert_scatter_rows(y):
        yt = jnp.concatenate([y, jnp.zeros((128 - 16, D), F32)], axis=0).T
        columns = [jnp.sum(jnp.where(lane_d == slot, yt, 0.0), axis=1, keepdims=True) for slot in range(2)]
        for _ in expert_scatter_parts(columns):
            pass

    def memory_read(s, g):
        sr = _state_rows(g)
        gw = GW[g]
        num_buf[g, 0:sr, :] = jnp.dot(mt_buf[g, 0:sr, 0:gw].astype(BF16), pq_buf.load(s, 128 * g, 128 * g + gw),
                                      preferred_element_type=F32)

    def memory_update(s, g):
        rg = _group_rows(g)
        a_g = _group_row_start(g)
        gw = GW[g]
        ones_row = 126 if g == 0 else 0
        lhs = _with_ones_row(vt_buf.load_words(s, a_g, a_g + rg), ones_row)
        upd = lax.dot_general(lhs, pk_buf.load(s, 128 * g, 128 * g + gw), NT_DIMS,
                              preferred_element_type=F32)
        er = lax.broadcasted_iota(I32, (rg, gw), 0) + (a_g - HPG * DH * g)
        el = lax.broadcasted_iota(I32, (rg, gw), 1)
        same_head = None
        for i in range(_heads_in_group(g)):
            t = ((er >= DH * i) & (er < DH * (i + 1)) & (el >= DH * i) & (el < DH * (i + 1)))
            same_head = t if same_head is None else (same_head | t)
        mt_buf[g, 0:rg, 0:gw] = mt_buf[g, 0:rg, 0:gw] + jnp.where(same_head, upd, 0.0)
        zr = lax.broadcasted_iota(I32, (8, gw), 0)
        zl = lax.broadcasted_iota(I32, (8, gw), 1)
        zmask = (zl >= zr * DH) & (zl < zr * DH + DH) & (zr < _heads_in_group(g))
        zs = upd[ones_row:ones_row + 1]
        z0 = _norm_row(g)
        mt_buf[g, z0:z0 + 8, 0:gw] = mt_buf[g, z0:z0 + 8, 0:gw] + jnp.where(zmask, zs, 0.0)

    def transpose_wo(g):
        hi = min(128 * (g + 1), D)
        wot.store(wo_raw[:, 128 * g:hi].T, lo=128 * g)

    def project_out(s):
        return jnp.dot(wot.load(), ot_buf[...].astype(BF16), preferred_element_type=F32)

    def residual(s, cols=slice(None)):
        return x_buf[s, :, cols].astype(F32) + xn_buf.load(s, cols=cols).astype(F32)

    def emit(s, val):
        out_buf[s] = val.astype(BF16)
        out_copy(s).start()

    zero = lax.shift_right_logical(i1, 16)

    def prow(start, size):
        return pl.ds(pl.multiple_of(zero + start, 8), size)

    P_OFFS = (0, 128, 384, 768)

    def fast_scores(s, g, hook, anchor):
        nh = _heads_in_group(g)
        gw = GW[g]
        pb = (p_buf0, p_buf1)[(s * NG + g) % 2]
        rowg = lax.broadcasted_iota(I32, (gw // 2, 128), 0)
        laneg = lax.broadcasted_iota(I32, (gw // 2, 128), 1)
        head_rows = [(rowg >= DH // 2 * i) & (rowg < DH // 2 * (i + 1)) for i in range(nh)]
        none = jnp.uint32(0)
        row64 = lax.broadcasted_iota(I32, (64, 128), 0)
        lane64 = lax.broadcasted_iota(I32, (64, 128), 1)
        visible_lo = row64 <= lane64
        row32 = lax.broadcasted_iota(I32, (32, 128), 0)
        lane32 = lax.broadcasted_iota(I32, (32, 128), 1)
        lane16 = lax.broadcasted_iota(I32, (16, 128), 1)
        for j in range(QT - 1, -1, -1):
            n = 128 * (j + 1)
            m = n - 64
            q = qs_buf.load_words(s, 128 * g, 128 * g + gw, slice(128 * j, 128 * (j + 1)))
            for h0, h1 in (((0, 3), (3, nh)) if nh == HPG else ((0, nh),)):
                q_in = anchor(q)
                qm = pltpu.bitcast(
                    jnp.concatenate([jnp.where(head_rows[i], q_in, none) for i in range(h0, h1)], axis=1),
                    BF16)
                st = jnp.dot(k_buf.load(s * NG + g, 0, m, slice(0, gw)), qm, preferred_element_type=F32)
                p = jnp.exp2(st)
                p_diag = jnp.where(jnp.concatenate([visible_lo] * (h1 - h0), axis=1), p[m - 64:], 0.0)
                p = jnp.concatenate([p[:m - 64], p_diag], axis=0) if j > 0 else p_diag
                pb[P_OFFS[j] // 2:(P_OFFS[j] + m) // 2, h0 * 128:h1 * 128] = pltpu.bitcast(p.astype(BF16), U32)
                hook(p)
            for width, k0 in ((64, m), (32, m + 32)):
                per = 128 // width
                q_top = q
                for t in range(per - 1):
                    q_top = jnp.where((laneg >= width * t) & (laneg < width * (t + 1)),
                                      pltpu.roll(q, width * (t + 1), 1), q_top)
                groups = [list(range(i, min(i + per, nh))) for i in range(0, nh, per)]
                tiles = []
                for heads in groups:
                    keep = None
                    for t, i in enumerate(heads):
                        slot = per - len(heads) + t
                        sel = head_rows[i] & (laneg >= width * slot) & (laneg < width * (slot + 1))
                        keep = sel if keep is None else (keep | sel)
                    tiles.append(jnp.where(keep, q_top, none))
                st = jnp.dot(k_buf.load(s * NG + g, k0, k0 + 32, slice(0, gw)),
                             pltpu.bitcast(jnp.concatenate(tiles, axis=1), BF16),
                             preferred_element_type=F32)
                visible = row32 + (k0 - m) <= (lane32 & (width - 1)) + (64 - width)
                p = jnp.where(jnp.concatenate([visible] * len(groups), axis=1), jnp.exp2(st), 0.0)
                p = pltpu.bitcast(p.astype(BF16), U32)
                rows = slice((P_OFFS[j] + k0) // 2, (P_OFFS[j] + k0 + 32) // 2)
                top = lane16 >= 128 - width
                for gi, heads in enumerate(groups):
                    shared = p[:, 128 * gi:128 * (gi + 1)]
                    for t, i in enumerate(heads):
                        slot = per - len(heads) + t
                        shift = width * (per - 1 - slot)
                        mine = shared if shift == 0 else pltpu.roll(shared, shift, 1)
                        pb[rows, 128 * i:128 * (i + 1)] = jnp.where(top, mine, jnp.uint32(0))

    def fast_values(s, g, after_tile=None):
        nh = _heads_in_group(g)
        a_g = _group_row_start(g)
        pb = (p_buf0, p_buf1)[(s * NG + g) % 2]
        for j in range(QT - 1, -1, -1):
            n = 128 * (j + 1)
            cols = slice(128 * j, 128 * (j + 1))
            for i in range(nh):
                h = HPG * g + i
                a = (h * DH // 16) * 16
                off = h * DH - a
                p = pltpu.bitcast(pb[prow(P_OFFS[j] // 2, n // 2), 128 * i:128 * (i + 1)], BF16)
                ones_row = 0 if off > 0 else 31
                lhs = _with_ones_row(vt_buf.load_words(s, a, a + 32, slice(0, n)), ones_row)
                o = jnp.dot(lhs, p, preferred_element_type=F32)
                lo = (off // 8) * 8
                hi = -(-(off + DH) // 8) * 8
                gate = gate_buf[h:h + 1, :]
                rl = 1.0 / o[ones_row:ones_row + 1]
                val = (1.0 - gate) * (o[lo:hi] * rl)
                if s > 0:
                    z = _norm_row(g) + i
                    rden = 1.0 / (num_buf[g, z:z + 1, cols] + 1e-6)
                    num = num_buf[g, a - a_g + lo:a - a_g + hi, cols]
                    val = gate * (num * rden) + val
                ot_buf[a + off:a + off + DH, cols] = val[off - lo:off - lo + DH]
            if after_tile is not None:
                after_tile(j)

    def fast_path():
        hidden = []
        up = expert_up_stream(hidden)
        n_down = FF // 128
        state = dict(down=0, wd_ready=False, up_done=False, y=[None] * 2, tail=None, tail_steps=0,
                     out_ready=False, pacer=None, anchor=None, anchor_next=None)

        def finish():
            yield from expert_scatter_parts([jnp.sum(acc, axis=1, keepdims=True) for acc in state["y"]])
            for u in range(NSEG - 1):
                for j in range(QT):
                    cols = slice(128 * j, 128 * (j + 1))
                    val = (paced(base[u, :, cols]) + x_buf[u, :, cols].astype(F32)
                           ) + xn_buf.load(u, cols=cols).astype(F32)
                    out_buf[u, :, cols] = val.astype(BF16)
                    state["anchor"] = val
                    if j == QT - 1:
                        out_copy(u).start()
                    yield

        def anchor(q):
            val, state["anchor_next"], state["anchor"] = state["anchor_next"], state["anchor"], None
            if val is None:
                return q
            return jnp.where(always[0][:, 0:128], q, pltpu.bitcast(val[D - q.shape[0]:D], U32))

        def paced(val):
            y = state["pacer"]
            if y is None:
                return val
            reps = -(-D // y.shape[0])
            y = jnp.concatenate([y[:, 128 * r:128 * (r + 1)] for r in range(reps)], axis=0)[0:D]
            return jnp.where(always[0][:, 0:128], val, y)

        def down_step():
            ft = state["down"]
            w = paced(wd_buf[:, 128 * ft:128 * (ft + 1)].astype(F32))
            hh = hidden[ft // 4][:, 128 * (ft % 4):128 * (ft % 4 + 1)]
            for slot in range(2):
                term = w * hh[slot:slot + 1]
                state["y"][slot] = term if state["y"][slot] is None else state["y"][slot] + term
            if ft % 6 == 5:
                state["anchor"] = state["y"][1]
            state["down"] += 1

        def hook(pacer=None):
            state["pacer"] = pacer if pacer is not None and pacer.shape[0] * (pacer.shape[1] // 128) >= D else None
            if not state["up_done"] and next(up, "done") == "done":
                state["up_done"] = True
            if state["down"] < n_down:
                if state["wd_ready"] and state["pacer"] is not None and state["down"] // 4 < len(hidden):
                    down_step()
            elif state["out_ready"]:
                if state["tail"] is None:
                    state["tail"] = finish()
                if state["pacer"] is not None or state["tail_steps"] < 2:
                    state["tail_steps"] += 1
                    next(state["tail"], None)

        steps = [(s, g) for s in range(NSEG) for g in range(NG)]
        last = NSEG - 1

        def last_tile(j):
            cols = slice(128 * j, 128 * (j + 1))
            attn = jnp.dot(wot.load(), ot_buf[:, cols].astype(BF16), preferred_element_type=F32)
            out_buf[last, :, cols] = (base[last, :, cols] + residual(last, cols) + attn).astype(BF16)
            out_tile_copy(j).start()

        fast_scores(0, 0, hook, anchor)
        for t, (s, g) in enumerate(steps):
            if t + 1 < len(steps):
                fast_scores(*steps[t + 1], hook, anchor)
            if s > 0:
                memory_read(s, g)
                hook()
            if t + 1 == len(steps):
                state["pacer"] = None
                assert state["down"] == n_down and state["tail"] is not None
                while next(state["tail"], "done") != "done":
                    pass
                pending = []

                def after_tile(j):
                    if pending:
                        last_tile(pending.pop())
                    pending.append(j)

                fast_values(s, g, after_tile)
                last_tile(pending.pop())
            else:
                fast_values(s, g)
            if s == 0:
                transpose_wo(g)
            if s + 1 < NSEG:
                memory_update(s, g)
                hook()
            if g == NG - 1 and s < last:
                base[s] = project_out(s)
                if s == 0:
                    cp_wd.wait()
                    state["wd_ready"] = True
                if s == last - 1:
                    state["out_ready"] = True
                hook()
        for u in range(NSEG - 1):
            out_copy(u).wait()
        for j in range(QT):
            out_tile_copy(j).wait()

    def slow_segment(s, carry):
        for g in range(NG):
            memory_read(s, g)
        key_i = lax.broadcasted_iota(I32, (L, L), 0)
        qry_i = lax.broadcasted_iota(I32, (L, L), 1)
        r32 = lax.broadcasted_iota(I32, (32, L), 0)
        for g in range(NG):
            gw = GW[g]
            a_g = _group_row_start(g)
            rowg = lax.broadcasted_iota(I32, (gw, L), 0)

            def head(i, c, g=g, gw=gw, a_g=a_g, rowg=rowg):
                h = HPG * g + i
                a = pl.multiple_of((h * DH // 16) * 16, 16)
                off = h * DH - a
                q = qs_buf.load(s, 128 * g, 128 * g + gw).astype(F32)
                qm = jnp.where((rowg >= DH * i) & (rowg < DH * (i + 1)), q, 0.0).astype(BF16)
                st = jnp.dot(k_buf.load(s * NG + g, cols=slice(0, gw)), qm, preferred_element_type=F32)
                st = jnp.where(key_i <= qry_i, st, NEG_BIG)
                p = jnp.exp2(st - jnp.max(st, axis=0, keepdims=True))
                rl = 1.0 / jnp.sum(p, axis=0, keepdims=True)
                o = jnp.dot(vt_buf.load(s, a, 32), p.astype(BF16), preferred_element_type=F32)
                gate = jnp.concatenate([gate_buf[pl.ds(h, 1), :]] * QT, axis=1)
                rden = 1.0 / (num_buf[g, pl.ds(_norm_row(g) + i, 1), :] + 1e-6)
                num = num_buf[g, pl.ds(pl.multiple_of(a - a_g, 16), 32), :]
                val = gate * (num * rden) + (1.0 - gate) * (o * rl)
                keep = (r32 >= off) & (r32 < off + DH)
                pltpu.store(ot_buf.at[pl.ds(a, 32), :], val, mask=keep)
                return c

            lax.fori_loop(0, _heads_in_group(g), head, 0)
        for g in range(NG):
            memory_update(s, g)
        emit(s, base[s] + residual(s) + project_out(s))
        return carry

    @pl.when(safe)
    def _():
        fast_path()

    @pl.when(jnp.logical_not(safe))
    def _():
        cp_wd.wait()
        for u in range(NSEG - 1):
            base[u] = jnp.zeros((D, L), F32)
        for g in range(NG):
            transpose_wo(g)
        expert_scatter_rows(expert_chunk(0, FF))
        lax.fori_loop(0, NSEG, slow_segment, 0)
        for u in range(NSEG):
            out_copy(u).wait()


@jax.jit
def pallas_parallel_sum__memory_aug_infini_attn__moe_arch_mod__prompt_kernel(
    A_x: jax.Array,
    A_wq: jax.Array,
    A_wk: jax.Array,
    A_wv: jax.Array,
    A_wo: jax.Array,
    A_beta: jax.Array,
    B_x: jax.Array,
    B_w_r: jax.Array,
    B_w_gate: jax.Array,
    B_w_up: jax.Array,
    B_w_down: jax.Array,
):
    del B_x
    hbm = pl.BlockSpec(memory_space=pl.ANY)
    scratch = [
        pltpu.VMEM((NSEG, D, L), BF16),
        pltpu.VMEM((D, D), BF16),
        pltpu.VMEM((D, D), BF16),
        pltpu.VMEM((D, D), BF16),
        pltpu.VMEM((D, D), BF16),
        pltpu.VMEM((H,), BF16),
        pltpu.VMEM((D,), BF16),
        pltpu.VMEM((D, FF), BF16),
        pltpu.VMEM((D, FF), BF16),
        pltpu.VMEM((D, FF), BF16),
        pltpu.VMEM((PR // 2, D), U32),
        pltpu.VMEM((PR // 2, D), U32),
        pltpu.VMEM((D // 2, D), U32),
        pltpu.VMEM((D // 2, D), U32),
        pltpu.VMEM((NSEG * D // 2, L), U32),
        pltpu.VMEM((NSEG, D, L), F32),
        pltpu.VMEM((NSEG * PR // 2, L), U32),
        pltpu.VMEM((NSEG * PR // 2, L), U32),
        pltpu.VMEM((NSEG * NG * L // 2, 128), U32),
        pltpu.VMEM((NSEG * PR // 2, L), U32),
        pltpu.VMEM((NSEG * D // 2, L), U32),
        pltpu.VMEM((8, S), F32),
        pltpu.VMEM((H, 128), F32),
        pltpu.VMEM((NG, MROWS, 128), F32),
        pltpu.VMEM((NG, MROWS, L), F32),
        pltpu.VMEM((640, HPG * 128), U32),
        pltpu.VMEM((640, HPG * 128), U32),
        pltpu.VMEM((D, L), F32),
        pltpu.VMEM((NSEG, D, L), BF16),
        pltpu.SemaphoreType.DMA((13,)),
        pltpu.SemaphoreType.DMA((NSEG + QT,)),
    ]
    out_t = pl.pallas_call(
        _kernel,
        out_shape=jax.ShapeDtypeStruct((1, D, S), BF16),
        in_specs=[hbm] * 10,
        out_specs=hbm,
        scratch_shapes=scratch,
        compiler_params=pltpu.CompilerParams(vmem_limit_bytes=128 * 1024 * 1024),
        name="infini_attn_moe",
    )(jnp.transpose(A_x, (0, 2, 1)), A_wq, A_wk, A_wv, A_wo, A_beta, B_w_r, B_w_gate, B_w_up,
      B_w_down.T)
    return jnp.transpose(out_t, (0, 2, 1))
```

```python
import jax
import jax.numpy as jnp
from jax import lax
import jax.experimental.pallas as pl
import jax.experimental.pallas.tpu as pltpu

F32 = jnp.float32
BF16 = jnp.bfloat16
U32 = jnp.uint32
I32 = jnp.int32

S = 2048
D = 576
H = 32
DH = 18
NSEG = 4
L = 512
FF = 4608
HPG = 7
NG = 5
QT = L // 128
GW = (128, 128, 128, 128, 80)
PR = sum(GW)
ROUTER_ROW = 126
MROWS = 144
LOG2E = 1.4426950408889634
QSCALE = (DH ** -0.5) * LOG2E
SAFE_LOG2_RANGE = 40.0
NEG_BIG = -1e30

NT_DIMS = (((1,), (1,)), ((), ()))


def _heads_in_group(g):
    return min(HPG, H - HPG * g)


def _group_row_start(g):
    return (HPG * g * DH // 16) * 16


def _group_rows(g):
    last = (HPG * g + _heads_in_group(g)) * DH
    return -(-(last - _group_row_start(g)) // 16) * 16


def _state_rows(g):
    return MROWS if g == 0 else _group_rows(g)


def _norm_row(g):
    return 128 if g == 0 else 0


def _round_bf16(x):
    return x.astype(BF16).astype(F32)


def _pad_heads_t(w):
    parts = []
    for g in range(NG):
        n = _heads_in_group(g) * DH
        parts.append(w[:, HPG * DH * g:HPG * DH * g + n])
        parts.append(jnp.zeros((D, 128 - n), w.dtype))
    return jnp.concatenate(parts, axis=1).T[0:PR]


def _recip(x):
    r = pl.reciprocal(x, approx=True)
    return r * (2.0 - x * r)


def _visible_words(rows, lanes_seen):
    k = 2 * lax.broadcasted_iota(I32, (rows // 2, 128), 0)
    return (jnp.where(k <= lanes_seen, jnp.uint32(0x0000FFFF), jnp.uint32(0))
            | jnp.where(k + 1 <= lanes_seen, jnp.uint32(0xFFFF0000), jnp.uint32(0)))


def _phi(t):
    return jnp.where(t > 0, t + 1.0, jnp.exp(t))


class _Packed:
    def __init__(self, ref, rows):
        self.ref = ref
        self.rows = rows

    def _slice(self, item, lo, size):
        start = item * (self.rows // 2) + lo // 2
        size = size // 2
        if isinstance(start, int):
            return slice(start, start + size)
        return pl.ds(pl.multiple_of(start, 8), size)

    def load_words(self, item=0, lo=0, hi=None, cols=slice(None)):
        size = hi if not isinstance(lo, int) else (self.rows if hi is None else hi) - lo
        return self.ref[self._slice(item, lo, size), cols]

    def load(self, item=0, lo=0, hi=None, cols=slice(None)):
        return pltpu.bitcast(self.load_words(item, lo, hi, cols), BF16)

    def store(self, val, item=0, lo=0, cols=slice(None)):
        self.ref[self._slice(item, lo, val.shape[0]), cols] = pltpu.bitcast(val.astype(BF16), U32)


def _with_ones_row(words, row):
    r = row // 2
    lo = (r // 8) * 8
    keep, one = (0x0000FFFF, 0x3F800000) if row % 2 else (0xFFFF0000, 0x00003F80)
    blk = words[lo:lo + 8]
    hit = lax.broadcasted_iota(I32, blk.shape, 0) == r - lo
    blk = jnp.where(hit, (blk & jnp.uint32(keep)) | jnp.uint32(one), blk)
    parts = [part for part in (words[0:lo], blk, words[lo + 8:]) if part.shape[0]]
    return pltpu.bitcast(jnp.concatenate(parts, axis=0), BF16)


def _kernel(x_hbm, wq_hbm, wk_hbm, wv_hbm, wo_hbm, beta_hbm, wr_hbm, wg_hbm, wu_hbm, wd_hbm,
            out_hbm,
            x_buf, wq_raw, wk_raw, wv_raw, wo_raw, beta_buf, wr_buf, wg_buf, wu_buf, wd_buf,
            wqt, wkt, wvt, wot, xn_buf, base, qs_buf, pq_buf, k_buf, pk_buf, vt_buf, r_buf,
            gate_buf, mt_buf, num_buf, p_buf0, p_buf1, ot_buf, out_buf, in_sems, out_sems):
    wqt, wkt = _Packed(wqt, PR), _Packed(wkt, PR)
    wvt, wot = _Packed(wvt, D), _Packed(wot, D)
    xn_buf, vt_buf = _Packed(xn_buf, D), _Packed(vt_buf, D)
    qs_buf, pq_buf, pk_buf = _Packed(qs_buf, PR), _Packed(pq_buf, PR), _Packed(pk_buf, PR)
    k_buf = _Packed(k_buf, L)

    def x_copy(c):
        return pltpu.make_async_copy(x_hbm.at[0, :, pl.ds(c * L, L)], x_buf.at[c], in_sems.at[c])

    cp_wv = pltpu.make_async_copy(wv_hbm, wv_raw, in_sems.at[4])
    cp_wq = pltpu.make_async_copy(wq_hbm, wq_raw, in_sems.at[5])
    cp_wk = pltpu.make_async_copy(wk_hbm, wk_raw, in_sems.at[6])
    cp_wo = pltpu.make_async_copy(wo_hbm, wo_raw, in_sems.at[7])
    cp_wg = pltpu.make_async_copy(wg_hbm, wg_buf, in_sems.at[8])
    cp_wu = pltpu.make_async_copy(wu_hbm, wu_buf, in_sems.at[9])
    cp_wd = pltpu.make_async_copy(wd_hbm, wd_buf, in_sems.at[10])
    cp_beta = pltpu.make_async_copy(beta_hbm, beta_buf, in_sems.at[11])
    cp_wr = pltpu.make_async_copy(wr_hbm, wr_buf, in_sems.at[12])

    def out_copy(s):
        cols = pl.ds(pl.multiple_of(s * L, L), L)
        return pltpu.make_async_copy(out_buf.at[s], out_hbm.at[0, :, cols], out_sems.at[s])

    def out_tile_copy(j):
        s = NSEG - 1
        return pltpu.make_async_copy(out_buf.at[s, :, pl.ds(128 * j, 128)],
                                     out_hbm.at[0, :, pl.ds(s * L + 128 * j, 128)], out_sems.at[NSEG + j])

    for cp in (x_copy(0), cp_wv, x_copy(1), cp_wq, cp_wr, cp_beta, x_copy(2), cp_wk, x_copy(3), cp_wo,
               cp_wg, cp_wu, cp_wd):
        cp.start()

    mt_buf[...] = jnp.zeros(mt_buf.shape, F32)

    always = []

    def pace(x, y):
        return x if y is None else jnp.where(always[0], x, y[0:D])

    def ln_stats(c, y):
        shift = x_buf[c, 0:16, :].astype(F32)[0:1]
        d = pace(x_buf[c].astype(F32), y) - shift
        m1 = jnp.sum(d, axis=0, keepdims=True) * (1.0 / D)
        m2 = jnp.sum(d * d, axis=0, keepdims=True) * (1.0 / D)
        var = jnp.maximum(m2 - m1 * m1, 0.0)
        inv = 1.0 / _round_bf16(jnp.sqrt(_round_bf16(_round_bf16(var) + 1e-5)))
        return _round_bf16(shift + m1), inv

    def ln_apply(c, mean_b, inv):
        x = x_buf[c].astype(F32)
        xn = (x - mean_b) * inv
        xn_buf.store(xn, c)
        if c == NSEG - 1:
            base[c] = jnp.zeros((D, L), F32)

    def project(w_ref, c, split):
        if not split:
            return jnp.dot(w_ref.load(), xn_buf.load(c), preferred_element_type=F32), None
        head = jnp.dot(w_ref.load(cols=slice(0, 256)), xn_buf.load(c, 0, 256), preferred_element_type=F32)
        tail = jnp.dot(w_ref.load(cols=slice(256, D)), xn_buf.load(c, 256, D), preferred_element_type=F32)
        return head + tail, head

    def project_v(c, mid=None):
        vt, head = project(wvt, c, mid is not None)
        if mid is not None:
            mid(head)
        vt_buf.store(vt, c)
        return vt

    def project_q(c, mid=None):
        qt, head = project(wqt, c, mid is not None)
        if mid is not None:
            mid(head)
        qsc = qt * QSCALE
        qs_buf.store(qsc, c)
        pq_buf.store(_phi(qt), c)
        r_buf[:, c * L:(c + 1) * L] = qt[120:128]
        mag = jnp.abs(qsc)
        r8 = lax.broadcasted_iota(I32, (8, L), 0)
        mag = jnp.concatenate([mag[0:120], jnp.where(r8 == ROUTER_ROW - 120, 0.0, mag[120:128]), mag[128:]], axis=0)
        return qt, jnp.max(mag.reshape(PR // 8, 8, L), axis=0)

    def project_k(c, mid=None, keep=False):
        kt, head = project(wkt, c, mid is not None)
        if mid is not None:
            mid(head)
        pk_buf.store(_phi(kt), c)
        for g in range(NG):
            ktg = kt[128 * g:128 * g + GW[g]]
            if GW[g] < 128:
                ktg = jnp.concatenate([ktg, jnp.zeros((128 - GW[g], L), F32)], axis=0)
            k_buf.store(ktg.T, c * NG + g)
        top = jnp.max(jnp.abs(kt).reshape(PR // 8, 8, L), axis=0)
        return (kt, top) if keep else top

    x_copy(0).wait()
    stats = ln_stats(0, None)
    always.append(jnp.logical_not(jnp.abs(stats[0]) < 0.0))
    ln_apply(0, *stats)
    cp_wv.wait()
    wvt.store(wv_raw[...].T)
    project_v(0)
    x_copy(1).wait()
    cp_wq.wait()
    cp_wr.wait()
    ln_apply(1, *ln_stats(1, None))

    def paced_weight(w_ref, y):
        w = w_ref[...].astype(F32)
        return jnp.concatenate([jnp.where(always[0], w[:, 0:L], y[0:D]), w[:, L:D]], axis=1)

    def prep_wq(y):
        wq_t = _pad_heads_t(paced_weight(wq_raw, y))
        wr_row = wr_buf[...].reshape(1, D).astype(F32)
        pr_row = lax.broadcasted_iota(I32, (8, D), 0)
        wq_t = jnp.concatenate(
            [wq_t[0:120], jnp.where(pr_row == ROUTER_ROW - 120, wr_row, wq_t[120:128]), wq_t[128:]], axis=0)
        wqt.store(wq_t)

    project_v(1, prep_wq)
    cp_wk.wait()
    cp_beta.wait()
    x_copy(2).wait()
    x_copy(3).wait()

    beta_row = beta_buf[...].reshape(1, H).astype(F32)
    beta_row = jnp.concatenate([beta_row, jnp.zeros((1, 128 - H), F32)], axis=1)
    h_row = lax.broadcasted_iota(I32, (H, 128), 0)
    h_lane = lax.broadcasted_iota(I32, (H, 128), 1)
    beta_col = jnp.sum(jnp.where(h_row == h_lane, beta_row, 0.0), axis=1, keepdims=True)
    gate_buf[...] = jnp.broadcast_to(jax.nn.sigmoid(beta_col), (H, 128))

    def prep_wk(y):
        wkt.store(_pad_heads_t(paced_weight(wk_raw, y)))

    def route():
        r = _round_bf16(r_buf[ROUTER_ROW - 120:ROUTER_ROW - 119, :])
        tok = lax.broadcasted_iota(I32, (1, S), 1).astype(F32)
        m1 = jnp.max(r)
        i1 = jnp.min(jnp.where(r == m1, tok, float(S)))
        r_rest = jnp.where(tok == i1, -jnp.inf, r)
        m2 = jnp.max(r_rest)
        i2 = jnp.min(jnp.where(r_rest == m2, tok, float(S)))
        i1 = jnp.clip(i1.astype(I32), 0, S - 1)
        i2 = jnp.clip(i2.astype(I32), 0, S - 1)
        return m1, m2, i1, i2

    qt, aq = project_q(0, prep_wk)
    qt, a = project_q(1)
    aq = jnp.maximum(aq, a)
    stats = ln_stats(2, qt)
    ak = project_k(0)
    ln_apply(2, *stats)
    kt, a = project_k(1, keep=True)
    ak = jnp.maximum(ak, a)
    stats = ln_stats(3, kt)
    project_v(2)
    ln_apply(3, *stats)
    qt, a = project_q(2)
    aq = jnp.maximum(aq, a)
    ak = jnp.maximum(ak, project_k(2))
    qt, a = project_q(3)
    aq = jnp.maximum(aq, a)
    m1, m2, i1, i2 = route()
    ak = jnp.maximum(ak, project_k(3))
    project_v(3)

    logit_bound = jnp.max(aq) * jnp.max(ak) * (DH * 1.02)
    safe = logit_bound <= SAFE_LOG2_RANGE

    sel_row = lax.broadcasted_iota(I32, (16, 128), 0)
    sel_lane = lax.broadcasted_iota(I32, (16, 128), 1)

    def token_tile(i):
        return i // L, pl.ds(pl.multiple_of(((i % L) // 128) * 128, 128), 128)

    def pick(i, slot):
        seg, cols = token_tile(i)
        onehot = jnp.where((sel_row == slot) & (sel_lane == i % 128), 1.0, 0.0).astype(BF16)
        return lax.dot_general(onehot, xn_buf.load(seg, cols=cols), NT_DIMS, preferred_element_type=F32)

    def routed_rows():
        return (pick(i1, 0) + pick(i2, 1)).astype(BF16)

    cp_wo.wait()
    cp_wg.wait()
    cp_wu.wait()

    def expert_chunk(lo, hi):
        xs = routed_rows()
        hg = jnp.dot(xs, wg_buf[:, lo:hi], preferred_element_type=F32)
        hu = jnp.dot(xs, wu_buf[:, lo:hi], preferred_element_type=F32)
        hh = (jax.nn.silu(hg) * hu).astype(BF16)
        return lax.dot_general(hh, wd_buf[:, lo:hi], NT_DIMS, preferred_element_type=F32)

    def expert_up_stream(hidden):
        kmain = 512
        xs = routed_rows()
        tail = xs[:, kmain:D].astype(F32)
        zero = jnp.zeros_like(tail)
        r16k = lax.broadcasted_iota(I32, (16, 128), 0)
        xs_rem = jnp.where(r16k < 2, jnp.concatenate([tail, zero], axis=1),
                           pltpu.roll(jnp.concatenate([zero, tail], axis=1), 2, 0)).astype(BF16)
        yield
        for c0 in range(0, FF, 512):
            w_rem = jnp.concatenate([wg_buf[kmain:D, c0:c0 + 512], wu_buf[kmain:D, c0:c0 + 512]], axis=0)
            both = jnp.dot(xs_rem, w_rem, preferred_element_type=F32)
            rem = (both, pltpu.roll(both, 14, 0))
            yield
            hs = []
            for f0 in range(c0, c0 + 512, 128):
                pre = []
                for w_ref, r in zip((wg_buf, wu_buf), rem):
                    pre.append(jnp.dot(xs[:, 0:kmain], w_ref[0:kmain, f0:f0 + 128], preferred_element_type=F32)
                               + r[:, f0 - c0:f0 - c0 + 128])
                    if len(pre) == 2:
                        hs.append(jax.nn.silu(pre[0]) * pre[1])
                        if len(hs) == 4:
                            hidden.append(_round_bf16(jnp.concatenate(hs, axis=1)))
                    yield

    lane_d = lax.broadcasted_iota(I32, (D, 128), 1)

    def expert_scatter_parts(columns):
        for col, i, score in zip(columns, (i1, i2), (m1, m2)):
            seg, cols = token_tile(i)
            col = col * jax.nn.sigmoid(jnp.full((D, 1), score, F32))
            base[seg, :, cols] = base[seg, :, cols] + jnp.where(lane_d == i % 128, col, 0.0)
            yield

    def expert_scatter_rows(y):
        yt = jnp.concatenate([y, jnp.zeros((128 - 16, D), F32)], axis=0).T
        columns = [jnp.sum(jnp.where(lane_d == slot, yt, 0.0), axis=1, keepdims=True) for slot in range(2)]
        for _ in expert_scatter_parts(columns):
            pass

    def memory_read(s, g):
        sr = _state_rows(g)
        gw = GW[g]
        num_buf[g, 0:sr, :] = jnp.dot(mt_buf[g, 0:sr, 0:gw].astype(BF16), pq_buf.load(s, 128 * g, 128 * g + gw),
                                      preferred_element_type=F32)

    def memory_update(s, g):
        rg = _group_rows(g)
        a_g = _group_row_start(g)
        gw = GW[g]
        ones_row = 126 if g == 0 else 0
        lhs = _with_ones_row(vt_buf.load_words(s, a_g, a_g + rg), ones_row)
        upd = lax.dot_general(lhs, pk_buf.load(s, 128 * g, 128 * g + gw), NT_DIMS,
                              preferred_element_type=F32)
        er = lax.broadcasted_iota(I32, (rg, gw), 0) + (a_g - HPG * DH * g)
        el = lax.broadcasted_iota(I32, (rg, gw), 1)
        same_head = None
        for i in range(_heads_in_group(g)):
            t = ((er >= DH * i) & (er < DH * (i + 1)) & (el >= DH * i) & (el < DH * (i + 1)))
            same_head = t if same_head is None else (same_head | t)
        mt_buf[g, 0:rg, 0:gw] = mt_buf[g, 0:rg, 0:gw] + jnp.where(same_head, upd, 0.0)
        zr = lax.broadcasted_iota(I32, (8, gw), 0)
        zl = lax.broadcasted_iota(I32, (8, gw), 1)
        zmask = (zl >= zr * DH) & (zl < zr * DH + DH) & (zr < _heads_in_group(g))
        zs = upd[ones_row:ones_row + 1]
        z0 = _norm_row(g)
        mt_buf[g, z0:z0 + 8, 0:gw] = mt_buf[g, z0:z0 + 8, 0:gw] + jnp.where(zmask, zs, 0.0)

    def transpose_wo(g):
        hi = min(128 * (g + 1), D)
        wot.store(wo_raw[:, 128 * g:hi].T, lo=128 * g)

    def project_out(s):
        return jnp.dot(wot.load(), ot_buf[...].astype(BF16), preferred_element_type=F32)

    def residual(s, cols=slice(None)):
        return x_buf[s, :, cols].astype(F32) + xn_buf.load(s, cols=cols).astype(F32)

    def emit(s, val):
        out_buf[s] = val.astype(BF16)
        out_copy(s).start()

    zero = lax.shift_right_logical(i1, 16)

    def prow(start, size):
        return pl.ds(pl.multiple_of(zero + start, 8), size)

    P_OFFS = (0, 128, 384, 768)

    def fast_scores(s, g, hook, anchor):
        nh = _heads_in_group(g)
        gw = GW[g]
        pb = (p_buf0, p_buf1)[(s * NG + g) % 2]
        rowg = lax.broadcasted_iota(I32, (gw // 2, 128), 0)
        laneg = lax.broadcasted_iota(I32, (gw // 2, 128), 1)
        head_rows = [(rowg >= DH // 2 * i) & (rowg < DH // 2 * (i + 1)) for i in range(nh)]
        none = jnp.uint32(0)
        visible_lo = _visible_words(64, lax.broadcasted_iota(I32, (32, 128), 1))
        lane16 = lax.broadcasted_iota(I32, (16, 128), 1)
        for j in range(QT - 1, -1, -1):
            n = 128 * (j + 1)
            m = n - 64
            q = qs_buf.load_words(s, 128 * g, 128 * g + gw, slice(128 * j, 128 * (j + 1)))
            for h0, h1 in (((0, 3), (3, nh)) if nh == HPG else ((0, nh),)):
                q_in = anchor(q)
                qm = pltpu.bitcast(
                    jnp.concatenate([jnp.where(head_rows[i], q_in, none) for i in range(h0, h1)], axis=1),
                    BF16)
                st = jnp.dot(k_buf.load(s * NG + g, 0, m, slice(0, gw)), qm, preferred_element_type=F32)
                p = jnp.exp2(st)
                words = pltpu.bitcast(p.astype(BF16), U32)
                diag = words[m // 2 - 32:] & jnp.concatenate([visible_lo] * (h1 - h0), axis=1)
                words = jnp.concatenate([words[:m // 2 - 32], diag], axis=0) if j > 0 else diag
                pb[P_OFFS[j] // 2:(P_OFFS[j] + m) // 2, h0 * 128:h1 * 128] = words
                hook(p)
            for width, k0 in ((64, m), (32, m + 32)):
                per = 128 // width
                q_top = q
                for t in range(per - 1):
                    q_top = jnp.where((laneg >= width * t) & (laneg < width * (t + 1)),
                                      pltpu.roll(q, width * (t + 1), 1), q_top)
                groups = [list(range(i, min(i + per, nh))) for i in range(0, nh, per)]
                tiles = []
                for heads in groups:
                    keep = None
                    for t, i in enumerate(heads):
                        slot = per - len(heads) + t
                        sel = head_rows[i] & (laneg >= width * slot) & (laneg < width * (slot + 1))
                        keep = sel if keep is None else (keep | sel)
                    tiles.append(jnp.where(keep, q_top, none))
                st = jnp.dot(k_buf.load(s * NG + g, k0, k0 + 32, slice(0, gw)),
                             pltpu.bitcast(jnp.concatenate(tiles, axis=1), BF16),
                             preferred_element_type=F32)
                visible = _visible_words(32, lane16 & (width - 1))
                p = pltpu.bitcast(jnp.exp2(st).astype(BF16), U32)
                p = p & jnp.concatenate([visible] * len(groups), axis=1)
                rows = slice((P_OFFS[j] + k0) // 2, (P_OFFS[j] + k0 + 32) // 2)
                top = lane16 >= 128 - width
                for gi, heads in enumerate(groups):
                    shared = p[:, 128 * gi:128 * (gi + 1)]
                    for t, i in enumerate(heads):
                        slot = per - len(heads) + t
                        shift = width * (per - 1 - slot)
                        mine = shared if shift == 0 else pltpu.roll(shared, shift, 1)
                        pb[rows, 128 * i:128 * (i + 1)] = jnp.where(top, mine, jnp.uint32(0))

    def fast_values(s, g, after_tile=None):
        nh = _heads_in_group(g)
        a_g = _group_row_start(g)
        pb = (p_buf0, p_buf1)[(s * NG + g) % 2]
        for j in range(QT - 1, -1, -1):
            n = 128 * (j + 1)
            cols = slice(128 * j, 128 * (j + 1))
            for i in range(nh):
                h = HPG * g + i
                a = (h * DH // 16) * 16
                off = h * DH - a
                p = pltpu.bitcast(pb[prow(P_OFFS[j] // 2, n // 2), 128 * i:128 * (i + 1)], BF16)
                ones_row = 0 if off > 0 else 31
                lhs = _with_ones_row(vt_buf.load_words(s, a, a + 32, slice(0, n)), ones_row)
                o = jnp.dot(lhs, p, preferred_element_type=F32)
                lo = (off // 8) * 8
                hi = -(-(off + DH) // 8) * 8
                gate = gate_buf[h:h + 1, :]
                rl = _recip(o[ones_row:ones_row + 1])
                val = (1.0 - gate) * (o[lo:hi] * rl)
                if s > 0:
                    z = _norm_row(g) + i
                    rden = _recip(num_buf[g, z:z + 1, cols] + 1e-6)
                    num = num_buf[g, a - a_g + lo:a - a_g + hi, cols]
                    val = gate * (num * rden) + val
                ot_buf[a + off:a + off + DH, cols] = val[off - lo:off - lo + DH]
            if after_tile is not None:
                after_tile(j)

    def fast_path():
        hidden = []
        up = expert_up_stream(hidden)
        n_down = FF // 128
        state = dict(down=0, wd_ready=False, up_done=False, y=[None] * 2, tail=None, tail_steps=0,
                     out_ready=False, pacer=None, anchor=None, anchor_next=None)

        def finish():
            yield from expert_scatter_parts([jnp.sum(acc, axis=1, keepdims=True) for acc in state["y"]])
            for u in range(NSEG - 1):
                for j in range(QT):
                    cols = slice(128 * j, 128 * (j + 1))
                    val = (paced(base[u, :, cols]) + x_buf[u, :, cols].astype(F32)
                           ) + xn_buf.load(u, cols=cols).astype(F32)
                    out_buf[u, :, cols] = val.astype(BF16)
                    state["anchor"] = val
                    if j == QT - 1:
                        out_copy(u).start()
                    yield

        def anchor(q):
            val, state["anchor_next"], state["anchor"] = state["anchor_next"], state["anchor"], None
            if val is None:
                return q
            return jnp.where(always[0][:, 0:128], q, pltpu.bitcast(val[D - q.shape[0]:D], U32))

        def paced(val):
            y = state["pacer"]
            if y is None:
                return val
            reps = -(-D // y.shape[0])
            y = jnp.concatenate([y[:, 128 * r:128 * (r + 1)] for r in range(reps)], axis=0)[0:D]
            return jnp.where(always[0][:, 0:128], val, y)

        def down_step():
            ft = state["down"]
            w = paced(wd_buf[:, 128 * ft:128 * (ft + 1)].astype(F32))
            hh = hidden[ft // 4][:, 128 * (ft % 4):128 * (ft % 4 + 1)]
            for slot in range(2):
                term = w * hh[slot:slot + 1]
                state["y"][slot] = term if state["y"][slot] is None else state["y"][slot] + term
            if ft % 6 == 5:
                state["anchor"] = state["y"][1]
            state["down"] += 1

        def hook(pacer=None):
            state["pacer"] = pacer if pacer is not None and pacer.shape[0] * (pacer.shape[1] // 128) >= D else None
            if not state["up_done"] and next(up, "done") == "done":
                state["up_done"] = True
            if state["down"] < n_down:
                if state["wd_ready"] and state["pacer"] is not None and state["down"] // 4 < len(hidden):
                    down_step()
            elif state["out_ready"]:
                if state["tail"] is None:
                    state["tail"] = finish()
                if state["pacer"] is not None or state["tail_steps"] < 2:
                    state["tail_steps"] += 1
                    next(state["tail"], None)

        steps = [(s, g) for s in range(NSEG) for g in range(NG)]
        last = NSEG - 1

        def last_tile(j):
            cols = slice(128 * j, 128 * (j + 1))
            attn = jnp.dot(wot.load(), ot_buf[:, cols].astype(BF16), preferred_element_type=F32)
            out_buf[last, :, cols] = (base[last, :, cols] + residual(last, cols) + attn).astype(BF16)
            out_tile_copy(j).start()

        fast_scores(0, 0, hook, anchor)
        for t, (s, g) in enumerate(steps):
            if t + 1 < len(steps):
                fast_scores(*steps[t + 1], hook, anchor)
            if s > 0:
                memory_read(s, g)
                hook()
            if t + 1 == len(steps):
                state["pacer"] = None
                assert state["down"] == n_down and state["tail"] is not None
                while next(state["tail"], "done") != "done":
                    pass
                pending = []

                def after_tile(j):
                    if pending:
                        last_tile(pending.pop())
                    pending.append(j)

                fast_values(s, g, after_tile)
                last_tile(pending.pop())
            else:
                fast_values(s, g)
            if s == 0:
                transpose_wo(g)
            if s + 1 < NSEG:
                memory_update(s, g)
                hook()
            if g == NG - 1 and s < last:
                base[s] = project_out(s)
                if s == 0:
                    cp_wd.wait()
                    state["wd_ready"] = True
                if s == last - 1:
                    state["out_ready"] = True
                hook()
        for u in range(NSEG - 1):
            out_copy(u).wait()
        for j in range(QT):
            out_tile_copy(j).wait()

    def slow_segment(s, carry):
        for g in range(NG):
            memory_read(s, g)
        key_i = lax.broadcasted_iota(I32, (L, L), 0)
        qry_i = lax.broadcasted_iota(I32, (L, L), 1)
        r32 = lax.broadcasted_iota(I32, (32, L), 0)
        for g in range(NG):
            gw = GW[g]
            a_g = _group_row_start(g)
            rowg = lax.broadcasted_iota(I32, (gw, L), 0)

            def head(i, c, g=g, gw=gw, a_g=a_g, rowg=rowg):
                h = HPG * g + i
                a = pl.multiple_of((h * DH // 16) * 16, 16)
                off = h * DH - a
                q = qs_buf.load(s, 128 * g, 128 * g + gw).astype(F32)
                qm = jnp.where((rowg >= DH * i) & (rowg < DH * (i + 1)), q, 0.0).astype(BF16)
                st = jnp.dot(k_buf.load(s * NG + g, cols=slice(0, gw)), qm, preferred_element_type=F32)
                st = jnp.where(key_i <= qry_i, st, NEG_BIG)
                p = jnp.exp2(st - jnp.max(st, axis=0, keepdims=True))
                rl = 1.0 / jnp.sum(p, axis=0, keepdims=True)
                o = jnp.dot(vt_buf.load(s, a, 32), p.astype(BF16), preferred_element_type=F32)
                gate = jnp.concatenate([gate_buf[pl.ds(h, 1), :]] * QT, axis=1)
                rden = 1.0 / (num_buf[g, pl.ds(_norm_row(g) + i, 1), :] + 1e-6)
                num = num_buf[g, pl.ds(pl.multiple_of(a - a_g, 16), 32), :]
                val = gate * (num * rden) + (1.0 - gate) * (o * rl)
                keep = (r32 >= off) & (r32 < off + DH)
                pltpu.store(ot_buf.at[pl.ds(a, 32), :], val, mask=keep)
                return c

            lax.fori_loop(0, _heads_in_group(g), head, 0)
        for g in range(NG):
            memory_update(s, g)
        emit(s, base[s] + residual(s) + project_out(s))
        return carry

    @pl.when(safe)
    def _():
        fast_path()

    @pl.when(jnp.logical_not(safe))
    def _():
        cp_wd.wait()
        for u in range(NSEG - 1):
            base[u] = jnp.zeros((D, L), F32)
        for g in range(NG):
            transpose_wo(g)
        expert_scatter_rows(expert_chunk(0, FF))
        lax.fori_loop(0, NSEG, slow_segment, 0)
        for u in range(NSEG):
            out_copy(u).wait()


@jax.jit
def pallas_parallel_sum__memory_aug_infini_attn__moe_arch_mod__prompt_kernel(
    A_x: jax.Array,
    A_wq: jax.Array,
    A_wk: jax.Array,
    A_wv: jax.Array,
    A_wo: jax.Array,
    A_beta: jax.Array,
    B_x: jax.Array,
    B_w_r: jax.Array,
    B_w_gate: jax.Array,
    B_w_up: jax.Array,
    B_w_down: jax.Array,
):
    del B_x
    hbm = pl.BlockSpec(memory_space=pl.ANY)
    scratch = [
        pltpu.VMEM((NSEG, D, L), BF16),
        pltpu.VMEM((D, D), BF16),
        pltpu.VMEM((D, D), BF16),
        pltpu.VMEM((D, D), BF16),
        pltpu.VMEM((D, D), BF16),
        pltpu.VMEM((H,), BF16),
        pltpu.VMEM((D,), BF16),
        pltpu.VMEM((D, FF), BF16),
        pltpu.VMEM((D, FF), BF16),
        pltpu.VMEM((D, FF), BF16),
        pltpu.VMEM((PR // 2, D), U32),
        pltpu.VMEM((PR // 2, D), U32),
        pltpu.VMEM((D // 2, D), U32),
        pltpu.VMEM((D // 2, D), U32),
        pltpu.VMEM((NSEG * D // 2, L), U32),
        pltpu.VMEM((NSEG, D, L), F32),
        pltpu.VMEM((NSEG * PR // 2, L), U32),
        pltpu.VMEM((NSEG * PR // 2, L), U32),
        pltpu.VMEM((NSEG * NG * L // 2, 128), U32),
        pltpu.VMEM((NSEG * PR // 2, L), U32),
        pltpu.VMEM((NSEG * D // 2, L), U32),
        pltpu.VMEM((8, S), F32),
        pltpu.VMEM((H, 128), F32),
        pltpu.VMEM((NG, MROWS, 128), F32),
        pltpu.VMEM((NG, MROWS, L), F32),
        pltpu.VMEM((640, HPG * 128), U32),
        pltpu.VMEM((640, HPG * 128), U32),
        pltpu.VMEM((D, L), F32),
        pltpu.VMEM((NSEG, D, L), BF16),
        pltpu.SemaphoreType.DMA((13,)),
        pltpu.SemaphoreType.DMA((NSEG + QT,)),
    ]
    out_t = pl.pallas_call(
        _kernel,
        out_shape=jax.ShapeDtypeStruct((1, D, S), BF16),
        in_specs=[hbm] * 10,
        out_specs=hbm,
        scratch_shapes=scratch,
        compiler_params=pltpu.CompilerParams(vmem_limit_bytes=128 * 1024 * 1024),
        name="infini_attn_moe",
    )(jnp.transpose(A_x, (0, 2, 1)), A_wq, A_wk, A_wv, A_wo, A_beta, B_w_r, B_w_gate, B_w_up,
      B_w_down.T)
    return jnp.transpose(out_t, (0, 2, 1))
```

```python
import jax
import jax.numpy as jnp
from jax import lax
import jax.experimental.pallas as pl
import jax.experimental.pallas.tpu as pltpu

F32 = jnp.float32
BF16 = jnp.bfloat16
U32 = jnp.uint32
I32 = jnp.int32

S = 2048
D = 576
H = 32
DH = 18
NSEG = 4
L = 512
FF = 4608
HPG = 7
NG = 5
QT = L // 128
GW = (128, 128, 128, 128, 80)
PR = sum(GW)
ROUTER_ROW = 126
MROWS = 144
LOG2E = 1.4426950408889634
QSCALE = (DH ** -0.5) * LOG2E
SAFE_LOG2_RANGE = 40.0
NEG_BIG = -1e30

NT_DIMS = (((1,), (1,)), ((), ()))


def _heads_in_group(g):
    return min(HPG, H - HPG * g)


def _group_row_start(g):
    return (HPG * g * DH // 16) * 16


def _group_rows(g):
    last = (HPG * g + _heads_in_group(g)) * DH
    return -(-(last - _group_row_start(g)) // 16) * 16


def _state_rows(g):
    return MROWS if g == 0 else _group_rows(g)


def _norm_row(g):
    return 128 if g == 0 else 0


def _round_bf16(x):
    return x.astype(BF16).astype(F32)


def _pad_heads_t(w):
    parts = []
    for g in range(NG):
        n = _heads_in_group(g) * DH
        parts.append(w[:, HPG * DH * g:HPG * DH * g + n])
        parts.append(jnp.zeros((D, 128 - n), w.dtype))
    return jnp.concatenate(parts, axis=1).T[0:PR]


def _recip(x):
    r = pl.reciprocal(x, approx=True)
    return r * (2.0 - x * r)


def _visible_words(rows, lanes_seen):
    k = 2 * lax.broadcasted_iota(I32, (rows // 2, 128), 0)
    return (jnp.where(k <= lanes_seen, jnp.uint32(0x0000FFFF), jnp.uint32(0))
            | jnp.where(k + 1 <= lanes_seen, jnp.uint32(0xFFFF0000), jnp.uint32(0)))


def _phi(t):
    return jnp.where(t > 0, t + 1.0, jnp.exp(t))


class _Packed:
    def __init__(self, ref, rows):
        self.ref = ref
        self.rows = rows

    def _slice(self, item, lo, size):
        start = item * (self.rows // 2) + lo // 2
        size = size // 2
        if isinstance(start, int):
            return slice(start, start + size)
        return pl.ds(pl.multiple_of(start, 8), size)

    def load_words(self, item=0, lo=0, hi=None, cols=slice(None)):
        size = hi if not isinstance(lo, int) else (self.rows if hi is None else hi) - lo
        return self.ref[self._slice(item, lo, size), cols]

    def load(self, item=0, lo=0, hi=None, cols=slice(None)):
        return pltpu.bitcast(self.load_words(item, lo, hi, cols), BF16)

    def store(self, val, item=0, lo=0, cols=slice(None)):
        self.ref[self._slice(item, lo, val.shape[0]), cols] = pltpu.bitcast(val.astype(BF16), U32)


def _with_ones_row(words, row):
    r = row // 2
    lo = (r // 8) * 8
    keep, one = (0x0000FFFF, 0x3F800000) if row % 2 else (0xFFFF0000, 0x00003F80)
    blk = words[lo:lo + 8]
    hit = lax.broadcasted_iota(I32, blk.shape, 0) == r - lo
    blk = jnp.where(hit, (blk & jnp.uint32(keep)) | jnp.uint32(one), blk)
    parts = [part for part in (words[0:lo], blk, words[lo + 8:]) if part.shape[0]]
    return pltpu.bitcast(jnp.concatenate(parts, axis=0), BF16)


def _kernel(x_hbm, wq_hbm, wk_hbm, wv_hbm, wo_hbm, beta_hbm, wr_hbm, wg_hbm, wu_hbm, wd_hbm,
            out_hbm,
            x_buf, wq_raw, wk_raw, wv_raw, wo_raw, beta_buf, wr_buf, wg_buf, wu_buf, wd_buf,
            wqt, wkt, wvt, wot, xn_buf, base, qs_buf, pq_buf, k_buf, pk_buf, vt_buf, r_buf,
            gate_buf, mt_buf, num_buf, p_buf0, p_buf1, ot_buf, out_buf, in_sems, out_sems):
    wqt, wkt = _Packed(wqt, PR), _Packed(wkt, PR)
    wvt, wot = _Packed(wvt, D), _Packed(wot, D)
    xn_buf, vt_buf = _Packed(xn_buf, D), _Packed(vt_buf, D)
    qs_buf, pq_buf, pk_buf = _Packed(qs_buf, PR), _Packed(pq_buf, PR), _Packed(pk_buf, PR)
    k_buf = _Packed(k_buf, L)

    def x_copy(c):
        return pltpu.make_async_copy(x_hbm.at[0, :, pl.ds(c * L, L)], x_buf.at[c], in_sems.at[c])

    cp_wv = pltpu.make_async_copy(wv_hbm, wv_raw, in_sems.at[4])
    cp_wq = pltpu.make_async_copy(wq_hbm, wq_raw, in_sems.at[5])
    cp_wk = pltpu.make_async_copy(wk_hbm, wk_raw, in_sems.at[6])
    cp_wo = pltpu.make_async_copy(wo_hbm, wo_raw, in_sems.at[7])
    cp_wg = pltpu.make_async_copy(wg_hbm, wg_buf, in_sems.at[8])
    cp_wu = pltpu.make_async_copy(wu_hbm, wu_buf, in_sems.at[9])
    cp_wd = pltpu.make_async_copy(wd_hbm, wd_buf, in_sems.at[10])
    cp_beta = pltpu.make_async_copy(beta_hbm, beta_buf, in_sems.at[11])
    cp_wr = pltpu.make_async_copy(wr_hbm, wr_buf, in_sems.at[12])

    def out_copy(s):
        cols = pl.ds(pl.multiple_of(s * L, L), L)
        return pltpu.make_async_copy(out_buf.at[s], out_hbm.at[0, :, cols], out_sems.at[s])

    def out_tile_copy(j):
        s = NSEG - 1
        return pltpu.make_async_copy(out_buf.at[s, :, pl.ds(128 * j, 128)],
                                     out_hbm.at[0, :, pl.ds(s * L + 128 * j, 128)], out_sems.at[NSEG + j])

    for cp in (x_copy(0), cp_wv, x_copy(1), cp_wq, cp_wr, cp_beta, x_copy(2), cp_wk, x_copy(3), cp_wo,
               cp_wg, cp_wu, cp_wd):
        cp.start()

    mt_buf[...] = jnp.zeros(mt_buf.shape, F32)

    always = []

    def pace(x, y):
        return x if y is None else jnp.where(always[0], x, y[0:D])

    def ln_stats(c, y):
        shift = x_buf[c, 0:16, :].astype(F32)[0:1]
        d = pace(x_buf[c].astype(F32), y) - shift
        m1 = jnp.sum(d, axis=0, keepdims=True) * (1.0 / D)
        m2 = jnp.sum(d * d, axis=0, keepdims=True) * (1.0 / D)
        var = jnp.maximum(m2 - m1 * m1, 0.0)
        inv = 1.0 / _round_bf16(jnp.sqrt(_round_bf16(_round_bf16(var) + 1e-5)))
        return _round_bf16(shift + m1), inv

    def ln_apply(c, mean_b, inv):
        x = x_buf[c].astype(F32)
        xn = (x - mean_b) * inv
        xn_buf.store(xn, c)
        if c == NSEG - 1:
            base[c] = jnp.zeros((D, L), F32)

    def project(w_ref, c, split):
        if not split:
            return jnp.dot(w_ref.load(), xn_buf.load(c), preferred_element_type=F32), None
        head = jnp.dot(w_ref.load(cols=slice(0, 256)), xn_buf.load(c, 0, 256), preferred_element_type=F32)
        tail = jnp.dot(w_ref.load(cols=slice(256, D)), xn_buf.load(c, 256, D), preferred_element_type=F32)
        return head + tail, head

    def project_v(c, mid=None):
        vt, head = project(wvt, c, mid is not None)
        if mid is not None:
            mid(head)
        vt_buf.store(vt, c)
        return vt

    def project_q(c, mid=None):
        qt, head = project(wqt, c, mid is not None)
        if mid is not None:
            mid(head)
        qsc = qt * QSCALE
        qs_buf.store(qsc, c)
        pq_buf.store(_phi(qt), c)
        r_buf[:, c * L:(c + 1) * L] = qt[120:128]
        mag = jnp.abs(qsc)
        r8 = lax.broadcasted_iota(I32, (8, L), 0)
        mag = jnp.concatenate([mag[0:120], jnp.where(r8 == ROUTER_ROW - 120, 0.0, mag[120:128]), mag[128:]], axis=0)
        return qt, jnp.max(mag.reshape(PR // 8, 8, L), axis=0)

    def project_k(c, mid=None, keep=False):
        kt, head = project(wkt, c, mid is not None)
        if mid is not None:
            mid(head)
        pk_buf.store(_phi(kt), c)
        for g in range(NG):
            ktg = kt[128 * g:128 * g + GW[g]]
            if GW[g] < 128:
                ktg = jnp.concatenate([ktg, jnp.zeros((128 - GW[g], L), F32)], axis=0)
            k_buf.store(ktg.T, c * NG + g)
        top = jnp.max(jnp.abs(kt).reshape(PR // 8, 8, L), axis=0)
        return (kt, top) if keep else top

    x_copy(0).wait()
    stats = ln_stats(0, None)
    always.append(jnp.logical_not(jnp.abs(stats[0]) < 0.0))
    ln_apply(0, *stats)
    cp_wv.wait()
    wvt.store(wv_raw[...].T)
    project_v(0)
    x_copy(1).wait()
    cp_wq.wait()
    cp_wr.wait()
    ln_apply(1, *ln_stats(1, None))

    def paced_weight(w_ref, y):
        w = w_ref[...].astype(F32)
        return jnp.concatenate([jnp.where(always[0], w[:, 0:L], y[0:D]), w[:, L:D]], axis=1)

    def prep_wq(y):
        wq_t = _pad_heads_t(paced_weight(wq_raw, y))
        wr_row = wr_buf[...].reshape(1, D).astype(F32)
        pr_row = lax.broadcasted_iota(I32, (8, D), 0)
        wq_t = jnp.concatenate(
            [wq_t[0:120], jnp.where(pr_row == ROUTER_ROW - 120, wr_row, wq_t[120:128]), wq_t[128:]], axis=0)
        wqt.store(wq_t)

    project_v(1, prep_wq)
    cp_wk.wait()
    cp_beta.wait()
    x_copy(2).wait()
    x_copy(3).wait()

    beta_row = beta_buf[...].reshape(1, H).astype(F32)
    beta_row = jnp.concatenate([beta_row, jnp.zeros((1, 128 - H), F32)], axis=1)
    h_row = lax.broadcasted_iota(I32, (H, 128), 0)
    h_lane = lax.broadcasted_iota(I32, (H, 128), 1)
    beta_col = jnp.sum(jnp.where(h_row == h_lane, beta_row, 0.0), axis=1, keepdims=True)
    gate_buf[...] = jnp.broadcast_to(jax.nn.sigmoid(beta_col), (H, 128))

    def prep_wk(y):
        wkt.store(_pad_heads_t(paced_weight(wk_raw, y)))

    def route():
        r = _round_bf16(r_buf[ROUTER_ROW - 120:ROUTER_ROW - 119, :])
        tok = lax.broadcasted_iota(I32, (1, S), 1).astype(F32)
        m1 = jnp.max(r)
        i1 = jnp.min(jnp.where(r == m1, tok, float(S)))
        r_rest = jnp.where(tok == i1, -jnp.inf, r)
        m2 = jnp.max(r_rest)
        i2 = jnp.min(jnp.where(r_rest == m2, tok, float(S)))
        i1 = jnp.clip(i1.astype(I32), 0, S - 1)
        i2 = jnp.clip(i2.astype(I32), 0, S - 1)
        return m1, m2, i1, i2

    qt, aq = project_q(0, prep_wk)
    qt, a = project_q(1)
    aq = jnp.maximum(aq, a)
    stats = ln_stats(2, qt)
    kt, ak = project_k(0, keep=True)
    ln_apply(2, *stats)
    stats = ln_stats(3, kt)
    ak = jnp.maximum(ak, project_k(1))
    ln_apply(3, *stats)
    project_v(2)
    qt, a = project_q(2)
    aq = jnp.maximum(aq, a)
    ak = jnp.maximum(ak, project_k(2))
    qt, a = project_q(3)
    aq = jnp.maximum(aq, a)
    m1, m2, i1, i2 = route()
    ak = jnp.maximum(ak, project_k(3))
    project_v(3)

    logit_bound = jnp.max(aq) * jnp.max(ak) * (DH * 1.02)
    safe = logit_bound <= SAFE_LOG2_RANGE

    sel_row = lax.broadcasted_iota(I32, (16, 128), 0)
    sel_lane = lax.broadcasted_iota(I32, (16, 128), 1)

    def token_tile(i):
        return i // L, pl.ds(pl.multiple_of(((i % L) // 128) * 128, 128), 128)

    def pick(i, slot):
        seg, cols = token_tile(i)
        onehot = jnp.where((sel_row == slot) & (sel_lane == i % 128), 1.0, 0.0).astype(BF16)
        return lax.dot_general(onehot, xn_buf.load(seg, cols=cols), NT_DIMS, preferred_element_type=F32)

    def routed_rows():
        return (pick(i1, 0) + pick(i2, 1)).astype(BF16)

    cp_wo.wait()
    cp_wg.wait()
    cp_wu.wait()

    def expert_chunk(lo, hi):
        xs = routed_rows()
        hg = jnp.dot(xs, wg_buf[:, lo:hi], preferred_element_type=F32)
        hu = jnp.dot(xs, wu_buf[:, lo:hi], preferred_element_type=F32)
        hh = (jax.nn.silu(hg) * hu).astype(BF16)
        return lax.dot_general(hh, wd_buf[:, lo:hi], NT_DIMS, preferred_element_type=F32)

    def expert_up_stream(hidden):
        kmain = 512
        xs = routed_rows()
        tail = xs[:, kmain:D].astype(F32)
        zero = jnp.zeros_like(tail)
        r16k = lax.broadcasted_iota(I32, (16, 128), 0)
        xs_rem = jnp.where(r16k < 2, jnp.concatenate([tail, zero], axis=1),
                           pltpu.roll(jnp.concatenate([zero, tail], axis=1), 2, 0)).astype(BF16)
        yield
        for c0 in range(0, FF, 512):
            w_rem = jnp.concatenate([wg_buf[kmain:D, c0:c0 + 512], wu_buf[kmain:D, c0:c0 + 512]], axis=0)
            both = jnp.dot(xs_rem, w_rem, preferred_element_type=F32)
            rem = (both, pltpu.roll(both, 14, 0))
            yield
            hs = []
            for f0 in range(c0, c0 + 512, 128):
                pre = []
                for w_ref, r in zip((wg_buf, wu_buf), rem):
                    pre.append(jnp.dot(xs[:, 0:kmain], w_ref[0:kmain, f0:f0 + 128], preferred_element_type=F32)
                               + r[:, f0 - c0:f0 - c0 + 128])
                    if len(pre) == 2:
                        hs.append(jax.nn.silu(pre[0]) * pre[1])
                        if len(hs) == 4:
                            hidden.append(_round_bf16(jnp.concatenate(hs, axis=1)))
                    yield

    lane_d = lax.broadcasted_iota(I32, (D, 128), 1)

    def expert_scatter_parts(columns):
        for col, i, score in zip(columns, (i1, i2), (m1, m2)):
            seg, cols = token_tile(i)
            col = col * jax.nn.sigmoid(jnp.full((D, 1), score, F32))
            base[seg, :, cols] = base[seg, :, cols] + jnp.where(lane_d == i % 128, col, 0.0)
            yield

    def expert_scatter_rows(y):
        yt = jnp.concatenate([y, jnp.zeros((128 - 16, D), F32)], axis=0).T
        columns = [jnp.sum(jnp.where(lane_d == slot, yt, 0.0), axis=1, keepdims=True) for slot in range(2)]
        for _ in expert_scatter_parts(columns):
            pass

    def memory_read(s, g):
        sr = _state_rows(g)
        gw = GW[g]
        num_buf[g, 0:sr, :] = jnp.dot(mt_buf[g, 0:sr, 0:gw].astype(BF16), pq_buf.load(s, 128 * g, 128 * g + gw),
                                      preferred_element_type=F32)

    def memory_update(s, g):
        rg = _group_rows(g)
        a_g = _group_row_start(g)
        gw = GW[g]
        ones_row = 126 if g == 0 else 0
        lhs = _with_ones_row(vt_buf.load_words(s, a_g, a_g + rg), ones_row)
        upd = lax.dot_general(lhs, pk_buf.load(s, 128 * g, 128 * g + gw), NT_DIMS,
                              preferred_element_type=F32)
        er = lax.broadcasted_iota(I32, (rg, gw), 0) + (a_g - HPG * DH * g)
        el = lax.broadcasted_iota(I32, (rg, gw), 1)
        same_head = None
        for i in range(_heads_in_group(g)):
            t = ((er >= DH * i) & (er < DH * (i + 1)) & (el >= DH * i) & (el < DH * (i + 1)))
            same_head = t if same_head is None else (same_head | t)
        mt_buf[g, 0:rg, 0:gw] = mt_buf[g, 0:rg, 0:gw] + jnp.where(same_head, upd, 0.0)
        zr = lax.broadcasted_iota(I32, (8, gw), 0)
        zl = lax.broadcasted_iota(I32, (8, gw), 1)
        zmask = (zl >= zr * DH) & (zl < zr * DH + DH) & (zr < _heads_in_group(g))
        zs = upd[ones_row:ones_row + 1]
        z0 = _norm_row(g)
        mt_buf[g, z0:z0 + 8, 0:gw] = mt_buf[g, z0:z0 + 8, 0:gw] + jnp.where(zmask, zs, 0.0)

    def transpose_wo(g):
        hi = min(128 * (g + 1), D)
        wot.store(wo_raw[:, 128 * g:hi].T, lo=128 * g)

    def project_out(s):
        return jnp.dot(wot.load(), ot_buf[...].astype(BF16), preferred_element_type=F32)

    def residual(s, cols=slice(None)):
        return x_buf[s, :, cols].astype(F32) + xn_buf.load(s, cols=cols).astype(F32)

    def emit(s, val):
        out_buf[s] = val.astype(BF16)
        out_copy(s).start()

    zero = lax.shift_right_logical(i1, 16)

    def prow(start, size):
        return pl.ds(pl.multiple_of(zero + start, 8), size)

    P_OFFS = (0, 128, 384, 768)

    def fast_scores(s, g, hook, anchor):
        nh = _heads_in_group(g)
        gw = GW[g]
        pb = (p_buf0, p_buf1)[(s * NG + g) % 2]
        rowg = lax.broadcasted_iota(I32, (gw // 2, 128), 0)
        laneg = lax.broadcasted_iota(I32, (gw // 2, 128), 1)
        head_rows = [(rowg >= DH // 2 * i) & (rowg < DH // 2 * (i + 1)) for i in range(nh)]
        none = jnp.uint32(0)
        visible_lo = _visible_words(64, lax.broadcasted_iota(I32, (32, 128), 1))
        lane16 = lax.broadcasted_iota(I32, (16, 128), 1)
        for j in range(QT - 1, -1, -1):
            n = 128 * (j + 1)
            m = n - 64
            q = qs_buf.load_words(s, 128 * g, 128 * g + gw, slice(128 * j, 128 * (j + 1)))
            for h0, h1 in (((0, 3), (3, nh)) if nh == HPG else ((0, nh),)):
                q_in = anchor(q)
                qm = pltpu.bitcast(
                    jnp.concatenate([jnp.where(head_rows[i], q_in, none) for i in range(h0, h1)], axis=1),
                    BF16)
                st = jnp.dot(k_buf.load(s * NG + g, 0, m, slice(0, gw)), qm, preferred_element_type=F32)
                p = jnp.exp2(st)
                words = pltpu.bitcast(p.astype(BF16), U32)
                diag = words[m // 2 - 32:] & jnp.concatenate([visible_lo] * (h1 - h0), axis=1)
                words = jnp.concatenate([words[:m // 2 - 32], diag], axis=0) if j > 0 else diag
                pb[P_OFFS[j] // 2:(P_OFFS[j] + m) // 2, h0 * 128:h1 * 128] = words
                hook(p)
            for width, k0 in ((64, m), (32, m + 32)):
                per = 128 // width
                q_top = q
                for t in range(per - 1):
                    q_top = jnp.where((laneg >= width * t) & (laneg < width * (t + 1)),
                                      pltpu.roll(q, width * (t + 1), 1), q_top)
                groups = [list(range(i, min(i + per, nh))) for i in range(0, nh, per)]
                tiles = []
                for heads in groups:
                    keep = None
                    for t, i in enumerate(heads):
                        slot = per - len(heads) + t
                        sel = head_rows[i] & (laneg >= width * slot) & (laneg < width * (slot + 1))
                        keep = sel if keep is None else (keep | sel)
                    tiles.append(jnp.where(keep, q_top, none))
                st = jnp.dot(k_buf.load(s * NG + g, k0, k0 + 32, slice(0, gw)),
                             pltpu.bitcast(jnp.concatenate(tiles, axis=1), BF16),
                             preferred_element_type=F32)
                visible = _visible_words(32, lane16 & (width - 1))
                p = pltpu.bitcast(jnp.exp2(st).astype(BF16), U32)
                p = p & jnp.concatenate([visible] * len(groups), axis=1)
                rows = slice((P_OFFS[j] + k0) // 2, (P_OFFS[j] + k0 + 32) // 2)
                top = lane16 >= 128 - width
                for gi, heads in enumerate(groups):
                    shared = p[:, 128 * gi:128 * (gi + 1)]
                    for t, i in enumerate(heads):
                        slot = per - len(heads) + t
                        shift = width * (per - 1 - slot)
                        mine = shared if shift == 0 else pltpu.roll(shared, shift, 1)
                        pb[rows, 128 * i:128 * (i + 1)] = jnp.where(top, mine, jnp.uint32(0))

    def fast_values(s, g, after_tile=None):
        nh = _heads_in_group(g)
        a_g = _group_row_start(g)
        pb = (p_buf0, p_buf1)[(s * NG + g) % 2]
        for j in range(QT - 1, -1, -1):
            n = 128 * (j + 1)
            cols = slice(128 * j, 128 * (j + 1))
            for i in range(nh):
                h = HPG * g + i
                a = (h * DH // 16) * 16
                off = h * DH - a
                p = pltpu.bitcast(pb[prow(P_OFFS[j] // 2, n // 2), 128 * i:128 * (i + 1)], BF16)
                ones_row = 0 if off > 0 else 31
                lhs = _with_ones_row(vt_buf.load_words(s, a, a + 32, slice(0, n)), ones_row)
                o = jnp.dot(lhs, p, preferred_element_type=F32)
                lo = (off // 8) * 8
                hi = -(-(off + DH) // 8) * 8
                gate = gate_buf[h:h + 1, :]
                rl = _recip(o[ones_row:ones_row + 1])
                val = (1.0 - gate) * (o[lo:hi] * rl)
                if s > 0:
                    z = _norm_row(g) + i
                    rden = _recip(num_buf[g, z:z + 1, cols] + 1e-6)
                    num = num_buf[g, a - a_g + lo:a - a_g + hi, cols]
                    val = gate * (num * rden) + val
                ot_buf[a + off:a + off + DH, cols] = val[off - lo:off - lo + DH]
            if after_tile is not None:
                after_tile(j)

    def fast_path():
        hidden = []
        up = expert_up_stream(hidden)
        n_down = FF // 128
        state = dict(down=0, wd_ready=False, up_done=False, y=[None] * 2, tail=None, tail_steps=0,
                     out_ready=False, pacer=None, anchor=None, anchor_next=None)

        def finish():
            yield from expert_scatter_parts([jnp.sum(acc, axis=1, keepdims=True) for acc in state["y"]])
            for u in range(NSEG - 1):
                for j in range(QT):
                    cols = slice(128 * j, 128 * (j + 1))
                    val = paced(base[u, :, cols])
                    out_buf[u, :, cols] = val.astype(BF16)
                    state["anchor"] = val
                    if j == QT - 1:
                        out_copy(u).start()
                    yield

        def anchor(q):
            val, state["anchor_next"], state["anchor"] = state["anchor_next"], state["anchor"], None
            if val is None:
                return q
            return jnp.where(always[0][:, 0:128], q, pltpu.bitcast(val[D - q.shape[0]:D], U32))

        def paced(val):
            y = state["pacer"]
            if y is None:
                return val
            reps = -(-D // y.shape[0])
            y = jnp.concatenate([y[:, 128 * r:128 * (r + 1)] for r in range(reps)], axis=0)[0:D]
            return jnp.where(always[0][:, 0:128], val, y)

        def down_step():
            ft = state["down"]
            w = paced(wd_buf[:, 128 * ft:128 * (ft + 1)].astype(F32))
            hh = hidden[ft // 4][:, 128 * (ft % 4):128 * (ft % 4 + 1)]
            for slot in range(2):
                term = w * hh[slot:slot + 1]
                state["y"][slot] = term if state["y"][slot] is None else state["y"][slot] + term
            if ft % 4 == 3:
                state["anchor"] = state["y"][1]
            state["down"] += 1

        def hook(pacer=None):
            state["pacer"] = pacer if pacer is not None and pacer.shape[0] * (pacer.shape[1] // 128) >= D else None
            if not state["up_done"] and next(up, "done") == "done":
                state["up_done"] = True
            if state["down"] < n_down:
                if (state["wd_ready"] and state["pacer"] is not None and state["pacer"].shape[0] >= 320
                        and state["down"] // 4 < len(hidden)):
                    down_step()
            elif state["out_ready"]:
                if state["tail"] is None:
                    state["tail"] = finish()
                if state["pacer"] is not None or state["tail_steps"] < 2:
                    state["tail_steps"] += 1
                    next(state["tail"], None)

        steps = [(s, g) for s in range(NSEG) for g in range(NG)]
        last = NSEG - 1

        def last_tile(j):
            cols = slice(128 * j, 128 * (j + 1))
            attn = jnp.dot(wot.load(), ot_buf[:, cols].astype(BF16), preferred_element_type=F32)
            out_buf[last, :, cols] = (base[last, :, cols] + residual(last, cols) + attn).astype(BF16)
            out_tile_copy(j).start()

        fast_scores(0, 0, hook, anchor)
        for t, (s, g) in enumerate(steps):
            if t + 1 < len(steps):
                fast_scores(*steps[t + 1], hook, anchor)
            if s > 0:
                memory_read(s, g)
                hook()
            if t + 1 == len(steps):
                state["pacer"] = None
                assert state["down"] == n_down and state["tail"] is not None
                while next(state["tail"], "done") != "done":
                    pass
                pending = []

                def after_tile(j):
                    if pending:
                        last_tile(pending.pop())
                    pending.append(j)

                fast_values(s, g, after_tile)
                last_tile(pending.pop())
            else:
                fast_values(s, g)
            if s == 0:
                transpose_wo(g)
            if s + 1 < NSEG:
                memory_update(s, g)
                hook()
            if g == NG - 1 and s < last:
                base[s] = project_out(s) + residual(s)
                if s == 0:
                    cp_wd.wait()
                    state["wd_ready"] = True
                if s == last - 1:
                    state["out_ready"] = True
                hook()
        for u in range(NSEG - 1):
            out_copy(u).wait()
        for j in range(QT):
            out_tile_copy(j).wait()

    def slow_segment(s, carry):
        for g in range(NG):
            memory_read(s, g)
        key_i = lax.broadcasted_iota(I32, (L, L), 0)
        qry_i = lax.broadcasted_iota(I32, (L, L), 1)
        r32 = lax.broadcasted_iota(I32, (32, L), 0)
        for g in range(NG):
            gw = GW[g]
            a_g = _group_row_start(g)
            rowg = lax.broadcasted_iota(I32, (gw, L), 0)

            def head(i, c, g=g, gw=gw, a_g=a_g, rowg=rowg):
                h = HPG * g + i
                a = pl.multiple_of((h * DH // 16) * 16, 16)
                off = h * DH - a
                q = qs_buf.load(s, 128 * g, 128 * g + gw).astype(F32)
                qm = jnp.where((rowg >= DH * i) & (rowg < DH * (i + 1)), q, 0.0).astype(BF16)
                st = jnp.dot(k_buf.load(s * NG + g, cols=slice(0, gw)), qm, preferred_element_type=F32)
                st = jnp.where(key_i <= qry_i, st, NEG_BIG)
                p = jnp.exp2(st - jnp.max(st, axis=0, keepdims=True))
                rl = 1.0 / jnp.sum(p, axis=0, keepdims=True)
                o = jnp.dot(vt_buf.load(s, a, 32), p.astype(BF16), preferred_element_type=F32)
                gate = jnp.concatenate([gate_buf[pl.ds(h, 1), :]] * QT, axis=1)
                rden = 1.0 / (num_buf[g, pl.ds(_norm_row(g) + i, 1), :] + 1e-6)
                num = num_buf[g, pl.ds(pl.multiple_of(a - a_g, 16), 32), :]
                val = gate * (num * rden) + (1.0 - gate) * (o * rl)
                keep = (r32 >= off) & (r32 < off + DH)
                pltpu.store(ot_buf.at[pl.ds(a, 32), :], val, mask=keep)
                return c

            lax.fori_loop(0, _heads_in_group(g), head, 0)
        for g in range(NG):
            memory_update(s, g)
        emit(s, base[s] + residual(s) + project_out(s))
        return carry

    @pl.when(safe)
    def _():
        fast_path()

    @pl.when(jnp.logical_not(safe))
    def _():
        cp_wd.wait()
        for u in range(NSEG - 1):
            base[u] = jnp.zeros((D, L), F32)
        for g in range(NG):
            transpose_wo(g)
        expert_scatter_rows(expert_chunk(0, FF))
        lax.fori_loop(0, NSEG, slow_segment, 0)
        for u in range(NSEG):
            out_copy(u).wait()


@jax.jit
def pallas_parallel_sum__memory_aug_infini_attn__moe_arch_mod__prompt_kernel(
    A_x: jax.Array,
    A_wq: jax.Array,
    A_wk: jax.Array,
    A_wv: jax.Array,
    A_wo: jax.Array,
    A_beta: jax.Array,
    B_x: jax.Array,
    B_w_r: jax.Array,
    B_w_gate: jax.Array,
    B_w_up: jax.Array,
    B_w_down: jax.Array,
):
    del B_x
    hbm = pl.BlockSpec(memory_space=pl.ANY)
    scratch = [
        pltpu.VMEM((NSEG, D, L), BF16),
        pltpu.VMEM((D, D), BF16),
        pltpu.VMEM((D, D), BF16),
        pltpu.VMEM((D, D), BF16),
        pltpu.VMEM((D, D), BF16),
        pltpu.VMEM((H,), BF16),
        pltpu.VMEM((D,), BF16),
        pltpu.VMEM((D, FF), BF16),
        pltpu.VMEM((D, FF), BF16),
        pltpu.VMEM((D, FF), BF16),
        pltpu.VMEM((PR // 2, D), U32),
        pltpu.VMEM((PR // 2, D), U32),
        pltpu.VMEM((D // 2, D), U32),
        pltpu.VMEM((D // 2, D), U32),
        pltpu.VMEM((NSEG * D // 2, L), U32),
        pltpu.VMEM((NSEG, D, L), F32),
        pltpu.VMEM((NSEG * PR // 2, L), U32),
        pltpu.VMEM((NSEG * PR // 2, L), U32),
        pltpu.VMEM((NSEG * NG * L // 2, 128), U32),
        pltpu.VMEM((NSEG * PR // 2, L), U32),
        pltpu.VMEM((NSEG * D // 2, L), U32),
        pltpu.VMEM((8, S), F32),
        pltpu.VMEM((H, 128), F32),
        pltpu.VMEM((NG, MROWS, 128), F32),
        pltpu.VMEM((NG, MROWS, L), F32),
        pltpu.VMEM((640, HPG * 128), U32),
        pltpu.VMEM((640, HPG * 128), U32),
        pltpu.VMEM((D, L), F32),
        pltpu.VMEM((NSEG, D, L), BF16),
        pltpu.SemaphoreType.DMA((13,)),
        pltpu.SemaphoreType.DMA((NSEG + QT,)),
    ]
    out_t = pl.pallas_call(
        _kernel,
        out_shape=jax.ShapeDtypeStruct((1, D, S), BF16),
        in_specs=[hbm] * 10,
        out_specs=hbm,
        scratch_shapes=scratch,
        compiler_params=pltpu.CompilerParams(vmem_limit_bytes=128 * 1024 * 1024),
        name="infini_attn_moe",
    )(jnp.transpose(A_x, (0, 2, 1)), A_wq, A_wk, A_wv, A_wo, A_beta, B_w_r, B_w_gate, B_w_up,
      B_w_down.T)
    return jnp.transpose(out_t, (0, 2, 1))
```
